```python
import jax
import jax.numpy as jnp

def _softmax(x, axis=-1):
    return jax.nn.softmax(x, axis=axis)

def _gelu(x):
    return jax.nn.gelu(x, approximate=True)

def _silu(x):
    return jax.nn.silu(x)

def _sigmoid(x):
    return jax.nn.sigmoid(x)

def _layernorm(x, axis=-1, eps=1e-05):
    m = jnp.mean(x, axis=axis, keepdims=True)
    v = jnp.var(x, axis=axis, keepdims=True)
    return (x - m) / jnp.sqrt(v + eps)

def _scatter_add(tgt, idx, src, axis=0):
    return tgt.at[idx].add(src)

def _segment_sum(src, seg, n):
    return jax.ops.segment_sum(src, seg, n)

class _Rng:

    def __init__(self, key):
        self._k = key

    def _next(self):
        self._k, sub = jax.random.split(self._k)
        return sub

    def normal(self, shape):
        return jax.random.normal(self._next(), shape, dtype=jnp.bfloat16)

    def randint(self, lo, hi, shape):
        return jax.random.randint(self._next(), shape, lo, hi, dtype=jnp.int32)

    def uniform(self, shape, lo=0.0, hi=1.0):
        return jax.random.uniform(self._next(), shape, jnp.bfloat16, lo, hi)

    def permutation(self, n):
        return jax.random.permutation(self._next(), n)
kernel_name = 'adaLN_cond__memory_aug_recurrent_mem_tr__moe_arch_mod__prompt'

def setup_inputs():
    _rng = _Rng(jax.random.key(int.from_bytes(__import__("os").urandom(4), "little")))
    _w = lambda a: (lambda t: t.astype(jnp.bfloat16) if jnp.issubdtype(t.dtype, jnp.floating) else t)(jnp.asarray(a))

    def _A_setup():
        B, S, Dm = (1, 2048, 1024)
        H, Dh = (32, 128)
        M, seg = (8, 32)
        seg = min(seg, S)
        S = S // seg * seg
        return {'x': _w((lambda *s: _rng.normal(s) * 0.05)(B, S, Dm)), 'mem0': _w((lambda *s: _rng.normal(s) * 0.05)(B, M, Dm)), 'Wq': _w((lambda *s: _rng.normal(s) * 0.05)(Dm, H, Dh) * Dm ** (-0.5)), 'Wk': _w((lambda *s: _rng.normal(s) * 0.05)(Dm, H, Dh) * Dm ** (-0.5)), 'Wv': _w((lambda *s: _rng.normal(s) * 0.05)(Dm, H, Dh) * Dm ** (-0.5)), 'Wo': _w((lambda *s: _rng.normal(s) * 0.05)(H, Dh, Dm) * (H * Dh) ** (-0.5)), 'seg_len': seg}
    _A_in = _A_setup()

    def _B_setup():
        B, S, D, F, C = (1, 2048, 1024, 3584, 2)
        return {'x': _w((lambda *s: _rng.normal(s) * 0.05)(B, S, D)), 'w_r': _w((lambda *s: _rng.normal(s) * 0.05)(D)), 'w_gate': _w((lambda *s: _rng.normal(s) * 0.05)(D, F)), 'w_up': _w((lambda *s: _rng.normal(s) * 0.05)(D, F)), 'w_down': _w((lambda *s: _rng.normal(s) * 0.05)(F, D))}
    _B_in = _B_setup()
    return {'A_x': _A_in['x'], 'A_mem0': _A_in['mem0'], 'A_Wq': _A_in['Wq'], 'A_Wk': _A_in['Wk'], 'A_Wv': _A_in['Wv'], 'A_Wo': _A_in['Wo'], 'A_seg_len': _A_in['seg_len'], 'B_x': _B_in['x'], 'B_w_r': _B_in['w_r'], 'B_w_gate': _B_in['w_gate'], 'B_w_up': _B_in['w_up'], 'B_w_down': _B_in['w_down'], 'c': _w((lambda *s: _rng.normal(s) * 0.05)(1, 1024)), 'w_mod': _w((lambda *s: _rng.normal(s) * 0.05)(1024, 6 * 1024) * 1024 ** (-0.5))}

def reference(A_x, A_mem0, A_Wq, A_Wk, A_Wv, A_Wo, A_seg_len, B_x, B_w_r, B_w_gate, B_w_up, B_w_down, c, w_mod):

    def _A_ref(x, mem0, Wq, Wk, Wv, Wo, seg_len):
        B, S, Dm = x.shape
        H, Dh = (Wq.shape[1], Wq.shape[2])
        M = mem0.shape[1]
        scale = Dh ** (-0.5)
        n_seg = S // seg_len
        L = M + seg_len
        idx = jnp.arange(L)
        mask = (idx[:, None] < M) | (idx[:, None] >= idx[None, :])
        mem = mem0
        outs = []
        for s in range(n_seg):
            xs = x[:, s * seg_len:(s + 1) * seg_len, :].copy()
            h = jnp.concatenate([mem, xs], axis=1)
            q = jnp.einsum('btd,dhe->bhte', h, Wq)
            k = jnp.einsum('btd,dhe->bhte', h, Wk)
            v = jnp.einsum('btd,dhe->bhte', h, Wv)
            scores = jnp.einsum('bhqe,bhke->bhqk', q, k) * scale
            scores = jnp.where(mask[None, None], scores, -1000000000.0)
            p = _softmax(scores, axis=-1)
            o = jnp.einsum('bhqk,bhke->bhqe', p, v)
            o = jnp.einsum('bhte,hed->btd', o, Wo)
            mem = o[:, :M, :].copy()
            outs.append(o[:, M:, :])
        return jnp.concatenate(outs, axis=1)

    def _B_ref(x, w_r, w_gate, w_up, w_down):
        B, S, D = x.shape
        C = 2
        r = x @ w_r
        idx = jnp.argsort(-r, axis=-1)[:, :C]
        idx_e = jnp.repeat(idx.reshape(B, C, 1), D, axis=2)
        x_sel = jnp.take_along_axis(x, idx_e, axis=1)
        g = _silu(x_sel @ w_gate)
        u = x_sel @ w_up
        y = g * u @ w_down
        r_sel = _sigmoid(jnp.take_along_axis(r, idx, axis=1))
        y = y * r_sel.reshape(B, C, 1)
        b_off = (jnp.arange(B) * S).reshape(B, 1)
        flat_idx = (idx + b_off).reshape(B * C)
        zero = (x * 0.0).reshape(B * S, D)
        upd = _scatter_add(zero, flat_idx, y.reshape(B * C, D), axis=0)
        return x + upd.reshape(B, S, D)
    x = A_x
    mod = (_silu(c) @ w_mod).reshape(c.shape[0], 6, 1, -1)
    sa, ca, ga, sb, cb, gb = (mod[:, 0].copy(), mod[:, 1].copy(), mod[:, 2].copy(), mod[:, 3].copy(), mod[:, 4].copy(), mod[:, 5].copy())
    h = _layernorm(x, axis=-1) * (1 + ca) + sa
    x = x + ga * _A_ref(h, A_mem0, A_Wq, A_Wk, A_Wv, A_Wo, A_seg_len)
    h = _layernorm(x, axis=-1) * (1 + cb) + sb
    x = x + gb * _B_ref(h, B_w_r, B_w_gate, B_w_up, B_w_down)
    return x
```

```python
import functools

import jax
import jax.numpy as jnp
import jax.experimental.pallas as pl
import jax.experimental.pallas.tpu as pltpu

F32 = jnp.float32
BF16 = jnp.bfloat16
U32 = jnp.uint32

D = 1024
H = 32
DH = 128
NP = H // 2
M = 8
SEG = 32
NSEG = 64
FF = 3584
NJ = SEG - M
NE = NSEG * M
EPS = 1e-5
SCALE = DH ** (-0.5)
NEG = -1000000000.0


def _rb(x):
    return x.astype(BF16).astype(F32)


def _layernorm(xf):
    m = jnp.mean(xf, axis=-1, keepdims=True)
    d = xf - m
    v = jnp.mean(d * d, axis=-1, keepdims=True)
    return d * jax.lax.rsqrt(v + EPS)


def _dot(a, b):
    return jnp.dot(a, b, preferred_element_type=F32)


def _dot_nt(a, b):
    return jax.lax.dot_general(a, b, (((1,), (1,)), ((), ())), preferred_element_type=F32)


def _kernel(x_hbm, mem0_ref, wq_hbm, wk_hbm, wv_hbm, wo_hbm, wr_ref, wg_hbm, wu_hbm, wd_hbm,
            c_ref, wm_hbm,
            out_hbm,
            wqkv, wo, wg, wu, wd, wm, xv, x1v, outv, early, oe, he, attn_e, lhs_ref, pend,
            mod, fill, rmat, patch,
            sem_pair, sem_misc, sem_out):
    w_u32 = [w.bitcast(U32) for w in (wq_hbm, wk_hbm, wv_hbm)]

    def pair_copies(p):
        return [pltpu.make_async_copy(w_u32[m].at[:, par, p, :], wqkv.at[m * H + 2 * p + par],
                                      sem_pair.at[p])
                for m in range(3) for par in range(2)]

    def col_copies(src, dst, lo, hi, sem):
        return [pltpu.make_async_copy(src.at[:, pl.ds(j * 128, 128)], dst.at[j], sem)
                for j in range(lo, hi)]

    cp_xe = [pltpu.make_async_copy(x_hbm.at[:, 3], xv.at[:, 3], sem_misc.at[0])]
    cp_wm1 = col_copies(wm_hbm, wm, 0, 16, sem_misc.at[1])
    cp_xj = [pltpu.make_async_copy(x_hbm.at[:, 0:3], xv.at[:, 0:3], sem_misc.at[2])]
    cp_wo = col_copies(wo_hbm, wo, 0, 8, sem_misc.at[3])
    cp_wm2 = col_copies(wm_hbm, wm, 16, 48, sem_misc.at[4])
    cp_ffn = (col_copies(wg_hbm, wg, 0, FF // 128, sem_misc.at[5])
              + col_copies(wu_hbm, wu, 0, FF // 128, sem_misc.at[5])
              + col_copies(wd_hbm, wd, 0, 8, sem_misc.at[5]))

    for cp in cp_xe + cp_wm1:
        cp.start()
    for p in range(NP):
        for cp in pair_copies(p):
            cp.start()
    for cp in cp_xj + cp_wo + cp_wm2 + cp_ffn:
        cp.start()

    ri = jax.lax.broadcasted_iota(jnp.int32, (80, 128), 0)
    ci = jax.lax.broadcasted_iota(jnp.int32, (80, 128), 1)

    def head_of(i):
        return jnp.where(i < 64, i // 32, (i - 64) // 8)

    def pos_of(i):
        return jnp.where(i < 64, i % 32, 32 + i % 8)

    same = (head_of(ri) == head_of(ci)) & (ci < 80)
    allowed = (pos_of(ri) < M) | (pos_of(ri) >= pos_of(ci))
    fill[...] = jnp.where(same, jnp.where(allowed, 0.0, NEG), -jnp.inf).astype(F32)
    rmat[...] = jnp.full(rmat.shape, -jnp.inf, F32)
    pend[...] = jnp.zeros(pend.shape, F32)

    cf = c_ref[...].astype(F32)
    sc = _rb(cf * jax.nn.sigmoid(cf))
    sc = jnp.broadcast_to(sc, (16, D)).astype(BF16)

    def mod_cols(lo, hi):
        for j in range(lo, hi):
            v = _rb(_dot(sc, wm[j])[0:8])
            if j // 8 in (1, 4):
                v = _rb(1.0 + v)
            mod[:, j * 128:(j + 1) * 128] = v

    def mod_vec(k):
        return mod[:, k * D:(k + 1) * D]

    def modulate1(xb):
        n = _rb(_layernorm(xb.astype(F32)))
        return _rb(n * mod_vec(1)) + mod_vec(0)

    for cp in cp_wm1:
        cp.wait()
    mod_cols(0, 16)
    for cp in cp_xe:
        cp.wait()

    def he_body(i, carry):
        hh = modulate1(xv[pl.ds(i * 8, 8), 3])
        he[pl.ds(pl.multiple_of(i * 64, 64), 64), :] = hh.reshape(64, D).astype(BF16)
        return carry

    jax.lax.fori_loop(0, NSEG // 8, he_body, 0)

    def relayout(p):
        for cp in pair_copies(p):
            cp.wait()
        for m in range(3):
            e = wqkv[m * H + 2 * p]
            o = wqkv[m * H + 2 * p + 1]
            wqkv[m * H + 2 * p] = (e & U32(0xFFFF)) | (o << 16)
            wqkv[m * H + 2 * p + 1] = (e >> 16) | (o & U32(0xFFFF0000))

    def w_head(m, h):
        return pltpu.bitcast(wqkv[m * H + h], BF16)

    def early_proj(p):
        for m in range(3):
            for c in range(2):
                hc = he[c * 256:(c + 1) * 256, :]
                r1 = _dot(hc, w_head(m, 2 * p)).reshape(32, 8, DH)
                r2 = _dot(hc, w_head(m, 2 * p + 1)).reshape(32, 8, DH)
                early[c * 32:(c + 1) * 32, m * NP + p] = (
                    jnp.concatenate([r1, r2], axis=1).astype(BF16))

    relayout(0)

    def pro_body(p, carry):
        relayout(p + 1)
        early_proj(p)
        return carry

    jax.lax.fori_loop(0, NP - 1, pro_body, 0)
    for cp in cp_xj + cp_wo + cp_wm2:
        cp.wait()
    early_proj(NP - 1)
    mod_cols(16, 48)
    lhs_ref[...] = jnp.concatenate(
        [mem0_ref[...].astype(F32), modulate1(xv[0, 0:3]).reshape(NJ, D)], axis=0).astype(BF16)

    wr = jnp.broadcast_to(wr_ref[...].astype(F32), (8, D))

    def second(x1):
        n = _rb(_layernorm(x1))
        h2 = _rb(_rb(n * mod_vec(4)) + mod_vec(3))
        r = _rb(jnp.sum(h2 * wr, axis=-1, keepdims=True))
        return h2, r

    def post(xb, attn):
        x1 = _rb(xb.astype(F32) + _rb(mod_vec(2) * _rb(attn)))
        h2, r = second(x1)
        out = x1 + _rb(mod_vec(5) * h2)
        return x1.astype(BF16), out.astype(BF16), r

    lane8 = jax.lax.broadcasted_iota(jnp.int32, (8, 128), 1)

    def post_j(s):
        x1, out, r = post(xv[s, 0:3], pend[...].reshape(3, 8, D))
        x1v[s, 0:3] = x1
        outv[s, 0:3] = out
        for g in range(3):
            rmat[g * 8:(g + 1) * 8, :] = jnp.where(lane8 == s, r[g], rmat[g * 8:(g + 1) * 8, :])

    zpad = jnp.zeros((48, DH), BF16)

    def step(s, carry):
        lhs = lhs_ref[...]
        post_j(jnp.maximum(s - 1, 0))
        hj_next = modulate1(xv[jnp.minimum(s + 1, NSEG - 1), 0:3]).reshape(NJ, D)

        def qkv(p):
            res = []
            for m in range(3):
                a = _dot(lhs, w_head(m, 2 * p)).astype(BF16)
                b = _dot(lhs, w_head(m, 2 * p + 1)).astype(BF16)
                parts = [a, b, early[s, m * NP + p]]
                if m > 0:
                    parts.append(zpad)
                res.append(jnp.concatenate(parts, axis=0))
            return res

        def scores(q, k):
            sc_ = _dot_nt(q, k) * SCALE
            f = fill[...]
            sc_ = jnp.where(f == 0.0, sc_, f)
            mx = jnp.max(sc_, axis=-1, keepdims=True)
            e = jnp.exp(sc_ - mx)
            return (e / jnp.sum(e, axis=-1, keepdims=True)).astype(BF16)

        def pv(p, pr, v):
            o = _dot(pr, v)
            row = pl.multiple_of(s * 8, 8)
            oe[pl.ds(row, 8), (2 * p) * DH:(2 * p + 1) * DH] = o[64:72]
            oe[pl.ds(row, 8), (2 * p + 1) * DH:(2 * p + 2) * DH] = o[72:80]
            return [o[0:32].astype(BF16), o[32:64].astype(BF16)]

        qkvs, probs, os_ = {}, {}, []
        for p in range(NP):
            qkvs[p] = qkv(p)
            if p >= 1:
                probs[p - 1] = scores(qkvs[p - 1][0], qkvs[p - 1][1])
            if p >= 2:
                os_ += pv(p - 2, probs[p - 2], qkvs[p - 2][2])
        ka = (NP - 2) * 2 * DH
        oa = jnp.concatenate(os_, axis=1)
        acc = []
        for n in range(8):
            acc.append(_dot(oa, wo[n, 0:ka, :]))
            if n == 1:
                probs[NP - 1] = scores(qkvs[NP - 1][0], qkvs[NP - 1][1])
                ob = pv(NP - 2, probs[NP - 2], qkvs[NP - 2][2])
            if n == 4:
                ob += pv(NP - 1, probs[NP - 1], qkvs[NP - 1][2])
        ob = jnp.concatenate(ob, axis=1)
        res = jnp.concatenate([acc[n] + _dot(ob, wo[n, ka:H * DH, :]) for n in range(8)], axis=1)
        pend[...] = res[M:SEG]
        lhs_ref[...] = jnp.concatenate([res[0:M], hj_next], axis=0).astype(BF16)
        return carry

    jax.lax.fori_loop(0, NSEG, step, 0)

    post_j(NSEG - 1)
    cp_oj = pltpu.make_async_copy(outv.at[:, 0:3], out_hbm.at[:, 0:3], sem_out.at[0])
    cp_oj.start()

    def epi_body(c, carry):
        row = pl.multiple_of(c * 128, 128)
        ol = oe[pl.ds(row, 128), :].astype(BF16)
        res = jnp.concatenate([_dot(ol, wo[n]) for n in range(8)], axis=1)
        sg = pl.multiple_of(c * 16, 16)
        x1, out, r = post(xv[pl.ds(sg, 16), 3], res.reshape(16, 8, D))
        x1v[pl.ds(sg, 16), 3] = x1
        outv[pl.ds(sg, 16), 3] = out
        rm = rmat[24:32, :]
        for g in range(16):
            rm = jnp.where(lane8 == sg + g, r[g], rm)
        rmat[24:32, :] = rm
        return carry

    jax.lax.fori_loop(0, NE // 128, epi_body, 0)
    cp_oe = pltpu.make_async_copy(outv.at[:, 3], out_hbm.at[:, 3], sem_out.at[1])
    cp_oe.start()

    rm = rmat[...]
    tok = (jax.lax.broadcasted_iota(jnp.int32, (SEG, 128), 1) * SEG
           + jax.lax.broadcasted_iota(jnp.int32, (SEG, 128), 0))
    big = NSEG * SEG - 1
    i1 = jnp.min(jnp.where(rm == jnp.max(rm), tok, big))
    rm2 = jnp.where(tok == i1, -jnp.inf, rm)
    i2 = jnp.min(jnp.where((rm2 == jnp.max(rm2)) & (tok != i1), tok, big))
    i1 = jnp.clip(i1, 0, big)
    i2 = jnp.clip(i2, 0, big)
    g1, g2 = i1 // 8, i2 // 8
    x1 = jnp.concatenate([x1v[g1 // 4, pl.ds(g1 % 4, 1)], x1v[g2 // 4, pl.ds(g2 % 4, 1)]],
                         axis=0).astype(F32)
    h2, r = second(x1)
    for cp in cp_ffn:
        cp.wait()
    hl = h2.reshape(16, D).astype(BF16)
    act = []
    for j in range(FF // 128):
        gt = _rb(_dot(hl, wg[j]))
        up = _rb(_dot(hl, wu[j]))
        act.append((_rb(gt * jax.nn.sigmoid(gt)) * up).astype(BF16))
    act = jnp.concatenate(act, axis=1)
    y = jnp.concatenate([_dot(act, wd[n]) for n in range(8)], axis=1).reshape(2, 8, D)
    y = _rb(_rb(y) * _rb(jax.nn.sigmoid(r)))
    rowi = jax.lax.broadcasted_iota(jnp.int32, (2, 8, 1), 1)
    gsel = jax.lax.broadcasted_iota(jnp.int32, (2, 8, 1), 0)
    tokp = jnp.where(gsel == 0, g1, g2) * 8 + rowi
    upd = jnp.where((tokp == i1) | (tokp == i2), y, 0.0)
    patch[...] = (x1 + _rb(mod_vec(5) * _rb(h2 + upd))).astype(BF16)
    cp_oj.wait()
    cp_oe.wait()
    cp1 = pltpu.make_async_copy(patch.at[0], out_hbm.at[g1 // 4, g1 % 4], sem_out.at[0])
    cp1.start()

    @pl.when(g1 != g2)
    def _():
        cp2 = pltpu.make_async_copy(patch.at[1], out_hbm.at[g2 // 4, g2 % 4], sem_out.at[1])
        cp2.start()
        cp2.wait()

    cp1.wait()


@functools.partial(jax.jit, static_argnames=("A_seg_len",))
def pallas_adaLN_cond__memory_aug_recurrent_mem_tr__moe_arch_mod__prompt_kernel(
    A_x: jax.Array,
    A_mem0: jax.Array,
    A_Wq: jax.Array,
    A_Wk: jax.Array,
    A_Wv: jax.Array,
    A_Wo: jax.Array,
    A_seg_len,
    B_x: jax.Array,
    B_w_r: jax.Array,
    B_w_gate: jax.Array,
    B_w_up: jax.Array,
    B_w_down: jax.Array,
    c: jax.Array,
    w_mod: jax.Array,
):
    assert A_seg_len == SEG and A_x.shape == (1, NSEG * SEG, D)
    any_spec = pl.BlockSpec(memory_space=pl.ANY)
    vmem_spec = pl.BlockSpec(memory_space=pltpu.VMEM)
    out = pl.pallas_call(
        _kernel,
        out_shape=jax.ShapeDtypeStruct((NSEG, 4, 8, D), BF16),
        in_specs=[any_spec, vmem_spec, any_spec, any_spec, any_spec, any_spec, vmem_spec,
                  any_spec, any_spec, any_spec, vmem_spec, any_spec],
        out_specs=any_spec,
        scratch_shapes=[
            pltpu.VMEM((3 * H, D // 2, DH), U32),
            pltpu.VMEM((8, H * DH, 128), BF16),
            pltpu.VMEM((FF // 128, D, 128), BF16),
            pltpu.VMEM((FF // 128, D, 128), BF16),
            pltpu.VMEM((8, FF, 128), BF16),
            pltpu.VMEM((48, D, 128), BF16),
            pltpu.VMEM((NSEG, 4, 8, D), BF16),
            pltpu.VMEM((NSEG, 4, 8, D), BF16),
            pltpu.VMEM((NSEG, 4, 8, D), BF16),
            pltpu.VMEM((NSEG, 3 * NP, 16, DH), BF16),
            pltpu.VMEM((NE, H * DH), F32),
            pltpu.VMEM((NE, D), BF16),
            pltpu.VMEM((8, 128), F32),
            pltpu.VMEM((SEG, D), BF16),
            pltpu.VMEM((NJ, D), F32),
            pltpu.VMEM((8, 6 * D), F32),
            pltpu.VMEM((80, 128), F32),
            pltpu.VMEM((SEG, 128), F32),
            pltpu.VMEM((2, 8, D), BF16),
            pltpu.SemaphoreType.DMA((NP,)),
            pltpu.SemaphoreType.DMA((6,)),
            pltpu.SemaphoreType.DMA((2,)),
        ],
        compiler_params=pltpu.CompilerParams(vmem_limit_bytes=120 * 1024 * 1024),
    )(
        A_x.reshape(NSEG, 4, 8, D),
        A_mem0.reshape(M, D),
        A_Wq.reshape(D // 2, 2, H, DH),
        A_Wk.reshape(D // 2, 2, H, DH),
        A_Wv.reshape(D // 2, 2, H, DH),
        A_Wo.reshape(H * DH, D),
        B_w_r.reshape(1, D),
        B_w_gate,
        B_w_up,
        B_w_down,
        c,
        w_mod,
    )
    return out.reshape(1, NSEG * SEG, D)
```

```python
import functools

import jax
import jax.numpy as jnp
import jax.experimental.pallas as pl
import jax.experimental.pallas.tpu as pltpu

F32 = jnp.float32
BF16 = jnp.bfloat16
U32 = jnp.uint32

D = 1024
H = 32
DH = 128
NP = H // 2
M = 8
SEG = 32
NSEG = 64
FF = 3584
NJ = SEG - M
NE = NSEG * M
EPS = 1e-5
SCALE = DH ** (-0.5)
NEG = -1000000000.0


def _rb(x):
    return x.astype(BF16).astype(F32)


def _layernorm(xf):
    m = jnp.mean(xf, axis=-1, keepdims=True)
    d = xf - m
    v = jnp.mean(d * d, axis=-1, keepdims=True)
    return d * jax.lax.rsqrt(v + EPS)


def _dot(a, b):
    return jnp.dot(a, b, preferred_element_type=F32)


def _dot_nt(a, b):
    return jax.lax.dot_general(a, b, (((1,), (1,)), ((), ())), preferred_element_type=F32)


def _kernel(x_hbm, mem0_ref, wq_hbm, wk_hbm, wv_hbm, wo_hbm, wr_ref, wg_hbm, wu_hbm, wd_hbm,
            c_ref, wm_hbm,
            out_hbm,
            wq, wk, wv, wo, wg, wu, wd, wm, xv, x1v, outv, early, oe, he, lhs_ref, pend,
            mod, fill, rmat, patch,
            sem_pair, sem_misc, sem_out):
    w_u32 = [w.bitcast(U32) for w in (wq_hbm, wk_hbm, wv_hbm)]

    wqkv = (wq, wk, wv)

    def w_copies(m, p, sem):
        return [pltpu.make_async_copy(w_u32[m].at[:, par, p, :], wqkv[m].at[2 * p + par], sem)
                for par in range(2)]

    def group_copies(p, last=False):
        cps = w_copies(1, p, sem_pair.at[p]) + w_copies(2, p, sem_pair.at[p])
        if not last:
            cps += w_copies(0, p + 1, sem_pair.at[p])
        return cps

    def col_copy(src, dst, j, sem):
        if not isinstance(j, int):
            return pltpu.make_async_copy(src.at[:, pl.ds(pl.multiple_of(j * 128, 128), 128)],
                                         dst.at[j], sem)
        return pltpu.make_async_copy(src.at[:, pl.ds(j * 128, 128)], dst.at[j], sem)

    def col_copies(src, dst, lo, hi, sem):
        return [col_copy(src, dst, j, sem) for j in range(lo, hi)]

    cp_xe = [pltpu.make_async_copy(x_hbm.at[:, 3], xv.at[:, 3], sem_misc.at[0])]
    cp_wm1 = col_copies(wm_hbm, wm, 0, 16, sem_misc.at[1])
    cp_xj = [pltpu.make_async_copy(x_hbm.at[:, 0:3], xv.at[:, 0:3], sem_misc.at[2])]
    cp_wo = col_copies(wo_hbm, wo, 0, 8, sem_misc.at[3])
    cp_wm2 = col_copies(wm_hbm, wm, 16, 48, sem_misc.at[4])
    cp_ffn = (col_copies(wg_hbm, wg, 0, FF // 128, sem_misc.at[5])
              + col_copies(wu_hbm, wu, 0, FF // 128, sem_misc.at[5])
              + col_copies(wd_hbm, wd, 0, 8, sem_misc.at[5]))

    cp_q0 = w_copies(0, 0, sem_misc.at[6])
    AHEAD = 3
    for cp in cp_xe + cp_wm1 + cp_q0:
        cp.start()
    for p in range(AHEAD):
        for cp in group_copies(p):
            cp.start()
    for cp in cp_xj:
        cp.start()

    ri = jax.lax.broadcasted_iota(jnp.int32, (80, 128), 0)
    ci = jax.lax.broadcasted_iota(jnp.int32, (80, 128), 1)

    def head_of(i):
        return jnp.where(i < 64, i // 32, (i - 64) // 8)

    def pos_of(i):
        return jnp.where(i < 64, i % 32, 32 + i % 8)

    same = (head_of(ri) == head_of(ci)) & (ci < 80)
    allowed = (pos_of(ri) < M) | (pos_of(ri) >= pos_of(ci))
    fill[...] = jnp.where(same, jnp.where(allowed, 0.0, NEG), -jnp.inf).astype(F32)
    rmat[...] = jnp.full(rmat.shape, -jnp.inf, F32)
    pend[...] = jnp.zeros(pend.shape, F32)

    cf = c_ref[...].astype(F32)
    sc = _rb(cf * jax.nn.sigmoid(cf))
    sc = jnp.broadcast_to(sc, (16, D)).astype(BF16)

    def mod_cols(lo, hi):
        for j in range(lo, hi):
            v = _rb(_dot(sc, wm[j])[0:8])
            if j // 8 in (1, 4):
                v = _rb(1.0 + v)
            mod[:, j * 128:(j + 1) * 128] = v

    def mod_vec(k):
        return mod[:, k * D:(k + 1) * D]

    def modulate1(xb):
        n = _rb(_layernorm(xb.astype(F32)))
        return _rb(n * mod_vec(1)) + mod_vec(0)

    for cp in cp_wm1:
        cp.wait()
    mod_cols(0, 16)
    for cp in cp_xe:
        cp.wait()

    def he_body(i, carry):
        hh = modulate1(xv[pl.ds(i * 8, 8), 3])
        he[pl.ds(pl.multiple_of(i * 64, 64), 64), :] = hh.reshape(64, D).astype(BF16)
        return carry

    with jax.named_scope("he_loop"):
        jax.lax.fori_loop(0, NSEG // 8, he_body, 0)

    def relayout(m, p):
        w = wqkv[m]
        e = w[2 * p]
        o = w[2 * p + 1]
        w[2 * p] = (e & U32(0xFFFF)) | (o << 16)
        w[2 * p + 1] = (e >> 16) | (o & U32(0xFFFF0000))

    def w_head(m, h):
        return pltpu.bitcast(wqkv[m][h], BF16)

    def early_proj(m, p):
        for c in range(2):
            hc = he[c * 256:(c + 1) * 256, :]
            r1 = _dot(hc, w_head(m, 2 * p)).reshape(32, 8, DH)
            r2 = _dot(hc, w_head(m, 2 * p + 1)).reshape(32, 8, DH)
            early[c * 32:(c + 1) * 32, m * NP + p] = (
                jnp.concatenate([r1, r2], axis=1).astype(BF16))

    def pro_compute(p, last=False):
        for cp in group_copies(p, last):
            cp.wait()
        relayout(1, p)
        early_proj(0, p)
        relayout(2, p)
        early_proj(1, p)
        if not last:
            relayout(0, p + 1)
        early_proj(2, p)

    for cp in cp_q0:
        cp.wait()
    relayout(0, 0)

    def pro_body(p, carry):
        @pl.when(p + AHEAD < NP - 1)
        def _():
            for cp in group_copies(p + AHEAD):
                cp.start()

        @pl.when(p + AHEAD == NP - 1)
        def _():
            for cp in group_copies(NP - 1, last=True):
                cp.start()

        @pl.when(p < 8)
        def _():
            col_copy(wo_hbm, wo, p, sem_misc.at[3]).start()

        @pl.when(p >= NP - 1 - 8)
        def _():
            for j in range(4):
                col_copy(wm_hbm, wm, 16 + (p - (NP - 1 - 8)) * 4 + j, sem_misc.at[4]).start()

        pro_compute(p)
        return carry

    with jax.named_scope("prologue_loop"):
        jax.lax.fori_loop(0, NP - 1, pro_body, 0)
    for cp in cp_xj + cp_wo + cp_wm2:
        cp.wait()
    for cp in cp_ffn[:56]:
        cp.start()
    pro_compute(NP - 1, last=True)
    mod_cols(16, 48)
    lhs_ref[...] = jnp.concatenate(
        [mem0_ref[...].astype(F32), modulate1(xv[0, 0:3]).reshape(NJ, D)], axis=0).astype(BF16)

    for cp in cp_ffn[56:]:
        cp.start()

    wr = jnp.broadcast_to(wr_ref[...].astype(F32), (8, D))

    def second(x1):
        n = _rb(_layernorm(x1))
        h2 = _rb(_rb(n * mod_vec(4)) + mod_vec(3))
        r = _rb(jnp.sum(h2 * wr, axis=-1, keepdims=True))
        return h2, r

    def post(xb, attn):
        x1 = _rb(xb.astype(F32) + _rb(mod_vec(2) * _rb(attn)))
        h2, r = second(x1)
        out = x1 + _rb(mod_vec(5) * h2)
        return x1.astype(BF16), out.astype(BF16), r

    lane8 = jax.lax.broadcasted_iota(jnp.int32, (8, 128), 1)

    def post_j(s):
        x1, out, r = post(xv[s, 0:3], pend[...].reshape(3, 8, D))
        x1v[s, 0:3] = x1
        outv[s, 0:3] = out
        for g in range(3):
            rmat[g * 8:(g + 1) * 8, :] = jnp.where(lane8 == s, r[g], rmat[g * 8:(g + 1) * 8, :])

    zpad = jnp.zeros((48, DH), BF16)

    def step(s, carry):
        lhs = lhs_ref[...]
        post_j(jnp.maximum(s - 1, 0))
        hj_next = modulate1(xv[jnp.minimum(s + 1, NSEG - 1), 0:3]).reshape(NJ, D)

        def qkv(p):
            res = []
            for m in range(3):
                a = _dot(lhs, w_head(m, 2 * p)).astype(BF16)
                b = _dot(lhs, w_head(m, 2 * p + 1)).astype(BF16)
                parts = [a, b, early[s, m * NP + p]]
                if m > 0:
                    parts.append(zpad)
                res.append(jnp.concatenate(parts, axis=0))
            return res

        def scores(q, k):
            sc_ = _dot_nt(q, k) * SCALE
            f = fill[...]
            sc_ = jnp.where(f == 0.0, sc_, f)
            mx = jnp.max(sc_, axis=-1, keepdims=True)
            e = jnp.exp(sc_ - mx)
            return e.astype(BF16), 1.0 / jnp.sum(e, axis=-1, keepdims=True)

        def pv(p, pr, v):
            o = _dot(pr[0], v) * pr[1]
            row = pl.multiple_of(s * 8, 8)
            oe[pl.ds(row, 8), (2 * p) * DH:(2 * p + 1) * DH] = o[64:72]
            oe[pl.ds(row, 8), (2 * p + 1) * DH:(2 * p + 2) * DH] = o[72:80]
            return [o[0:32].astype(BF16), o[32:64].astype(BF16)]

        qkvs, probs, os_ = {}, {}, []
        for p in range(NP):
            qkvs[p] = qkv(p)
            if p >= 1:
                probs[p - 1] = scores(qkvs[p - 1][0], qkvs[p - 1][1])
            if p >= 2:
                os_ += pv(p - 2, probs[p - 2], qkvs[p - 2][2])
        ka = (NP - 2) * 2 * DH
        oa = jnp.concatenate(os_, axis=1)
        acc = []
        for n in range(8):
            acc.append(_dot(oa, wo[n, 0:ka, :]))
            if n == 1:
                probs[NP - 1] = scores(qkvs[NP - 1][0], qkvs[NP - 1][1])
                ob = pv(NP - 2, probs[NP - 2], qkvs[NP - 2][2])
            if n == 4:
                ob += pv(NP - 1, probs[NP - 1], qkvs[NP - 1][2])
        ob = jnp.concatenate(ob, axis=1)
        res = jnp.concatenate([_dot(ob, wo[n, ka:H * DH, :]) + acc[n] for n in range(8)], axis=1)
        pend[...] = res[M:SEG]
        lhs_ref[...] = jnp.concatenate([res[0:M], hj_next], axis=0).astype(BF16)
        return carry

    with jax.named_scope("main_loop"):
        jax.lax.fori_loop(0, NSEG, step, 0)

    post_j(NSEG - 1)
    cp_oj = pltpu.make_async_copy(outv.at[:, 0:3], out_hbm.at[:, 0:3], sem_out.at[0])
    cp_oj.start()

    def epi_body(c, carry):
        row = pl.multiple_of(c * 128, 128)
        ol = oe[pl.ds(row, 128), :].astype(BF16)
        res = jnp.concatenate([_dot(ol, wo[n]) for n in range(8)], axis=1)
        sg = pl.multiple_of(c * 16, 16)
        x1, out, r = post(xv[pl.ds(sg, 16), 3], res.reshape(16, 8, D))
        x1v[pl.ds(sg, 16), 3] = x1
        outv[pl.ds(sg, 16), 3] = out
        rm = rmat[24:32, :]
        for g in range(16):
            rm = jnp.where(lane8 == sg + g, r[g], rm)
        rmat[24:32, :] = rm
        return carry

    with jax.named_scope("epilogue_loop"):
        jax.lax.fori_loop(0, NE // 128, epi_body, 0)
    cp_oe = pltpu.make_async_copy(outv.at[:, 3], out_hbm.at[:, 3], sem_out.at[1])
    cp_oe.start()

    rm = rmat[...]
    tok = (jax.lax.broadcasted_iota(jnp.int32, (SEG, 128), 1) * SEG
           + jax.lax.broadcasted_iota(jnp.int32, (SEG, 128), 0))
    big = NSEG * SEG - 1
    i1 = jnp.min(jnp.where(rm == jnp.max(rm), tok, big))
    rm2 = jnp.where(tok == i1, -jnp.inf, rm)
    i2 = jnp.min(jnp.where((rm2 == jnp.max(rm2)) & (tok != i1), tok, big))
    i1 = jnp.clip(i1, 0, big)
    i2 = jnp.clip(i2, 0, big)
    g1, g2 = i1 // 8, i2 // 8
    x1 = jnp.concatenate([x1v[g1 // 4, pl.ds(g1 % 4, 1)], x1v[g2 // 4, pl.ds(g2 % 4, 1)]],
                         axis=0).astype(F32)
    h2, r = second(x1)
    for cp in cp_ffn:
        cp.wait()
    hl = h2.reshape(16, D).astype(BF16)
    act = []
    for j in range(FF // 128):
        gt = _rb(_dot(hl, wg[j]))
        up = _rb(_dot(hl, wu[j]))
        act.append((_rb(gt * jax.nn.sigmoid(gt)) * up).astype(BF16))
    act = jnp.concatenate(act, axis=1)
    y = jnp.concatenate([_dot(act, wd[n]) for n in range(8)], axis=1).reshape(2, 8, D)
    y = _rb(_rb(y) * _rb(jax.nn.sigmoid(r)))
    rowi = jax.lax.broadcasted_iota(jnp.int32, (2, 8, 1), 1)
    gsel = jax.lax.broadcasted_iota(jnp.int32, (2, 8, 1), 0)
    tokp = jnp.where(gsel == 0, g1, g2) * 8 + rowi
    upd = jnp.where((tokp == i1) | (tokp == i2), y, 0.0)
    patch[...] = (x1 + _rb(mod_vec(5) * _rb(h2 + upd))).astype(BF16)
    cp_oj.wait()
    cp_oe.wait()
    cp1 = pltpu.make_async_copy(patch.at[0], out_hbm.at[g1 // 4, g1 % 4], sem_out.at[0])
    cp1.start()

    @pl.when(g1 != g2)
    def _():
        cp2 = pltpu.make_async_copy(patch.at[1], out_hbm.at[g2 // 4, g2 % 4], sem_out.at[1])
        cp2.start()
        cp2.wait()

    cp1.wait()


@functools.partial(jax.jit, static_argnames=("A_seg_len",))
def pallas_adaLN_cond__memory_aug_recurrent_mem_tr__moe_arch_mod__prompt_kernel(
    A_x: jax.Array,
    A_mem0: jax.Array,
    A_Wq: jax.Array,
    A_Wk: jax.Array,
    A_Wv: jax.Array,
    A_Wo: jax.Array,
    A_seg_len,
    B_x: jax.Array,
    B_w_r: jax.Array,
    B_w_gate: jax.Array,
    B_w_up: jax.Array,
    B_w_down: jax.Array,
    c: jax.Array,
    w_mod: jax.Array,
):
    assert A_seg_len == SEG and A_x.shape == (1, NSEG * SEG, D)
    any_spec = pl.BlockSpec(memory_space=pl.ANY)
    vmem_spec = pl.BlockSpec(memory_space=pltpu.VMEM)
    out = pl.pallas_call(
        _kernel,
        out_shape=jax.ShapeDtypeStruct((NSEG, 4, 8, D), BF16),
        in_specs=[any_spec, vmem_spec, any_spec, any_spec, any_spec, any_spec, vmem_spec,
                  any_spec, any_spec, any_spec, vmem_spec, any_spec],
        out_specs=any_spec,
        scratch_shapes=[
            pltpu.VMEM((H, D // 2, DH), U32),
            pltpu.VMEM((H, D // 2, DH), U32),
            pltpu.VMEM((H, D // 2, DH), U32),
            pltpu.VMEM((8, H * DH, 128), BF16),
            pltpu.VMEM((FF // 128, D, 128), BF16),
            pltpu.VMEM((FF // 128, D, 128), BF16),
            pltpu.VMEM((8, FF, 128), BF16),
            pltpu.VMEM((48, D, 128), BF16),
            pltpu.VMEM((NSEG, 4, 8, D), BF16),
            pltpu.VMEM((NSEG, 4, 8, D), BF16),
            pltpu.VMEM((NSEG, 4, 8, D), BF16),
            pltpu.VMEM((NSEG, 3 * NP, 16, DH), BF16),
            pltpu.VMEM((NE, H * DH), F32),
            pltpu.VMEM((NE, D), BF16),
            pltpu.VMEM((SEG, D), BF16),
            pltpu.VMEM((NJ, D), F32),
            pltpu.VMEM((8, 6 * D), F32),
            pltpu.VMEM((80, 128), F32),
            pltpu.VMEM((SEG, 128), F32),
            pltpu.VMEM((2, 8, D), BF16),
            pltpu.SemaphoreType.DMA((NP,)),
            pltpu.SemaphoreType.DMA((7,)),
            pltpu.SemaphoreType.DMA((2,)),
        ],
        compiler_params=pltpu.CompilerParams(vmem_limit_bytes=120 * 1024 * 1024),
    )(
        A_x.reshape(NSEG, 4, 8, D),
        A_mem0.reshape(M, D),
        A_Wq.reshape(D // 2, 2, H, DH),
        A_Wk.reshape(D // 2, 2, H, DH),
        A_Wv.reshape(D // 2, 2, H, DH),
        A_Wo.reshape(H * DH, D),
        B_w_r.reshape(1, D),
        B_w_gate,
        B_w_up,
        B_w_down,
        c,
        w_mod,
    )
    return out.reshape(1, NSEG * SEG, D)
```

```python
import functools

import jax
import jax.numpy as jnp
import jax.experimental.pallas as pl
import jax.experimental.pallas.tpu as pltpu

F32 = jnp.float32
BF16 = jnp.bfloat16
U32 = jnp.uint32

D = 1024
H = 32
DH = 128
NP = H // 2
M = 8
SEG = 32
NSEG = 64
FF = 3584
NJ = SEG - M
NE = NSEG * M
EPS = 1e-5
SCALE = DH ** (-0.5)
NEG = -1000000000.0


def _rb(x):
    return x.astype(BF16).astype(F32)


def _layernorm(xf):
    m = jnp.mean(xf, axis=-1, keepdims=True)
    d = xf - m
    v = jnp.mean(d * d, axis=-1, keepdims=True)
    return d * jax.lax.rsqrt(v + EPS)


def _dot(a, b):
    return jnp.dot(a, b, preferred_element_type=F32)


def _dot_nt(a, b):
    return jax.lax.dot_general(a, b, (((1,), (1,)), ((), ())), preferred_element_type=F32)


def _kernel(x_hbm, mem0_ref, wq_hbm, wk_hbm, wv_hbm, wo_hbm, wr_ref, wg_hbm, wu_hbm, wd_hbm,
            c_ref, wm_hbm,
            out_hbm,
            wq, wk, wv, wo, wg, wu, wd, wm, xv, x1v, outv, early, oe, he, lhs_ref, pend,
            mod, fill, rmat, patch,
            sem_pair, sem_misc, sem_out):
    w_u32 = [w.bitcast(U32) for w in (wq_hbm, wk_hbm, wv_hbm)]

    wqkv = (wq, wk, wv)
    wo_hbm, wg_hbm, wu_hbm, wd_hbm, wm_hbm = [
        w.bitcast(U32) for w in (wo_hbm, wg_hbm, wu_hbm, wd_hbm, wm_hbm)]

    def wblk(w, j, lo=None, hi=None):
        v = w[j] if lo is None else w[j, lo // 2:hi // 2, :]
        return pltpu.bitcast(v, BF16)

    def w_copies(m, p, sem):
        return [pltpu.make_async_copy(w_u32[m].at[:, par, p, :], wqkv[m].at[2 * p + par], sem)
                for par in range(2)]

    def group_copies(p, last=False):
        cps = w_copies(1, p, sem_pair.at[p]) + w_copies(2, p, sem_pair.at[p])
        if not last:
            cps += w_copies(0, p + 1, sem_pair.at[p])
        return cps

    def col_copy(src, dst, j, sem):
        if not isinstance(j, int):
            return pltpu.make_async_copy(src.at[:, pl.ds(pl.multiple_of(j * 128, 128), 128)],
                                         dst.at[j], sem)
        return pltpu.make_async_copy(src.at[:, pl.ds(j * 128, 128)], dst.at[j], sem)

    def col_copies(src, dst, lo, hi, sem):
        return [col_copy(src, dst, j, sem) for j in range(lo, hi)]

    cp_xe = [pltpu.make_async_copy(x_hbm.at[:, 3], xv.at[:, 3], sem_misc.at[0])]
    cp_wm1 = col_copies(wm_hbm, wm, 0, 16, sem_misc.at[1])
    cp_xj = [pltpu.make_async_copy(x_hbm.at[:, 0:3], xv.at[:, 0:3], sem_misc.at[2])]
    cp_wo = col_copies(wo_hbm, wo, 0, 8, sem_misc.at[3])
    cp_wm2 = col_copies(wm_hbm, wm, 16, 48, sem_misc.at[4])
    cp_ffn = (col_copies(wg_hbm, wg, 0, FF // 128, sem_misc.at[5])
              + col_copies(wu_hbm, wu, 0, FF // 128, sem_misc.at[5])
              + col_copies(wd_hbm, wd, 0, 8, sem_misc.at[5]))

    cp_q0 = w_copies(0, 0, sem_misc.at[6])
    AHEAD = 3
    for cp in cp_xe + cp_wm1 + cp_q0:
        cp.start()
    for p in range(AHEAD):
        for cp in group_copies(p):
            cp.start()
    for cp in cp_xj:
        cp.start()

    ri = jax.lax.broadcasted_iota(jnp.int32, (80, 128), 0)
    ci = jax.lax.broadcasted_iota(jnp.int32, (80, 128), 1)

    def head_of(i):
        return jnp.where(i < 64, i // 32, (i - 64) // 8)

    def pos_of(i):
        return jnp.where(i < 64, i % 32, 32 + i % 8)

    same = (head_of(ri) == head_of(ci)) & (ci < 80)
    allowed = (pos_of(ri) < M) | (pos_of(ri) >= pos_of(ci))
    fill[...] = jnp.where(same, jnp.where(allowed, 0.0, NEG), -jnp.inf).astype(F32)
    rmat[...] = jnp.full(rmat.shape, -jnp.inf, F32)
    pend[...] = jnp.zeros(pend.shape, F32)

    cf = c_ref[...].astype(F32)
    sc = _rb(cf * jax.nn.sigmoid(cf))
    sc = jnp.broadcast_to(sc, (16, D)).astype(BF16)

    def mod_cols(lo, hi):
        for j in range(lo, hi):
            v = _rb(_dot(sc, wblk(wm, j))[0:8])
            if j // 8 in (1, 4):
                v = _rb(1.0 + v)
            mod[:, j * 128:(j + 1) * 128] = v

    def mod_vec(k):
        return mod[:, k * D:(k + 1) * D]

    def modulate1(xb):
        n = _rb(_layernorm(xb.astype(F32)))
        return _rb(n * mod_vec(1)) + mod_vec(0)

    for cp in cp_wm1:
        cp.wait()
    mod_cols(0, 16)
    for cp in cp_xe:
        cp.wait()

    def he_body(i, carry):
        hh = modulate1(xv[pl.ds(i * 8, 8), 3])
        he[pl.ds(pl.multiple_of(i * 64, 64), 64), :] = hh.reshape(64, D).astype(BF16)
        return carry

    with jax.named_scope("he_loop"):
        jax.lax.fori_loop(0, NSEG // 8, he_body, 0)

    def relayout(m, p):
        w = wqkv[m]
        e = w[2 * p]
        o = w[2 * p + 1]
        w[2 * p] = (e & U32(0xFFFF)) | (o << 16)
        w[2 * p + 1] = (e >> 16) | (o & U32(0xFFFF0000))

    def w_head(m, h):
        return pltpu.bitcast(wqkv[m][h], BF16)

    def early_proj(m, p):
        for c in range(2):
            hc = he[c * 256:(c + 1) * 256, :]
            r1 = _dot(hc, w_head(m, 2 * p)).reshape(32, 8, DH)
            r2 = _dot(hc, w_head(m, 2 * p + 1)).reshape(32, 8, DH)
            early[c * 32:(c + 1) * 32, m * NP + p] = (
                jnp.concatenate([r1, r2], axis=1).astype(BF16))

    def pro_compute(p, last=False):
        for cp in group_copies(p, last):
            cp.wait()
        relayout(1, p)
        early_proj(0, p)
        relayout(2, p)
        early_proj(1, p)
        if not last:
            relayout(0, p + 1)
        early_proj(2, p)

    for cp in cp_q0:
        cp.wait()
    relayout(0, 0)

    def pro_body(p, carry):
        @pl.when(p + AHEAD < NP - 1)
        def _():
            for cp in group_copies(p + AHEAD):
                cp.start()

        @pl.when(p + AHEAD == NP - 1)
        def _():
            for cp in group_copies(NP - 1, last=True):
                cp.start()

        @pl.when(p < 8)
        def _():
            col_copy(wo_hbm, wo, p, sem_misc.at[3]).start()

        @pl.when(p >= NP - 1 - 8)
        def _():
            for j in range(4):
                col_copy(wm_hbm, wm, 16 + (p - (NP - 1 - 8)) * 4 + j, sem_misc.at[4]).start()

        pro_compute(p)
        return carry

    with jax.named_scope("prologue_loop"):
        jax.lax.fori_loop(0, NP - 1, pro_body, 0)
    for cp in cp_xj + cp_wo + cp_wm2:
        cp.wait()
    for cp in cp_ffn[:56]:
        cp.start()
    pro_compute(NP - 1, last=True)
    mod_cols(16, 48)
    lhs_ref[...] = jnp.concatenate(
        [mem0_ref[...].astype(F32), modulate1(xv[0, 0:3]).reshape(NJ, D)], axis=0).astype(BF16)

    for cp in cp_ffn[56:]:
        cp.start()

    wr = jnp.broadcast_to(wr_ref[...].astype(F32), (8, D))

    def second(x1):
        n = _rb(_layernorm(x1))
        h2 = _rb(_rb(n * mod_vec(4)) + mod_vec(3))
        r = _rb(jnp.sum(h2 * wr, axis=-1, keepdims=True))
        return h2, r

    def post(xb, attn):
        x1 = _rb(xb.astype(F32) + _rb(mod_vec(2) * _rb(attn)))
        h2, r = second(x1)
        out = x1 + _rb(mod_vec(5) * h2)
        return x1.astype(BF16), out.astype(BF16), r

    lane8 = jax.lax.broadcasted_iota(jnp.int32, (8, 128), 1)

    def post_j(s):
        x1, out, r = post(xv[s, 0:3], pend[...].reshape(3, 8, D))
        x1v[s, 0:3] = x1
        outv[s, 0:3] = out
        for g in range(3):
            rmat[g * 8:(g + 1) * 8, :] = jnp.where(lane8 == s, r[g], rmat[g * 8:(g + 1) * 8, :])

    zpad = jnp.zeros((48, DH), BF16)

    def step(s, carry):
        lhs = lhs_ref[...]
        post_j(jnp.maximum(s - 1, 0))
        hj_next = modulate1(xv[jnp.minimum(s + 1, NSEG - 1), 0:3]).reshape(NJ, D)

        def qkv(p):
            res = []
            for m in range(3):
                a = _dot(lhs, w_head(m, 2 * p)).astype(BF16)
                b = _dot(lhs, w_head(m, 2 * p + 1)).astype(BF16)
                parts = [a, b, early[s, m * NP + p]]
                if m > 0:
                    parts.append(zpad)
                res.append(jnp.concatenate(parts, axis=0))
            return res

        def scores(q, k):
            sc_ = _dot_nt(q, k) * SCALE
            f = fill[...]
            sc_ = jnp.where(f == 0.0, sc_, f)
            mx = jnp.max(sc_, axis=-1, keepdims=True)
            e = jnp.exp(sc_ - mx)
            den = jnp.sum(e, axis=-1, keepdims=True)
            inv = pl.reciprocal(den, approx=True)
            return e.astype(BF16), inv * (2.0 - den * inv)

        def pv(p, pr, v):
            o = _dot(pr[0], v) * pr[1]
            row = pl.multiple_of(s * 8, 8)
            oe[pl.ds(row, 8), (2 * p) * DH:(2 * p + 1) * DH] = o[64:72]
            oe[pl.ds(row, 8), (2 * p + 1) * DH:(2 * p + 2) * DH] = o[72:80]
            return [o[0:32].astype(BF16), o[32:64].astype(BF16)]

        qkvs, probs, os_ = {}, {}, []
        for p in range(NP):
            qkvs[p] = qkv(p)
            if p >= 1:
                probs[p - 1] = scores(qkvs[p - 1][0], qkvs[p - 1][1])
            if p >= 2:
                os_ += pv(p - 2, probs[p - 2], qkvs[p - 2][2])
        ka = (NP - 2) * 2 * DH
        oa = jnp.concatenate(os_, axis=1)
        acc = []
        for n in range(8):
            acc.append(_dot(oa, wblk(wo, n, 0, ka)))
            if n == 1:
                probs[NP - 1] = scores(qkvs[NP - 1][0], qkvs[NP - 1][1])
                ob = pv(NP - 2, probs[NP - 2], qkvs[NP - 2][2])
            if n == 4:
                ob += pv(NP - 1, probs[NP - 1], qkvs[NP - 1][2])
        ob = jnp.concatenate(ob, axis=1)
        res = jnp.concatenate([_dot(ob, wblk(wo, n, ka, H * DH)) + acc[n] for n in range(8)], axis=1)
        pend[...] = res[M:SEG]
        lhs_ref[...] = jnp.concatenate([res[0:M], hj_next], axis=0).astype(BF16)
        return carry

    with jax.named_scope("main_loop"):
        jax.lax.fori_loop(0, NSEG, step, 0)

    post_j(NSEG - 1)
    cp_oj = pltpu.make_async_copy(outv.at[:, 0:3], out_hbm.at[:, 0:3], sem_out.at[0])
    cp_oj.start()

    def epi_body(c, carry):
        row = pl.multiple_of(c * 128, 128)
        ol = oe[pl.ds(row, 128), :].astype(BF16)
        res = jnp.concatenate([_dot(ol, wblk(wo, n)) for n in range(8)], axis=1)
        sg = pl.multiple_of(c * 16, 16)
        x1, out, r = post(xv[pl.ds(sg, 16), 3], res.reshape(16, 8, D))
        x1v[pl.ds(sg, 16), 3] = x1
        outv[pl.ds(sg, 16), 3] = out
        rm = rmat[24:32, :]
        for g in range(16):
            rm = jnp.where(lane8 == sg + g, r[g], rm)
        rmat[24:32, :] = rm
        return carry

    with jax.named_scope("epilogue_loop"):
        jax.lax.fori_loop(0, NE // 128, epi_body, 0)
    cp_oe = pltpu.make_async_copy(outv.at[:, 3], out_hbm.at[:, 3], sem_out.at[1])
    cp_oe.start()

    rm = rmat[...]
    tok = (jax.lax.broadcasted_iota(jnp.int32, (SEG, 128), 1) * SEG
           + jax.lax.broadcasted_iota(jnp.int32, (SEG, 128), 0))
    big = NSEG * SEG - 1
    i1 = jnp.min(jnp.where(rm == jnp.max(rm), tok, big))
    rm2 = jnp.where(tok == i1, -jnp.inf, rm)
    i2 = jnp.min(jnp.where((rm2 == jnp.max(rm2)) & (tok != i1), tok, big))
    i1 = jnp.clip(i1, 0, big)
    i2 = jnp.clip(i2, 0, big)
    g1, g2 = i1 // 8, i2 // 8
    x1 = jnp.concatenate([x1v[g1 // 4, pl.ds(g1 % 4, 1)], x1v[g2 // 4, pl.ds(g2 % 4, 1)]],
                         axis=0).astype(F32)
    h2, r = second(x1)
    for cp in cp_ffn:
        cp.wait()
    hl = h2.reshape(16, D).astype(BF16)
    act = []
    for j in range(FF // 128):
        gt = _rb(_dot(hl, wblk(wg, j)))
        up = _rb(_dot(hl, wblk(wu, j)))
        act.append((_rb(gt * jax.nn.sigmoid(gt)) * up).astype(BF16))
    act = jnp.concatenate(act, axis=1)
    y = jnp.concatenate([_dot(act, wblk(wd, n)) for n in range(8)], axis=1).reshape(2, 8, D)
    y = _rb(_rb(y) * _rb(jax.nn.sigmoid(r)))
    rowi = jax.lax.broadcasted_iota(jnp.int32, (2, 8, 1), 1)
    gsel = jax.lax.broadcasted_iota(jnp.int32, (2, 8, 1), 0)
    tokp = jnp.where(gsel == 0, g1, g2) * 8 + rowi
    upd = jnp.where((tokp == i1) | (tokp == i2), y, 0.0)
    patch[...] = (x1 + _rb(mod_vec(5) * _rb(h2 + upd))).astype(BF16)
    cp_oj.wait()
    cp_oe.wait()
    cp1 = pltpu.make_async_copy(patch.at[0], out_hbm.at[g1 // 4, g1 % 4], sem_out.at[0])
    cp1.start()

    @pl.when(g1 != g2)
    def _():
        cp2 = pltpu.make_async_copy(patch.at[1], out_hbm.at[g2 // 4, g2 % 4], sem_out.at[1])
        cp2.start()
        cp2.wait()

    cp1.wait()


@functools.partial(jax.jit, static_argnames=("A_seg_len",))
def pallas_adaLN_cond__memory_aug_recurrent_mem_tr__moe_arch_mod__prompt_kernel(
    A_x: jax.Array,
    A_mem0: jax.Array,
    A_Wq: jax.Array,
    A_Wk: jax.Array,
    A_Wv: jax.Array,
    A_Wo: jax.Array,
    A_seg_len,
    B_x: jax.Array,
    B_w_r: jax.Array,
    B_w_gate: jax.Array,
    B_w_up: jax.Array,
    B_w_down: jax.Array,
    c: jax.Array,
    w_mod: jax.Array,
):
    assert A_seg_len == SEG and A_x.shape == (1, NSEG * SEG, D)
    any_spec = pl.BlockSpec(memory_space=pl.ANY)
    vmem_spec = pl.BlockSpec(memory_space=pltpu.VMEM)
    out = pl.pallas_call(
        _kernel,
        out_shape=jax.ShapeDtypeStruct((NSEG, 4, 8, D), BF16),
        in_specs=[any_spec, vmem_spec, any_spec, any_spec, any_spec, any_spec, vmem_spec,
                  any_spec, any_spec, any_spec, vmem_spec, any_spec],
        out_specs=any_spec,
        scratch_shapes=[
            pltpu.VMEM((H, D // 2, DH), U32),
            pltpu.VMEM((H, D // 2, DH), U32),
            pltpu.VMEM((H, D // 2, DH), U32),
            pltpu.VMEM((8, H * DH // 2, 128), U32),
            pltpu.VMEM((FF // 128, D // 2, 128), U32),
            pltpu.VMEM((FF // 128, D // 2, 128), U32),
            pltpu.VMEM((8, FF // 2, 128), U32),
            pltpu.VMEM((48, D // 2, 128), U32),
            pltpu.VMEM((NSEG, 4, 8, D), BF16),
            pltpu.VMEM((NSEG, 4, 8, D), BF16),
            pltpu.VMEM((NSEG, 4, 8, D), BF16),
            pltpu.VMEM((NSEG, 3 * NP, 16, DH), BF16),
            pltpu.VMEM((NE, H * DH), F32),
            pltpu.VMEM((NE, D), BF16),
            pltpu.VMEM((SEG, D), BF16),
            pltpu.VMEM((NJ, D), F32),
            pltpu.VMEM((8, 6 * D), F32),
            pltpu.VMEM((80, 128), F32),
            pltpu.VMEM((SEG, 128), F32),
            pltpu.VMEM((2, 8, D), BF16),
            pltpu.SemaphoreType.DMA((NP,)),
            pltpu.SemaphoreType.DMA((7,)),
            pltpu.SemaphoreType.DMA((2,)),
        ],
        compiler_params=pltpu.CompilerParams(vmem_limit_bytes=120 * 1024 * 1024),
    )(
        A_x.reshape(NSEG, 4, 8, D),
        A_mem0.reshape(M, D),
        A_Wq.reshape(D // 2, 2, H, DH),
        A_Wk.reshape(D // 2, 2, H, DH),
        A_Wv.reshape(D // 2, 2, H, DH),
        A_Wo.reshape(H * DH, D),
        B_w_r.reshape(1, D),
        B_w_gate,
        B_w_up,
        B_w_down,
        c,
        w_mod,
    )
    return out.reshape(1, NSEG * SEG, D)
```

```python
import functools

import jax
import jax.numpy as jnp
import jax.experimental.pallas as pl
import jax.experimental.pallas.tpu as pltpu

F32 = jnp.float32
BF16 = jnp.bfloat16
U32 = jnp.uint32

D = 1024
H = 32
DH = 128
NP = H // 2
M = 8
SEG = 32
NSEG = 64
FF = 3584
NJ = SEG - M
NE = NSEG * M
EPS = 1e-5
SCALE = DH ** (-0.5)
NEG = -1000000000.0
OUT_SPLIT = 58


def _rb(x):
    return x.astype(BF16).astype(F32)


def _layernorm(xf):
    m = jnp.mean(xf, axis=-1, keepdims=True)
    d = xf - m
    v = jnp.mean(d * d, axis=-1, keepdims=True)
    return d * jax.lax.rsqrt(v + EPS)


def _dot(a, b):
    return jnp.dot(a, b, preferred_element_type=F32)


def _dot_nt(a, b):
    return jax.lax.dot_general(a, b, (((1,), (1,)), ((), ())), preferred_element_type=F32)


def _kernel(x_hbm, mem0_ref, wq_hbm, wk_hbm, wv_hbm, wo_hbm, wr_ref, wg_hbm, wu_hbm, wd_hbm,
            c_ref, wm_hbm,
            out_hbm,
            wq, wk, wv, wo, wg, wu, wd, wm, xv, x1v, outv, early, he, hj, lhs_ref, pend,
            mod, fill, rmat, patch, zero,
            sem_pair, sem_misc, sem_out):
    w_u32 = [w.bitcast(U32) for w in (wq_hbm, wk_hbm, wv_hbm)]
    wqkv = (wq, wk, wv)
    wo_hbm, wg_hbm, wu_hbm, wd_hbm, wm_hbm = [
        w.bitcast(U32) for w in (wo_hbm, wg_hbm, wu_hbm, wd_hbm, wm_hbm)]

    def wblk(w, j, lo=None, hi=None):
        rows = slice(None) if lo is None else slice(lo // 2, hi // 2)
        return pltpu.bitcast(w[rows, j * 128:(j + 1) * 128], BF16)

    def wm_copy(lo, n, sem):
        return pltpu.make_async_copy(wm_hbm.at[:, pl.ds(lo, n)], wm.at[:, pl.ds(lo, n)], sem)

    def group_copies(p):
        cps = [pltpu.make_async_copy(w_u32[m].at[:, par, p, :], wqkv[m].at[2 * p + par],
                                     sem_pair.at[p])
               for m in range(3) for par in range(2)]
        segs = pl.ds(4 * p, 4)
        cps.append(pltpu.make_async_copy(x_hbm.at[segs, 0:3], xv.at[segs, 0:3], sem_pair.at[p]))
        return cps

    cp_xe = pltpu.make_async_copy(x_hbm.at[:, 3], xv.at[:, 3], sem_misc.at[0])
    cp_wm1 = [wm_copy(j * 512, 512, sem_misc.at[1 + j]) for j in range(4)]
    cp_wm2 = wm_copy(2 * D, 4 * D, sem_misc.at[6])
    cp_wo = pltpu.make_async_copy(wo_hbm, wo, sem_misc.at[7])
    cp_ffn = [pltpu.make_async_copy(wg_hbm, wg, sem_misc.at[8]),
              pltpu.make_async_copy(wu_hbm, wu, sem_misc.at[9]),
              pltpu.make_async_copy(wd_hbm, wd, sem_misc.at[10])]

    cp_xe.start()
    for cp in cp_wm1:
        cp.start()
    for p in range(8):
        for cp in group_copies(p):
            cp.start()

    ri = jax.lax.broadcasted_iota(jnp.int32, (80, 128), 0)
    ci = jax.lax.broadcasted_iota(jnp.int32, (80, 128), 1)

    def head_of(i):
        return jnp.where(i < 64, i >> 5, (i - 64) >> 3)

    def pos_of(i):
        return jnp.where(i < 64, i & 31, 32 + (i & 7))

    same = (head_of(ri) == head_of(ci)) & (ci < 80)
    allowed = (pos_of(ri) < M) | (pos_of(ri) >= pos_of(ci))
    fill[...] = jnp.where(same, jnp.where(allowed, 0.0, NEG), -jnp.inf).astype(F32)
    rmat[...] = jnp.full(rmat.shape, -jnp.inf, F32)
    pend[...] = jnp.zeros(pend.shape, F32)
    zero[...] = jnp.zeros(zero.shape, U32)

    def pin_bits(v):
        return pltpu.bitcast(v, U32) & zero[...]

    cf = c_ref[...].astype(F32)
    sc = _rb(cf * jax.nn.sigmoid(cf))
    sc = jnp.broadcast_to(sc, (16, D)).astype(BF16)

    def mod_cols(lo, hi):
        for j in range(lo, hi):
            v = _rb(_dot(sc, wblk(wm, j))[0:8])
            if j // 8 in (1, 4):
                v = _rb(1.0 + v)
            mod[:, j * 128:(j + 1) * 128] = v

    def mod_vec(k):
        return mod[:, k * D:(k + 1) * D]

    def affine1(n):
        return _rb(n * mod_vec(1)) + mod_vec(0)

    cp_xe.wait()

    def ne_body(i, carry):
        n = _layernorm(xv[pl.ds(i * 16, 16), 3].astype(F32))
        he[pl.ds(pl.multiple_of(i * 128, 128), 128), :] = n.reshape(128, D).astype(BF16)
        return carry

    jax.lax.fori_loop(0, NSEG // 16, ne_body, 0)
    for j in range(4):
        cp_wm1[j].wait()
        mod_cols(4 * j, 4 * j + 4)

    def he_body(i, carry):
        rows = pl.ds(pl.multiple_of(i * 128, 128), 128)
        n = he[rows, :].astype(F32).reshape(16, 8, D)
        he[rows, :] = affine1(n).reshape(128, D).astype(BF16)
        return carry

    jax.lax.fori_loop(0, NSEG // 16, he_body, 0)

    def w_head(m, h, lo=0, hi=D):
        return pltpu.bitcast(wqkv[m][h, lo // 2:hi // 2, :], BF16)

    def pro_body(p, carry):
        @pl.when(p == 4)
        def _():
            for pp in range(8, NP):
                for cp in group_copies(pp):
                    cp.start()
            cp_wo.start()
            cp_wm2.start()
            for cp in cp_ffn:
                cp.start()

        for cp in group_copies(p):
            cp.wait()
        for m in range(3):
            w = wqkv[m]
            e = w[2 * p]
            o = w[2 * p + 1]
            w[2 * p] = (e & U32(0xFFFF)) | (o << 16)
            w[2 * p + 1] = (e >> 16) | (o & U32(0xFFFF0000))
            for c in range(2):
                hc = he[c * 256:(c + 1) * 256, :]
                r1 = _dot(hc, w_head(m, 2 * p)).reshape(32, 8, DH)
                r2 = _dot(hc, w_head(m, 2 * p + 1)).reshape(32, 8, DH)
                early[c * 32:(c + 1) * 32, m * NP + p] = (
                    jnp.concatenate([r1, r2], axis=1).astype(BF16))
        for t in range(4):
            s = p * 4 + t
            hj[s] = affine1(_rb(_layernorm(xv[s, 0:3].astype(F32))))
        return carry

    with jax.named_scope("prologue_loop"):
        jax.lax.fori_loop(0, NP, pro_body, 0)
    cp_wm2.wait()
    cp_wo.wait()
    mod_cols(16, 48)
    lhs_ref[...] = jnp.concatenate(
        [mem0_ref[...].astype(F32), hj[0].reshape(NJ, D)], axis=0).astype(BF16)

    wr = jnp.broadcast_to(wr_ref[...].astype(F32).reshape(1, D), (8, D))

    def second(x1):
        n = _rb(_layernorm(x1))
        h2 = _rb(_rb(n * mod_vec(4)) + mod_vec(3))
        r = _rb(jnp.sum(h2 * wr, axis=-1, keepdims=True))
        return h2, r

    lane8 = jax.lax.broadcasted_iota(jnp.int32, (8, 128), 1)

    def post(s, g0, g1, attn):
        attn = attn.reshape(g1 - g0, 8, D)
        x1 = _rb(xv[s, g0:g1].astype(F32) + _rb(mod_vec(2) * _rb(attn)))
        h2, r = second(x1)
        x1v[s, g0:g1] = x1.astype(BF16)
        outv[s, g0:g1] = (x1 + _rb(mod_vec(5) * h2)).astype(BF16)
        pins = []
        for g in range(g0, g1):
            rows = slice(g * 8, (g + 1) * 8)
            rnew = jnp.where(lane8 == s, r[g - g0], rmat[rows, :])
            rmat[rows, :] = rnew
            pins.append(rnew)
        return pins

    def post_pending(i):
        return (post(2 * i + 1, 0, 4, pend[0:SEG, :])
                + post(2 * i, 3, 4, pend[SEG:SEG + M, :]))

    zpad = jnp.zeros((48, DH), BF16)
    LAG = 3
    KA = (NP - LAG) * 2 * DH
    KS = D - 128

    def segment(s, lhs_cols, split_first, extra, pins):
        lhs = jnp.concatenate(lhs_cols, axis=1)
        qkvs, probs = {}, {}

        def qkv(p):
            keys = [(m, 2 * p + b) for m in range(3) for b in range(2)]
            if p == 0 and split_first:
                la = jnp.concatenate(lhs_cols[:-1], axis=1)
                part = [_dot(la, w_head(m, h, 0, KS)) for m, h in keys]
                full = [_dot(lhs_cols[-1], w_head(m, h, KS, D)) + part[i]
                        for i, (m, h) in enumerate(keys)]
            else:
                full = [_dot(lhs, w_head(m, h)) for m, h in keys]
            res = []
            for m in range(3):
                parts = [full[2 * m].astype(BF16), full[2 * m + 1].astype(BF16),
                         early[s, m * NP + p]]
                if m > 0:
                    parts.append(zpad)
                res.append(jnp.concatenate(parts, axis=0))
            return res

        def scores(p):
            sc_ = _dot_nt(qkvs[p][0], qkvs[p][1]) * SCALE
            f = fill[...]
            if p in pins:
                z = pltpu.bitcast(pin_bits(pins[p]), F32)
                f = jnp.concatenate([f[0:8] + z, f[8:]], axis=0)
            sc_ = jnp.where(f == 0.0, sc_, f)
            mx = jnp.max(sc_, axis=-1, keepdims=True)
            e = jnp.exp(sc_ - mx)
            den = jnp.sum(e, axis=-1, keepdims=True)
            inv = pl.reciprocal(den, approx=True)
            probs[p] = (e * (inv * (2.0 - den * inv))).astype(BF16)

        oe = []

        def pv(p):
            o = _dot(probs[p], qkvs[p][2])
            res = []
            for b in range(2):
                rows, erows = o[32 * b:32 * b + 32], o[64 + 8 * b:72 + 8 * b]
                oe.append(erows)
                if extra is not None:
                    rows = jnp.concatenate([rows, erows, extra[2 * p + b]], axis=0)
                res.append(rows.astype(BF16))
            return res

        os_ = []
        for p in range(NP):
            qkvs[p] = qkv(p)
            if p >= 1:
                scores(p - 1)
            if p >= LAG:
                os_ += pv(p - LAG)
        oa = jnp.concatenate(os_, axis=1)
        acc, ob = [], []
        for n in range(7):
            acc.append(_dot(oa, wblk(wo, n, 0, KA)))
            if n == 0:
                scores(NP - 1)
                ob += pv(NP - 3)
            if n == 2:
                ob += pv(NP - 2)
            if n == 4:
                ob += pv(NP - 1)
        ob = jnp.concatenate(ob, axis=1)
        res = [_dot(ob, wblk(wo, n, KA, H * DH)) + acc[n] for n in range(7)]
        res.append(_dot(jnp.concatenate([oa, ob], axis=1), wblk(wo, 7)))
        return res, oe

    def next_lhs(res, s):
        hjs = hj[s].reshape(NJ, D)
        return [jnp.concatenate([res[n][0:M], hjs[:, n * 128:(n + 1) * 128]], axis=0).astype(BF16)
                for n in range(8)]

    cp_o1 = pltpu.make_async_copy(outv.at[0:OUT_SPLIT], out_hbm.at[0:OUT_SPLIT], sem_out.at[0])
    cp_o2 = pltpu.make_async_copy(outv.at[OUT_SPLIT:NSEG], out_hbm.at[OUT_SPLIT:NSEG],
                                  sem_out.at[1])

    def step(i, carry):
        @pl.when(i == OUT_SPLIT // 2 + 1)
        def _():
            cp_o1.start()

        a = 2 * i
        pins = post_pending(jnp.maximum(i - 1, 0))
        lhs_a = [lhs_ref[:, n * 128:(n + 1) * 128] for n in range(8)]
        res_a, oe_a = segment(a, lhs_a, False, None, {2 + 2 * g: v for g, v in enumerate(pins)})
        pins = post(a, 0, 3, jnp.concatenate([r[M:SEG] for r in res_a], axis=1))
        res_b, _ = segment(a + 1, next_lhs(res_a, a + 1), True, oe_a,
                           {3 + 3 * g: v for g, v in enumerate(pins)})
        nxt = next_lhs(res_b, jnp.minimum(a + 2, NSEG - 1))
        for n in range(8):
            pend[:, n * 128:(n + 1) * 128] = res_b[n][M:]
            lhs_ref[:, n * 128:(n + 1) * 128] = nxt[n]
        return carry

    with jax.named_scope("main_loop"):
        jax.lax.fori_loop(0, NSEG // 2, step, 0)
    post_pending(NSEG // 2 - 1)
    cp_o2.start()

    rm = rmat[...]
    tok = (jax.lax.broadcasted_iota(jnp.int32, (SEG, 128), 1) * SEG
           + jax.lax.broadcasted_iota(jnp.int32, (SEG, 128), 0))
    big = NSEG * SEG - 1
    i1 = jnp.min(jnp.where(rm == jnp.max(rm), tok, big))
    rm2 = jnp.where(tok == i1, -jnp.inf, rm)
    i2 = jnp.min(jnp.where((rm2 == jnp.max(rm2)) & (tok != i1), tok, big))
    i1 = jnp.clip(i1, 0, big)
    i2 = jnp.clip(i2, 0, big)
    g1, g2 = i1 >> 3, i2 >> 3
    x1 = jnp.concatenate([x1v[g1 >> 2, pl.ds(g1 & 3, 1)], x1v[g2 >> 2, pl.ds(g2 & 3, 1)]],
                         axis=0).astype(F32)
    h2, r = second(x1)
    for cp in cp_ffn:
        cp.wait()
    hl = h2.reshape(16, D).astype(BF16)
    act = []
    for j in range(FF // 128):
        gt = _rb(_dot(hl, wblk(wg, j)))
        up = _rb(_dot(hl, wblk(wu, j)))
        act.append((_rb(gt * jax.nn.sigmoid(gt)) * up).astype(BF16))
    act = jnp.concatenate(act, axis=1)
    y = jnp.concatenate([_dot(act, wblk(wd, n)) for n in range(8)], axis=1).reshape(2, 8, D)
    y = _rb(_rb(y) * _rb(jax.nn.sigmoid(r)))
    rowi = jax.lax.broadcasted_iota(jnp.int32, (2, 8, 1), 1)
    gsel = jax.lax.broadcasted_iota(jnp.int32, (2, 8, 1), 0)
    tokp = jnp.where(gsel == 0, g1, g2) * 8 + rowi
    upd = jnp.where((tokp == i1) | (tokp == i2), y, 0.0)
    patch[...] = (x1 + _rb(mod_vec(5) * _rb(h2 + upd))).astype(BF16)
    cp_o1.wait()
    cp_o2.wait()
    cp1 = pltpu.make_async_copy(patch.at[0], out_hbm.at[g1 >> 2, g1 & 3], sem_out.at[0])
    cp1.start()

    @pl.when(g1 != g2)
    def _():
        cp2 = pltpu.make_async_copy(patch.at[1], out_hbm.at[g2 >> 2, g2 & 3], sem_out.at[1])
        cp2.start()
        cp2.wait()

    cp1.wait()


@functools.partial(jax.jit, static_argnames=("A_seg_len",))
def pallas_adaLN_cond__memory_aug_recurrent_mem_tr__moe_arch_mod__prompt_kernel(
    A_x: jax.Array,
    A_mem0: jax.Array,
    A_Wq: jax.Array,
    A_Wk: jax.Array,
    A_Wv: jax.Array,
    A_Wo: jax.Array,
    A_seg_len,
    B_x: jax.Array,
    B_w_r: jax.Array,
    B_w_gate: jax.Array,
    B_w_up: jax.Array,
    B_w_down: jax.Array,
    c: jax.Array,
    w_mod: jax.Array,
):
    assert A_seg_len == SEG and A_x.shape == (1, NSEG * SEG, D)
    any_spec = pl.BlockSpec(memory_space=pl.ANY)
    vmem_spec = pl.BlockSpec(memory_space=pltpu.VMEM)
    out = pl.pallas_call(
        _kernel,
        out_shape=jax.ShapeDtypeStruct((NSEG, 4, 8, D), BF16),
        in_specs=[any_spec, vmem_spec, any_spec, any_spec, any_spec, any_spec, vmem_spec,
                  any_spec, any_spec, any_spec, vmem_spec, any_spec],
        out_specs=any_spec,
        scratch_shapes=[
            pltpu.VMEM((H, D // 2, DH), U32),
            pltpu.VMEM((H, D // 2, DH), U32),
            pltpu.VMEM((H, D // 2, DH), U32),
            pltpu.VMEM((H * DH // 2, D), U32),
            pltpu.VMEM((D // 2, FF), U32),
            pltpu.VMEM((D // 2, FF), U32),
            pltpu.VMEM((FF // 2, D), U32),
            pltpu.VMEM((D // 2, 6 * D), U32),
            pltpu.VMEM((NSEG, 4, 8, D), BF16),
            pltpu.VMEM((NSEG, 4, 8, D), BF16),
            pltpu.VMEM((NSEG, 4, 8, D), BF16),
            pltpu.VMEM((NSEG, 3 * NP, 16, DH), BF16),
            pltpu.VMEM((NE, D), BF16),
            pltpu.VMEM((NSEG, 3, 8, D), F32),
            pltpu.VMEM((SEG, D), BF16),
            pltpu.VMEM((SEG + M, D), F32),
            pltpu.VMEM((8, 6 * D), F32),
            pltpu.VMEM((80, 128), F32),
            pltpu.VMEM((SEG, 128), F32),
            pltpu.VMEM((2, 8, D), BF16),
            pltpu.VMEM((8, 128), U32),
            pltpu.SemaphoreType.DMA((NP,)),
            pltpu.SemaphoreType.DMA((11,)),
            pltpu.SemaphoreType.DMA((2,)),
        ],
        compiler_params=pltpu.CompilerParams(vmem_limit_bytes=120 * 1024 * 1024),
    )(
        A_x.reshape(NSEG, 4, 8, D),
        A_mem0.reshape(M, D),
        A_Wq.reshape(D // 2, 2, H, DH),
        A_Wk.reshape(D // 2, 2, H, DH),
        A_Wv.reshape(D // 2, 2, H, DH),
        A_Wo.reshape(H * DH, D),
        B_w_r,
        B_w_gate,
        B_w_up,
        B_w_down,
        c,
        w_mod,
    )
    return out.reshape(1, NSEG * SEG, D)
```

```python
import functools

import jax
import jax.numpy as jnp
import jax.experimental.pallas as pl
import jax.experimental.pallas.tpu as pltpu

F32 = jnp.float32
BF16 = jnp.bfloat16
U32 = jnp.uint32

D = 1024
H = 32
DH = 128
NP = H // 2
M = 8
SEG = 32
NSEG = 64
FF = 3584
NJ = SEG - M
NE = NSEG * M
EPS = 1e-5
SCALE = DH ** (-0.5)
NEG = -1000000000.0
OUT_SPLIT = 58


def _rb(x):
    return x.astype(BF16).astype(F32)


def _layernorm(xf):
    m = jnp.mean(xf, axis=-1, keepdims=True)
    d = xf - m
    v = jnp.mean(d * d, axis=-1, keepdims=True)
    return d * jax.lax.rsqrt(v + EPS)


def _dot(a, b):
    return jnp.dot(a, b, preferred_element_type=F32)


def _dot_nt(a, b):
    return jax.lax.dot_general(a, b, (((1,), (1,)), ((), ())), preferred_element_type=F32)


def _kernel(x_hbm, mem0_ref, wq_hbm, wk_hbm, wv_hbm, wo_hbm, wr_ref, wg_hbm, wu_hbm, wd_hbm,
            c_ref, wm_hbm,
            out_hbm,
            wq, wk, wv, wo, wg, wu, wd, wm, xv, x1v, outv, early, he, hj, lhs_ref, pend,
            mod, fill, rmat, patch, zero,
            sem_pair, sem_misc, sem_out):
    w_u32 = [w.bitcast(U32) for w in (wq_hbm, wk_hbm, wv_hbm)]
    wqkv = (wq, wk, wv)
    wo_hbm, wg_hbm, wu_hbm, wd_hbm, wm_hbm = [
        w.bitcast(U32) for w in (wo_hbm, wg_hbm, wu_hbm, wd_hbm, wm_hbm)]

    def wblk(w, j, lo=None, hi=None):
        rows = slice(None) if lo is None else slice(lo // 2, hi // 2)
        return pltpu.bitcast(w[rows, j * 128:(j + 1) * 128], BF16)

    def wm_copy(lo, n, sem):
        return pltpu.make_async_copy(wm_hbm.at[:, pl.ds(lo, n)], wm.at[:, pl.ds(lo, n)], sem)

    def group_copies(p):
        cps = [pltpu.make_async_copy(w_u32[m].at[:, par, p, :], wqkv[m].at[2 * p + par],
                                     sem_pair.at[p])
               for m in range(3) for par in range(2)]
        segs = pl.ds(4 * p, 4)
        cps.append(pltpu.make_async_copy(x_hbm.at[segs, 0:3], xv.at[segs, 0:3], sem_pair.at[p]))
        return cps

    cp_xe = pltpu.make_async_copy(x_hbm.at[:, 3], xv.at[:, 3], sem_misc.at[0])
    cp_wm1 = [wm_copy(j * 512, 512, sem_misc.at[1 + j]) for j in range(4)]
    cp_wm2 = wm_copy(2 * D, 4 * D, sem_misc.at[6])
    cp_wo = pltpu.make_async_copy(wo_hbm, wo, sem_misc.at[7])
    cp_ffn = [pltpu.make_async_copy(wg_hbm, wg, sem_misc.at[8]),
              pltpu.make_async_copy(wu_hbm, wu, sem_misc.at[9]),
              pltpu.make_async_copy(wd_hbm, wd, sem_misc.at[10])]

    cp_xe.start()
    for cp in cp_wm1:
        cp.start()
    for p in range(8):
        for cp in group_copies(p):
            cp.start()

    ri = jax.lax.broadcasted_iota(jnp.int32, (80, 128), 0)
    ci = jax.lax.broadcasted_iota(jnp.int32, (80, 128), 1)

    def head_of(i):
        return jnp.where(i < 64, i >> 5, (i - 64) >> 3)

    def pos_of(i):
        return jnp.where(i < 64, i & 31, 32 + (i & 7))

    same = (head_of(ri) == head_of(ci)) & (ci < 80)
    allowed = (pos_of(ri) < M) | (pos_of(ri) >= pos_of(ci))
    fill[...] = jnp.where(same, jnp.where(allowed, 0.0, NEG), -jnp.inf).astype(F32)
    rmat[...] = jnp.full(rmat.shape, -jnp.inf, F32)
    pend[...] = jnp.zeros(pend.shape, F32)
    zero[...] = jnp.zeros(zero.shape, U32)

    def pin_bits(v):
        return pltpu.bitcast(v, U32) & zero[...]

    cf = c_ref[...].astype(F32)
    sc = _rb(cf * jax.nn.sigmoid(cf))
    sc = jnp.broadcast_to(sc, (16, D)).astype(BF16)

    def mod_cols(lo, hi):
        for j in range(lo, hi):
            v = _rb(_dot(sc, wblk(wm, j))[0:8])
            if j // 8 in (1, 4):
                v = _rb(1.0 + v)
            mod[:, j * 128:(j + 1) * 128] = v

    def mod_vec(k):
        return mod[:, k * D:(k + 1) * D]

    def affine1(n):
        return _rb(n * mod_vec(1)) + mod_vec(0)

    cp_xe.wait()

    def ne_body(i, carry):
        n = _layernorm(xv[pl.ds(i * 16, 16), 3].astype(F32))
        he[pl.ds(pl.multiple_of(i * 128, 128), 128), :] = n.reshape(128, D).astype(BF16)
        return carry

    jax.lax.fori_loop(0, NSEG // 16, ne_body, 0)
    for j in range(4):
        cp_wm1[j].wait()
        mod_cols(4 * j, 4 * j + 4)

    def he_body(i, carry):
        rows = pl.ds(pl.multiple_of(i * 128, 128), 128)
        n = he[rows, :].astype(F32).reshape(16, 8, D)
        he[rows, :] = affine1(n).reshape(128, D).astype(BF16)
        return carry

    jax.lax.fori_loop(0, NSEG // 16, he_body, 0)

    def w_head(m, h, lo=0, hi=D):
        return pltpu.bitcast(wqkv[m][h, lo // 2:hi // 2, :], BF16)

    def pro_body(p, carry):
        @pl.when(p == 4)
        def _():
            for pp in range(8, NP):
                for cp in group_copies(pp):
                    cp.start()
            cp_wo.start()
            cp_wm2.start()
            for cp in cp_ffn:
                cp.start()

        for cp in group_copies(p):
            cp.wait()
        for m in range(3):
            w = wqkv[m]
            e = w[2 * p]
            o = w[2 * p + 1]
            w[2 * p] = (e & U32(0xFFFF)) | (o << 16)
            w[2 * p + 1] = (e >> 16) | (o & U32(0xFFFF0000))
            for c in range(2):
                hc = he[c * 256:(c + 1) * 256, :]
                r1 = _dot(hc, w_head(m, 2 * p)).reshape(32, 8, DH)
                r2 = _dot(hc, w_head(m, 2 * p + 1)).reshape(32, 8, DH)
                early[c * 32:(c + 1) * 32, m * NP + p] = (
                    jnp.concatenate([r1, r2], axis=1).astype(BF16))
        for t in range(4):
            s = p * 4 + t
            hj[s] = affine1(_rb(_layernorm(xv[s, 0:3].astype(F32))))
        return carry

    with jax.named_scope("prologue_loop"):
        jax.lax.fori_loop(0, NP, pro_body, 0)
    cp_wm2.wait()
    cp_wo.wait()
    mod_cols(16, 48)
    lhs_ref[...] = jnp.concatenate(
        [mem0_ref[...].astype(F32), hj[0].reshape(NJ, D)], axis=0).astype(BF16)

    wr = jnp.broadcast_to(wr_ref[...].astype(F32).reshape(1, D), (8, D))

    def second(x1):
        n = _rb(_layernorm(x1))
        h2 = _rb(_rb(n * mod_vec(4)) + mod_vec(3))
        r = _rb(jnp.sum(h2 * wr, axis=-1, keepdims=True))
        return h2, r

    lane8 = jax.lax.broadcasted_iota(jnp.int32, (8, 128), 1)

    def post(s, g0, g1, attn):
        attn = attn.reshape(g1 - g0, 8, D)
        x1 = _rb(xv[s, g0:g1].astype(F32) + _rb(mod_vec(2) * _rb(attn)))
        h2, r = second(x1)
        x1v[s, g0:g1] = x1.astype(BF16)
        outv[s, g0:g1] = (x1 + _rb(mod_vec(5) * h2)).astype(BF16)
        pins = []
        for g in range(g0, g1):
            rows = slice(g * 8, (g + 1) * 8)
            rnew = jnp.where(lane8 == s, r[g - g0], rmat[rows, :])
            rmat[rows, :] = rnew
            pins.append(rnew)
        return pins

    def post_pending(i):
        return (post(2 * i + 1, 0, 4, pend[0:SEG, :])
                + post(2 * i, 3, 4, pend[SEG:SEG + M, :]))

    zpad = jnp.zeros((48, DH), BF16)
    KA = (NP - 4) * 2 * DH
    KS = D - 128

    def segment(s, lhs_cols, split_first, extra, pins):
        lhs = jnp.concatenate(lhs_cols, axis=1)
        qkvs, probs = {}, {}

        def qkv2(p):
            keys = [(m, 2 * p + b) for m in range(3) for b in range(4)]
            nsplit = 6 if (p == 0 and split_first) else 0
            la = jnp.concatenate(lhs_cols[:-1], axis=1)
            part = [_dot(la, w_head(m, h, 0, KS)) for m, h in keys[:nsplit]]
            full = [_dot(lhs_cols[-1], w_head(m, h, KS, D)) + part[i]
                    for i, (m, h) in enumerate(keys[:nsplit])]
            full += [_dot(lhs, w_head(m, h)) for m, h in keys[nsplit:]]
            for t in range(2):
                res = []
                for m in range(3):
                    parts = [full[4 * m + 2 * t].astype(BF16), full[4 * m + 2 * t + 1].astype(BF16),
                             early[s, m * NP + p + t]]
                    if m > 0:
                        parts.append(zpad)
                    res.append(jnp.concatenate(parts, axis=0))
                qkvs[p + t] = res

        def scores(p):
            sc_ = _dot_nt(qkvs[p][0], qkvs[p][1]) * SCALE
            f = fill[...]
            if p in pins:
                z = pltpu.bitcast(pin_bits(pins[p]), F32)
                f = jnp.concatenate([f[0:8] + z, f[8:]], axis=0)
            sc_ = jnp.where(f == 0.0, sc_, f)
            mx = jnp.max(sc_, axis=-1, keepdims=True)
            e = jnp.exp(sc_ - mx)
            den = jnp.sum(e, axis=-1, keepdims=True)
            inv = pl.reciprocal(den, approx=True)
            probs[p] = (e * (inv * (2.0 - den * inv))).astype(BF16)

        oe = []

        def pv(p):
            o = _dot(probs[p], qkvs[p][2])
            res = []
            for b in range(2):
                rows, erows = o[32 * b:32 * b + 32], o[64 + 8 * b:72 + 8 * b]
                oe.append(erows)
                if extra is not None:
                    rows = jnp.concatenate([rows, erows, extra[2 * p + b]], axis=0)
                res.append(rows.astype(BF16))
            return res

        os_ = []
        for p in range(0, NP, 2):
            qkv2(p)
            scores(p)
            scores(p + 1)
            if p >= 2:
                os_ += pv(p - 2)
                os_ += pv(p - 1)
        oa = jnp.concatenate(os_[:KA // DH], axis=1)
        acc, ob = [], os_[KA // DH:]
        for n in range(7):
            acc.append(_dot(oa, wblk(wo, n, 0, KA)))
            if n == 2:
                ob += pv(NP - 2)
                ob += pv(NP - 1)
        ob = jnp.concatenate(ob, axis=1)
        res = [_dot(ob, wblk(wo, n, KA, H * DH)) + acc[n] for n in range(7)]
        res.append(_dot(jnp.concatenate([oa, ob], axis=1), wblk(wo, 7)))
        return res, oe

    def next_lhs(res, s):
        hjs = hj[s].reshape(NJ, D)
        return [jnp.concatenate([res[n][0:M], hjs[:, n * 128:(n + 1) * 128]], axis=0).astype(BF16)
                for n in range(8)]

    cp_o1 = pltpu.make_async_copy(outv.at[0:OUT_SPLIT], out_hbm.at[0:OUT_SPLIT], sem_out.at[0])
    cp_o2 = pltpu.make_async_copy(outv.at[OUT_SPLIT:NSEG], out_hbm.at[OUT_SPLIT:NSEG],
                                  sem_out.at[1])

    def step(i, carry):
        @pl.when(i == OUT_SPLIT // 2 + 1)
        def _():
            cp_o1.start()

        a = 2 * i
        pins = post_pending(jnp.maximum(i - 1, 0))
        lhs_a = [lhs_ref[:, n * 128:(n + 1) * 128] for n in range(8)]
        res_a, oe_a = segment(a, lhs_a, False, None, {2 + 2 * g: v for g, v in enumerate(pins)})
        pins = post(a, 0, 3, jnp.concatenate([r[M:SEG] for r in res_a], axis=1))
        res_b, _ = segment(a + 1, next_lhs(res_a, a + 1), True, oe_a,
                           {3 + 3 * g: v for g, v in enumerate(pins)})
        nxt = next_lhs(res_b, jnp.minimum(a + 2, NSEG - 1))
        for n in range(8):
            pend[:, n * 128:(n + 1) * 128] = res_b[n][M:]
            lhs_ref[:, n * 128:(n + 1) * 128] = nxt[n]
        return carry

    with jax.named_scope("main_loop"):
        jax.lax.fori_loop(0, NSEG // 2, step, 0)
    post_pending(NSEG // 2 - 1)
    cp_o2.start()

    rm = rmat[...]
    tok = (jax.lax.broadcasted_iota(jnp.int32, (SEG, 128), 1) * SEG
           + jax.lax.broadcasted_iota(jnp.int32, (SEG, 128), 0))
    big = NSEG * SEG - 1
    i1 = jnp.min(jnp.where(rm == jnp.max(rm), tok, big))
    rm2 = jnp.where(tok == i1, -jnp.inf, rm)
    i2 = jnp.min(jnp.where((rm2 == jnp.max(rm2)) & (tok != i1), tok, big))
    i1 = jnp.clip(i1, 0, big)
    i2 = jnp.clip(i2, 0, big)
    g1, g2 = i1 >> 3, i2 >> 3
    x1 = jnp.concatenate([x1v[g1 >> 2, pl.ds(g1 & 3, 1)], x1v[g2 >> 2, pl.ds(g2 & 3, 1)]],
                         axis=0).astype(F32)
    h2, r = second(x1)
    for cp in cp_ffn:
        cp.wait()
    hl = h2.reshape(16, D).astype(BF16)
    act = []
    for j in range(FF // 128):
        gt = _rb(_dot(hl, wblk(wg, j)))
        up = _rb(_dot(hl, wblk(wu, j)))
        act.append((_rb(gt * jax.nn.sigmoid(gt)) * up).astype(BF16))
    act = jnp.concatenate(act, axis=1)
    y = jnp.concatenate([_dot(act, wblk(wd, n)) for n in range(8)], axis=1).reshape(2, 8, D)
    y = _rb(_rb(y) * _rb(jax.nn.sigmoid(r)))
    rowi = jax.lax.broadcasted_iota(jnp.int32, (2, 8, 1), 1)
    gsel = jax.lax.broadcasted_iota(jnp.int32, (2, 8, 1), 0)
    tokp = jnp.where(gsel == 0, g1, g2) * 8 + rowi
    upd = jnp.where((tokp == i1) | (tokp == i2), y, 0.0)
    patch[...] = (x1 + _rb(mod_vec(5) * _rb(h2 + upd))).astype(BF16)
    cp_o1.wait()
    cp_o2.wait()
    cp1 = pltpu.make_async_copy(patch.at[0], out_hbm.at[g1 >> 2, g1 & 3], sem_out.at[0])
    cp1.start()

    @pl.when(g1 != g2)
    def _():
        cp2 = pltpu.make_async_copy(patch.at[1], out_hbm.at[g2 >> 2, g2 & 3], sem_out.at[1])
        cp2.start()
        cp2.wait()

    cp1.wait()


@functools.partial(jax.jit, static_argnames=("A_seg_len",))
def pallas_adaLN_cond__memory_aug_recurrent_mem_tr__moe_arch_mod__prompt_kernel(
    A_x: jax.Array,
    A_mem0: jax.Array,
    A_Wq: jax.Array,
    A_Wk: jax.Array,
    A_Wv: jax.Array,
    A_Wo: jax.Array,
    A_seg_len,
    B_x: jax.Array,
    B_w_r: jax.Array,
    B_w_gate: jax.Array,
    B_w_up: jax.Array,
    B_w_down: jax.Array,
    c: jax.Array,
    w_mod: jax.Array,
):
    assert A_seg_len == SEG and A_x.shape == (1, NSEG * SEG, D)
    any_spec = pl.BlockSpec(memory_space=pl.ANY)
    vmem_spec = pl.BlockSpec(memory_space=pltpu.VMEM)
    out = pl.pallas_call(
        _kernel,
        out_shape=jax.ShapeDtypeStruct((NSEG, 4, 8, D), BF16),
        in_specs=[any_spec, vmem_spec, any_spec, any_spec, any_spec, any_spec, vmem_spec,
                  any_spec, any_spec, any_spec, vmem_spec, any_spec],
        out_specs=any_spec,
        scratch_shapes=[
            pltpu.VMEM((H, D // 2, DH), U32),
            pltpu.VMEM((H, D // 2, DH), U32),
            pltpu.VMEM((H, D // 2, DH), U32),
            pltpu.VMEM((H * DH // 2, D), U32),
            pltpu.VMEM((D // 2, FF), U32),
            pltpu.VMEM((D // 2, FF), U32),
            pltpu.VMEM((FF // 2, D), U32),
            pltpu.VMEM((D // 2, 6 * D), U32),
            pltpu.VMEM((NSEG, 4, 8, D), BF16),
            pltpu.VMEM((NSEG, 4, 8, D), BF16),
            pltpu.VMEM((NSEG, 4, 8, D), BF16),
            pltpu.VMEM((NSEG, 3 * NP, 16, DH), BF16),
            pltpu.VMEM((NE, D), BF16),
            pltpu.VMEM((NSEG, 3, 8, D), F32),
            pltpu.VMEM((SEG, D), BF16),
            pltpu.VMEM((SEG + M, D), F32),
            pltpu.VMEM((8, 6 * D), F32),
            pltpu.VMEM((80, 128), F32),
            pltpu.VMEM((SEG, 128), F32),
            pltpu.VMEM((2, 8, D), BF16),
            pltpu.VMEM((8, 128), U32),
            pltpu.SemaphoreType.DMA((NP,)),
            pltpu.SemaphoreType.DMA((11,)),
            pltpu.SemaphoreType.DMA((2,)),
        ],
        compiler_params=pltpu.CompilerParams(vmem_limit_bytes=120 * 1024 * 1024),
    )(
        A_x.reshape(NSEG, 4, 8, D),
        A_mem0.reshape(M, D),
        A_Wq.reshape(D // 2, 2, H, DH),
        A_Wk.reshape(D // 2, 2, H, DH),
        A_Wv.reshape(D // 2, 2, H, DH),
        A_Wo.reshape(H * DH, D),
        B_w_r,
        B_w_gate,
        B_w_up,
        B_w_down,
        c,
        w_mod,
    )
    return out.reshape(1, NSEG * SEG, D)
```

```python
import functools

import jax
import jax.numpy as jnp
import jax.experimental.pallas as pl
import jax.experimental.pallas.tpu as pltpu

F32 = jnp.float32
BF16 = jnp.bfloat16
U32 = jnp.uint32

D = 1024
H = 32
DH = 128
NP = H // 2
M = 8
SEG = 32
NSEG = 64
FF = 3584
NJ = SEG - M
NE = NSEG * M
EPS = 1e-5
SCALE = DH ** (-0.5)
NEG = -1000000000.0
UNROLL = 2
NIT = NSEG // (2 * UNROLL)
OUT_SPLIT = NSEG - 2 * UNROLL - 2


def _rb(x):
    return x.astype(BF16).astype(F32)


def _layernorm(xf):
    m = jnp.mean(xf, axis=-1, keepdims=True)
    d = xf - m
    v = jnp.mean(d * d, axis=-1, keepdims=True)
    return d * jax.lax.rsqrt(v + EPS)


def _dot(a, b):
    return jnp.dot(a, b, preferred_element_type=F32)


def _dot_nt(a, b):
    return jax.lax.dot_general(a, b, (((1,), (1,)), ((), ())), preferred_element_type=F32)


def _kernel(x_hbm, mem0_ref, wq_hbm, wk_hbm, wv_hbm, wo_hbm, wr_ref, wg_hbm, wu_hbm, wd_hbm,
            c_ref, wm_hbm,
            out_hbm,
            wq, wk, wv, wo, wg, wu, wd, wm, xv, x1v, outv, early, he, hj, pend,
            mod, fill, rmat, patch, zero,
            sem_pair, sem_misc, sem_out):
    w_u32 = [w.bitcast(U32) for w in (wq_hbm, wk_hbm, wv_hbm)]
    wqkv = (wq, wk, wv)
    wo_hbm, wg_hbm, wu_hbm, wd_hbm, wm_hbm = [
        w.bitcast(U32) for w in (wo_hbm, wg_hbm, wu_hbm, wd_hbm, wm_hbm)]

    def wblk(w, j, lo=None, hi=None):
        rows = slice(None) if lo is None else slice(lo // 2, hi // 2)
        return pltpu.bitcast(w[rows, j * 128:(j + 1) * 128], BF16)

    def wm_copy(lo, n, sem):
        return pltpu.make_async_copy(wm_hbm.at[:, pl.ds(lo, n)], wm.at[:, pl.ds(lo, n)], sem)

    def group_copies(p):
        cps = [pltpu.make_async_copy(w_u32[m].at[:, par, p, :], wqkv[m].at[2 * p + par],
                                     sem_pair.at[p])
               for m in range(3) for par in range(2)]
        segs = pl.ds(4 * p, 4)
        cps.append(pltpu.make_async_copy(x_hbm.at[segs, 0:3], xv.at[segs, 0:3], sem_pair.at[p]))
        return cps

    cp_xe = pltpu.make_async_copy(x_hbm.at[:, 3], xv.at[:, 3], sem_misc.at[0])
    cp_wm1 = [wm_copy(j * 512, 512, sem_misc.at[1 + j]) for j in range(4)]
    cp_wm2 = wm_copy(2 * D, 4 * D, sem_misc.at[6])
    cp_wo = pltpu.make_async_copy(wo_hbm, wo, sem_misc.at[7])
    cp_ffn = [pltpu.make_async_copy(wg_hbm, wg, sem_misc.at[8]),
              pltpu.make_async_copy(wu_hbm, wu, sem_misc.at[9]),
              pltpu.make_async_copy(wd_hbm, wd, sem_misc.at[10])]

    cp_xe.start()
    for cp in cp_wm1:
        cp.start()
    for p in range(8):
        for cp in group_copies(p):
            cp.start()

    ri = jax.lax.broadcasted_iota(jnp.int32, (80, 128), 0)
    ci = jax.lax.broadcasted_iota(jnp.int32, (80, 128), 1)

    def head_of(i):
        return jnp.where(i < 64, i >> 5, (i - 64) >> 3)

    def pos_of(i):
        return jnp.where(i < 64, i & 31, 32 + (i & 7))

    same = (head_of(ri) == head_of(ci)) & (ci < 80)
    allowed = (pos_of(ri) < M) | (pos_of(ri) >= pos_of(ci))
    fill[...] = jnp.where(same, jnp.where(allowed, 0.0, NEG), -jnp.inf).astype(F32)
    rmat[...] = jnp.full(rmat.shape, -jnp.inf, F32)
    pend[0:M, :] = mem0_ref[...].astype(F32)
    pend[M:, :] = jnp.zeros((SEG + M, D), F32)
    zero[...] = jnp.zeros(zero.shape, U32)

    def pin_zero(vals):
        acc = None
        for v in vals:
            v = pltpu.bitcast(v, U32)
            for r in range(0, v.shape[0], 8):
                acc = v[r:r + 8] if acc is None else acc | v[r:r + 8]
        return pltpu.bitcast(acc & zero[...], F32)

    cf = c_ref[...].astype(F32)
    sc = _rb(cf * jax.nn.sigmoid(cf))
    sc = jnp.broadcast_to(sc, (16, D)).astype(BF16)

    def mod_cols(lo, hi):
        for j in range(lo, hi):
            v = _rb(_dot(sc, wblk(wm, j))[0:8])
            if j // 8 in (1, 4):
                v = _rb(1.0 + v)
            mod[:, j * 128:(j + 1) * 128] = v

    def mod_vec(k):
        return mod[:, k * D:(k + 1) * D]

    def affine1(n):
        return _rb(n * mod_vec(1)) + mod_vec(0)

    cp_xe.wait()

    def ne_body(i, carry):
        n = _layernorm(xv[pl.ds(i * 16, 16), 3].astype(F32))
        he[pl.ds(pl.multiple_of(i * 128, 128), 128), :] = n.reshape(128, D).astype(BF16)
        return carry

    jax.lax.fori_loop(0, NSEG // 16, ne_body, 0)
    for j in range(4):
        cp_wm1[j].wait()
        mod_cols(4 * j, 4 * j + 4)

    def he_body(i, carry):
        rows = pl.ds(pl.multiple_of(i * 128, 128), 128)
        n = he[rows, :].astype(F32).reshape(16, 8, D)
        he[rows, :] = affine1(n).reshape(128, D).astype(BF16)
        return carry

    jax.lax.fori_loop(0, NSEG // 16, he_body, 0)

    def w_head(m, h, lo=0, hi=D):
        return pltpu.bitcast(wqkv[m][h, lo // 2:hi // 2, :], BF16)

    def pro_body(p, carry):
        @pl.when(p == 4)
        def _():
            for pp in range(8, NP):
                for cp in group_copies(pp):
                    cp.start()
            cp_wo.start()
            cp_wm2.start()
            for cp in cp_ffn:
                cp.start()

        for cp in group_copies(p):
            cp.wait()
        for m in range(3):
            w = wqkv[m]
            e = w[2 * p]
            o = w[2 * p + 1]
            w[2 * p] = (e & U32(0xFFFF)) | (o << 16)
            w[2 * p + 1] = (e >> 16) | (o & U32(0xFFFF0000))
            for c in range(2):
                hc = he[c * 256:(c + 1) * 256, :]
                r1 = _dot(hc, w_head(m, 2 * p)).reshape(32, 8, DH)
                r2 = _dot(hc, w_head(m, 2 * p + 1)).reshape(32, 8, DH)
                r12 = jnp.concatenate([r1, r2], axis=1).reshape(512, DH)
                early[c * 32:(c + 1) * 32, m * NP + p] = pltpu.bitcast(
                    r12.astype(BF16), U32).reshape(32, 8, DH)
        for t in range(4):
            s = p * 4 + t
            hj[s] = affine1(_rb(_layernorm(xv[s, 0:3].astype(F32))))
        return carry

    with jax.named_scope("prologue_loop"):
        jax.lax.fori_loop(0, NP, pro_body, 0)
    cp_wm2.wait()
    cp_wo.wait()
    mod_cols(16, 48)

    wr = jnp.broadcast_to(wr_ref[...].astype(F32).reshape(1, D), (8, D))

    def second(x1):
        n = _rb(_layernorm(x1))
        h2 = _rb(_rb(n * mod_vec(4)) + mod_vec(3))
        r = _rb(jnp.sum(h2 * wr, axis=-1, keepdims=True))
        return h2, r

    lane8 = jax.lax.broadcasted_iota(jnp.int32, (8, 128), 1)

    def post(s, g0, g1, attn):
        attn = attn.reshape(g1 - g0, 8, D)
        x1 = _rb(xv[s, g0:g1].astype(F32) + _rb(mod_vec(2) * _rb(attn)))
        h2, r = second(x1)
        x1v[s, g0:g1] = x1.astype(BF16)
        outv[s, g0:g1] = (x1 + _rb(mod_vec(5) * h2)).astype(BF16)
        pins = []
        for g in range(g0, g1):
            rows = slice(g * 8, (g + 1) * 8)
            rnew = jnp.where(lane8 == s, r[g - g0], rmat[rows, :])
            rmat[rows, :] = rnew
            pins.append(rnew)
        return pins

    def post_pair(a, rows):
        return post(a + 1, 0, 4, rows[0:SEG]) + post(a, 3, 4, rows[SEG:])

    zpad = jnp.zeros((48, DH), F32)
    G = 4
    KA = (NP - G) * 2 * DH
    KS = D - 128

    def segment(s, lhs, lhs_split, extra, pins):
        qkvs, probs = {}, {}

        def qkv_group(p):
            keys = [(m, 2 * p + b) for m in range(3) for b in range(2 * G)]
            nsplit = 6 if (p == 0 and lhs_split is not None) else 0
            part = [_dot(lhs_split[0], w_head(m, h, 0, KS)) for m, h in keys[:nsplit]]
            full = [_dot(lhs_split[1], w_head(m, h, KS, D)) + part[i]
                    for i, (m, h) in enumerate(keys[:nsplit])]
            full += [_dot(lhs, w_head(m, h)) for m, h in keys[nsplit:]]
            for t in range(G):
                res = []
                for m in range(3):
                    i = 2 * G * m + 2 * t
                    parts = [full[i], full[i + 1],
                             pltpu.bitcast(early[s, m * NP + p + t], BF16).astype(F32)]
                    if m > 0:
                        parts.append(zpad)
                    res.append(jnp.concatenate(parts, axis=0).astype(BF16))
                qkvs[p + t] = res

        def scores(p):
            sc_ = _dot_nt(qkvs[p][0], qkvs[p][1]) * SCALE
            f = fill[...]
            if pins.get(p):
                f = jnp.concatenate([f[0:8] + pin_zero(pins[p]), f[8:]], axis=0)
            sc_ = jnp.where(f == 0.0, sc_, f)
            mx = jnp.max(sc_, axis=-1, keepdims=True)
            e = jnp.exp(sc_ - mx)
            den = jnp.sum(e, axis=-1, keepdims=True)
            inv = pl.reciprocal(den, approx=True)
            probs[p] = e.astype(BF16), inv * (2.0 - den * inv)

        oe = []

        def pv(p):
            o = _dot(probs[p][0], qkvs[p][2]) * probs[p][1]
            res = []
            for b in range(2):
                rows, erows = o[32 * b:32 * b + 32], o[64 + 8 * b:72 + 8 * b]
                oe.append(erows)
                if extra is not None:
                    rows = jnp.concatenate([rows, erows, extra[2 * p + b]], axis=0)
                res.append(rows)
            pins.setdefault(p + G, []).append(o)
            return res

        os_ = []
        for p in range(0, NP, G):
            qkv_group(p)
            if p >= G:
                for t in range(G):
                    os_ += pv(p - G + t)
            for t in range(G):
                scores(p + t)
        oa = jnp.concatenate(os_, axis=1).astype(BF16)
        acc, ob = [], []
        for n in range(7):
            acc.append(_dot(oa, wblk(wo, n, 0, KA)))
            if n == 2:
                for t in range(G):
                    ob += pv(NP - G + t)
        ob = jnp.concatenate(ob, axis=1).astype(BF16)
        res = [_dot(ob, wblk(wo, n, KA, H * DH)) + acc[n] for n in range(7)]
        res.append(_dot(ob, wblk(wo, 7, KA, H * DH)) + _dot(oa, wblk(wo, 7, 0, KA)))
        return res, oe

    def make_lhs(mem, s):
        return jnp.concatenate([mem, hj[s].reshape(NJ, D)], axis=0)

    cp_o1 = pltpu.make_async_copy(outv.at[0:OUT_SPLIT], out_hbm.at[0:OUT_SPLIT], sem_out.at[0])
    cp_o2 = pltpu.make_async_copy(outv.at[OUT_SPLIT:NSEG], out_hbm.at[OUT_SPLIT:NSEG],
                                  sem_out.at[1])

    def split_lhs(lhs):
        return lhs.astype(BF16), (lhs[:, :KS].astype(BF16), lhs[:, KS:].astype(BF16))

    def step(i, carry):
        @pl.when(i == NIT - 1)
        def _():
            cp_o1.start()

        prev = pend[...]
        for u in range(UNROLL):
            a = 2 * (UNROLL * i + u)
            pins = post_pair(jnp.maximum(a - 2, 0) if u == 0 else a - 2, prev[M:])
            lhs_a = make_lhs(prev[0:M], a)
            lhs_a = (lhs_a.astype(BF16), None) if u == 0 else split_lhs(lhs_a)
            res_a, oe_a = segment(a, *lhs_a, None,
                                  {k: [v] for k, v in zip((4, 5, 8, 9, 12), pins)})
            res_a = jnp.concatenate(res_a, axis=1)
            pins = post(a, 0, 3, res_a[M:])
            res_b, _ = segment(a + 1, *split_lhs(make_lhs(res_a[0:M], a + 1)), oe_a,
                               {k: [v] for k, v in zip((4, 8, 12), pins)})
            prev = jnp.concatenate(res_b, axis=1)
        pend[...] = prev
        return carry

    with jax.named_scope("main_loop"):
        jax.lax.fori_loop(0, NIT, step, 0)
    post_pair(NSEG - 2, pend[M:, :])
    cp_o2.start()

    rm = rmat[...]
    tok = (jax.lax.broadcasted_iota(jnp.int32, (SEG, 128), 1) * SEG
           + jax.lax.broadcasted_iota(jnp.int32, (SEG, 128), 0))
    big = NSEG * SEG - 1
    i1 = jnp.min(jnp.where(rm == jnp.max(rm), tok, big))
    rm2 = jnp.where(tok == i1, -jnp.inf, rm)
    i2 = jnp.min(jnp.where((rm2 == jnp.max(rm2)) & (tok != i1), tok, big))
    i1 = jnp.clip(i1, 0, big)
    i2 = jnp.clip(i2, 0, big)
    g1, g2 = i1 >> 3, i2 >> 3
    x1 = jnp.concatenate([x1v[g1 >> 2, pl.ds(g1 & 3, 1)], x1v[g2 >> 2, pl.ds(g2 & 3, 1)]],
                         axis=0).astype(F32)
    h2, r = second(x1)
    for cp in cp_ffn:
        cp.wait()
    hl = h2.reshape(16, D).astype(BF16)
    act = []
    for j in range(FF // 128):
        gt = _rb(_dot(hl, wblk(wg, j)))
        up = _rb(_dot(hl, wblk(wu, j)))
        act.append((_rb(gt * jax.nn.sigmoid(gt)) * up).astype(BF16))
    act = jnp.concatenate(act, axis=1)
    y = jnp.concatenate([_dot(act, wblk(wd, n)) for n in range(8)], axis=1).reshape(2, 8, D)
    y = _rb(_rb(y) * _rb(jax.nn.sigmoid(r)))
    rowi = jax.lax.broadcasted_iota(jnp.int32, (2, 8, 1), 1)
    gsel = jax.lax.broadcasted_iota(jnp.int32, (2, 8, 1), 0)
    tokp = jnp.where(gsel == 0, g1, g2) * 8 + rowi
    upd = jnp.where((tokp == i1) | (tokp == i2), y, 0.0)
    patch[...] = (x1 + _rb(mod_vec(5) * _rb(h2 + upd))).astype(BF16)
    cp_o1.wait()
    cp_o2.wait()
    cp1 = pltpu.make_async_copy(patch.at[0], out_hbm.at[g1 >> 2, g1 & 3], sem_out.at[0])
    cp1.start()

    @pl.when(g1 != g2)
    def _():
        cp2 = pltpu.make_async_copy(patch.at[1], out_hbm.at[g2 >> 2, g2 & 3], sem_out.at[1])
        cp2.start()
        cp2.wait()

    cp1.wait()


@functools.partial(jax.jit, static_argnames=("A_seg_len",))
def pallas_adaLN_cond__memory_aug_recurrent_mem_tr__moe_arch_mod__prompt_kernel(
    A_x: jax.Array,
    A_mem0: jax.Array,
    A_Wq: jax.Array,
    A_Wk: jax.Array,
    A_Wv: jax.Array,
    A_Wo: jax.Array,
    A_seg_len,
    B_x: jax.Array,
    B_w_r: jax.Array,
    B_w_gate: jax.Array,
    B_w_up: jax.Array,
    B_w_down: jax.Array,
    c: jax.Array,
    w_mod: jax.Array,
):
    assert A_seg_len == SEG and A_x.shape == (1, NSEG * SEG, D)
    any_spec = pl.BlockSpec(memory_space=pl.ANY)
    vmem_spec = pl.BlockSpec(memory_space=pltpu.VMEM)
    out = pl.pallas_call(
        _kernel,
        out_shape=jax.ShapeDtypeStruct((NSEG, 4, 8, D), BF16),
        in_specs=[any_spec, vmem_spec, any_spec, any_spec, any_spec, any_spec, vmem_spec,
                  any_spec, any_spec, any_spec, vmem_spec, any_spec],
        out_specs=any_spec,
        scratch_shapes=[
            pltpu.VMEM((H, D // 2, DH), U32),
            pltpu.VMEM((H, D // 2, DH), U32),
            pltpu.VMEM((H, D // 2, DH), U32),
            pltpu.VMEM((H * DH // 2, D), U32),
            pltpu.VMEM((D // 2, FF), U32),
            pltpu.VMEM((D // 2, FF), U32),
            pltpu.VMEM((FF // 2, D), U32),
            pltpu.VMEM((D // 2, 6 * D), U32),
            pltpu.VMEM((NSEG, 4, 8, D), BF16),
            pltpu.VMEM((NSEG, 4, 8, D), BF16),
            pltpu.VMEM((NSEG, 4, 8, D), BF16),
            pltpu.VMEM((NSEG, 3 * NP, 8, DH), U32),
            pltpu.VMEM((NE, D), BF16),
            pltpu.VMEM((NSEG, 3, 8, D), F32),
            pltpu.VMEM((M + SEG + M, D), F32),
            pltpu.VMEM((8, 6 * D), F32),
            pltpu.VMEM((80, 128), F32),
            pltpu.VMEM((SEG, 128), F32),
            pltpu.VMEM((2, 8, D), BF16),
            pltpu.VMEM((8, 128), U32),
            pltpu.SemaphoreType.DMA((NP,)),
            pltpu.SemaphoreType.DMA((11,)),
            pltpu.SemaphoreType.DMA((2,)),
        ],
        compiler_params=pltpu.CompilerParams(vmem_limit_bytes=120 * 1024 * 1024),
    )(
        A_x.reshape(NSEG, 4, 8, D),
        A_mem0.reshape(M, D),
        A_Wq.reshape(D // 2, 2, H, DH),
        A_Wk.reshape(D // 2, 2, H, DH),
        A_Wv.reshape(D // 2, 2, H, DH),
        A_Wo.reshape(H * DH, D),
        B_w_r,
        B_w_gate,
        B_w_up,
        B_w_down,
        c,
        w_mod,
    )
    return out.reshape(1, NSEG * SEG, D)
```

```python
import functools

import jax
import jax.numpy as jnp
import jax.experimental.pallas as pl
import jax.experimental.pallas.tpu as pltpu

F32 = jnp.float32
BF16 = jnp.bfloat16
U32 = jnp.uint32

D = 1024
H = 32
DH = 128
NP = H // 2
M = 8
SEG = 32
NSEG = 64
FF = 3584
NJ = SEG - M
NE = NSEG * M
EPS = 1e-5
SCALE = DH ** (-0.5)
NEG = -1000000000.0
UNROLL = 1
NIT = NSEG // (2 * UNROLL)
OUT_SPLIT = NSEG - 2 * UNROLL - 2


def _rb(x):
    return x.astype(BF16).astype(F32)


def _layernorm(xf):
    m = jnp.mean(xf, axis=-1, keepdims=True)
    d = xf - m
    v = jnp.mean(d * d, axis=-1, keepdims=True)
    return d * jax.lax.rsqrt(v + EPS)


def _dot(a, b):
    return jnp.dot(a, b, preferred_element_type=F32)


def _dot_nt(a, b):
    return jax.lax.dot_general(a, b, (((1,), (1,)), ((), ())), preferred_element_type=F32)


def _kernel(x_hbm, mem0_hbm, wq_hbm, wk_hbm, wv_hbm, wo_hbm, wr_hbm, wg_hbm, wu_hbm, wd_hbm,
            c_hbm, wm_hbm,
            out_hbm,
            wq, wk, wv, wo, wg, wu, wd, wm, xv, x1v, h2v, outv, early, he, hj, pend,
            mod, fill, keys, patch, zero, mem0_ref, wr_ref, c_ref,
            sem, sem_out):
    w_u32 = [w.bitcast(U32) for w in (wq_hbm, wk_hbm, wv_hbm)]
    wqkv = (wq, wk, wv)
    wo_hbm, wg_hbm, wu_hbm, wd_hbm, wm_hbm = [
        w.bitcast(U32) for w in (wo_hbm, wg_hbm, wu_hbm, wd_hbm, wm_hbm)]

    def wblk(w, j, lo=None, hi=None):
        rows = slice(None) if lo is None else slice(lo // 2, hi // 2)
        return pltpu.bitcast(w[rows, j * 128:(j + 1) * 128], BF16)

    def wm_copy(lo, n, k):
        return pltpu.make_async_copy(wm_hbm.at[:, pl.ds(lo, n)], wm.at[:, pl.ds(lo, n)], sem.at[k])

    def w_copies(m, p, k):
        return [pltpu.make_async_copy(w_u32[m].at[:, par, p, :], wqkv[m].at[2 * p + par], sem.at[k])
                for par in range(2)]

    def xj_copy(p, k):
        segs = pl.ds(4 * p, 4)
        return pltpu.make_async_copy(x_hbm.at[segs, 0:3], xv.at[segs, 0:3], sem.at[k])

    def group_copies(p):
        k = 16 + p
        return w_copies(0, p, k) + w_copies(1, p, k) + w_copies(2, p, k) + [xj_copy(p, k)]

    cp_small = [pltpu.make_async_copy(c_hbm, c_ref, sem.at[5]),
                pltpu.make_async_copy(mem0_hbm, mem0_ref, sem.at[5]),
                pltpu.make_async_copy(wr_hbm, wr_ref, sem.at[5])]
    cp_xe = pltpu.make_async_copy(x_hbm.at[:, 3], xv.at[:, 3], sem.at[0])
    cp_wm1 = [wm_copy(j * 512, 512, 1 + j) for j in range(4)]
    cp_w0 = [w_copies(m, 0, 6 + m) for m in range(3)]
    cp_late = [wm_copy(2 * D, 4 * D, 9), xj_copy(0, 14),
               pltpu.make_async_copy(wo_hbm, wo, sem.at[10])]
    cp_ffn = [pltpu.make_async_copy(wg_hbm, wg, sem.at[11]),
              pltpu.make_async_copy(wu_hbm, wu, sem.at[12]),
              pltpu.make_async_copy(wd_hbm, wd, sem.at[13])]

    for cp in [cp_xe] + cp_small + cp_wm1 + cp_w0[0] + cp_w0[1] + cp_w0[2]:
        cp.start()
    for p in range(1, 8):
        for cp in group_copies(p):
            cp.start()

    ri = jax.lax.broadcasted_iota(jnp.int32, (80, 128), 0)
    ci = jax.lax.broadcasted_iota(jnp.int32, (80, 128), 1)

    def head_of(i):
        return jnp.where(i < 64, i >> 5, (i - 64) >> 3)

    def pos_of(i):
        return jnp.where(i < 64, i & 31, 32 + (i & 7))

    same = (head_of(ri) == head_of(ci)) & (ci < 80)
    allowed = (pos_of(ri) < M) | (pos_of(ri) >= pos_of(ci))
    fill[...] = jnp.where(same, jnp.where(allowed, 0.0, NEG), -jnp.inf).astype(F32)
    keys[...] = jnp.zeros(keys.shape, F32)
    pend[M:, :] = jnp.zeros((SEG + M, D), F32)
    zero[...] = jnp.zeros(zero.shape, U32)

    def pin_zero(vals):
        acc = None
        for v in vals:
            v = pltpu.bitcast(v, U32)
            for r in range(0, v.shape[0], 8):
                acc = v[r:r + 8] if acc is None else acc | v[r:r + 8]
        return acc & zero[...]

    cp_xe.wait()
    for cp in cp_small:
        cp.wait()
    pend[0:M, :] = mem0_ref[...].astype(F32)
    cf = c_ref[...].astype(F32)
    sc = _rb(cf * jax.nn.sigmoid(cf))
    sc = jnp.broadcast_to(sc, (16, D)).astype(BF16)

    def mod_cols(lo, hi):
        for j in range(lo, hi):
            v = _rb(_dot(sc, wblk(wm, j))[0:8])
            if j // 8 in (1, 4):
                v = _rb(1.0 + v)
            mod[:, j * 128:(j + 1) * 128] = v

    def mod_vec(k):
        return mod[:, k * D:(k + 1) * D]

    def affine1(n):
        return _rb(n * mod_vec(1)) + mod_vec(0)

    def ne_body(i, carry):
        n = _layernorm(xv[pl.ds(i * 16, 16), 3].astype(F32))
        he[pl.ds(pl.multiple_of(i * 128, 128), 128), :] = n.reshape(128, D).astype(BF16)
        return carry

    jax.lax.fori_loop(0, NSEG // 16, ne_body, 0)
    for j in range(4):
        cp_wm1[j].wait()
        mod_cols(4 * j, 4 * j + 4)

    def he_body(i, carry):
        rows = pl.ds(pl.multiple_of(i * 128, 128), 128)
        n = he[rows, :].astype(F32).reshape(16, 8, D)
        he[rows, :] = affine1(n).reshape(128, D).astype(BF16)
        return carry

    jax.lax.fori_loop(0, NSEG // 16, he_body, 0)

    def w_head(m, h, lo=0, hi=D):
        return pltpu.bitcast(wqkv[m][h, lo // 2:hi // 2, :], BF16)

    def early_proj(m, p, pins=(), rows=256, between=None):
        w = wqkv[m]
        e = w[2 * p]
        o = w[2 * p + 1]
        lo = (e & U32(0xFFFF)) | (o << 16)
        if pins:
            lo = jnp.concatenate([lo[0:8] | pin_zero(pins), lo[8:]], axis=0)
        w[2 * p] = lo
        w[2 * p + 1] = (e >> 16) | (o & U32(0xFFFF0000))
        ns = rows // 8
        for c in range(NE // rows):
            hc = he[c * rows:(c + 1) * rows, :]
            r12 = []
            for b in range(2):
                r12.append(_dot(hc, w_head(m, 2 * p + b)).reshape(ns, 8, DH))
                if between is not None:
                    between()
            r12 = jnp.concatenate(r12, axis=1).reshape(2 * rows, DH)
            early[c * ns:(c + 1) * ns, m * NP + p] = pltpu.bitcast(
                r12.astype(BF16), U32).reshape(ns, 8, DH)

    def make_hj(s):
        h = affine1(_rb(_layernorm(xv[s, 0:3].astype(F32))))
        hj[s] = h
        return h[:, :, 0:128].reshape(NJ, 128)

    for m in range(3):
        for cp in cp_w0[m]:
            cp.wait()
        early_proj(m, 0)

    def pro_body(p, carry):
        @pl.when(p == 4)
        def _():
            for pp in range(8, NP):
                for cp in group_copies(pp):
                    cp.start()
            for cp in cp_late + cp_ffn:
                cp.start()

        for cp in group_copies(p):
            cp.wait()
        pins = [make_hj(p * 4 + t) for t in range(4)]
        early_proj(0, p)
        early_proj(1, p, pins[0:2])
        early_proj(2, p, pins[2:4])
        return carry

    with jax.named_scope("prologue_loop"):
        jax.lax.fori_loop(1, NP - 1, pro_body, 0)

    for cp in group_copies(NP - 1) + cp_late:
        cp.wait()
    todo = list(range(16, 48))

    def some_mod_cols():
        n = 2 if len(todo) % 4 == 0 else 1
        for _ in range(n):
            j = todo.pop(0)
            mod_cols(j, j + 1)

    pins = [make_hj(s) for s in (0, 1, 2, 3, 60, 61, 62, 63)]
    early_proj(0, NP - 1, rows=128, between=some_mod_cols)
    early_proj(1, NP - 1, pins[0:4], rows=128, between=some_mod_cols)
    early_proj(2, NP - 1, pins[4:8], rows=128, between=some_mod_cols)
    assert not todo

    wr = jnp.broadcast_to(wr_ref[...].astype(F32).reshape(1, D), (8, D))

    lane8 = jax.lax.broadcasted_iota(jnp.int32, (8, 128), 1)
    sub8 = jax.lax.broadcasted_iota(jnp.int32, (8, 128), 0)
    LAST = NSEG * SEG - 1

    def post(s, g0, g1, attn):
        attn = attn.reshape(g1 - g0, 8, D)
        x1 = _rb(xv[s, g0:g1].astype(F32) + _rb(mod_vec(2) * _rb(attn)))
        n = _rb(_layernorm(x1))
        h2 = _rb(_rb(n * mod_vec(4)) + mod_vec(3))
        r = _rb(jnp.sum(h2 * wr, axis=-1, keepdims=True)) + 0.0
        x1v[s, g0:g1] = x1.astype(BF16)
        h2v[s, g0:g1] = h2.astype(BF16)
        outv[s, g0:g1] = (x1 + _rb(mod_vec(5) * h2)).astype(BF16)
        pins = []
        for g in range(g0, g1):
            bits = pltpu.bitcast(jnp.broadcast_to(r[g - g0], (8, 128)), jnp.int32)
            hi = jax.lax.shift_right_logical(bits, 16)
            code = jnp.where(bits < 0, hi ^ 0xFFFF, hi | 0x8000)
            key = (code << 11) | (LAST - (s * SEG + g * 8) - sub8) | 0x40000000
            rows = slice(g * 8, (g + 1) * 8)
            knew = jnp.where(lane8 == s, pltpu.bitcast(key, F32), keys[rows, :])
            keys[rows, :] = knew
            pins.append(knew)
        return pins

    def post_pair(a, rows):
        return post(a + 1, 0, 4, rows[0:SEG]) + post(a, 3, 4, rows[SEG:])

    zpad = jnp.zeros((48, DH), F32)
    G = 4
    KA = (NP - G) * 2 * DH
    KS = D - 128

    def segment(s, lhs, lhs_split, extra, pins):
        qkvs, probs = {}, {}

        def qkv_group(p):
            keys = [(m, 2 * p + b) for m in range(3) for b in range(2 * G)]
            nsplit = 6 if (p == 0 and lhs_split is not None) else 0
            part = [_dot(lhs_split[0], w_head(m, h, 0, KS)) for m, h in keys[:nsplit]]
            full = [_dot(lhs_split[1], w_head(m, h, KS, D)) + part[i]
                    for i, (m, h) in enumerate(keys[:nsplit])]
            full += [_dot(lhs, w_head(m, h)) for m, h in keys[nsplit:]]
            for t in range(G):
                res = []
                for m in range(3):
                    i = 2 * G * m + 2 * t
                    parts = [full[i], full[i + 1],
                             pltpu.bitcast(early[s, m * NP + p + t], BF16).astype(F32)]
                    if m > 0:
                        parts.append(zpad)
                    res.append(jnp.concatenate(parts, axis=0).astype(BF16))
                qkvs[p + t] = res

        def scores(p):
            sc_ = _dot_nt(qkvs[p][0], qkvs[p][1]) * SCALE
            f = fill[...]
            if pins.get(p):
                f = jnp.concatenate([f[0:8] + pltpu.bitcast(pin_zero(pins[p]), F32), f[8:]], axis=0)
            sc_ = jnp.where(f == 0.0, sc_, f)
            mx = jnp.max(sc_, axis=-1, keepdims=True)
            e = jnp.exp(sc_ - mx)
            den = jnp.sum(e, axis=-1, keepdims=True)
            inv = pl.reciprocal(den, approx=True)
            probs[p] = e.astype(BF16), inv * (2.0 - den * inv)

        oe = []

        def pv(p):
            o = _dot(probs[p][0], qkvs[p][2]) * probs[p][1]
            res = []
            for b in range(2):
                rows, erows = o[32 * b:32 * b + 32], o[64 + 8 * b:72 + 8 * b]
                oe.append(erows)
                if extra is not None:
                    rows = jnp.concatenate([rows, erows, extra[2 * p + b]], axis=0)
                res.append(rows)
            pins.setdefault(p + G, []).append(o)
            return res

        os_ = []
        for p in range(0, NP, G):
            qkv_group(p)
            if p >= G:
                for t in range(G):
                    os_ += pv(p - G + t)
            for t in range(G):
                scores(p + t)
        oa = jnp.concatenate(os_, axis=1).astype(BF16)
        acc, ob = [], []
        for n in range(7):
            acc.append(_dot(oa, wblk(wo, n, 0, KA)))
            if n == 2:
                for t in range(G):
                    ob += pv(NP - G + t)
        ob = jnp.concatenate(ob, axis=1).astype(BF16)
        res = [_dot(ob, wblk(wo, n, KA, H * DH)) + acc[n] for n in range(7)]
        res.append(_dot(ob, wblk(wo, 7, KA, H * DH)) + _dot(oa, wblk(wo, 7, 0, KA)))
        return res, oe

    def make_lhs(mem, s):
        return jnp.concatenate([mem, hj[s].reshape(NJ, D)], axis=0)

    cp_o1 = pltpu.make_async_copy(outv.at[0:OUT_SPLIT], out_hbm.at[0:OUT_SPLIT], sem_out.at[0])
    cp_o2 = pltpu.make_async_copy(outv.at[OUT_SPLIT:NSEG], out_hbm.at[OUT_SPLIT:NSEG],
                                  sem_out.at[1])

    def split_lhs(lhs):
        return lhs.astype(BF16), (lhs[:, :KS].astype(BF16), lhs[:, KS:].astype(BF16))

    def step(i, carry):
        @pl.when(i == NIT - 1)
        def _():
            cp_o1.start()

        prev = pend[...]
        for u in range(UNROLL):
            a = 2 * (UNROLL * i + u)
            pins = post_pair(jnp.maximum(a - 2, 0) if u == 0 else a - 2, prev[M:])
            lhs_a = make_lhs(prev[0:M], a)
            lhs_a = (lhs_a.astype(BF16), None) if u == 0 else split_lhs(lhs_a)
            res_a, oe_a = segment(a, *lhs_a, None,
                                  {k: [v] for k, v in zip((4, 5, 8, 9, 12), pins)})
            res_a = jnp.concatenate(res_a, axis=1)
            pins = post(a, 0, 3, res_a[M:])
            res_b, _ = segment(a + 1, *split_lhs(make_lhs(res_a[0:M], a + 1)), oe_a,
                               {k: [v] for k, v in zip((4, 8, 12), pins)})
            prev = jnp.concatenate(res_b, axis=1)
        pend[...] = prev
        return carry

    with jax.named_scope("main_loop"):
        jax.lax.fori_loop(0, NIT, step, 0)
    post_pair(NSEG - 2, pend[M:, :])
    cp_o2.start()

    def max_all(v):
        return jnp.max(jnp.max(v, axis=0, keepdims=True), axis=1, keepdims=True)

    def decode(k):
        kb = pltpu.bitcast(jnp.broadcast_to(k, (8, 128)), jnp.int32)
        code = (kb >> 11) & 0xFFFF
        hi = jnp.where(code >= 0x8000, code & 0x7FFF, code ^ 0xFFFF)
        return (LAST - (kb & LAST))[0, 0], pltpu.bitcast(hi << 16, F32)[:, 0:1]

    kv = keys[...]
    k1 = max_all(kv)
    k2 = max_all(jnp.where(kv == k1, 0.0, kv))
    i1, r1 = decode(k1)
    i2, r2 = decode(k2)
    g1, g2 = i1 >> 3, i2 >> 3

    def rows_of(ref):
        return jnp.concatenate([ref[g1 >> 2, pl.ds(g1 & 3, 1)], ref[g2 >> 2, pl.ds(g2 & 3, 1)]],
                               axis=0).astype(F32)

    x1, h2 = rows_of(x1v), rows_of(h2v)
    for cp in cp_ffn:
        cp.wait()
    hl = h2.reshape(16, D).astype(BF16)
    act = []
    for j in range(FF // 128):
        gt = _rb(_dot(hl, wblk(wg, j)))
        up = _rb(_dot(hl, wblk(wu, j)))
        act.append((_rb(gt * jax.nn.sigmoid(gt)) * up).astype(BF16))
    act = jnp.concatenate(act, axis=1)
    y = jnp.concatenate([_dot(act, wblk(wd, n)) for n in range(8)], axis=1).reshape(2, 8, D)
    rowi = jax.lax.broadcasted_iota(jnp.int32, (2, 8, 1), 1)
    gsel = jax.lax.broadcasted_iota(jnp.int32, (2, 8, 1), 0)
    tokp = jnp.where(gsel == 0, g1, g2) * 8 + rowi
    gate = _rb(jax.nn.sigmoid(jnp.where(tokp == i1, r1[None], r2[None])))
    upd = jnp.where((tokp == i1) | (tokp == i2), _rb(_rb(y) * gate), 0.0)
    patch[...] = (x1 + _rb(mod_vec(5) * _rb(h2 + upd))).astype(BF16)
    cp_o1.wait()
    cp_o2.wait()
    cp1 = pltpu.make_async_copy(patch.at[0], out_hbm.at[g1 >> 2, g1 & 3], sem_out.at[0])
    cp1.start()

    @pl.when(g1 != g2)
    def _():
        cp2 = pltpu.make_async_copy(patch.at[1], out_hbm.at[g2 >> 2, g2 & 3], sem_out.at[1])
        cp2.start()
        cp2.wait()

    cp1.wait()


@functools.partial(jax.jit, static_argnames=("A_seg_len",))
def pallas_adaLN_cond__memory_aug_recurrent_mem_tr__moe_arch_mod__prompt_kernel(
    A_x: jax.Array,
    A_mem0: jax.Array,
    A_Wq: jax.Array,
    A_Wk: jax.Array,
    A_Wv: jax.Array,
    A_Wo: jax.Array,
    A_seg_len,
    B_x: jax.Array,
    B_w_r: jax.Array,
    B_w_gate: jax.Array,
    B_w_up: jax.Array,
    B_w_down: jax.Array,
    c: jax.Array,
    w_mod: jax.Array,
):
    assert A_seg_len == SEG and A_x.shape == (1, NSEG * SEG, D)
    any_spec = pl.BlockSpec(memory_space=pl.ANY)
    out = pl.pallas_call(
        _kernel,
        out_shape=jax.ShapeDtypeStruct((NSEG, 4, 8, D), BF16),
        in_specs=[any_spec] * 12,
        out_specs=any_spec,
        scratch_shapes=[
            pltpu.VMEM((H, D // 2, DH), U32),
            pltpu.VMEM((H, D // 2, DH), U32),
            pltpu.VMEM((H, D // 2, DH), U32),
            pltpu.VMEM((H * DH // 2, D), U32),
            pltpu.VMEM((D // 2, FF), U32),
            pltpu.VMEM((D // 2, FF), U32),
            pltpu.VMEM((FF // 2, D), U32),
            pltpu.VMEM((D // 2, 6 * D), U32),
            pltpu.VMEM((NSEG, 4, 8, D), BF16),
            pltpu.VMEM((NSEG, 4, 8, D), BF16),
            pltpu.VMEM((NSEG, 4, 8, D), BF16),
            pltpu.VMEM((NSEG, 4, 8, D), BF16),
            pltpu.VMEM((NSEG, 3 * NP, 8, DH), U32),
            pltpu.VMEM((NE, D), BF16),
            pltpu.VMEM((NSEG, 3, 8, D), F32),
            pltpu.VMEM((M + SEG + M, D), F32),
            pltpu.VMEM((8, 6 * D), F32),
            pltpu.VMEM((80, 128), F32),
            pltpu.VMEM((SEG, 128), F32),
            pltpu.VMEM((2, 8, D), BF16),
            pltpu.VMEM((8, 128), U32),
            pltpu.VMEM((M, D), BF16),
            pltpu.VMEM((D,), BF16),
            pltpu.VMEM((1, D), BF16),
            pltpu.SemaphoreType.DMA((16 + NP,)),
            pltpu.SemaphoreType.DMA((2,)),
        ],
        compiler_params=pltpu.CompilerParams(vmem_limit_bytes=120 * 1024 * 1024),
    )(
        A_x.reshape(NSEG, 4, 8, D),
        A_mem0.reshape(M, D),
        A_Wq.reshape(D // 2, 2, H, DH),
        A_Wk.reshape(D // 2, 2, H, DH),
        A_Wv.reshape(D // 2, 2, H, DH),
        A_Wo.reshape(H * DH, D),
        B_w_r,
        B_w_gate,
        B_w_up,
        B_w_down,
        c,
        w_mod,
    )
    return out.reshape(1, NSEG * SEG, D)
```

```python
import functools

import jax
import jax.numpy as jnp
import jax.experimental.pallas as pl
import jax.experimental.pallas.tpu as pltpu

F32 = jnp.float32
BF16 = jnp.bfloat16
U32 = jnp.uint32

D = 1024
H = 32
DH = 128
NP = H // 2
M = 8
SEG = 32
NSEG = 64
FF = 3584
NJ = SEG - M
NE = NSEG * M
EPS = 1e-5
SCALE = DH ** (-0.5)
NEG = -1000000000.0
UNROLL = 1
NIT = NSEG // (2 * UNROLL)
OUT_SPLIT = NSEG - 2 * UNROLL - 2


def _rb(x):
    return x.astype(BF16).astype(F32)


def _layernorm(xf):
    m = jnp.mean(xf, axis=-1, keepdims=True)
    d = xf - m
    v = jnp.mean(d * d, axis=-1, keepdims=True)
    return d * jax.lax.rsqrt(v + EPS)


def _dot(a, b):
    return jnp.dot(a, b, preferred_element_type=F32)


def _dot_nt(a, b):
    return jax.lax.dot_general(a, b, (((1,), (1,)), ((), ())), preferred_element_type=F32)


def _kernel(x_hbm, mem0_hbm, wq_hbm, wk_hbm, wv_hbm, wo_hbm, wr_hbm, wg_hbm, wu_hbm, wd_hbm,
            c_hbm, wm_hbm,
            out_hbm,
            wq, wk, wv, wo, wg, wu, wd, wm, xv, x1v, h2v, outv, early, he, hj, pend,
            mod, fill, keys, patch, zero, mem0_ref, wr_ref, c_ref,
            sem, sem_out):
    w_u32 = [w.bitcast(U32) for w in (wq_hbm, wk_hbm, wv_hbm)]
    wqkv = (wq, wk, wv)
    wo_hbm, wg_hbm, wu_hbm, wd_hbm, wm_hbm = [
        w.bitcast(U32) for w in (wo_hbm, wg_hbm, wu_hbm, wd_hbm, wm_hbm)]

    def wblk(w, j, lo=None, hi=None):
        rows = slice(None) if lo is None else slice(lo // 2, hi // 2)
        return pltpu.bitcast(w[rows, j * 128:(j + 1) * 128], BF16)

    def wm_copy(lo, n, k):
        return pltpu.make_async_copy(wm_hbm.at[:, pl.ds(lo, n)], wm.at[:, pl.ds(lo, n)], sem.at[k])

    def w_copies(m, p, k):
        return [pltpu.make_async_copy(w_u32[m].at[:, par, p, :], wqkv[m].at[2 * p + par], sem.at[k])
                for par in range(2)]

    def xj_copy(p, k):
        segs = pl.ds(4 * p, 4)
        return pltpu.make_async_copy(x_hbm.at[segs, 0:3], xv.at[segs, 0:3], sem.at[k])

    def group_copies(p):
        k = 16 + p
        return w_copies(0, p, k) + w_copies(1, p, k) + w_copies(2, p, k) + [xj_copy(p, k)]

    cp_small = [pltpu.make_async_copy(c_hbm, c_ref, sem.at[5]),
                pltpu.make_async_copy(mem0_hbm, mem0_ref, sem.at[5]),
                pltpu.make_async_copy(wr_hbm, wr_ref, sem.at[5])]
    cp_xe = pltpu.make_async_copy(x_hbm.at[:, 3], xv.at[:, 3], sem.at[0])
    cp_wm1 = [wm_copy(j * 512, 512, 1 + j) for j in range(4)]
    cp_w0 = [w_copies(m, 0, 6 + m) for m in range(3)]
    cp_w0[1].append(xj_copy(0, 7))
    cp_late = [wm_copy(2 * D, 4 * D, 9), pltpu.make_async_copy(wo_hbm, wo, sem.at[10])]
    cp_ffn = [pltpu.make_async_copy(wg_hbm, wg, sem.at[11]),
              pltpu.make_async_copy(wu_hbm, wu, sem.at[12]),
              pltpu.make_async_copy(wd_hbm, wd, sem.at[13])]

    for cp in [cp_xe] + cp_small + cp_wm1 + cp_w0[0] + cp_w0[1] + cp_w0[2]:
        cp.start()
    for p in range(1, 8):
        for cp in group_copies(p):
            cp.start()

    ri = jax.lax.broadcasted_iota(jnp.int32, (80, 128), 0)
    ci = jax.lax.broadcasted_iota(jnp.int32, (80, 128), 1)

    def head_of(i):
        return jnp.where(i < 64, i >> 5, (i - 64) >> 3)

    def pos_of(i):
        return jnp.where(i < 64, i & 31, 32 + (i & 7))

    same = (head_of(ri) == head_of(ci)) & (ci < 80)
    allowed = (pos_of(ri) < M) | (pos_of(ri) >= pos_of(ci))
    fill[...] = jnp.where(same, jnp.where(allowed, 0.0, NEG), -jnp.inf).astype(F32)
    keys[...] = jnp.zeros(keys.shape, F32)
    pend[M:, :] = jnp.zeros((SEG + M, D), F32)
    zero[...] = jnp.zeros(zero.shape, U32)

    def pin_zero(vals):
        acc = None
        for v in vals:
            v = pltpu.bitcast(v, U32)
            for r in range(0, v.shape[0], 8):
                acc = v[r:r + 8] if acc is None else acc | v[r:r + 8]
        return acc & zero[...]

    cp_xe.wait()
    for cp in cp_small:
        cp.wait()
    pend[0:M, :] = mem0_ref[...].astype(F32)
    cf = c_ref[...].astype(F32)
    sc = _rb(cf * jax.nn.sigmoid(cf))
    sc = jnp.broadcast_to(sc, (16, D)).astype(BF16)

    def mod_cols(lo, hi):
        for j in range(lo, hi):
            v = _rb(_dot(sc, wblk(wm, j))[0:8])
            if j // 8 in (1, 4):
                v = _rb(1.0 + v)
            mod[:, j * 128:(j + 1) * 128] = v

    def mod_vec(k):
        return mod[:, k * D:(k + 1) * D]

    def affine1(n):
        return _rb(n * mod_vec(1)) + mod_vec(0)

    def ne_body(i, carry):
        n = _layernorm(xv[pl.ds(i * 16, 16), 3].astype(F32))
        he[pl.ds(pl.multiple_of(i * 128, 128), 128), :] = n.reshape(128, D).astype(BF16)
        return carry

    jax.lax.fori_loop(0, NSEG // 16, ne_body, 0)
    for j in range(4):
        cp_wm1[j].wait()
        mod_cols(4 * j, 4 * j + 4)

    def he_body(i, carry):
        rows = pl.ds(pl.multiple_of(i * 128, 128), 128)
        n = he[rows, :].astype(F32).reshape(16, 8, D)
        he[rows, :] = affine1(n).reshape(128, D).astype(BF16)
        return carry

    jax.lax.fori_loop(0, NSEG // 16, he_body, 0)

    def w_head(m, h, lo=0, hi=D):
        return pltpu.bitcast(wqkv[m][h, lo // 2:hi // 2, :], BF16)

    def early_proj(m, p, pins=None, rows=256, between=None):
        w = wqkv[m]
        e = w[2 * p]
        o = w[2 * p + 1]
        w[2 * p] = (e & U32(0xFFFF)) | (o << 16)
        w[2 * p + 1] = (e >> 16) | (o & U32(0xFFFF0000))
        ns = rows // 8
        for c in range(NE // rows):
            hc = he[c * rows:(c + 1) * rows, :]
            r12 = []
            for b in range(2):
                wv_ = w[2 * p + b]
                if pins and 2 * c + b in pins:
                    wv_ = jnp.concatenate([wv_[0:8] | pin_zero([pins[2 * c + b]]), wv_[8:]], axis=0)
                r12.append(_dot(hc, pltpu.bitcast(wv_, BF16)).reshape(ns, 8, DH))
                if between is not None:
                    between()
            r12 = jnp.concatenate(r12, axis=1).reshape(2 * rows, DH)
            early[c * ns:(c + 1) * ns, m * NP + p] = pltpu.bitcast(
                r12.astype(BF16), U32).reshape(ns, 8, DH)

    def make_hj(s):
        h = affine1(_rb(_layernorm(xv[s, 0:3].astype(F32))))
        hj[s] = h
        return h[:, :, 0:128].reshape(NJ, 128)

    for m in range(3):
        for cp in cp_w0[m]:
            cp.wait()
        early_proj(m, 0, {2: make_hj(2 * m - 2), 3: make_hj(2 * m - 1)} if m else None)

    def pro_body(p, carry):
        @pl.when(p == 4)
        def _():
            for pp in range(8, NP):
                for cp in group_copies(pp):
                    cp.start()
            for cp in cp_late + cp_ffn:
                cp.start()

        for cp in group_copies(p):
            cp.wait()
        pins = [make_hj(p * 4 + t) for t in range(4)]
        early_proj(0, p, {3: pins[0]})
        early_proj(1, p, {3: pins[1]})
        early_proj(2, p, {2: pins[2], 3: pins[3]})
        return carry

    with jax.named_scope("prologue_loop"):
        jax.lax.fori_loop(1, NP - 1, pro_body, 0)

    for cp in group_copies(NP - 1) + cp_late:
        cp.wait()
    todo = list(range(16, 48))

    def one_mod_col():
        j = todo.pop(0)
        mod_cols(j, j + 1)

    pins = [make_hj(s) for s in range(NSEG - 4, NSEG)]
    early_proj(0, NP - 1, rows=64, between=one_mod_col)
    early_proj(1, NP - 1, {3: pins[0], 6: pins[1]}, rows=128, between=one_mod_col)
    early_proj(2, NP - 1, {3: pins[2], 6: pins[3]}, rows=128, between=one_mod_col)
    assert not todo

    wr = jnp.broadcast_to(wr_ref[...].astype(F32).reshape(1, D), (8, D))

    lane8 = jax.lax.broadcasted_iota(jnp.int32, (8, 128), 1)
    sub8 = jax.lax.broadcasted_iota(jnp.int32, (8, 128), 0)
    LAST = NSEG * SEG - 1

    def post(s, g0, g1, attn):
        attn = attn.reshape(g1 - g0, 8, D)
        x1 = _rb(xv[s, g0:g1].astype(F32) + _rb(mod_vec(2) * _rb(attn)))
        n = _rb(_layernorm(x1))
        h2 = _rb(_rb(n * mod_vec(4)) + mod_vec(3))
        r = _rb(jnp.sum(h2 * wr, axis=-1, keepdims=True)) + 0.0
        x1v[s, g0:g1] = x1.astype(BF16)
        h2v[s, g0:g1] = h2.astype(BF16)
        outv[s, g0:g1] = (x1 + _rb(mod_vec(5) * h2)).astype(BF16)
        pins = []
        for g in range(g0, g1):
            bits = pltpu.bitcast(jnp.broadcast_to(r[g - g0], (8, 128)), jnp.int32)
            hi = jax.lax.shift_right_logical(bits, 16)
            code = jnp.where(bits < 0, hi ^ 0xFFFF, hi | 0x8000)
            key = (code << 11) | (LAST - (s * SEG + g * 8) - sub8) | 0x40000000
            rows = slice(g * 8, (g + 1) * 8)
            knew = jnp.where(lane8 == s, pltpu.bitcast(key, F32), keys[rows, :])
            keys[rows, :] = knew
            pins.append(knew)
        return pins

    def post_pair(a, rows):
        return post(a + 1, 0, 4, rows[0:SEG]) + post(a, 3, 4, rows[SEG:])

    zpad = jnp.zeros((48, DH), F32)
    G = 4
    KA = (NP - G) * 2 * DH
    KS = D - 128

    def segment(s, lhs, lhs_split, extra, pins):
        qkvs, probs = {}, {}

        def qkv_group(p):
            keys = [(m, 2 * p + b) for m in range(3) for b in range(2 * G)]
            nsplit = 6 if (p == 0 and lhs_split is not None) else 0
            part = [_dot(lhs_split[0], w_head(m, h, 0, KS)) for m, h in keys[:nsplit]]
            full = [_dot(lhs_split[1], w_head(m, h, KS, D)) + part[i]
                    for i, (m, h) in enumerate(keys[:nsplit])]
            full += [_dot(lhs, w_head(m, h)) for m, h in keys[nsplit:]]
            for t in range(G):
                res = []
                for m in range(3):
                    i = 2 * G * m + 2 * t
                    parts = [full[i], full[i + 1],
                             pltpu.bitcast(early[s, m * NP + p + t], BF16).astype(F32)]
                    if m > 0:
                        parts.append(zpad)
                    res.append(jnp.concatenate(parts, axis=0).astype(BF16))
                qkvs[p + t] = res

        def scores(p):
            sc_ = _dot_nt(qkvs[p][0], qkvs[p][1]) * SCALE
            f = fill[...]
            if pins.get(p):
                f = jnp.concatenate([f[0:8] + pltpu.bitcast(pin_zero(pins[p]), F32), f[8:]], axis=0)
            sc_ = jnp.where(f == 0.0, sc_, f)
            mx = jnp.max(sc_, axis=-1, keepdims=True)
            e = jnp.exp(sc_ - mx)
            den = jnp.sum(e, axis=-1, keepdims=True)
            inv = pl.reciprocal(den, approx=True)
            probs[p] = e.astype(BF16), inv * (2.0 - den * inv)

        oe = []

        def pv(p):
            o = _dot(probs[p][0], qkvs[p][2]) * probs[p][1]
            res = []
            for b in range(2):
                rows, erows = o[32 * b:32 * b + 32], o[64 + 8 * b:72 + 8 * b]
                oe.append(erows)
                if extra is not None:
                    rows = jnp.concatenate([rows, erows, extra[2 * p + b]], axis=0)
                res.append(rows)
            pins.setdefault(p + G, []).append(o)
            return res

        os_ = []
        for p in range(0, NP, G):
            qkv_group(p)
            if p >= G:
                for t in range(G):
                    os_ += pv(p - G + t)
            for t in range(G):
                scores(p + t)
        oa = jnp.concatenate(os_, axis=1).astype(BF16)
        acc, ob = [], []
        for n in range(7):
            acc.append(_dot(oa, wblk(wo, n, 0, KA)))
            if n == 2:
                for t in range(G):
                    ob += pv(NP - G + t)
        ob = jnp.concatenate(ob, axis=1).astype(BF16)
        res = [_dot(ob, wblk(wo, n, KA, H * DH)) + acc[n] for n in range(7)]
        res.append(_dot(ob, wblk(wo, 7, KA, H * DH)) + _dot(oa, wblk(wo, 7, 0, KA)))
        return res, oe

    def make_lhs(mem, s):
        return jnp.concatenate([mem, hj[s].reshape(NJ, D)], axis=0)

    cp_o1 = pltpu.make_async_copy(outv.at[0:OUT_SPLIT], out_hbm.at[0:OUT_SPLIT], sem_out.at[0])
    cp_o2 = pltpu.make_async_copy(outv.at[OUT_SPLIT:NSEG], out_hbm.at[OUT_SPLIT:NSEG],
                                  sem_out.at[1])

    def split_lhs(lhs):
        return lhs.astype(BF16), (lhs[:, :KS].astype(BF16), lhs[:, KS:].astype(BF16))

    def step(i, carry):
        @pl.when(i == NIT - 1)
        def _():
            cp_o1.start()

        prev = pend[...]
        for u in range(UNROLL):
            a = 2 * (UNROLL * i + u)
            pins = post_pair(jnp.maximum(a - 2, 0) if u == 0 else a - 2, prev[M:])
            lhs_a = make_lhs(prev[0:M], a)
            lhs_a = (lhs_a.astype(BF16), None) if u == 0 else split_lhs(lhs_a)
            res_a, oe_a = segment(a, *lhs_a, None,
                                  {k: [v] for k, v in zip((4, 5, 8, 9, 12), pins)})
            res_a = jnp.concatenate(res_a, axis=1)
            pins = post(a, 0, 3, res_a[M:])
            res_b, _ = segment(a + 1, *split_lhs(make_lhs(res_a[0:M], a + 1)), oe_a,
                               {k: [v] for k, v in zip((4, 8, 12), pins)})
            prev = jnp.concatenate(res_b, axis=1)
        pend[...] = prev
        return carry

    with jax.named_scope("main_loop"):
        jax.lax.fori_loop(0, NIT, step, 0)
    post_pair(NSEG - 2, pend[M:, :])
    cp_o2.start()

    def max_all(v):
        return jnp.max(jnp.max(v, axis=0, keepdims=True), axis=1, keepdims=True)

    def decode(k):
        kb = pltpu.bitcast(jnp.broadcast_to(k, (8, 128)), jnp.int32)
        code = (kb >> 11) & 0xFFFF
        hi = jnp.where(code >= 0x8000, code & 0x7FFF, code ^ 0xFFFF)
        return (LAST - (kb & LAST))[0, 0], pltpu.bitcast(hi << 16, F32)[:, 0:1]

    kv = keys[...]
    k1 = max_all(kv)
    k2 = max_all(jnp.where(kv == k1, 0.0, kv))
    i1, r1 = decode(k1)
    i2, r2 = decode(k2)
    g1, g2 = i1 >> 3, i2 >> 3

    def rows_of(ref):
        return jnp.concatenate([ref[g1 >> 2, pl.ds(g1 & 3, 1)], ref[g2 >> 2, pl.ds(g2 & 3, 1)]],
                               axis=0).astype(F32)

    x1, h2 = rows_of(x1v), rows_of(h2v)
    for cp in cp_ffn:
        cp.wait()
    hl = h2.reshape(16, D).astype(BF16)
    act = []
    for j in range(FF // 128):
        gt = _rb(_dot(hl, wblk(wg, j)))
        up = _rb(_dot(hl, wblk(wu, j)))
        act.append((_rb(gt * jax.nn.sigmoid(gt)) * up).astype(BF16))
    act = jnp.concatenate(act, axis=1)
    y = jnp.concatenate([_dot(act, wblk(wd, n)) for n in range(8)], axis=1).reshape(2, 8, D)
    rowi = jax.lax.broadcasted_iota(jnp.int32, (2, 8, 1), 1)
    gsel = jax.lax.broadcasted_iota(jnp.int32, (2, 8, 1), 0)
    tokp = jnp.where(gsel == 0, g1, g2) * 8 + rowi
    gate = _rb(jax.nn.sigmoid(jnp.where(tokp == i1, r1[None], r2[None])))
    upd = jnp.where((tokp == i1) | (tokp == i2), _rb(_rb(y) * gate), 0.0)
    patch[...] = (x1 + _rb(mod_vec(5) * _rb(h2 + upd))).astype(BF16)
    cp_o1.wait()
    cp_o2.wait()
    cp1 = pltpu.make_async_copy(patch.at[0], out_hbm.at[g1 >> 2, g1 & 3], sem_out.at[0])
    cp1.start()

    @pl.when(g1 != g2)
    def _():
        cp2 = pltpu.make_async_copy(patch.at[1], out_hbm.at[g2 >> 2, g2 & 3], sem_out.at[1])
        cp2.start()
        cp2.wait()

    cp1.wait()


@functools.partial(jax.jit, static_argnames=("A_seg_len",))
def pallas_adaLN_cond__memory_aug_recurrent_mem_tr__moe_arch_mod__prompt_kernel(
    A_x: jax.Array,
    A_mem0: jax.Array,
    A_Wq: jax.Array,
    A_Wk: jax.Array,
    A_Wv: jax.Array,
    A_Wo: jax.Array,
    A_seg_len,
    B_x: jax.Array,
    B_w_r: jax.Array,
    B_w_gate: jax.Array,
    B_w_up: jax.Array,
    B_w_down: jax.Array,
    c: jax.Array,
    w_mod: jax.Array,
):
    assert A_seg_len == SEG and A_x.shape == (1, NSEG * SEG, D)
    any_spec = pl.BlockSpec(memory_space=pl.ANY)
    out = pl.pallas_call(
        _kernel,
        out_shape=jax.ShapeDtypeStruct((NSEG, 4, 8, D), BF16),
        in_specs=[any_spec] * 12,
        out_specs=any_spec,
        scratch_shapes=[
            pltpu.VMEM((H, D // 2, DH), U32),
            pltpu.VMEM((H, D // 2, DH), U32),
            pltpu.VMEM((H, D // 2, DH), U32),
            pltpu.VMEM((H * DH // 2, D), U32),
            pltpu.VMEM((D // 2, FF), U32),
            pltpu.VMEM((D // 2, FF), U32),
            pltpu.VMEM((FF // 2, D), U32),
            pltpu.VMEM((D // 2, 6 * D), U32),
            pltpu.VMEM((NSEG, 4, 8, D), BF16),
            pltpu.VMEM((NSEG, 4, 8, D), BF16),
            pltpu.VMEM((NSEG, 4, 8, D), BF16),
            pltpu.VMEM((NSEG, 4, 8, D), BF16),
            pltpu.VMEM((NSEG, 3 * NP, 8, DH), U32),
            pltpu.VMEM((NE, D), BF16),
            pltpu.VMEM((NSEG, 3, 8, D), F32),
            pltpu.VMEM((M + SEG + M, D), F32),
            pltpu.VMEM((8, 6 * D), F32),
            pltpu.VMEM((80, 128), F32),
            pltpu.VMEM((SEG, 128), F32),
            pltpu.VMEM((2, 8, D), BF16),
            pltpu.VMEM((8, 128), U32),
            pltpu.VMEM((M, D), BF16),
            pltpu.VMEM((D,), BF16),
            pltpu.VMEM((1, D), BF16),
            pltpu.SemaphoreType.DMA((16 + NP,)),
            pltpu.SemaphoreType.DMA((2,)),
        ],
        compiler_params=pltpu.CompilerParams(vmem_limit_bytes=120 * 1024 * 1024),
    )(
        A_x.reshape(NSEG, 4, 8, D),
        A_mem0.reshape(M, D),
        A_Wq.reshape(D // 2, 2, H, DH),
        A_Wk.reshape(D // 2, 2, H, DH),
        A_Wv.reshape(D // 2, 2, H, DH),
        A_Wo.reshape(H * DH, D),
        B_w_r,
        B_w_gate,
        B_w_up,
        B_w_down,
        c,
        w_mod,
    )
    return out.reshape(1, NSEG * SEG, D)
```

```python
import functools

import jax
import jax.numpy as jnp
import jax.experimental.pallas as pl
import jax.experimental.pallas.tpu as pltpu

F32 = jnp.float32
BF16 = jnp.bfloat16
U32 = jnp.uint32

D = 1024
H = 32
DH = 128
NP = H // 2
M = 8
SEG = 32
NSEG = 64
FF = 3584
NJ = SEG - M
NE = NSEG * M
EPS = 1e-5
SCALE = DH ** (-0.5)
NEG = -1000000000.0
UNROLL = 2
NIT = NSEG // (2 * UNROLL)
OUT_SPLIT = NSEG - 2 * UNROLL - 2


def _rb(x):
    return x.astype(BF16).astype(F32)


def _layernorm(xf):
    m = jnp.mean(xf, axis=-1, keepdims=True)
    d = xf - m
    v = jnp.mean(d * d, axis=-1, keepdims=True)
    return d * jax.lax.rsqrt(v + EPS)


def _dot(a, b):
    return jnp.dot(a, b, preferred_element_type=F32)


def _dot_nt(a, b):
    return jax.lax.dot_general(a, b, (((1,), (1,)), ((), ())), preferred_element_type=F32)


def _kernel(x_hbm, mem0_hbm, wq_hbm, wk_hbm, wv_hbm, wo_hbm, wr_hbm, wg_hbm, wu_hbm, wd_hbm,
            c_hbm, wm_hbm,
            out_hbm,
            wq, wk, wv, wo, wg, wu, wd, wm, xv, x1v, h2v, outv, early, he, hj, pend,
            mod, fill, keys, patch, zero, opnd, mem0_ref, wr_ref, c_ref,
            sem, sem_out):
    w_u32 = [w.bitcast(U32) for w in (wq_hbm, wk_hbm, wv_hbm)]
    wqkv = (wq, wk, wv)
    wo_hbm, wg_hbm, wu_hbm, wd_hbm, wm_hbm = [
        w.bitcast(U32) for w in (wo_hbm, wg_hbm, wu_hbm, wd_hbm, wm_hbm)]

    def wblk(w, j, lo=None, hi=None):
        rows = slice(None) if lo is None else slice(lo // 2, hi // 2)
        return pltpu.bitcast(w[rows, j * 128:(j + 1) * 128], BF16)

    def wm_copy(lo, n, k):
        return pltpu.make_async_copy(wm_hbm.at[:, pl.ds(lo, n)], wm.at[:, pl.ds(lo, n)], sem.at[k])

    def w_copies(m, p, k):
        return [pltpu.make_async_copy(w_u32[m].at[:, par, p, :], wqkv[m].at[2 * p + par], sem.at[k])
                for par in range(2)]

    def xj_copy(p, k):
        segs = pl.ds(4 * p, 4)
        return pltpu.make_async_copy(x_hbm.at[segs, 0:3], xv.at[segs, 0:3], sem.at[k])

    def group_copies(p):
        k = 16 + p
        return w_copies(0, p, k) + w_copies(1, p, k) + w_copies(2, p, k) + [xj_copy(p, k)]

    cp_small = [pltpu.make_async_copy(c_hbm, c_ref, sem.at[5]),
                pltpu.make_async_copy(mem0_hbm, mem0_ref, sem.at[5]),
                pltpu.make_async_copy(wr_hbm, wr_ref, sem.at[5])]
    cp_xe = pltpu.make_async_copy(x_hbm.at[:, 3], xv.at[:, 3], sem.at[0])
    cp_wm1 = [wm_copy(j * 512, 512, 1 + j) for j in range(4)]
    cp_w0 = [w_copies(m, 0, 6 + m) for m in range(3)]
    cp_w0[1].append(xj_copy(0, 7))
    cp_late = [wm_copy(2 * D, 4 * D, 9), pltpu.make_async_copy(wo_hbm, wo, sem.at[10])]
    cp_ffn = [pltpu.make_async_copy(wg_hbm, wg, sem.at[11]),
              pltpu.make_async_copy(wu_hbm, wu, sem.at[12]),
              pltpu.make_async_copy(wd_hbm, wd, sem.at[13])]

    for cp in [cp_xe] + cp_small + cp_wm1 + cp_w0[0] + cp_w0[1] + cp_w0[2]:
        cp.start()
    for p in range(1, 8):
        for cp in group_copies(p):
            cp.start()

    ri = jax.lax.broadcasted_iota(jnp.int32, (80, 128), 0)
    ci = jax.lax.broadcasted_iota(jnp.int32, (80, 128), 1)

    def head_of(i):
        return jnp.where(i < 64, i >> 5, (i - 64) >> 3)

    def pos_of(i):
        return jnp.where(i < 64, i & 31, 32 + (i & 7))

    same = (head_of(ri) == head_of(ci)) & (ci < 80)
    allowed = (pos_of(ri) < M) | (pos_of(ri) >= pos_of(ci))
    fill[...] = jnp.where(same, jnp.where(allowed, 0.0, NEG), -jnp.inf).astype(F32)
    keys[...] = jnp.zeros(keys.shape, F32)
    pend[M:, :] = jnp.zeros((SEG + M, D), F32)
    zero[...] = jnp.zeros(zero.shape, U32)
    opnd[...] = jnp.zeros(opnd.shape, U32)

    def pin_zero(vals):
        acc = None
        for v in vals:
            v = pltpu.bitcast(v, U32)
            for r in range(0, v.shape[0], 8):
                acc = v[r:r + 8] if acc is None else acc | v[r:r + 8]
        return acc & zero[...]

    cp_xe.wait()
    for cp in cp_small:
        cp.wait()
    pend[0:M, :] = mem0_ref[...].astype(F32)
    cf = c_ref[...].astype(F32)
    sc = _rb(cf * jax.nn.sigmoid(cf))
    sc = jnp.broadcast_to(sc, (16, D)).astype(BF16)

    def mod_cols(lo, hi):
        for j in range(lo, hi):
            v = _rb(_dot(sc, wblk(wm, j))[0:8])
            if j // 8 in (1, 4):
                v = _rb(1.0 + v)
            mod[:, j * 128:(j + 1) * 128] = v

    def mod_vec(k):
        return mod[:, k * D:(k + 1) * D]

    def affine1(n):
        return _rb(n * mod_vec(1)) + mod_vec(0)

    def ne_body(i, carry):
        n = _layernorm(xv[pl.ds(i * 16, 16), 3].astype(F32))
        he[pl.ds(pl.multiple_of(i * 128, 128), 128), :] = n.reshape(128, D).astype(BF16)
        return carry

    jax.lax.fori_loop(0, NSEG // 16, ne_body, 0)
    for j in range(4):
        cp_wm1[j].wait()
        mod_cols(4 * j, 4 * j + 4)

    def he_body(i, carry):
        rows = pl.ds(pl.multiple_of(i * 128, 128), 128)
        n = he[rows, :].astype(F32).reshape(16, 8, D)
        he[rows, :] = affine1(n).reshape(128, D).astype(BF16)
        return carry

    jax.lax.fori_loop(0, NSEG // 16, he_body, 0)

    def w_head(m, h, lo=0, hi=D):
        return pltpu.bitcast(wqkv[m][h, lo // 2:hi // 2, :], BF16)

    def early_proj(m, p, pins=None, rows=256, between=None):
        w = wqkv[m]
        e = w[2 * p]
        o = w[2 * p + 1]
        w[2 * p] = (e & U32(0xFFFF)) | (o << 16)
        w[2 * p + 1] = (e >> 16) | (o & U32(0xFFFF0000))
        ns = rows // 8
        for c in range(NE // rows):
            hc = he[c * rows:(c + 1) * rows, :]
            r12 = []
            for b in range(2):
                wv_ = w[2 * p + b]
                if pins and 2 * c + b in pins:
                    wv_ = jnp.concatenate([wv_[0:8] | pin_zero([pins[2 * c + b]]), wv_[8:]], axis=0)
                r12.append(_dot(hc, pltpu.bitcast(wv_, BF16)).reshape(ns, 8, DH))
                if between is not None:
                    between()
            r12 = jnp.concatenate(r12, axis=1).reshape(2 * rows, DH)
            early[c * ns:(c + 1) * ns, m * NP + p] = pltpu.bitcast(
                r12.astype(BF16), U32).reshape(ns, 8, DH)

    def make_hj(s):
        h = affine1(_rb(_layernorm(xv[s, 0:3].astype(F32))))
        hj[s] = h
        return h[:, :, 0:128].reshape(NJ, 128)

    for m in range(3):
        for cp in cp_w0[m]:
            cp.wait()
        early_proj(m, 0, {2: make_hj(2 * m - 2), 3: make_hj(2 * m - 1)} if m else None)

    def pro_body(p, carry):
        @pl.when(p == 4)
        def _():
            for pp in range(8, NP):
                for cp in group_copies(pp):
                    cp.start()
            for cp in cp_late + cp_ffn:
                cp.start()

        for cp in group_copies(p):
            cp.wait()
        pins = [make_hj(p * 4 + t) for t in range(4)]
        early_proj(0, p, {3: pins[0]})
        early_proj(1, p, {3: pins[1]})
        early_proj(2, p, {2: pins[2], 3: pins[3]})
        return carry

    with jax.named_scope("prologue_loop"):
        jax.lax.fori_loop(1, NP - 1, pro_body, 0)

    for cp in group_copies(NP - 1) + cp_late:
        cp.wait()
    todo = list(range(16, 48))

    def one_mod_col():
        j = todo.pop(0)
        mod_cols(j, j + 1)

    pins = [make_hj(s) for s in range(NSEG - 4, NSEG)]
    early_proj(0, NP - 1, rows=64, between=one_mod_col)
    early_proj(1, NP - 1, {3: pins[0], 6: pins[1]}, rows=128, between=one_mod_col)
    early_proj(2, NP - 1, {3: pins[2], 6: pins[3]}, rows=128, between=one_mod_col)
    assert not todo

    wr = jnp.broadcast_to(wr_ref[...].astype(F32).reshape(1, D), (8, D))

    lane8 = jax.lax.broadcasted_iota(jnp.int32, (8, 128), 1)
    sub8 = jax.lax.broadcasted_iota(jnp.int32, (8, 128), 0)
    LAST = NSEG * SEG - 1

    def post(s, g0, g1, attn):
        attn = attn.reshape(g1 - g0, 8, D)
        x1 = _rb(xv[s, g0:g1].astype(F32) + _rb(mod_vec(2) * _rb(attn)))
        n = _rb(_layernorm(x1))
        h2 = _rb(_rb(n * mod_vec(4)) + mod_vec(3))
        r = _rb(jnp.sum(h2 * wr, axis=-1, keepdims=True)) + 0.0
        x1v[s, g0:g1] = x1.astype(BF16)
        h2v[s, g0:g1] = h2.astype(BF16)
        outv[s, g0:g1] = (x1 + _rb(mod_vec(5) * h2)).astype(BF16)
        pins = []
        for g in range(g0, g1):
            bits = pltpu.bitcast(jnp.broadcast_to(r[g - g0], (8, 128)), jnp.int32)
            hi = jax.lax.shift_right_logical(bits, 16)
            code = jnp.where(bits < 0, hi ^ 0xFFFF, hi | 0x8000)
            key = (code << 11) | (LAST - (s * SEG + g * 8) - sub8) | 0x40000000
            rows = slice(g * 8, (g + 1) * 8)
            knew = jnp.where(lane8 == s, pltpu.bitcast(key, F32), keys[rows, :])
            keys[rows, :] = knew
            pins.append(knew)
        return pins

    def post_pair(a, rows):
        return post(a + 1, 0, 4, rows[0:SEG]) + post(a, 3, 4, rows[SEG:])

    zpad = jnp.zeros((24, DH), U32)
    G = 4
    KA = (NP - G) * 2 * DH
    KS = D - 128

    def segment(s, lhs, lhs_split, extra, pins):
        probs = {}
        always = zero[...] == 0

        def stash(p, m, v):
            v = pltpu.bitcast(v.astype(BF16), U32)
            n = v.shape[0]
            pltpu.store(opnd.at[p, m, 0:n, :], v, mask=jnp.concatenate([always] * (n // 8), axis=0))

        def qkv_group(p):
            keys = [(m, 2 * p + b) for m in range(3) for b in range(2 * G)]
            nsplit = 6 if (p == 0 and lhs_split is not None) else 0
            part = [_dot(lhs_split[0], w_head(m, h, 0, KS)) for m, h in keys[:nsplit]]
            full = [_dot(lhs_split[1], w_head(m, h, KS, D)) + part[i]
                    for i, (m, h) in enumerate(keys[:nsplit])]
            full += [_dot(lhs, w_head(m, h)) for m, h in keys[nsplit:]]
            for m in range(3):
                for t in range(G):
                    i = 2 * G * m + 2 * t
                    stash(p + t, m, jnp.concatenate([full[i], full[i + 1]], axis=0))

        def operand(p, m):
            parts = [opnd[p, m, 0:32, :], early[s, m * NP + p]]
            if m > 0:
                parts.append(zpad)
            return pltpu.bitcast(jnp.concatenate(parts, axis=0), BF16)

        def scores(p):
            sc_ = _dot_nt(operand(p, 0), operand(p, 1)) * SCALE
            f = fill[...]
            if pins.get(p):
                f = jnp.concatenate([f[0:8] + pltpu.bitcast(pin_zero(pins[p]), F32), f[8:]], axis=0)
            sc_ = jnp.where(f == 0.0, sc_, f)
            mx = jnp.max(sc_, axis=-1, keepdims=True)
            e = jnp.exp(sc_ - mx)
            den = jnp.sum(e, axis=-1, keepdims=True)
            inv = pl.reciprocal(den, approx=True)
            stash(p, 3, e)
            probs[p] = inv * (2.0 - den * inv)

        oe = []

        def pv(p):
            o = _dot(pltpu.bitcast(opnd[p, 3], BF16), operand(p, 2)) * probs[p]
            res = []
            for b in range(2):
                rows, erows = o[32 * b:32 * b + 32], o[64 + 8 * b:72 + 8 * b]
                oe.append(erows)
                if extra is not None:
                    rows = jnp.concatenate([rows, erows, extra[2 * p + b]], axis=0)
                res.append(rows)
            pins.setdefault(p + G, []).append(o)
            return res

        os_ = []
        for p in range(0, NP, G):
            qkv_group(p)
            if p >= G:
                for t in range(G):
                    os_ += pv(p - G + t)
            for t in range(G):
                scores(p + t)
        oa = jnp.concatenate(os_, axis=1).astype(BF16)
        acc, ob = [], []
        for n in range(7):
            acc.append(_dot(oa, wblk(wo, n, 0, KA)))
            if n == 2:
                for t in range(G):
                    ob += pv(NP - G + t)
        ob = jnp.concatenate(ob, axis=1).astype(BF16)
        res = [_dot(ob, wblk(wo, n, KA, H * DH)) + acc[n] for n in range(7)]
        res.append(_dot(ob, wblk(wo, 7, KA, H * DH)) + _dot(oa, wblk(wo, 7, 0, KA)))
        return res, oe

    def make_lhs(mem, s):
        return jnp.concatenate([mem, hj[s].reshape(NJ, D)], axis=0)

    cp_o1 = pltpu.make_async_copy(outv.at[0:OUT_SPLIT], out_hbm.at[0:OUT_SPLIT], sem_out.at[0])
    cp_o2 = pltpu.make_async_copy(outv.at[OUT_SPLIT:NSEG], out_hbm.at[OUT_SPLIT:NSEG],
                                  sem_out.at[1])

    def split_lhs(lhs):
        return lhs.astype(BF16), (lhs[:, :KS].astype(BF16), lhs[:, KS:].astype(BF16))

    def step(i, carry):
        @pl.when(i == NIT - 1)
        def _():
            cp_o1.start()

        prev = pend[...]
        for u in range(UNROLL):
            a = 2 * (UNROLL * i + u)
            pins = post_pair(jnp.maximum(a - 2, 0) if u == 0 else a - 2, prev[M:])
            lhs_a = make_lhs(prev[0:M], a)
            lhs_a = (lhs_a.astype(BF16), None) if u == 0 else split_lhs(lhs_a)
            res_a, oe_a = segment(a, *lhs_a, None,
                                  {k: [v] for k, v in zip((0, 4, 8, 12), pins[:4])})
            res_a = jnp.concatenate(res_a, axis=1)
            pins = pins[4:] + post(a, 0, 3, res_a[M:])
            res_b, _ = segment(a + 1, *split_lhs(make_lhs(res_a[0:M], a + 1)), oe_a,
                               {k: [v] for k, v in zip((0, 4, 8, 12), pins)})
            prev = jnp.concatenate(res_b, axis=1)
        pend[...] = prev
        return carry

    with jax.named_scope("main_loop"):
        jax.lax.fori_loop(0, NIT, step, 0)
    post_pair(NSEG - 2, pend[M:, :])
    cp_o2.start()

    def max_all(v):
        return jnp.max(jnp.max(v, axis=0, keepdims=True), axis=1, keepdims=True)

    def decode(k):
        kb = pltpu.bitcast(jnp.broadcast_to(k, (8, 128)), jnp.int32)
        code = (kb >> 11) & 0xFFFF
        hi = jnp.where(code >= 0x8000, code & 0x7FFF, code ^ 0xFFFF)
        return (LAST - (kb & LAST))[0, 0], pltpu.bitcast(hi << 16, F32)[:, 0:1]

    kv = keys[...]
    k1 = max_all(kv)
    k2 = max_all(jnp.where(kv == k1, 0.0, kv))
    i1, r1 = decode(k1)
    i2, r2 = decode(k2)
    g1, g2 = i1 >> 3, i2 >> 3

    def rows_of(ref):
        return jnp.concatenate([ref[g1 >> 2, pl.ds(g1 & 3, 1)], ref[g2 >> 2, pl.ds(g2 & 3, 1)]],
                               axis=0).astype(F32)

    x1, h2 = rows_of(x1v), rows_of(h2v)
    for cp in cp_ffn:
        cp.wait()
    hl = h2.reshape(16, D).astype(BF16)
    act = []
    for j in range(FF // 128):
        gt = _rb(_dot(hl, wblk(wg, j)))
        up = _rb(_dot(hl, wblk(wu, j)))
        act.append((_rb(gt * jax.nn.sigmoid(gt)) * up).astype(BF16))
    act = jnp.concatenate(act, axis=1)
    y = jnp.concatenate([_dot(act, wblk(wd, n)) for n in range(8)], axis=1).reshape(2, 8, D)
    rowi = jax.lax.broadcasted_iota(jnp.int32, (2, 8, 1), 1)
    gsel = jax.lax.broadcasted_iota(jnp.int32, (2, 8, 1), 0)
    tokp = jnp.where(gsel == 0, g1, g2) * 8 + rowi
    gate = _rb(jax.nn.sigmoid(jnp.where(tokp == i1, r1[None], r2[None])))
    upd = jnp.where((tokp == i1) | (tokp == i2), _rb(_rb(y) * gate), 0.0)
    patch[...] = (x1 + _rb(mod_vec(5) * _rb(h2 + upd))).astype(BF16)
    cp_o1.wait()
    cp_o2.wait()
    cp1 = pltpu.make_async_copy(patch.at[0], out_hbm.at[g1 >> 2, g1 & 3], sem_out.at[0])
    cp1.start()

    @pl.when(g1 != g2)
    def _():
        cp2 = pltpu.make_async_copy(patch.at[1], out_hbm.at[g2 >> 2, g2 & 3], sem_out.at[1])
        cp2.start()
        cp2.wait()

    cp1.wait()


@functools.partial(jax.jit, static_argnames=("A_seg_len",))
def pallas_adaLN_cond__memory_aug_recurrent_mem_tr__moe_arch_mod__prompt_kernel(
    A_x: jax.Array,
    A_mem0: jax.Array,
    A_Wq: jax.Array,
    A_Wk: jax.Array,
    A_Wv: jax.Array,
    A_Wo: jax.Array,
    A_seg_len,
    B_x: jax.Array,
    B_w_r: jax.Array,
    B_w_gate: jax.Array,
    B_w_up: jax.Array,
    B_w_down: jax.Array,
    c: jax.Array,
    w_mod: jax.Array,
):
    assert A_seg_len == SEG and A_x.shape == (1, NSEG * SEG, D)
    any_spec = pl.BlockSpec(memory_space=pl.ANY)
    out = pl.pallas_call(
        _kernel,
        out_shape=jax.ShapeDtypeStruct((NSEG, 4, 8, D), BF16),
        in_specs=[any_spec] * 12,
        out_specs=any_spec,
        scratch_shapes=[
            pltpu.VMEM((H, D // 2, DH), U32),
            pltpu.VMEM((H, D // 2, DH), U32),
            pltpu.VMEM((H, D // 2, DH), U32),
            pltpu.VMEM((H * DH // 2, D), U32),
            pltpu.VMEM((D // 2, FF), U32),
            pltpu.VMEM((D // 2, FF), U32),
            pltpu.VMEM((FF // 2, D), U32),
            pltpu.VMEM((D // 2, 6 * D), U32),
            pltpu.VMEM((NSEG, 4, 8, D), BF16),
            pltpu.VMEM((NSEG, 4, 8, D), BF16),
            pltpu.VMEM((NSEG, 4, 8, D), BF16),
            pltpu.VMEM((NSEG, 4, 8, D), BF16),
            pltpu.VMEM((NSEG, 3 * NP, 8, DH), U32),
            pltpu.VMEM((NE, D), BF16),
            pltpu.VMEM((NSEG, 3, 8, D), F32),
            pltpu.VMEM((M + SEG + M, D), F32),
            pltpu.VMEM((8, 6 * D), F32),
            pltpu.VMEM((80, 128), F32),
            pltpu.VMEM((SEG, 128), F32),
            pltpu.VMEM((2, 8, D), BF16),
            pltpu.VMEM((8, 128), U32),
            pltpu.VMEM((NP, 4, 40, DH), U32),
            pltpu.VMEM((M, D), BF16),
            pltpu.VMEM((D,), BF16),
            pltpu.VMEM((1, D), BF16),
            pltpu.SemaphoreType.DMA((16 + NP,)),
            pltpu.SemaphoreType.DMA((2,)),
        ],
        compiler_params=pltpu.CompilerParams(vmem_limit_bytes=120 * 1024 * 1024),
    )(
        A_x.reshape(NSEG, 4, 8, D),
        A_mem0.reshape(M, D),
        A_Wq.reshape(D // 2, 2, H, DH),
        A_Wk.reshape(D // 2, 2, H, DH),
        A_Wv.reshape(D // 2, 2, H, DH),
        A_Wo.reshape(H * DH, D),
        B_w_r,
        B_w_gate,
        B_w_up,
        B_w_down,
        c,
        w_mod,
    )
    return out.reshape(1, NSEG * SEG, D)
```

```python
import jax
import jax.numpy as jnp
import jax.experimental.pallas as pl
import jax.experimental.pallas.tpu as pltpu

F32 = jnp.float32
BF16 = jnp.bfloat16
U32 = jnp.uint32

D = 1024
H = 32
DH = 128
NP = H // 2
M = 8
SEG = 32
NSEG = 64
FF = 3584
NJ = SEG - M
NE = NSEG * M
EPS = 1e-5
SCALE = DH ** (-0.5)
NEG = -1000000000.0
UNROLL = 2
NIT = NSEG // (2 * UNROLL)
OUT_SPLIT = NSEG - 2 * UNROLL - 2


def _rb(x):
    return x.astype(BF16).astype(F32)


def _layernorm(xf):
    m = jnp.mean(xf, axis=-1, keepdims=True)
    d = xf - m
    v = jnp.mean(d * d, axis=-1, keepdims=True)
    return d * jax.lax.rsqrt(v + EPS)


def _dot(a, b):
    return jnp.dot(a, b, preferred_element_type=F32)


def _dot_nt(a, b):
    return jax.lax.dot_general(a, b, (((1,), (1,)), ((), ())), preferred_element_type=F32)


def _kernel(x_hbm, mem0_hbm, wq_hbm, wk_hbm, wv_hbm, wo_hbm, wr_hbm, wg_hbm, wu_hbm, wd_hbm,
            c_hbm, wm_hbm,
            out_hbm,
            wq, wk, wv, wo, wg, wu, wd, wm, xv, x1v, h2v, outv, early, he, hj, pend,
            mod, fill, keys, patch, zero, opnd, mem0_ref, wr_ref, c_ref,
            sem, sem_out):
    w_u32 = [w.bitcast(U32) for w in (wq_hbm, wk_hbm, wv_hbm)]
    wqkv = (wq, wk, wv)
    wo_hbm, wg_hbm, wu_hbm, wd_hbm, wm_hbm = [
        w.bitcast(U32) for w in (wo_hbm, wg_hbm, wu_hbm, wd_hbm, wm_hbm)]

    def wblk(w, j, lo=None, hi=None):
        rows = slice(None) if lo is None else slice(lo // 2, hi // 2)
        return pltpu.bitcast(w[rows, j * 128:(j + 1) * 128], BF16)

    def wm_copy(lo, n, k):
        return pltpu.make_async_copy(wm_hbm.at[:, pl.ds(lo, n)], wm.at[:, pl.ds(lo, n)], sem.at[k])

    def w_copies(m, p, k):
        return [pltpu.make_async_copy(w_u32[m].at[:, par, p, :], wqkv[m].at[2 * p + par], sem.at[k])
                for par in range(2)]

    def xj_copy(p, k):
        segs = pl.ds(4 * p, 4)
        return pltpu.make_async_copy(x_hbm.at[segs, 0:3], xv.at[segs, 0:3], sem.at[k])

    def group_copies(p):
        k = 16 + p
        return w_copies(0, p, k) + w_copies(1, p, k) + w_copies(2, p, k) + [xj_copy(p, k)]

    cp_small = [pltpu.make_async_copy(c_hbm, c_ref, sem.at[5]),
                pltpu.make_async_copy(mem0_hbm, mem0_ref, sem.at[5]),
                pltpu.make_async_copy(wr_hbm, wr_ref, sem.at[5])]
    cp_xe = pltpu.make_async_copy(x_hbm.at[:, 3], xv.at[:, 3], sem.at[0])
    cp_wm1 = [wm_copy(j * 512, 512, 1 + j) for j in range(4)]
    cp_w0 = [w_copies(m, 0, 6 + m) for m in range(3)]
    cp_w0[1].append(xj_copy(0, 7))
    cp_late = [wm_copy(2 * D, 4 * D, 9), pltpu.make_async_copy(wo_hbm, wo, sem.at[10])]
    cp_ffn = [pltpu.make_async_copy(wg_hbm, wg, sem.at[11]),
              pltpu.make_async_copy(wu_hbm, wu, sem.at[12]),
              pltpu.make_async_copy(wd_hbm, wd, sem.at[13])]

    for cp in [cp_xe] + cp_small + cp_wm1 + cp_w0[0] + cp_w0[1] + cp_w0[2]:
        cp.start()
    for p in range(1, 8):
        for cp in group_copies(p):
            cp.start()

    ri = jax.lax.broadcasted_iota(jnp.int32, (80, 128), 0)
    ci = jax.lax.broadcasted_iota(jnp.int32, (80, 128), 1)

    def head_of(i):
        return jnp.where(i < 64, i >> 5, (i - 64) >> 3)

    def pos_of(i):
        return jnp.where(i < 64, i & 31, 32 + (i & 7))

    same = (head_of(ri) == head_of(ci)) & (ci < 80)
    allowed = (pos_of(ri) < M) | (pos_of(ri) >= pos_of(ci))
    fill[...] = jnp.where(same, jnp.where(allowed, 0.0, NEG), -jnp.inf).astype(F32)
    keys[...] = jnp.zeros(keys.shape, F32)
    pend[M:, :] = jnp.zeros((SEG + M, D), F32)
    zero[...] = jnp.zeros(zero.shape, U32)
    opnd[...] = jnp.zeros(opnd.shape, U32)

    def pin_zero(vals):
        acc = None
        for v in vals:
            v = pltpu.bitcast(v, U32)
            for r in range(0, v.shape[0], 8):
                acc = v[r:r + 8] if acc is None else acc | v[r:r + 8]
        return acc & zero[...]

    cp_xe.wait()
    for cp in cp_small:
        cp.wait()
    pend[0:M, :] = mem0_ref[...].astype(F32)
    cf = c_ref[...].astype(F32)
    sc = _rb(cf * jax.nn.sigmoid(cf))
    sc = jnp.broadcast_to(sc, (16, D)).astype(BF16)

    def mod_cols(lo, hi):
        for j in range(lo, hi):
            v = _rb(_dot(sc, wblk(wm, j))[0:8])
            if j // 8 in (1, 4):
                v = _rb(1.0 + v)
            mod[:, j * 128:(j + 1) * 128] = v

    def mod_vec(k):
        return mod[:, k * D:(k + 1) * D]

    def affine1(n):
        return _rb(n * mod_vec(1)) + mod_vec(0)

    def ne_body(i, carry):
        n = _layernorm(xv[pl.ds(i * 16, 16), 3].astype(F32))
        he[pl.ds(pl.multiple_of(i * 128, 128), 128), :] = n.reshape(128, D).astype(BF16)
        return carry

    jax.lax.fori_loop(0, NSEG // 16, ne_body, 0)
    for j in range(4):
        cp_wm1[j].wait()
        mod_cols(4 * j, 4 * j + 4)

    def he_body(i, carry):
        rows = pl.ds(pl.multiple_of(i * 128, 128), 128)
        n = he[rows, :].astype(F32).reshape(16, 8, D)
        he[rows, :] = affine1(n).reshape(128, D).astype(BF16)
        return carry

    jax.lax.fori_loop(0, NSEG // 16, he_body, 0)

    def w_head(m, h, lo=0, hi=D):
        return pltpu.bitcast(wqkv[m][h, lo // 2:hi // 2, :], BF16)

    def early_proj(m, p, pins=None, rows=256, between=None):
        w = wqkv[m]
        e = w[2 * p]
        o = w[2 * p + 1]
        w[2 * p] = (e & U32(0xFFFF)) | (o << 16)
        w[2 * p + 1] = (e >> 16) | (o & U32(0xFFFF0000))
        ns = rows // 8
        for c in range(NE // rows):
            hc = he[c * rows:(c + 1) * rows, :]
            r12 = []
            for b in range(2):
                wv_ = w[2 * p + b]
                if pins and 2 * c + b in pins:
                    wv_ = jnp.concatenate([wv_[0:8] | pin_zero([pins[2 * c + b]]), wv_[8:]], axis=0)
                r12.append(_dot(hc, pltpu.bitcast(wv_, BF16)).reshape(ns, 8, DH))
                if between is not None:
                    between()
            r12 = jnp.concatenate(r12, axis=1).reshape(2 * rows, DH)
            early[c * ns:(c + 1) * ns, m * NP + p] = pltpu.bitcast(
                r12.astype(BF16), U32).reshape(ns, 8, DH)

    def make_hj(s):
        h = affine1(_rb(_layernorm(xv[s, 0:3].astype(F32))))
        hj[s] = h
        return h[:, :, 0:128].reshape(NJ, 128)

    for m in range(3):
        for cp in cp_w0[m]:
            cp.wait()
        early_proj(m, 0, {2: make_hj(2 * m - 2), 3: make_hj(2 * m - 1)} if m else None)

    def pro_body(p, carry):
        @pl.when(p == 4)
        def _():
            for pp in range(8, NP):
                for cp in group_copies(pp):
                    cp.start()
            for cp in cp_late + cp_ffn:
                cp.start()

        for cp in group_copies(p):
            cp.wait()
        pins = [make_hj(p * 4 + t) for t in range(4)]
        early_proj(0, p, {3: pins[0]})
        early_proj(1, p, {3: pins[1]})
        early_proj(2, p, {2: pins[2], 3: pins[3]})
        return carry

    with jax.named_scope("prologue_loop"):
        jax.lax.fori_loop(1, NP - 1, pro_body, 0)

    for cp in group_copies(NP - 1) + cp_late:
        cp.wait()
    todo = list(range(16, 48))

    def one_mod_col():
        j = todo.pop(0)
        mod_cols(j, j + 1)

    pins = [make_hj(s) for s in range(NSEG - 4, NSEG)]
    early_proj(0, NP - 1, rows=64, between=one_mod_col)
    early_proj(1, NP - 1, {3: pins[0], 6: pins[1]}, rows=128, between=one_mod_col)
    early_proj(2, NP - 1, {3: pins[2], 6: pins[3]}, rows=128, between=one_mod_col)
    assert not todo

    wr = jnp.broadcast_to(wr_ref[...].astype(F32).reshape(1, D), (8, D))

    lane8 = jax.lax.broadcasted_iota(jnp.int32, (8, 128), 1)
    sub8 = jax.lax.broadcasted_iota(jnp.int32, (8, 128), 0)
    LAST = NSEG * SEG - 1

    def post(s, g0, g1, attn):
        attn = attn.reshape(g1 - g0, 8, D)
        x1 = _rb(xv[s, g0:g1].astype(F32) + _rb(mod_vec(2) * _rb(attn)))
        n = _rb(_layernorm(x1))
        h2 = _rb(_rb(n * mod_vec(4)) + mod_vec(3))
        r = _rb(jnp.sum(h2 * wr, axis=-1, keepdims=True)) + 0.0
        x1v[s, g0:g1] = x1.astype(BF16)
        h2v[s, g0:g1] = h2.astype(BF16)
        outv[s, g0:g1] = (x1 + _rb(mod_vec(5) * h2)).astype(BF16)
        pins = []
        for g in range(g0, g1):
            bits = pltpu.bitcast(jnp.broadcast_to(r[g - g0], (8, 128)), jnp.int32)
            hi = jax.lax.shift_right_logical(bits, 16)
            code = jnp.where(bits < 0, hi ^ 0xFFFF, hi | 0x8000)
            key = (code << 11) | (LAST - (s * SEG + g * 8) - sub8) | 0x40000000
            rows = slice(g * 8, (g + 1) * 8)
            knew = jnp.where(lane8 == s, pltpu.bitcast(key, F32), keys[rows, :])
            keys[rows, :] = knew
            pins.append(knew)
        return pins

    def post_pair(a, rows):
        return post(a + 1, 0, 4, rows[0:SEG]) + post(a, 3, 4, rows[SEG:])

    zpad = jnp.zeros((24, DH), U32)
    G = 4
    KA = (NP - G) * 2 * DH
    KS = D - 128

    def segment(s, lhs, lhs_split, extra, pins):
        probs = {}
        always = zero[...] == 0

        def stash(p, m, v):
            v = pltpu.bitcast(v.astype(BF16), U32)
            n = v.shape[0]
            pltpu.store(opnd.at[p, m, 0:n, :], v, mask=jnp.concatenate([always] * (n // 8), axis=0))

        def qkv_group(p):
            keys = [(m, 2 * p + b) for m in range(3) for b in range(2 * G)]
            nsplit = 6 if (p == 0 and lhs_split is not None) else 0
            part = [_dot(lhs_split[0], w_head(m, h, 0, KS)) for m, h in keys[:nsplit]]
            full = [_dot(lhs_split[1], w_head(m, h, KS, D)) + part[i]
                    for i, (m, h) in enumerate(keys[:nsplit])]
            full += [_dot(lhs, w_head(m, h)) for m, h in keys[nsplit:]]
            for m in range(3):
                for t in range(G):
                    i = 2 * G * m + 2 * t
                    stash(p + t, m, jnp.concatenate([full[i], full[i + 1]], axis=0))

        def operand(p, m):
            parts = [opnd[p, m, 0:32, :], early[s, m * NP + p]]
            if m > 0:
                parts.append(zpad)
            return pltpu.bitcast(jnp.concatenate(parts, axis=0), BF16)

        def scores(p):
            sc_ = _dot_nt(operand(p, 0), operand(p, 1)) * SCALE
            f = fill[...]
            if pins.get(p):
                f = jnp.concatenate([f[0:8] + pltpu.bitcast(pin_zero(pins[p]), F32), f[8:]], axis=0)
            sc_ = jnp.where(f == 0.0, sc_, f)
            mx = jnp.max(sc_, axis=-1, keepdims=True)
            e = jnp.exp(sc_ - mx)
            den = jnp.sum(e, axis=-1, keepdims=True)
            inv = pl.reciprocal(den, approx=True)
            stash(p, 3, e)
            probs[p] = inv * (2.0 - den * inv)

        oe = []

        def pv(p):
            o = _dot(pltpu.bitcast(opnd[p, 3], BF16), operand(p, 2)) * probs[p]
            res = []
            for b in range(2):
                rows, erows = o[32 * b:32 * b + 32], o[64 + 8 * b:72 + 8 * b]
                oe.append(erows)
                if extra is not None:
                    rows = jnp.concatenate([rows, erows, extra[2 * p + b]], axis=0)
                res.append(rows)
            pins.setdefault(p + G, []).append(o)
            return res

        os_ = []
        for p in range(0, NP, G):
            qkv_group(p)
            if p >= G:
                for t in range(G):
                    os_ += pv(p - G + t)
            for t in range(G):
                scores(p + t)
        oa = jnp.concatenate(os_, axis=1).astype(BF16)
        acc, ob = [], []
        for n in range(7):
            acc.append(_dot(oa, wblk(wo, n, 0, KA)))
            if n == 2:
                for t in range(G):
                    ob += pv(NP - G + t)
        ob = jnp.concatenate(ob, axis=1).astype(BF16)
        res = [_dot(ob, wblk(wo, n, KA, H * DH)) + acc[n] for n in range(7)]
        res.append(_dot(ob, wblk(wo, 7, KA, H * DH)) + _dot(oa, wblk(wo, 7, 0, KA)))
        return res, oe

    def make_lhs(mem, s):
        return jnp.concatenate([mem, hj[s].reshape(NJ, D)], axis=0)

    cp_o1 = pltpu.make_async_copy(outv.at[0:OUT_SPLIT], out_hbm.at[0:OUT_SPLIT], sem_out.at[0])
    cp_o2 = pltpu.make_async_copy(outv.at[OUT_SPLIT:NSEG], out_hbm.at[OUT_SPLIT:NSEG],
                                  sem_out.at[1])

    def split_lhs(lhs):
        return lhs.astype(BF16), (lhs[:, :KS].astype(BF16), lhs[:, KS:].astype(BF16))

    def step(i, carry):
        @pl.when(i == NIT - 1)
        def _():
            cp_o1.start()

        prev = pend[...]
        for u in range(UNROLL):
            a = 2 * (UNROLL * i + u)
            pins = post_pair(jnp.maximum(a - 2, 0) if u == 0 else a - 2, prev[M:])
            lhs_a = make_lhs(prev[0:M], a)
            lhs_a = (lhs_a.astype(BF16), None) if u == 0 else split_lhs(lhs_a)
            res_a, oe_a = segment(a, *lhs_a, None,
                                  {k: [v] for k, v in zip((0, 4, 8, 12), pins[:4])})
            res_a = jnp.concatenate(res_a, axis=1)
            pins = pins[4:] + post(a, 0, 3, res_a[M:])
            res_b, _ = segment(a + 1, *split_lhs(make_lhs(res_a[0:M], a + 1)), oe_a,
                               {k: [v] for k, v in zip((0, 4, 8, 12), pins)})
            prev = jnp.concatenate(res_b, axis=1)
        pend[...] = prev
        return carry

    with jax.named_scope("main_loop"):
        jax.lax.fori_loop(0, NIT, step, 0)
    post_pair(NSEG - 2, pend[M:, :])
    cp_o2.start()

    def max_all(v):
        return jnp.max(jnp.max(v, axis=0, keepdims=True), axis=1, keepdims=True)

    def decode(k):
        kb = pltpu.bitcast(jnp.broadcast_to(k, (8, 128)), jnp.int32)
        code = (kb >> 11) & 0xFFFF
        hi = jnp.where(code >= 0x8000, code & 0x7FFF, code ^ 0xFFFF)
        tok = jnp.clip((LAST - (kb & LAST))[0, 0], 0, LAST)
        return tok, pltpu.bitcast(hi << 16, F32)[:, 0:1]

    kv = keys[...]
    k1 = max_all(kv)
    k2 = max_all(jnp.where(kv == k1, 0.0, kv))
    i1, r1 = decode(k1)
    i2, r2 = decode(k2)
    g1, g2 = i1 >> 3, i2 >> 3

    def rows_of(ref):
        return jnp.concatenate([ref[g1 >> 2, pl.ds(g1 & 3, 1)], ref[g2 >> 2, pl.ds(g2 & 3, 1)]],
                               axis=0).astype(F32)

    x1, h2 = rows_of(x1v), rows_of(h2v)
    for cp in cp_ffn:
        cp.wait()
    hl = h2.reshape(16, D).astype(BF16)
    act = []
    for j in range(FF // 128):
        gt = _rb(_dot(hl, wblk(wg, j)))
        up = _rb(_dot(hl, wblk(wu, j)))
        act.append((_rb(gt * jax.nn.sigmoid(gt)) * up).astype(BF16))
    act = jnp.concatenate(act, axis=1)
    y = jnp.concatenate([_dot(act, wblk(wd, n)) for n in range(8)], axis=1).reshape(2, 8, D)
    rowi = jax.lax.broadcasted_iota(jnp.int32, (2, 8, 1), 1)
    gsel = jax.lax.broadcasted_iota(jnp.int32, (2, 8, 1), 0)
    tokp = jnp.where(gsel == 0, g1, g2) * 8 + rowi
    gate = _rb(jax.nn.sigmoid(jnp.where(tokp == i1, r1[None], r2[None])))
    upd = jnp.where((tokp == i1) | (tokp == i2), _rb(_rb(y) * gate), 0.0)
    patch[...] = (x1 + _rb(mod_vec(5) * _rb(h2 + upd))).astype(BF16)
    cp_o1.wait()
    cp_o2.wait()
    cp1 = pltpu.make_async_copy(patch.at[0], out_hbm.at[g1 >> 2, g1 & 3], sem_out.at[0])
    cp1.start()

    @pl.when(g1 != g2)
    def _():
        cp2 = pltpu.make_async_copy(patch.at[1], out_hbm.at[g2 >> 2, g2 & 3], sem_out.at[1])
        cp2.start()
        cp2.wait()

    cp1.wait()


@jax.jit
def pallas_adaLN_cond__memory_aug_recurrent_mem_tr__moe_arch_mod__prompt_kernel(
    A_x: jax.Array,
    A_mem0: jax.Array,
    A_Wq: jax.Array,
    A_Wk: jax.Array,
    A_Wv: jax.Array,
    A_Wo: jax.Array,
    A_seg_len,
    B_x: jax.Array,
    B_w_r: jax.Array,
    B_w_gate: jax.Array,
    B_w_up: jax.Array,
    B_w_down: jax.Array,
    c: jax.Array,
    w_mod: jax.Array,
):
    assert A_x.shape == (1, NSEG * SEG, D)
    any_spec = pl.BlockSpec(memory_space=pl.ANY)
    out = pl.pallas_call(
        _kernel,
        out_shape=jax.ShapeDtypeStruct((NSEG, 4, 8, D), BF16),
        in_specs=[any_spec] * 12,
        out_specs=any_spec,
        scratch_shapes=[
            pltpu.VMEM((H, D // 2, DH), U32),
            pltpu.VMEM((H, D // 2, DH), U32),
            pltpu.VMEM((H, D // 2, DH), U32),
            pltpu.VMEM((H * DH // 2, D), U32),
            pltpu.VMEM((D // 2, FF), U32),
            pltpu.VMEM((D // 2, FF), U32),
            pltpu.VMEM((FF // 2, D), U32),
            pltpu.VMEM((D // 2, 6 * D), U32),
            pltpu.VMEM((NSEG, 4, 8, D), BF16),
            pltpu.VMEM((NSEG, 4, 8, D), BF16),
            pltpu.VMEM((NSEG, 4, 8, D), BF16),
            pltpu.VMEM((NSEG, 4, 8, D), BF16),
            pltpu.VMEM((NSEG, 3 * NP, 8, DH), U32),
            pltpu.VMEM((NE, D), BF16),
            pltpu.VMEM((NSEG, 3, 8, D), F32),
            pltpu.VMEM((M + SEG + M, D), F32),
            pltpu.VMEM((8, 6 * D), F32),
            pltpu.VMEM((80, 128), F32),
            pltpu.VMEM((SEG, 128), F32),
            pltpu.VMEM((2, 8, D), BF16),
            pltpu.VMEM((8, 128), U32),
            pltpu.VMEM((NP, 4, 40, DH), U32),
            pltpu.VMEM((M, D), BF16),
            pltpu.VMEM((D,), BF16),
            pltpu.VMEM((1, D), BF16),
            pltpu.SemaphoreType.DMA((16 + NP,)),
            pltpu.SemaphoreType.DMA((2,)),
        ],
        compiler_params=pltpu.CompilerParams(vmem_limit_bytes=120 * 1024 * 1024),
    )(
        A_x.reshape(NSEG, 4, 8, D),
        A_mem0.reshape(M, D),
        A_Wq.reshape(D // 2, 2, H, DH),
        A_Wk.reshape(D // 2, 2, H, DH),
        A_Wv.reshape(D // 2, 2, H, DH),
        A_Wo.reshape(H * DH, D),
        B_w_r,
        B_w_gate,
        B_w_up,
        B_w_down,
        c,
        w_mod,
    )
    return out.reshape(1, NSEG * SEG, D)
```

```python
import jax
import jax.numpy as jnp
import jax.experimental.pallas as pl
import jax.experimental.pallas.tpu as pltpu

F32 = jnp.float32
BF16 = jnp.bfloat16
U32 = jnp.uint32

D = 1024
H = 32
DH = 128
NP = H // 2
M = 8
SEG = 32
NSEG = 64
FF = 3584
NJ = SEG - M
NE = NSEG * M
EPS = 1e-5
SCALE = DH ** (-0.5)
NEG = -1000000000.0
LOG2E = 1.4426950408889634
UNROLL = 2
NIT = NSEG // (2 * UNROLL)
OUT_SPLIT = NSEG - 2 * UNROLL - 2


def _rb(x):
    return x.astype(BF16).astype(F32)


def _layernorm(xf):
    m = jnp.mean(xf, axis=-1, keepdims=True)
    d = xf - m
    v = jnp.mean(d * d, axis=-1, keepdims=True)
    return d * jax.lax.rsqrt(v + EPS)


def _dot(a, b):
    return jnp.dot(a, b, preferred_element_type=F32)


def _dot_nt(a, b):
    return jax.lax.dot_general(a, b, (((1,), (1,)), ((), ())), preferred_element_type=F32)


def _kernel(x_hbm, mem0_hbm, wq_hbm, wk_hbm, wv_hbm, wo_hbm, wr_hbm, wg_hbm, wu_hbm, wd_hbm,
            c_hbm, wm_hbm,
            out_hbm,
            wq, wk, wv, wo, wg, wu, wd, wm, xv, x1v, h2v, outv, early, he, hj, pend,
            mod, fill, keys, patch, zero, opnd, mem0_ref, wr_ref, c_ref,
            sem, sem_out):
    w_u32 = [w.bitcast(U32) for w in (wq_hbm, wk_hbm, wv_hbm)]
    wqkv = (wq, wk, wv)
    wo_hbm, wg_hbm, wu_hbm, wd_hbm, wm_hbm = [
        w.bitcast(U32) for w in (wo_hbm, wg_hbm, wu_hbm, wd_hbm, wm_hbm)]

    def wblk(w, j, lo=None, hi=None):
        rows = slice(None) if lo is None else slice(lo // 2, hi // 2)
        return pltpu.bitcast(w[rows, j * 128:(j + 1) * 128], BF16)

    def wm_copy(lo, n, k):
        return pltpu.make_async_copy(wm_hbm.at[:, pl.ds(lo, n)], wm.at[:, pl.ds(lo, n)], sem.at[k])

    def w_copies(m, p, k):
        return [pltpu.make_async_copy(w_u32[m].at[:, par, p, :], wqkv[m].at[2 * p + par], sem.at[k])
                for par in range(2)]

    def xj_copy(p, k):
        segs = pl.ds(4 * p, 4)
        return pltpu.make_async_copy(x_hbm.at[segs, 0:3], xv.at[segs, 0:3], sem.at[k])

    def group_copies(p):
        k = 16 + p
        return w_copies(0, p, k) + w_copies(1, p, k) + w_copies(2, p, k) + [xj_copy(p, k)]

    cp_small = [pltpu.make_async_copy(c_hbm, c_ref, sem.at[5]),
                pltpu.make_async_copy(mem0_hbm, mem0_ref, sem.at[5]),
                pltpu.make_async_copy(wr_hbm, wr_ref, sem.at[5])]
    cp_xe = pltpu.make_async_copy(x_hbm.at[:, 3], xv.at[:, 3], sem.at[0])
    cp_wm1 = [wm_copy(j * 512, 512, 1 + j) for j in range(4)]
    cp_w0 = [w_copies(m, 0, 6 + m) for m in range(3)]
    cp_w0[1].append(xj_copy(0, 7))
    cp_late = [wm_copy(2 * D, 4 * D, 9), pltpu.make_async_copy(wo_hbm, wo, sem.at[10])]
    cp_ffn = [pltpu.make_async_copy(wg_hbm, wg, sem.at[11]),
              pltpu.make_async_copy(wu_hbm, wu, sem.at[12]),
              pltpu.make_async_copy(wd_hbm, wd, sem.at[13])]

    for cp in [cp_xe] + cp_small + cp_wm1 + cp_w0[0] + cp_w0[1] + cp_w0[2]:
        cp.start()
    for p in range(1, 8):
        for cp in group_copies(p):
            cp.start()

    ri = jax.lax.broadcasted_iota(jnp.int32, (80, 128), 0)
    ci = jax.lax.broadcasted_iota(jnp.int32, (80, 128), 1)

    def head_of(i):
        return jnp.where(i < 64, i >> 5, (i - 64) >> 3)

    def pos_of(i):
        return jnp.where(i < 64, i & 31, 32 + (i & 7))

    same = (head_of(ri) == head_of(ci)) & (ci < 80)
    allowed = (pos_of(ri) < M) | (pos_of(ri) >= pos_of(ci))
    fill[...] = jnp.where(same, jnp.where(allowed, 0.0, NEG / SCALE), -jnp.inf).astype(F32)
    keys[...] = jnp.zeros(keys.shape, F32)
    pend[M:, :] = jnp.zeros((SEG + M, D), F32)
    zero[...] = jnp.zeros(zero.shape, U32)

    def pin_zero(vals):
        acc = None
        for v in vals:
            v = pltpu.bitcast(v, U32)
            for r in range(0, v.shape[0], 8):
                acc = v[r:r + 8] if acc is None else acc | v[r:r + 8]
        return acc & zero[...]

    cp_xe.wait()
    for cp in cp_small:
        cp.wait()
    pend[0:M, :] = mem0_ref[...].astype(F32)
    cf = c_ref[...].astype(F32)
    sc = _rb(cf * jax.nn.sigmoid(cf))
    sc = jnp.broadcast_to(sc, (16, D)).astype(BF16)

    def mod_cols(lo, hi):
        for j in range(lo, hi):
            v = _rb(_dot(sc, wblk(wm, j))[0:8])
            if j // 8 in (1, 4):
                v = _rb(1.0 + v)
            mod[:, j * 128:(j + 1) * 128] = v

    def mod_vec(k):
        return mod[:, k * D:(k + 1) * D]

    def affine1(n):
        return _rb(n * mod_vec(1)) + mod_vec(0)

    def ne_body(i, carry):
        n = _layernorm(xv[pl.ds(i * 16, 16), 3].astype(F32))
        he[pl.ds(pl.multiple_of(i * 128, 128), 128), :] = n.reshape(128, D).astype(BF16)
        return carry

    jax.lax.fori_loop(0, NSEG // 16, ne_body, 0)
    for j in range(4):
        cp_wm1[j].wait()
        mod_cols(4 * j, 4 * j + 4)

    def he_body(i, carry):
        rows = pl.ds(pl.multiple_of(i * 128, 128), 128)
        n = he[rows, :].astype(F32).reshape(16, 8, D)
        he[rows, :] = affine1(n).reshape(128, D).astype(BF16)
        return carry

    jax.lax.fori_loop(0, NSEG // 16, he_body, 0)

    def w_head(m, h, lo=0, hi=D):
        return pltpu.bitcast(wqkv[m][h, lo // 2:hi // 2, :], BF16)

    def early_proj(m, p, pins=None, rows=256, between=None):
        w = wqkv[m]
        e = w[2 * p]
        o = w[2 * p + 1]
        w[2 * p] = (e & U32(0xFFFF)) | (o << 16)
        w[2 * p + 1] = (e >> 16) | (o & U32(0xFFFF0000))
        ns = rows // 8
        for c in range(NE // rows):
            hc = he[c * rows:(c + 1) * rows, :]
            r12 = []
            for b in range(2):
                wv_ = w[2 * p + b]
                if pins and 2 * c + b in pins:
                    wv_ = jnp.concatenate([wv_[0:8] | pin_zero([pins[2 * c + b]]), wv_[8:]], axis=0)
                r12.append(_dot(hc, pltpu.bitcast(wv_, BF16)).reshape(ns, 8, DH))
                if between is not None:
                    between()
            r12 = jnp.concatenate(r12, axis=1).reshape(2 * rows, DH)
            early[c * ns:(c + 1) * ns, m * NP + p] = pltpu.bitcast(
                r12.astype(BF16), U32).reshape(ns, 8, DH)

    def make_hj(s):
        h = affine1(_rb(_layernorm(xv[s, 0:3].astype(F32))))
        hj[s] = h
        return h[:, :, 0:128].reshape(NJ, 128)

    for m in range(3):
        for cp in cp_w0[m]:
            cp.wait()
        early_proj(m, 0, {2: make_hj(2 * m - 2), 3: make_hj(2 * m - 1)} if m else None)

    def pro_body(p, carry):
        @pl.when(p == 4)
        def _():
            for pp in range(8, NP):
                for cp in group_copies(pp):
                    cp.start()
            for cp in cp_late + cp_ffn:
                cp.start()

        for cp in group_copies(p):
            cp.wait()
        pins = [make_hj(p * 4 + t) for t in range(4)]
        early_proj(0, p, {3: pins[0]})
        early_proj(1, p, {3: pins[1]})
        early_proj(2, p, {2: pins[2], 3: pins[3]})
        return carry

    with jax.named_scope("prologue_loop"):
        jax.lax.fori_loop(1, NP - 1, pro_body, 0)

    for cp in group_copies(NP - 1) + cp_late:
        cp.wait()
    todo = list(range(16, 48))

    def one_mod_col():
        j = todo.pop(0)
        mod_cols(j, j + 1)

    pins = [make_hj(s) for s in range(NSEG - 4, NSEG)]
    early_proj(0, NP - 1, rows=64, between=one_mod_col)
    early_proj(1, NP - 1, {3: pins[0], 6: pins[1]}, rows=128, between=one_mod_col)
    early_proj(2, NP - 1, {3: pins[2], 6: pins[3]}, rows=128, between=one_mod_col)
    assert not todo

    wr = jnp.broadcast_to(wr_ref[...].astype(F32).reshape(1, D), (8, D))

    lane8 = jax.lax.broadcasted_iota(jnp.int32, (8, 128), 1)
    sub8 = jax.lax.broadcasted_iota(jnp.int32, (8, 128), 0)
    LAST = NSEG * SEG - 1

    def post(s, g0, g1, attn):
        attn = attn.reshape(g1 - g0, 8, D)
        x1 = _rb(xv[s, g0:g1].astype(F32) + _rb(mod_vec(2) * _rb(attn)))
        n = _rb(_layernorm(x1))
        h2 = _rb(_rb(n * mod_vec(4)) + mod_vec(3))
        r = _rb(jnp.sum(h2 * wr, axis=-1, keepdims=True)) + 0.0
        x1v[s, g0:g1] = x1.astype(BF16)
        h2v[s, g0:g1] = h2.astype(BF16)
        outv[s, g0:g1] = (x1 + _rb(mod_vec(5) * h2)).astype(BF16)
        pins = []
        for g in range(g0, g1):
            bits = pltpu.bitcast(jnp.broadcast_to(r[g - g0], (8, 128)), jnp.int32)
            hi = jax.lax.shift_right_logical(bits, 16)
            code = jnp.where(bits < 0, hi ^ 0xFFFF, hi | 0x8000)
            key = (code << 11) | (LAST - (s * SEG + g * 8) - sub8) | 0x40000000
            rows = slice(g * 8, (g + 1) * 8)
            knew = jnp.where(lane8 == s, pltpu.bitcast(key, F32), keys[rows, :])
            keys[rows, :] = knew
            pins.append(knew)
        return pins

    def post_pair(a, rows):
        return post(a + 1, 0, 4, rows[0:SEG]) + post(a, 3, 4, rows[SEG:])

    zpad = jnp.zeros((48, DH), BF16)
    G = 4
    KA = (NP - G) * 2 * DH
    KS = D - 128

    def segment(s, lhs, lhs_split, extra, pins):
        probs = {}

        def stash(p, m, v):
            opnd[p, m, 0:v.shape[0], :] = v.astype(BF16)

        def qkv_group(p):
            keys = [(m, 2 * p + b) for m in range(3) for b in range(2 * G)]
            nsplit = 6 if (p == 0 and lhs_split is not None) else 0
            part = [_dot(lhs_split[0], w_head(m, h, 0, KS)) for m, h in keys[:nsplit]]
            full = [_dot(lhs_split[1], w_head(m, h, KS, D)) + part[i]
                    for i, (m, h) in enumerate(keys[:nsplit])]
            full += [_dot(lhs, w_head(m, h)) for m, h in keys[nsplit:]]
            for m in range(3):
                for t in range(G):
                    i = 2 * G * m + 2 * t
                    stash(p + t, m, jnp.concatenate([full[i], full[i + 1]], axis=0))

        def operand(p, m):
            parts = [opnd[p, m, 0:64, :], pltpu.bitcast(early[s, m * NP + p], BF16)]
            if m > 0:
                parts.append(zpad)
            return jnp.concatenate(parts, axis=0)

        def scores(p):
            sc_ = _dot_nt(operand(p, 0), operand(p, 1))
            f = fill[...]
            if pins.get(p):
                f = jnp.concatenate([f[0:8] + pltpu.bitcast(pin_zero(pins[p]), F32), f[8:]], axis=0)
            sc_ = jnp.where(f == 0.0, sc_, f)
            mx = jnp.max(sc_, axis=-1, keepdims=True)
            e = jnp.exp2((sc_ - mx) * (SCALE * LOG2E))
            den = jnp.sum(e, axis=-1, keepdims=True)
            inv = pl.reciprocal(den, approx=True)
            stash(p, 3, e)
            probs[p] = inv * (2.0 - den * inv)

        oe = []

        def pv(p):
            o = _dot(opnd[p, 3], operand(p, 2)) * probs[p]
            res = []
            for b in range(2):
                rows, erows = o[32 * b:32 * b + 32], o[64 + 8 * b:72 + 8 * b]
                oe.append(erows)
                if extra is not None:
                    rows = jnp.concatenate([rows, erows, extra[2 * p + b]], axis=0)
                res.append(rows)
            pins.setdefault(p + G, []).append(o)
            return res

        os_ = []
        for p in range(0, NP, G):
            qkv_group(p)
            if p >= G:
                for t in range(G):
                    os_ += pv(p - G + t)
            for t in range(G):
                scores(p + t)
        oa = jnp.concatenate(os_, axis=1).astype(BF16)
        acc, ob = [], []
        for n in range(7):
            acc.append(_dot(oa, wblk(wo, n, 0, KA)))
            if n == 2:
                for t in range(G):
                    ob += pv(NP - G + t)
        ob = jnp.concatenate(ob, axis=1).astype(BF16)
        res = [_dot(ob, wblk(wo, n, KA, H * DH)) + acc[n] for n in range(7)]
        res.append(_dot(ob, wblk(wo, 7, KA, H * DH)) + _dot(oa, wblk(wo, 7, 0, KA)))
        return res, oe

    def make_lhs(mem, s):
        return jnp.concatenate([mem, hj[s].reshape(NJ, D)], axis=0)

    cp_o1 = pltpu.make_async_copy(outv.at[0:OUT_SPLIT], out_hbm.at[0:OUT_SPLIT], sem_out.at[0])
    cp_o2 = pltpu.make_async_copy(outv.at[OUT_SPLIT:NSEG], out_hbm.at[OUT_SPLIT:NSEG],
                                  sem_out.at[1])

    def split_lhs(lhs):
        return lhs.astype(BF16), (lhs[:, :KS].astype(BF16), lhs[:, KS:].astype(BF16))

    def step(i, carry):
        @pl.when(i == NIT - 1)
        def _():
            cp_o1.start()

        prev = pend[...]
        for u in range(UNROLL):
            a = 2 * (UNROLL * i + u)
            pins = post_pair(jnp.maximum(a - 2, 0) if u == 0 else a - 2, prev[M:])
            lhs_a = make_lhs(prev[0:M], a)
            lhs_a = (lhs_a.astype(BF16), None) if u == 0 else split_lhs(lhs_a)
            res_a, oe_a = segment(a, *lhs_a, None,
                                  {k: [v] for k, v in zip((0, 4, 8, 12), pins[:4])})
            res_a = jnp.concatenate(res_a, axis=1)
            pins = pins[4:] + post(a, 0, 3, res_a[M:])
            res_b, _ = segment(a + 1, *split_lhs(make_lhs(res_a[0:M], a + 1)), oe_a,
                               {k: [v] for k, v in zip((0, 4, 8, 12), pins)})
            prev = jnp.concatenate(res_b, axis=1)
        pend[...] = prev
        return carry

    with jax.named_scope("main_loop"):
        jax.lax.fori_loop(0, NIT, step, 0)
    post_pair(NSEG - 2, pend[M:, :])
    cp_o2.start()

    def max_all(v):
        return jnp.max(jnp.max(v, axis=0, keepdims=True), axis=1, keepdims=True)

    def decode(k):
        kb = pltpu.bitcast(jnp.broadcast_to(k, (8, 128)), jnp.int32)
        code = (kb >> 11) & 0xFFFF
        hi = jnp.where(code >= 0x8000, code & 0x7FFF, code ^ 0xFFFF)
        tok = jnp.clip((LAST - (kb & LAST))[0, 0], 0, LAST)
        return tok, pltpu.bitcast(hi << 16, F32)[:, 0:1]

    kv = keys[...]
    k1 = max_all(kv)
    k2 = max_all(jnp.where(kv == k1, 0.0, kv))
    i1, r1 = decode(k1)
    i2, r2 = decode(k2)
    g1, g2 = i1 >> 3, i2 >> 3

    def rows_of(ref):
        return jnp.concatenate([ref[g1 >> 2, pl.ds(g1 & 3, 1)], ref[g2 >> 2, pl.ds(g2 & 3, 1)]],
                               axis=0).astype(F32)

    x1, h2 = rows_of(x1v), rows_of(h2v)
    for cp in cp_ffn:
        cp.wait()
    hl = h2.reshape(16, D).astype(BF16)
    act = []
    for j in range(FF // 128):
        gt = _rb(_dot(hl, wblk(wg, j)))
        up = _rb(_dot(hl, wblk(wu, j)))
        act.append((_rb(gt * jax.nn.sigmoid(gt)) * up).astype(BF16))
    act = jnp.concatenate(act, axis=1)
    y = jnp.concatenate([_dot(act, wblk(wd, n)) for n in range(8)], axis=1).reshape(2, 8, D)
    rowi = jax.lax.broadcasted_iota(jnp.int32, (2, 8, 1), 1)
    gsel = jax.lax.broadcasted_iota(jnp.int32, (2, 8, 1), 0)
    tokp = jnp.where(gsel == 0, g1, g2) * 8 + rowi
    gate = _rb(jax.nn.sigmoid(jnp.where(tokp == i1, r1[None], r2[None])))
    upd = jnp.where((tokp == i1) | (tokp == i2), _rb(_rb(y) * gate), 0.0)
    patch[...] = (x1 + _rb(mod_vec(5) * _rb(h2 + upd))).astype(BF16)
    cp_o1.wait()
    cp_o2.wait()
    cp1 = pltpu.make_async_copy(patch.at[0], out_hbm.at[g1 >> 2, g1 & 3], sem_out.at[0])
    cp1.start()

    @pl.when(g1 != g2)
    def _():
        cp2 = pltpu.make_async_copy(patch.at[1], out_hbm.at[g2 >> 2, g2 & 3], sem_out.at[1])
        cp2.start()
        cp2.wait()

    cp1.wait()


@jax.jit
def pallas_adaLN_cond__memory_aug_recurrent_mem_tr__moe_arch_mod__prompt_kernel(
    A_x: jax.Array,
    A_mem0: jax.Array,
    A_Wq: jax.Array,
    A_Wk: jax.Array,
    A_Wv: jax.Array,
    A_Wo: jax.Array,
    A_seg_len,
    B_x: jax.Array,
    B_w_r: jax.Array,
    B_w_gate: jax.Array,
    B_w_up: jax.Array,
    B_w_down: jax.Array,
    c: jax.Array,
    w_mod: jax.Array,
):
    assert A_x.shape == (1, NSEG * SEG, D)
    any_spec = pl.BlockSpec(memory_space=pl.ANY)
    out = pl.pallas_call(
        _kernel,
        out_shape=jax.ShapeDtypeStruct((NSEG, 4, 8, D), BF16),
        in_specs=[any_spec] * 12,
        out_specs=any_spec,
        scratch_shapes=[
            pltpu.VMEM((H, D // 2, DH), U32),
            pltpu.VMEM((H, D // 2, DH), U32),
            pltpu.VMEM((H, D // 2, DH), U32),
            pltpu.VMEM((H * DH // 2, D), U32),
            pltpu.VMEM((D // 2, FF), U32),
            pltpu.VMEM((D // 2, FF), U32),
            pltpu.VMEM((FF // 2, D), U32),
            pltpu.VMEM((D // 2, 6 * D), U32),
            pltpu.VMEM((NSEG, 4, 8, D), BF16),
            pltpu.VMEM((NSEG, 4, 8, D), BF16),
            pltpu.VMEM((NSEG, 4, 8, D), BF16),
            pltpu.VMEM((NSEG, 4, 8, D), BF16),
            pltpu.VMEM((NSEG, 3 * NP, 8, DH), U32),
            pltpu.VMEM((NE, D), BF16),
            pltpu.VMEM((NSEG, 3, 8, D), F32),
            pltpu.VMEM((M + SEG + M, D), F32),
            pltpu.VMEM((8, 6 * D), F32),
            pltpu.VMEM((80, 128), F32),
            pltpu.VMEM((SEG, 128), F32),
            pltpu.VMEM((2, 8, D), BF16),
            pltpu.VMEM((8, 128), U32),
            pltpu.VMEM((NP, 4, 80, DH), BF16),
            pltpu.VMEM((M, D), BF16),
            pltpu.VMEM((D,), BF16),
            pltpu.VMEM((1, D), BF16),
            pltpu.SemaphoreType.DMA((16 + NP,)),
            pltpu.SemaphoreType.DMA((2,)),
        ],
        compiler_params=pltpu.CompilerParams(vmem_limit_bytes=120 * 1024 * 1024),
    )(
        A_x.reshape(NSEG, 4, 8, D),
        A_mem0.reshape(M, D),
        A_Wq.reshape(D // 2, 2, H, DH),
        A_Wk.reshape(D // 2, 2, H, DH),
        A_Wv.reshape(D // 2, 2, H, DH),
        A_Wo.reshape(H * DH, D),
        B_w_r,
        B_w_gate,
        B_w_up,
        B_w_down,
        c,
        w_mod,
    )
    return out.reshape(1, NSEG * SEG, D)
```

```python
import jax
import jax.numpy as jnp
import jax.experimental.pallas as pl
import jax.experimental.pallas.tpu as pltpu

F32 = jnp.float32
BF16 = jnp.bfloat16
U32 = jnp.uint32

D = 1024
H = 32
DH = 128
NP = H // 2
M = 8
SEG = 32
NSEG = 64
FF = 3584
NJ = SEG - M
NE = NSEG * M
EPS = 1e-5
SCALE = DH ** (-0.5)
NEG = -1000000000.0
LOG2E = 1.4426950408889634
KQ = 256
FIRST = 7
UNROLL = 1
NIT = NSEG // (2 * UNROLL)
OUT_SPLIT = NSEG - 2 * UNROLL - 2


def _rb(x):
    return x.astype(BF16).astype(F32)


def _layernorm(xf):
    m = jnp.mean(xf, axis=-1, keepdims=True)
    d = xf - m
    v = jnp.mean(d * d, axis=-1, keepdims=True)
    return d * jax.lax.rsqrt(v + EPS)


def _dot(a, b):
    return jnp.dot(a, b, preferred_element_type=F32)


def _dot_nt(a, b):
    return jax.lax.dot_general(a, b, (((1,), (1,)), ((), ())), preferred_element_type=F32)


def _kernel(x_hbm, mem0_hbm, wq_hbm, wk_hbm, wv_hbm, wo_hbm, wr_hbm, wg_hbm, wu_hbm, wd_hbm,
            c_hbm, wm_hbm,
            out_hbm,
            wq, wk, wv, wo, wg, wu, wd, wm, xv, x1v, h2v, outv, early, he, hj, pend,
            mod, fill, keys, patch, zero, opnd, acc0, mem0_ref, wr_ref, c_ref,
            sem, sem_out):
    w_u32 = [w.bitcast(U32) for w in (wq_hbm, wk_hbm, wv_hbm)]
    wqkv = (wq, wk, wv)
    wo_hbm, wg_hbm, wu_hbm, wd_hbm, wm_hbm = [
        w.bitcast(U32) for w in (wo_hbm, wg_hbm, wu_hbm, wd_hbm, wm_hbm)]

    def wblk(w, j, lo=None, hi=None):
        rows = slice(None) if lo is None else slice(lo // 2, hi // 2)
        return pltpu.bitcast(w[rows, j * 128:(j + 1) * 128], BF16)

    def wm_copy(lo, n, k):
        return pltpu.make_async_copy(wm_hbm.at[:, pl.ds(lo, n)], wm.at[:, pl.ds(lo, n)], sem.at[k])

    def w_copies(m, p, k):
        return [pltpu.make_async_copy(w_u32[m].at[:, par, p, :], wqkv[m].at[2 * p + par], sem.at[k])
                for par in range(2)]

    def xj_copy(p, k):
        segs = pl.ds(4 * p, 4)
        return pltpu.make_async_copy(x_hbm.at[segs, 0:3], xv.at[segs, 0:3], sem.at[k])

    def group_copies(p, last=False):
        k = 16 + p
        return (w_copies(1, p, k) + w_copies(2, p, k) + ([] if last else w_copies(0, p + 1, k))
                + [xj_copy(p, k)])

    cp_small = [pltpu.make_async_copy(c_hbm, c_ref, sem.at[5]),
                pltpu.make_async_copy(mem0_hbm, mem0_ref, sem.at[5]),
                pltpu.make_async_copy(wr_hbm, wr_ref, sem.at[5])]
    cp_xe = pltpu.make_async_copy(x_hbm.at[:, 3], xv.at[:, 3], sem.at[0])
    cp_w0 = w_copies(0, 0, 6) + w_copies(1, 0, 6) + w_copies(2, 0, 6)
    cp_wm1 = [[wm_copy(j * KQ, KQ, 1 + j), wm_copy(D + j * KQ, KQ, 1 + j)] for j in range(D // KQ)]
    cp_q1 = w_copies(0, 1, 7) + [xj_copy(0, 7)]
    cp_late = [wm_copy(2 * D, 4 * D, 9), pltpu.make_async_copy(wo_hbm, wo, sem.at[10])]
    cp_ffn = [pltpu.make_async_copy(wg_hbm, wg, sem.at[11]),
              pltpu.make_async_copy(wu_hbm, wu, sem.at[12]),
              pltpu.make_async_copy(wd_hbm, wd, sem.at[13])]

    for cp in [cp_xe] + cp_small + cp_w0 + sum(cp_wm1, []) + cp_q1:
        cp.start()
    for p in range(1, FIRST):
        for cp in group_copies(p):
            cp.start()

    ri = jax.lax.broadcasted_iota(jnp.int32, (80, 128), 0)
    ci = jax.lax.broadcasted_iota(jnp.int32, (80, 128), 1)

    def head_of(i):
        return jnp.where(i < 64, i >> 5, (i - 64) >> 3)

    def pos_of(i):
        return jnp.where(i < 64, i & 31, 32 + (i & 7))

    same = (head_of(ri) == head_of(ci)) & (ci < 80)
    allowed = (pos_of(ri) < M) | (pos_of(ri) >= pos_of(ci))
    fill[...] = jnp.where(same, jnp.where(allowed, 0.0, NEG / SCALE), -jnp.inf).astype(F32)
    keys[...] = jnp.zeros(keys.shape, F32)
    pend[M:, :] = jnp.zeros((SEG + M, D), F32)
    zero[...] = jnp.zeros(zero.shape, U32)

    def pin_zero(vals):
        acc = None
        for v in vals:
            v = pltpu.bitcast(v, U32)
            for r in range(0, v.shape[0], 8):
                acc = v[r:r + 8] if acc is None else acc | v[r:r + 8]
        return acc & zero[...]

    cp_xe.wait()
    for cp in cp_small:
        cp.wait()
    pend[0:M, :] = mem0_ref[...].astype(F32)
    cf = c_ref[...].astype(F32)
    sc = _rb(cf * jax.nn.sigmoid(cf))
    sc = jnp.broadcast_to(sc, (16, D)).astype(BF16)

    def mod_cols(lo, hi):
        for j in range(lo, hi):
            v = _rb(_dot(sc, wblk(wm, j))[0:8])
            if j // 8 in (1, 4):
                v = _rb(1.0 + v)
            mod[:, j * 128:(j + 1) * 128] = v

    def mod_vec(k):
        return mod[:, k * D:(k + 1) * D]

    def affine1(n):
        return _rb(n * mod_vec(1)) + mod_vec(0)

    def ne_body(i, carry):
        n = _layernorm(xv[pl.ds(i * 16, 16), 3].astype(F32))
        he[pl.ds(pl.multiple_of(i * 128, 128), 128), :] = n.reshape(128, D).astype(BF16)
        return carry

    jax.lax.fori_loop(0, NSEG // 16, ne_body, 0)

    def w_head(m, h, lo=0, hi=D):
        return pltpu.bitcast(wqkv[m][h, lo // 2:hi // 2, :], BF16)

    def relayout(m, p):
        w = wqkv[m]
        e = w[2 * p]
        o = w[2 * p + 1]
        w[2 * p] = (e & U32(0xFFFF)) | (o << 16)
        w[2 * p + 1] = (e >> 16) | (o & U32(0xFFFF0000))

    def store_early(m, p, row0, r1, r2):
        ns = r1.shape[0] // 8
        r12 = jnp.concatenate([r1.reshape(ns, 8, DH), r2.reshape(ns, 8, DH)], axis=1)
        early[row0 // 8:row0 // 8 + ns, m * NP + p] = pltpu.bitcast(
            r12.reshape(16 * ns, DH).astype(BF16), U32).reshape(ns, 8, DH)

    for cp in cp_w0:
        cp.wait()
    for m in range(3):
        relayout(m, 0)
    for j in range(D // KQ):
        for cp in cp_wm1[j]:
            cp.wait()
        lo, hi = j * KQ, (j + 1) * KQ
        mod_cols(lo // 128, hi // 128)
        mod_cols((D + lo) // 128, (D + hi) // 128)
        for c in range(2):
            rows = slice(c * 256, (c + 1) * 256)
            n = he[rows, lo:hi].astype(F32).reshape(32, 8, KQ)
            h = (_rb(n * mod[:, D + lo:D + hi]) + mod[:, lo:hi]).reshape(256, KQ)
            he[rows, lo:hi] = h.astype(BF16)
            hb = h.astype(BF16)
            for m in range(3):
                w2 = jnp.concatenate([w_head(m, 0, lo, hi), w_head(m, 1, lo, hi)], axis=1)
                r = _dot(hb, w2)
                if j > 0:
                    r = r + acc0[m, rows, :]
                if hi < D:
                    acc0[m, rows, :] = r
                else:
                    store_early(m, 0, c * 256, r[:, :DH], r[:, DH:])

    def early_proj(m, p, pins=None, rows=256, between=None):
        relayout(m, p)
        for c in range(NE // rows):
            hc = he[c * rows:(c + 1) * rows, :]
            r12 = []
            for b in range(2):
                wv_ = wqkv[m][2 * p + b]
                if pins and 2 * c + b in pins:
                    wv_ = jnp.concatenate([wv_[0:8] | pin_zero(pins[2 * c + b]), wv_[8:]], axis=0)
                r12.append(_dot(hc, pltpu.bitcast(wv_, BF16)))
                if between is not None:
                    between()
            store_early(m, p, c * rows, *r12)

    def make_hj(s):
        h = affine1(_rb(_layernorm(xv[s, 0:3].astype(F32))))
        hj[s] = h
        return h[:, :, 0:128].reshape(NJ, 128)

    for cp in cp_q1:
        cp.wait()
    pins = [make_hj(s) for s in range(4)]
    early_proj(0, 1, {2: pins[0:2], 3: pins[2:4]})

    def pro_body(p, carry):
        @pl.when(p == 3)
        def _():
            for pp in range(FIRST, NP):
                for cp in group_copies(pp, pp == NP - 1):
                    cp.start()
            for cp in cp_late:
                cp.start()

        for cp in group_copies(p):
            cp.wait()
        pins = [[make_hj(p * 4 + t)] for t in range(4)]
        early_proj(1, p, {3: pins[0]})
        early_proj(2, p, {3: pins[1]})
        early_proj(0, p + 1, {2: pins[2], 3: pins[3]})
        return carry

    with jax.named_scope("prologue_loop"):
        jax.lax.fori_loop(1, NP - 1, pro_body, 0)

    for cp in cp_ffn:
        cp.start()
    for cp in group_copies(NP - 1, True) + cp_late:
        cp.wait()
    todo = list(range(16, 48))

    def one_mod_col():
        j = todo.pop(0)
        mod_cols(j, j + 1)

    pins = [[make_hj(s)] for s in range(NSEG - 4, NSEG)]
    early_proj(1, NP - 1, {6: pins[0], 12: pins[1]}, rows=64, between=one_mod_col)
    early_proj(2, NP - 1, {4: pins[2], 10: pins[3]}, rows=64, between=one_mod_col)
    assert not todo

    wr = jnp.broadcast_to(wr_ref[...].astype(F32).reshape(1, D), (8, D))

    lane8 = jax.lax.broadcasted_iota(jnp.int32, (8, 128), 1)
    sub8 = jax.lax.broadcasted_iota(jnp.int32, (8, 128), 0)
    LAST = NSEG * SEG - 1

    def post(s, g0, g1, attn):
        attn = attn.reshape(g1 - g0, 8, D)
        x1 = _rb(xv[s, g0:g1].astype(F32) + _rb(mod_vec(2) * _rb(attn)))
        n = _rb(_layernorm(x1))
        h2 = _rb(_rb(n * mod_vec(4)) + mod_vec(3))
        r = _rb(jnp.sum(h2 * wr, axis=-1, keepdims=True)) + 0.0
        x1v[s, g0:g1] = x1.astype(BF16)
        h2v[s, g0:g1] = h2.astype(BF16)
        outv[s, g0:g1] = (x1 + _rb(mod_vec(5) * h2)).astype(BF16)
        pins = []
        for g in range(g0, g1):
            bits = pltpu.bitcast(jnp.broadcast_to(r[g - g0], (8, 128)), jnp.int32)
            hi = jax.lax.shift_right_logical(bits, 16)
            code = jnp.where(bits < 0, hi ^ 0xFFFF, hi | 0x8000)
            key = (code << 11) | (LAST - (s * SEG + g * 8) - sub8) | 0x40000000
            rows = slice(g * 8, (g + 1) * 8)
            knew = jnp.where(lane8 == s, pltpu.bitcast(key, F32), keys[rows, :])
            keys[rows, :] = knew
            pins.append(knew)
        return pins

    def post_pair(a, rows):
        return post(a + 1, 0, 4, rows[0:SEG]) + post(a, 3, 4, rows[SEG:])

    zpad = jnp.zeros((48, DH), BF16)
    G = 4
    KA = (NP - G) * 2 * DH
    KS = D - 128

    def segment(s, lhs, lhs_split, extra, pins):
        probs = {}

        def stash(p, m, v):
            opnd[p, m, 0:v.shape[0], :] = v.astype(BF16)

        def qkv_group(p):
            keys = [(m, 2 * p + b) for m in range(3) for b in range(2 * G)]
            nsplit = 6 if (p == 0 and lhs_split is not None) else 0
            part = [_dot(lhs_split[0], w_head(m, h, 0, KS)) for m, h in keys[:nsplit]]
            full = [_dot(lhs_split[1], w_head(m, h, KS, D)) + part[i]
                    for i, (m, h) in enumerate(keys[:nsplit])]
            full += [_dot(lhs, w_head(m, h)) for m, h in keys[nsplit:]]
            for m in range(3):
                for t in range(G):
                    i = 2 * G * m + 2 * t
                    stash(p + t, m, jnp.concatenate([full[i], full[i + 1]], axis=0))

        def operand(p, m):
            parts = [opnd[p, m, 0:64, :], pltpu.bitcast(early[s, m * NP + p], BF16)]
            if m > 0:
                parts.append(zpad)
            return jnp.concatenate(parts, axis=0)

        def scores(p):
            sc_ = _dot_nt(operand(p, 0), operand(p, 1))
            f = fill[...]
            if pins.get(p):
                f = jnp.concatenate([f[0:8] + pltpu.bitcast(pin_zero(pins[p]), F32), f[8:]], axis=0)
            sc_ = jnp.where(f == 0.0, sc_, f)
            mx = jnp.max(sc_, axis=-1, keepdims=True)
            e = jnp.exp2((sc_ - mx) * (SCALE * LOG2E))
            den = jnp.sum(e, axis=-1, keepdims=True)
            inv = pl.reciprocal(den, approx=True)
            stash(p, 3, e)
            probs[p] = inv * (2.0 - den * inv)

        oe = []

        def pv(p):
            o = _dot(opnd[p, 3], operand(p, 2)) * probs[p]
            res = []
            for b in range(2):
                rows, erows = o[32 * b:32 * b + 32], o[64 + 8 * b:72 + 8 * b]
                oe.append(erows)
                if extra is not None:
                    rows = jnp.concatenate([rows, erows, extra[2 * p + b]], axis=0)
                res.append(rows)
            pins.setdefault(p + G, []).append(o)
            return res

        os_ = []
        for p in range(0, NP, G):
            qkv_group(p)
            if p >= G:
                for t in range(G):
                    os_ += pv(p - G + t)
            for t in range(G):
                scores(p + t)
        oa = jnp.concatenate(os_, axis=1).astype(BF16)
        acc, ob = [], []
        for n in range(7):
            acc.append(_dot(oa, wblk(wo, n, 0, KA)))
            if n == 2:
                for t in range(G):
                    ob += pv(NP - G + t)
        ob = jnp.concatenate(ob, axis=1).astype(BF16)
        res = [_dot(ob, wblk(wo, n, KA, H * DH)) + acc[n] for n in range(7)]
        res.append(_dot(ob, wblk(wo, 7, KA, H * DH)) + _dot(oa, wblk(wo, 7, 0, KA)))
        return res, oe

    def make_lhs(mem, s):
        return jnp.concatenate([mem, hj[s].reshape(NJ, D)], axis=0)

    cp_o1 = pltpu.make_async_copy(outv.at[0:OUT_SPLIT], out_hbm.at[0:OUT_SPLIT], sem_out.at[0])
    cp_o2 = pltpu.make_async_copy(outv.at[OUT_SPLIT:NSEG], out_hbm.at[OUT_SPLIT:NSEG],
                                  sem_out.at[1])

    def split_lhs(lhs):
        return lhs.astype(BF16), (lhs[:, :KS].astype(BF16), lhs[:, KS:].astype(BF16))

    def step(i, carry):
        @pl.when(i == NIT - 1)
        def _():
            cp_o1.start()

        prev = pend[...]
        for u in range(UNROLL):
            a = 2 * (UNROLL * i + u)
            pins = post_pair(jnp.maximum(a - 2, 0) if u == 0 else a - 2, prev[M:])
            lhs_a = make_lhs(prev[0:M], a)
            lhs_a = (lhs_a.astype(BF16), None) if u == 0 else split_lhs(lhs_a)
            res_a, oe_a = segment(a, *lhs_a, None,
                                  {k: [v] for k, v in zip((0, 4, 8, 12), pins[:4])})
            res_a = jnp.concatenate(res_a, axis=1)
            pins = pins[4:] + post(a, 0, 3, res_a[M:])
            res_b, _ = segment(a + 1, *split_lhs(make_lhs(res_a[0:M], a + 1)), oe_a,
                               {k: [v] for k, v in zip((0, 4, 8, 12), pins)})
            prev = jnp.concatenate(res_b, axis=1)
        pend[...] = prev
        return carry

    with jax.named_scope("main_loop"):
        jax.lax.fori_loop(0, NIT, step, 0)
    post_pair(NSEG - 2, pend[M:, :])
    cp_o2.start()

    def max_all(v):
        return jnp.max(jnp.max(v, axis=0, keepdims=True), axis=1, keepdims=True)

    def decode(k):
        kb = pltpu.bitcast(jnp.broadcast_to(k, (8, 128)), jnp.int32)
        code = (kb >> 11) & 0xFFFF
        hi = jnp.where(code >= 0x8000, code & 0x7FFF, code ^ 0xFFFF)
        tok = jnp.clip((LAST - (kb & LAST))[0, 0], 0, LAST)
        return tok, pltpu.bitcast(hi << 16, F32)[:, 0:1]

    kv = keys[...]
    k1 = max_all(kv)
    k2 = max_all(jnp.where(kv == k1, 0.0, kv))
    i1, r1 = decode(k1)
    i2, r2 = decode(k2)
    g1, g2 = i1 >> 3, i2 >> 3

    def rows_of(ref):
        return jnp.concatenate([ref[g1 >> 2, pl.ds(g1 & 3, 1)], ref[g2 >> 2, pl.ds(g2 & 3, 1)]],
                               axis=0).astype(F32)

    x1, h2 = rows_of(x1v), rows_of(h2v)
    for cp in cp_ffn:
        cp.wait()
    hl = h2.reshape(16, D).astype(BF16)
    act = []
    for j in range(FF // 128):
        gt = _rb(_dot(hl, wblk(wg, j)))
        up = _rb(_dot(hl, wblk(wu, j)))
        act.append((_rb(gt * jax.nn.sigmoid(gt)) * up).astype(BF16))
    act = jnp.concatenate(act, axis=1)
    y = jnp.concatenate([_dot(act, wblk(wd, n)) for n in range(8)], axis=1).reshape(2, 8, D)
    rowi = jax.lax.broadcasted_iota(jnp.int32, (2, 8, 1), 1)
    gsel = jax.lax.broadcasted_iota(jnp.int32, (2, 8, 1), 0)
    tokp = jnp.where(gsel == 0, g1, g2) * 8 + rowi
    gate = _rb(jax.nn.sigmoid(jnp.where(tokp == i1, r1[None], r2[None])))
    upd = jnp.where((tokp == i1) | (tokp == i2), _rb(_rb(y) * gate), 0.0)
    patch[...] = (x1 + _rb(mod_vec(5) * _rb(h2 + upd))).astype(BF16)
    cp_o1.wait()
    cp_o2.wait()
    cp1 = pltpu.make_async_copy(patch.at[0], out_hbm.at[g1 >> 2, g1 & 3], sem_out.at[0])
    cp1.start()

    @pl.when(g1 != g2)
    def _():
        cp2 = pltpu.make_async_copy(patch.at[1], out_hbm.at[g2 >> 2, g2 & 3], sem_out.at[1])
        cp2.start()
        cp2.wait()

    cp1.wait()


@jax.jit
def pallas_adaLN_cond__memory_aug_recurrent_mem_tr__moe_arch_mod__prompt_kernel(
    A_x: jax.Array,
    A_mem0: jax.Array,
    A_Wq: jax.Array,
    A_Wk: jax.Array,
    A_Wv: jax.Array,
    A_Wo: jax.Array,
    A_seg_len,
    B_x: jax.Array,
    B_w_r: jax.Array,
    B_w_gate: jax.Array,
    B_w_up: jax.Array,
    B_w_down: jax.Array,
    c: jax.Array,
    w_mod: jax.Array,
):
    assert A_x.shape == (1, NSEG * SEG, D)
    any_spec = pl.BlockSpec(memory_space=pl.ANY)
    out = pl.pallas_call(
        _kernel,
        out_shape=jax.ShapeDtypeStruct((NSEG, 4, 8, D), BF16),
        in_specs=[any_spec] * 12,
        out_specs=any_spec,
        scratch_shapes=[
            pltpu.VMEM((H, D // 2, DH), U32),
            pltpu.VMEM((H, D // 2, DH), U32),
            pltpu.VMEM((H, D // 2, DH), U32),
            pltpu.VMEM((H * DH // 2, D), U32),
            pltpu.VMEM((D // 2, FF), U32),
            pltpu.VMEM((D // 2, FF), U32),
            pltpu.VMEM((FF // 2, D), U32),
            pltpu.VMEM((D // 2, 6 * D), U32),
            pltpu.VMEM((NSEG, 4, 8, D), BF16),
            pltpu.VMEM((NSEG, 4, 8, D), BF16),
            pltpu.VMEM((NSEG, 4, 8, D), BF16),
            pltpu.VMEM((NSEG, 4, 8, D), BF16),
            pltpu.VMEM((NSEG, 3 * NP, 8, DH), U32),
            pltpu.VMEM((NE, D), BF16),
            pltpu.VMEM((NSEG, 3, 8, D), F32),
            pltpu.VMEM((M + SEG + M, D), F32),
            pltpu.VMEM((8, 6 * D), F32),
            pltpu.VMEM((80, 128), F32),
            pltpu.VMEM((SEG, 128), F32),
            pltpu.VMEM((2, 8, D), BF16),
            pltpu.VMEM((8, 128), U32),
            pltpu.VMEM((NP, 4, 80, DH), BF16),
            pltpu.VMEM((3, NE, 2 * DH), F32),
            pltpu.VMEM((M, D), BF16),
            pltpu.VMEM((D,), BF16),
            pltpu.VMEM((1, D), BF16),
            pltpu.SemaphoreType.DMA((16 + NP,)),
            pltpu.SemaphoreType.DMA((2,)),
        ],
        compiler_params=pltpu.CompilerParams(vmem_limit_bytes=120 * 1024 * 1024),
    )(
        A_x.reshape(NSEG, 4, 8, D),
        A_mem0.reshape(M, D),
        A_Wq.reshape(D // 2, 2, H, DH),
        A_Wk.reshape(D // 2, 2, H, DH),
        A_Wv.reshape(D // 2, 2, H, DH),
        A_Wo.reshape(H * DH, D),
        B_w_r,
        B_w_gate,
        B_w_up,
        B_w_down,
        c,
        w_mod,
    )
    return out.reshape(1, NSEG * SEG, D)
```

```python
import jax
import jax.numpy as jnp
import jax.experimental.pallas as pl
import jax.experimental.pallas.tpu as pltpu

F32 = jnp.float32
BF16 = jnp.bfloat16
U32 = jnp.uint32

D = 1024
H = 32
DH = 128
NP = H // 2
M = 8
SEG = 32
NSEG = 64
FF = 3584
NJ = SEG - M
NE = NSEG * M
EPS = 1e-5
SCALE = DH ** (-0.5)
NEG = -1000000000.0
LOG2E = 1.4426950408889634
KQ = 256
FIRST = 7
UNROLL = 2
NIT = NSEG // (2 * UNROLL)
OUT_SPLIT = NSEG - 2 * UNROLL - 2


def _rb(x):
    return x.astype(BF16).astype(F32)


def _layernorm(xf):
    m = jnp.mean(xf, axis=-1, keepdims=True)
    d = xf - m
    v = jnp.mean(d * d, axis=-1, keepdims=True)
    return d * jax.lax.rsqrt(v + EPS)


def _dot(a, b):
    return jnp.dot(a, b, preferred_element_type=F32)


def _dot_nt(a, b):
    return jax.lax.dot_general(a, b, (((1,), (1,)), ((), ())), preferred_element_type=F32)


def _kernel(x_hbm, mem0_hbm, wq_hbm, wk_hbm, wv_hbm, wo_hbm, wr_hbm, wg_hbm, wu_hbm, wd_hbm,
            c_hbm, wm_hbm,
            out_hbm,
            wq, wk, wv, wo, wg, wu, wd, wm, xv, x1v, h2v, outv, early, he, hj, pend,
            mod, fill, keys, patch, zero, opnd, acc0, mem0_ref, wr_ref, c_ref,
            sem, sem_out):
    w_u32 = [w.bitcast(U32) for w in (wq_hbm, wk_hbm, wv_hbm)]
    wqkv = (wq, wk, wv)
    wo_hbm, wg_hbm, wu_hbm, wd_hbm, wm_hbm = [
        w.bitcast(U32) for w in (wo_hbm, wg_hbm, wu_hbm, wd_hbm, wm_hbm)]

    def wblk(w, j, lo=None, hi=None):
        rows = slice(None) if lo is None else slice(lo // 2, hi // 2)
        return pltpu.bitcast(w[rows, j * 128:(j + 1) * 128], BF16)

    def wm_copy(lo, n, k):
        return pltpu.make_async_copy(wm_hbm.at[:, pl.ds(lo, n)], wm.at[:, pl.ds(lo, n)], sem.at[k])

    def w_copies(m, p, k):
        return [pltpu.make_async_copy(w_u32[m].at[:, par, p, :], wqkv[m].at[2 * p + par], sem.at[k])
                for par in range(2)]

    def xj_copy(p, k):
        segs = pl.ds(4 * p, 4)
        return pltpu.make_async_copy(x_hbm.at[segs, 0:3], xv.at[segs, 0:3], sem.at[k])

    def group_copies(p, last=False):
        k = 16 + p
        return (w_copies(1, p, k) + w_copies(2, p, k) + ([] if last else w_copies(0, p + 1, k))
                + [xj_copy(p, k)])

    cp_c = pltpu.make_async_copy(c_hbm, c_ref, sem.at[5])
    cp_xe = pltpu.make_async_copy(x_hbm.at[:, 3], xv.at[:, 3], sem.at[0])
    cp_w0 = w_copies(0, 0, 6) + w_copies(1, 0, 6) + w_copies(2, 0, 6)
    cp_wm1 = [[wm_copy(j * KQ, KQ, 1 + j), wm_copy(D + j * KQ, KQ, 1 + j)] for j in range(D // KQ)]
    cp_q1 = w_copies(0, 1, 7) + [xj_copy(0, 7)]
    cp_late = [wm_copy(2 * D, 4 * D, 9), pltpu.make_async_copy(wo_hbm, wo, sem.at[10]),
               pltpu.make_async_copy(mem0_hbm, mem0_ref, sem.at[14]),
               pltpu.make_async_copy(wr_hbm, wr_ref, sem.at[15])]
    cp_ffn = [pltpu.make_async_copy(wg_hbm, wg, sem.at[11]),
              pltpu.make_async_copy(wu_hbm, wu, sem.at[12]),
              pltpu.make_async_copy(wd_hbm, wd, sem.at[13])]

    for cp in [cp_c, cp_xe] + cp_w0 + sum(cp_wm1, []) + cp_q1:
        cp.start()
    for p in range(1, FIRST):
        for cp in group_copies(p):
            cp.start()

    ri = jax.lax.broadcasted_iota(jnp.int32, (80, 128), 0)
    ci = jax.lax.broadcasted_iota(jnp.int32, (80, 128), 1)

    def head_of(i):
        return jnp.where(i < 64, i >> 5, (i - 64) >> 3)

    def pos_of(i):
        return jnp.where(i < 64, i & 31, 32 + (i & 7))

    same = (head_of(ri) == head_of(ci)) & (ci < 80)
    allowed = (pos_of(ri) < M) | (pos_of(ri) >= pos_of(ci))
    fill[...] = jnp.where(same, jnp.where(allowed, 0.0, NEG / SCALE), -jnp.inf).astype(F32)
    keys[...] = jnp.zeros(keys.shape, F32)
    pend[M:, :] = jnp.zeros((SEG + M, D), F32)
    zero[...] = jnp.zeros(zero.shape, U32)

    def pin_zero(vals):
        acc = None
        for v in vals:
            v = pltpu.bitcast(v, U32)
            for r in range(0, v.shape[0], 8):
                acc = v[r:r + 8] if acc is None else acc | v[r:r + 8]
        return acc & zero[...]

    cp_xe.wait()
    cp_c.wait()
    cf = c_ref[...].astype(F32)
    sc = _rb(cf * jax.nn.sigmoid(cf))
    sc = jnp.broadcast_to(sc, (16, D)).astype(BF16)

    def mod_cols(lo, hi):
        for j in range(lo, hi):
            v = _rb(_dot(sc, wblk(wm, j))[0:8])
            if j // 8 in (1, 4):
                v = _rb(1.0 + v)
            mod[:, j * 128:(j + 1) * 128] = v

    def mod_vec(k):
        return mod[:, k * D:(k + 1) * D]

    def affine1(n):
        return _rb(n * mod_vec(1)) + mod_vec(0)

    def ne_body(i, carry):
        n = _layernorm(xv[pl.ds(i * 16, 16), 3].astype(F32))
        he[pl.ds(pl.multiple_of(i * 128, 128), 128), :] = n.reshape(128, D).astype(BF16)
        return carry

    jax.lax.fori_loop(0, NSEG // 16, ne_body, 0)

    def w_head(m, h, lo=0, hi=D):
        return pltpu.bitcast(wqkv[m][h, lo // 2:hi // 2, :], BF16)

    def relayout(m, p):
        w = wqkv[m]
        e = w[2 * p]
        o = w[2 * p + 1]
        w[2 * p] = (e & U32(0xFFFF)) | (o << 16)
        w[2 * p + 1] = (e >> 16) | (o & U32(0xFFFF0000))

    def store_early(m, p, row0, r1, r2):
        ns = r1.shape[0] // 8
        r12 = jnp.concatenate([r1.reshape(ns, 8, DH), r2.reshape(ns, 8, DH)], axis=1)
        early[row0 // 8:row0 // 8 + ns, m * NP + p] = pltpu.bitcast(
            r12.reshape(16 * ns, DH).astype(BF16), U32).reshape(ns, 8, DH)

    for cp in cp_w0:
        cp.wait()
    for m in range(3):
        relayout(m, 0)
    for j in range(D // KQ):
        for cp in cp_wm1[j]:
            cp.wait()
        lo, hi = j * KQ, (j + 1) * KQ
        mod_cols(lo // 128, hi // 128)
        mod_cols((D + lo) // 128, (D + hi) // 128)
        for c in range(2):
            rows = slice(c * 256, (c + 1) * 256)
            n = he[rows, lo:hi].astype(F32).reshape(32, 8, KQ)
            h = (_rb(n * mod[:, D + lo:D + hi]) + mod[:, lo:hi]).reshape(256, KQ)
            he[rows, lo:hi] = h.astype(BF16)
            hb = h.astype(BF16)
            for m in range(3):
                w2 = jnp.concatenate([w_head(m, 0, lo, hi), w_head(m, 1, lo, hi)], axis=1)
                r = _dot(hb, w2)
                if j > 0:
                    r = r + acc0[m, rows, :]
                if hi < D:
                    acc0[m, rows, :] = r
                else:
                    store_early(m, 0, c * 256, r[:, :DH], r[:, DH:])

    def early_proj(m, p, pins=None, rows=256, between=None):
        relayout(m, p)
        for c in range(NE // rows):
            hc = he[c * rows:(c + 1) * rows, :]
            r12 = []
            for b in range(2):
                wv_ = wqkv[m][2 * p + b]
                if pins and 2 * c + b in pins:
                    wv_ = jnp.concatenate([wv_[0:8] | pin_zero(pins[2 * c + b]), wv_[8:]], axis=0)
                r12.append(_dot(hc, pltpu.bitcast(wv_, BF16)))
                if between is not None:
                    between()
            store_early(m, p, c * rows, *r12)

    def make_hj(s):
        h = affine1(_rb(_layernorm(xv[s, 0:3].astype(F32))))
        hj[s] = h
        return h[:, :, 0:128].reshape(NJ, 128)

    for cp in cp_q1:
        cp.wait()
    pins = [make_hj(s) for s in range(4)]
    early_proj(0, 1, {2: pins[0:2], 3: pins[2:4]})

    def pro_body(p, carry):
        @pl.when(p == 4)
        def _():
            for pp in range(FIRST, NP):
                for cp in group_copies(pp, pp == NP - 1):
                    cp.start()
            for cp in cp_late:
                cp.start()

        for cp in group_copies(p):
            cp.wait()
        pins = [[make_hj(p * 4 + t)] for t in range(4)]
        early_proj(1, p, {3: pins[0]})
        early_proj(2, p, {3: pins[1]})
        early_proj(0, p + 1, {2: pins[2], 3: pins[3]})
        return carry

    with jax.named_scope("prologue_loop"):
        jax.lax.fori_loop(1, NP - 1, pro_body, 0)

    for cp in cp_ffn:
        cp.start()
    for cp in group_copies(NP - 1, True) + cp_late:
        cp.wait()
    pend[0:M, :] = mem0_ref[...].astype(F32)
    todo = list(range(16, 48))

    def one_mod_col():
        j = todo.pop(0)
        mod_cols(j, j + 1)

    pins = [[make_hj(s)] for s in range(NSEG - 4, NSEG)]
    early_proj(1, NP - 1, {6: pins[0], 12: pins[1]}, rows=64, between=one_mod_col)
    early_proj(2, NP - 1, {4: pins[2], 10: pins[3]}, rows=64, between=one_mod_col)
    assert not todo

    wr = jnp.broadcast_to(wr_ref[...].astype(F32).reshape(1, D), (8, D))

    lane8 = jax.lax.broadcasted_iota(jnp.int32, (8, 128), 1)
    sub8 = jax.lax.broadcasted_iota(jnp.int32, (8, 128), 0)
    LAST = NSEG * SEG - 1

    def post(s, g0, g1, attn):
        attn = attn.reshape(g1 - g0, 8, D)
        x1 = _rb(xv[s, g0:g1].astype(F32) + _rb(mod_vec(2) * _rb(attn)))
        n = _rb(_layernorm(x1))
        h2 = _rb(_rb(n * mod_vec(4)) + mod_vec(3))
        r = _rb(jnp.sum(h2 * wr, axis=-1, keepdims=True)) + 0.0
        x1v[s, g0:g1] = x1.astype(BF16)
        h2v[s, g0:g1] = h2.astype(BF16)
        outv[s, g0:g1] = (x1 + _rb(mod_vec(5) * h2)).astype(BF16)
        pins = []
        for g in range(g0, g1):
            bits = pltpu.bitcast(jnp.broadcast_to(r[g - g0], (8, 128)), jnp.int32)
            hi = jax.lax.shift_right_logical(bits, 16)
            code = jnp.where(bits < 0, hi ^ 0xFFFF, hi | 0x8000)
            key = (code << 11) | (LAST - (s * SEG + g * 8) - sub8) | 0x40000000
            rows = slice(g * 8, (g + 1) * 8)
            knew = jnp.where(lane8 == s, pltpu.bitcast(key, F32), keys[rows, :])
            keys[rows, :] = knew
            pins.append(knew)
        return pins

    def post_pair(a, rows):
        return post(a + 1, 0, 4, rows[0:SEG]) + post(a, 3, 4, rows[SEG:])

    zpad = jnp.zeros((48, DH), BF16)
    G = 4
    KA = (NP - G) * 2 * DH
    KS = D - 128

    def segment(s, lhs, lhs_split, extra, pins):
        probs = {}

        def stash(p, m, v):
            opnd[p, m, 0:v.shape[0], :] = v.astype(BF16)

        def qkv_group(p):
            keys = [(m, 2 * p + b) for m in range(3) for b in range(2 * G)]
            nsplit = 6 if (p == 0 and lhs_split is not None) else 0
            part = [_dot(lhs_split[0], w_head(m, h, 0, KS)) for m, h in keys[:nsplit]]
            full = [_dot(lhs_split[1], w_head(m, h, KS, D)) + part[i]
                    for i, (m, h) in enumerate(keys[:nsplit])]
            full += [_dot(lhs, w_head(m, h)) for m, h in keys[nsplit:]]
            for m in range(3):
                for t in range(G):
                    i = 2 * G * m + 2 * t
                    stash(p + t, m, jnp.concatenate([full[i], full[i + 1]], axis=0))

        def operand(p, m):
            parts = [opnd[p, m, 0:64, :], pltpu.bitcast(early[s, m * NP + p], BF16)]
            if m > 0:
                parts.append(zpad)
            return jnp.concatenate(parts, axis=0)

        def scores(p):
            sc_ = _dot_nt(operand(p, 0), operand(p, 1))
            f = fill[...]
            if pins.get(p):
                f = jnp.concatenate([f[0:8] + pltpu.bitcast(pin_zero(pins[p]), F32), f[8:]], axis=0)
            sc_ = jnp.where(f == 0.0, sc_, f)
            mx = jnp.max(sc_, axis=-1, keepdims=True)
            e = jnp.exp2((sc_ - mx) * (SCALE * LOG2E))
            den = jnp.sum(e, axis=-1, keepdims=True)
            inv = pl.reciprocal(den, approx=True)
            stash(p, 3, e)
            probs[p] = inv * (2.0 - den * inv)

        oe = []

        def pv(p):
            o = _dot(opnd[p, 3], operand(p, 2)) * probs[p]
            res = []
            for b in range(2):
                rows, erows = o[32 * b:32 * b + 32], o[64 + 8 * b:72 + 8 * b]
                oe.append(erows)
                if extra is not None:
                    rows = jnp.concatenate([rows, erows, extra[2 * p + b]], axis=0)
                res.append(rows)
            pins.setdefault(p + G, []).append(o)
            return res

        os_ = []
        for p in range(0, NP, G):
            qkv_group(p)
            if p >= G:
                for t in range(G):
                    os_ += pv(p - G + t)
            for t in range(G):
                scores(p + t)
        oa = jnp.concatenate(os_, axis=1).astype(BF16)
        acc, ob = [], []
        for n in range(7):
            acc.append(_dot(oa, wblk(wo, n, 0, KA)))
            if n == 2:
                for t in range(G):
                    ob += pv(NP - G + t)
        ob = jnp.concatenate(ob, axis=1).astype(BF16)
        res = [_dot(ob, wblk(wo, n, KA, H * DH)) + acc[n] for n in range(7)]
        res.append(_dot(ob, wblk(wo, 7, KA, H * DH)) + _dot(oa, wblk(wo, 7, 0, KA)))
        return res, oe

    def make_lhs(mem, s):
        return jnp.concatenate([mem, hj[s].reshape(NJ, D)], axis=0)

    cp_o1 = pltpu.make_async_copy(outv.at[0:OUT_SPLIT], out_hbm.at[0:OUT_SPLIT], sem_out.at[0])
    cp_o2 = pltpu.make_async_copy(outv.at[OUT_SPLIT:NSEG], out_hbm.at[OUT_SPLIT:NSEG],
                                  sem_out.at[1])

    def split_lhs(lhs):
        return lhs.astype(BF16), (lhs[:, :KS].astype(BF16), lhs[:, KS:].astype(BF16))

    def step(i, carry):
        @pl.when(i == NIT - 1)
        def _():
            cp_o1.start()

        prev = pend[...]
        for u in range(UNROLL):
            a = 2 * (UNROLL * i + u)
            pins = post_pair(jnp.maximum(a - 2, 0) if u == 0 else a - 2, prev[M:])
            lhs_a = make_lhs(prev[0:M], a)
            lhs_a = (lhs_a.astype(BF16), None) if u == 0 else split_lhs(lhs_a)
            res_a, oe_a = segment(a, *lhs_a, None,
                                  {k: [v] for k, v in zip((0, 4, 8, 12), pins[:4])})
            res_a = jnp.concatenate(res_a, axis=1)
            pins = pins[4:] + post(a, 0, 3, res_a[M:])
            res_b, _ = segment(a + 1, *split_lhs(make_lhs(res_a[0:M], a + 1)), oe_a,
                               {k: [v] for k, v in zip((0, 4, 8, 12), pins)})
            prev = jnp.concatenate(res_b, axis=1)
        pend[...] = prev
        return carry

    with jax.named_scope("main_loop"):
        jax.lax.fori_loop(0, NIT, step, 0)
    post_pair(NSEG - 2, pend[M:, :])
    cp_o2.start()

    def max_all(v):
        return jnp.max(jnp.max(v, axis=0, keepdims=True), axis=1, keepdims=True)

    def decode(k):
        kb = pltpu.bitcast(jnp.broadcast_to(k, (8, 128)), jnp.int32)
        code = (kb >> 11) & 0xFFFF
        hi = jnp.where(code >= 0x8000, code & 0x7FFF, code ^ 0xFFFF)
        tok = jnp.clip((LAST - (kb & LAST))[0, 0], 0, LAST)
        return tok, pltpu.bitcast(hi << 16, F32)[:, 0:1]

    kv = keys[...]
    k1 = max_all(kv)
    k2 = max_all(jnp.where(kv == k1, 0.0, kv))
    i1, r1 = decode(k1)
    i2, r2 = decode(k2)
    g1, g2 = i1 >> 3, i2 >> 3

    def rows_of(ref):
        return jnp.concatenate([ref[g1 >> 2, pl.ds(g1 & 3, 1)], ref[g2 >> 2, pl.ds(g2 & 3, 1)]],
                               axis=0).astype(F32)

    x1, h2 = rows_of(x1v), rows_of(h2v)
    for cp in cp_ffn:
        cp.wait()
    hl = h2.reshape(16, D).astype(BF16)
    act = []
    for j in range(FF // 128):
        gt = _rb(_dot(hl, wblk(wg, j)))
        up = _rb(_dot(hl, wblk(wu, j)))
        act.append((_rb(gt * jax.nn.sigmoid(gt)) * up).astype(BF16))
    act = jnp.concatenate(act, axis=1)
    y = jnp.concatenate([_dot(act, wblk(wd, n)) for n in range(8)], axis=1).reshape(2, 8, D)
    rowi = jax.lax.broadcasted_iota(jnp.int32, (2, 8, 1), 1)
    gsel = jax.lax.broadcasted_iota(jnp.int32, (2, 8, 1), 0)
    tokp = jnp.where(gsel == 0, g1, g2) * 8 + rowi
    gate = _rb(jax.nn.sigmoid(jnp.where(tokp == i1, r1[None], r2[None])))
    upd = jnp.where((tokp == i1) | (tokp == i2), _rb(_rb(y) * gate), 0.0)
    patch[...] = (x1 + _rb(mod_vec(5) * _rb(h2 + upd))).astype(BF16)
    cp_o1.wait()
    cp_o2.wait()
    cp1 = pltpu.make_async_copy(patch.at[0], out_hbm.at[g1 >> 2, g1 & 3], sem_out.at[0])
    cp1.start()

    @pl.when(g1 != g2)
    def _():
        cp2 = pltpu.make_async_copy(patch.at[1], out_hbm.at[g2 >> 2, g2 & 3], sem_out.at[1])
        cp2.start()
        cp2.wait()

    cp1.wait()


@jax.jit
def pallas_adaLN_cond__memory_aug_recurrent_mem_tr__moe_arch_mod__prompt_kernel(
    A_x: jax.Array,
    A_mem0: jax.Array,
    A_Wq: jax.Array,
    A_Wk: jax.Array,
    A_Wv: jax.Array,
    A_Wo: jax.Array,
    A_seg_len,
    B_x: jax.Array,
    B_w_r: jax.Array,
    B_w_gate: jax.Array,
    B_w_up: jax.Array,
    B_w_down: jax.Array,
    c: jax.Array,
    w_mod: jax.Array,
):
    assert A_x.shape == (1, NSEG * SEG, D)
    any_spec = pl.BlockSpec(memory_space=pl.ANY)
    out = pl.pallas_call(
        _kernel,
        out_shape=jax.ShapeDtypeStruct((NSEG, 4, 8, D), BF16),
        in_specs=[any_spec] * 12,
        out_specs=any_spec,
        scratch_shapes=[
            pltpu.VMEM((H, D // 2, DH), U32),
            pltpu.VMEM((H, D // 2, DH), U32),
            pltpu.VMEM((H, D // 2, DH), U32),
            pltpu.VMEM((H * DH // 2, D), U32),
            pltpu.VMEM((D // 2, FF), U32),
            pltpu.VMEM((D // 2, FF), U32),
            pltpu.VMEM((FF // 2, D), U32),
            pltpu.VMEM((D // 2, 6 * D), U32),
            pltpu.VMEM((NSEG, 4, 8, D), BF16),
            pltpu.VMEM((NSEG, 4, 8, D), BF16),
            pltpu.VMEM((NSEG, 4, 8, D), BF16),
            pltpu.VMEM((NSEG, 4, 8, D), BF16),
            pltpu.VMEM((NSEG, 3 * NP, 8, DH), U32),
            pltpu.VMEM((NE, D), BF16),
            pltpu.VMEM((NSEG, 3, 8, D), F32),
            pltpu.VMEM((M + SEG + M, D), F32),
            pltpu.VMEM((8, 6 * D), F32),
            pltpu.VMEM((80, 128), F32),
            pltpu.VMEM((SEG, 128), F32),
            pltpu.VMEM((2, 8, D), BF16),
            pltpu.VMEM((8, 128), U32),
            pltpu.VMEM((NP, 4, 80, DH), BF16),
            pltpu.VMEM((3, NE, 2 * DH), F32),
            pltpu.VMEM((M, D), BF16),
            pltpu.VMEM((D,), BF16),
            pltpu.VMEM((1, D), BF16),
            pltpu.SemaphoreType.DMA((16 + NP,)),
            pltpu.SemaphoreType.DMA((2,)),
        ],
        compiler_params=pltpu.CompilerParams(vmem_limit_bytes=120 * 1024 * 1024),
    )(
        A_x.reshape(NSEG, 4, 8, D),
        A_mem0.reshape(M, D),
        A_Wq.reshape(D // 2, 2, H, DH),
        A_Wk.reshape(D // 2, 2, H, DH),
        A_Wv.reshape(D // 2, 2, H, DH),
        A_Wo.reshape(H * DH, D),
        B_w_r,
        B_w_gate,
        B_w_up,
        B_w_down,
        c,
        w_mod,
    )
    return out.reshape(1, NSEG * SEG, D)
```

```python
import jax
import jax.numpy as jnp
import jax.experimental.pallas as pl
import jax.experimental.pallas.tpu as pltpu

F32 = jnp.float32
BF16 = jnp.bfloat16
U32 = jnp.uint32

D = 1024
H = 32
DH = 128
NP = H // 2
M = 8
SEG = 32
NSEG = 64
FF = 3584
NJ = SEG - M
NE = NSEG * M
EPS = 1e-5
SCALE = DH ** (-0.5)
NEG = -1000000000.0
LOG2E = 1.4426950408889634
KQ = 256
FIRST = 7
UNROLL = 2
NIT = NSEG // (2 * UNROLL)
OUT_SPLIT = NSEG - 2 * UNROLL - 2


def _rb(x):
    return x.astype(BF16).astype(F32)


def _layernorm(xf):
    m = jnp.mean(xf, axis=-1, keepdims=True)
    d = xf - m
    v = jnp.mean(d * d, axis=-1, keepdims=True)
    return d * jax.lax.rsqrt(v + EPS)


def _dot(a, b):
    return jnp.dot(a, b, preferred_element_type=F32)


def _dot_nt(a, b):
    return jax.lax.dot_general(a, b, (((1,), (1,)), ((), ())), preferred_element_type=F32)


def _kernel(x_hbm, mem0_hbm, wq_hbm, wk_hbm, wv_hbm, wo_hbm, wr_hbm, wg_hbm, wu_hbm, wd_hbm,
            c_hbm, wm_hbm,
            out_hbm,
            wq, wk, wv, wo, wg, wu, wd, wm, xv, x1v, h2v, outv, early, he, hj, pend,
            mod, fill, keys, patch, zero, opnd, acc0, mem0_ref, wr_ref, c_ref,
            sem, sem_out):
    w_u32 = [w.bitcast(U32) for w in (wq_hbm, wk_hbm, wv_hbm)]
    wqkv = (wq, wk, wv)
    wo_hbm, wg_hbm, wu_hbm, wd_hbm, wm_hbm = [
        w.bitcast(U32) for w in (wo_hbm, wg_hbm, wu_hbm, wd_hbm, wm_hbm)]

    def wblk(w, j, lo=None, hi=None):
        rows = slice(None) if lo is None else slice(lo // 2, hi // 2)
        return pltpu.bitcast(w[rows, j * 128:(j + 1) * 128], BF16)

    def wm_copy(lo, n, k):
        return pltpu.make_async_copy(wm_hbm.at[:, pl.ds(lo, n)], wm.at[:, pl.ds(lo, n)], sem.at[k])

    def w_copies(m, p, k):
        return [pltpu.make_async_copy(w_u32[m].at[:, par, p, :], wqkv[m].at[2 * p + par], sem.at[k])
                for par in range(2)]

    def xj_copy(p, k):
        segs = pl.ds(4 * p, 4)
        return pltpu.make_async_copy(x_hbm.at[segs, 0:3], xv.at[segs, 0:3], sem.at[k])

    def group_copies(p, last=False):
        k = 16 + p
        return (w_copies(1, p, k) + w_copies(2, p, k) + ([] if last else w_copies(0, p + 1, k))
                + [xj_copy(p, k)])

    cp_c = pltpu.make_async_copy(c_hbm, c_ref, sem.at[5])
    cp_xe = pltpu.make_async_copy(x_hbm.at[:, 3], xv.at[:, 3], sem.at[0])
    cp_w0 = w_copies(0, 0, 6) + w_copies(1, 0, 6) + w_copies(2, 0, 6)
    cp_wm1 = [[wm_copy(j * KQ, KQ, 1 + j), wm_copy(D + j * KQ, KQ, 1 + j)] for j in range(D // KQ)]
    cp_q1 = w_copies(0, 1, 7) + [xj_copy(0, 7)]
    cp_late = [wm_copy(2 * D, 4 * D, 9), pltpu.make_async_copy(wo_hbm, wo, sem.at[10]),
               pltpu.make_async_copy(mem0_hbm, mem0_ref, sem.at[14]),
               pltpu.make_async_copy(wr_hbm, wr_ref, sem.at[15])]
    cp_ffn = [pltpu.make_async_copy(wg_hbm, wg, sem.at[11]),
              pltpu.make_async_copy(wu_hbm, wu, sem.at[12]),
              pltpu.make_async_copy(wd_hbm, wd, sem.at[13])]

    for cp in [cp_c, cp_xe] + cp_w0 + sum(cp_wm1, []) + cp_q1:
        cp.start()
    for p in range(1, FIRST):
        for cp in group_copies(p):
            cp.start()

    ri = jax.lax.broadcasted_iota(jnp.int32, (80, 128), 0)
    ci = jax.lax.broadcasted_iota(jnp.int32, (80, 128), 1)

    def head_of(i):
        return jnp.where(i < 64, i >> 5, (i - 64) >> 3)

    def pos_of(i):
        return jnp.where(i < 64, i & 31, 32 + (i & 7))

    same = (head_of(ri) == head_of(ci)) & (ci < 80)
    allowed = (pos_of(ri) < M) | (pos_of(ri) >= pos_of(ci))
    fill[...] = jnp.where(same, jnp.where(allowed, 0.0, NEG / SCALE), -jnp.inf).astype(F32)
    keys[...] = jnp.zeros(keys.shape, F32)
    pend[M:, :] = jnp.zeros((SEG + M, D), F32)
    zero[...] = jnp.zeros(zero.shape, U32)

    def pin_zero(vals):
        acc = None
        for v in vals:
            v = pltpu.bitcast(v, U32)
            for r in range(0, v.shape[0], 8):
                acc = v[r:r + 8] if acc is None else acc | v[r:r + 8]
        return acc & zero[...]

    cp_xe.wait()
    cp_c.wait()
    cf = c_ref[...].astype(F32)
    sc = _rb(cf * jax.nn.sigmoid(cf))
    sc = jnp.broadcast_to(sc, (16, D)).astype(BF16)

    def mod_cols(lo, hi):
        for j in range(lo, hi):
            v = _rb(_dot(sc, wblk(wm, j))[0:8])
            if j // 8 in (1, 4):
                v = _rb(1.0 + v)
            mod[:, j * 128:(j + 1) * 128] = v

    def mod_vec(k):
        return mod[:, k * D:(k + 1) * D]

    def affine1(n):
        return _rb(n * mod_vec(1)) + mod_vec(0)

    def ne_body(i, carry):
        n = _layernorm(xv[pl.ds(i * 16, 16), 3].astype(F32))
        he[pl.ds(pl.multiple_of(i * 128, 128), 128), :] = n.reshape(128, D).astype(BF16)
        return carry

    jax.lax.fori_loop(0, NSEG // 16, ne_body, 0)

    def w_head(m, h, lo=0, hi=D):
        return pltpu.bitcast(wqkv[m][h, lo // 2:hi // 2, :], BF16)

    def relayout(m, p):
        w = wqkv[m]
        e = w[2 * p]
        o = w[2 * p + 1]
        w[2 * p] = (e & U32(0xFFFF)) | (o << 16)
        w[2 * p + 1] = (e >> 16) | (o & U32(0xFFFF0000))

    def store_early(m, p, row0, r1, r2):
        ns = r1.shape[0] // 8
        r12 = jnp.concatenate([r1.reshape(ns, 8, DH), r2.reshape(ns, 8, DH)], axis=1)
        early[row0 // 8:row0 // 8 + ns, m * NP + p] = pltpu.bitcast(
            r12.reshape(16 * ns, DH).astype(BF16), U32).reshape(ns, 8, DH)

    for cp in cp_w0:
        cp.wait()
    for m in range(3):
        relayout(m, 0)
    for j in range(D // KQ):
        for cp in cp_wm1[j]:
            cp.wait()
        lo, hi = j * KQ, (j + 1) * KQ
        mod_cols(lo // 128, hi // 128)
        mod_cols((D + lo) // 128, (D + hi) // 128)
        for c in range(2):
            rows = slice(c * 256, (c + 1) * 256)
            n = he[rows, lo:hi].astype(F32).reshape(32, 8, KQ)
            h = (_rb(n * mod[:, D + lo:D + hi]) + mod[:, lo:hi]).reshape(256, KQ)
            he[rows, lo:hi] = h.astype(BF16)
            hb = h.astype(BF16)
            for m in range(3):
                w2 = jnp.concatenate([w_head(m, 0, lo, hi), w_head(m, 1, lo, hi)], axis=1)
                r = _dot(hb, w2)
                if j > 0:
                    r = r + acc0[m, rows, :]
                if hi < D:
                    acc0[m, rows, :] = r
                else:
                    store_early(m, 0, c * 256, r[:, :DH], r[:, DH:])

    def early_proj(m, p, pins=None, rows=256, between=None):
        relayout(m, p)
        for c in range(NE // rows):
            hc = he[c * rows:(c + 1) * rows, :]
            r12 = []
            for b in range(2):
                wv_ = wqkv[m][2 * p + b]
                if pins and 2 * c + b in pins:
                    wv_ = jnp.concatenate([wv_[0:8] | pin_zero(pins[2 * c + b]), wv_[8:]], axis=0)
                r12.append(_dot(hc, pltpu.bitcast(wv_, BF16)))
                if between is not None:
                    between()
            store_early(m, p, c * rows, *r12)

    def make_hj(s):
        h = affine1(_rb(_layernorm(xv[s, 0:3].astype(F32))))
        hj[s] = h
        return h[:, :, 0:128].reshape(NJ, 128)

    for cp in cp_q1:
        cp.wait()
    pins = [make_hj(s) for s in range(4)]
    early_proj(0, 1, {2: pins[0:2], 3: pins[2:4]})

    def pro_body(p, carry):
        @pl.when(p == 4)
        def _():
            for pp in range(FIRST, NP):
                for cp in group_copies(pp, pp == NP - 1):
                    cp.start()
            for cp in cp_late:
                cp.start()

        for cp in group_copies(p):
            cp.wait()
        pins = [[make_hj(p * 4 + t)] for t in range(4)]
        early_proj(1, p, {3: pins[0]})
        early_proj(2, p, {3: pins[1]})
        early_proj(0, p + 1, {2: pins[2], 3: pins[3]})
        return carry

    with jax.named_scope("prologue_loop"):
        jax.lax.fori_loop(1, NP - 1, pro_body, 0)

    for cp in cp_ffn:
        cp.start()
    for cp in group_copies(NP - 1, True) + cp_late:
        cp.wait()
    pend[0:M, :] = mem0_ref[...].astype(F32)
    todo = list(range(16, 48))

    def one_mod_col():
        j = todo.pop(0)
        mod_cols(j, j + 1)

    pins = [[make_hj(s)] for s in range(NSEG - 4, NSEG)]
    early_proj(1, NP - 1, {6: pins[0], 12: pins[1]}, rows=64, between=one_mod_col)
    early_proj(2, NP - 1, {4: pins[2], 10: pins[3]}, rows=64, between=one_mod_col)
    assert not todo

    wr = jnp.broadcast_to(wr_ref[...].astype(F32).reshape(1, D), (8, D))

    lane8 = jax.lax.broadcasted_iota(jnp.int32, (8, 128), 1)
    sub8 = jax.lax.broadcasted_iota(jnp.int32, (8, 128), 0)
    LAST = NSEG * SEG - 1

    def post(s, g0, g1, attn):
        attn = attn.reshape(g1 - g0, 8, D)
        x1 = _rb(xv[s, g0:g1].astype(F32) + _rb(mod_vec(2) * _rb(attn)))
        n = _rb(_layernorm(x1))
        h2 = _rb(_rb(n * mod_vec(4)) + mod_vec(3))
        r = _rb(jnp.sum(h2 * wr, axis=-1, keepdims=True)) + 0.0
        x1v[s, g0:g1] = x1.astype(BF16)
        h2v[s, g0:g1] = h2.astype(BF16)
        outv[s, g0:g1] = (x1 + _rb(mod_vec(5) * h2)).astype(BF16)
        pins = []
        for g in range(g0, g1):
            bits = pltpu.bitcast(jnp.broadcast_to(r[g - g0], (8, 128)), jnp.int32)
            hi = jax.lax.shift_right_logical(bits, 16)
            code = jnp.where(bits < 0, hi ^ 0xFFFF, hi | 0x8000)
            key = (code << 11) | (LAST - (s * SEG + g * 8) - sub8) | 0x40000000
            rows = slice(g * 8, (g + 1) * 8)
            knew = jnp.where(lane8 == s, pltpu.bitcast(key, F32), keys[rows, :])
            keys[rows, :] = knew
            pins.append(knew)
        return pins

    def post_pair(a, rows):
        return post(a + 1, 0, 4, rows[0:SEG]) + post(a, 3, 4, rows[SEG:])

    zpad = jnp.zeros((48, DH), BF16)
    G = 4
    KA = (NP - G) * 2 * DH
    KS = D - 128

    def segment(s, lhs, lhs_split, extra, pins):
        probs = {}

        def stash(p, m, v):
            opnd[p, m, 0:v.shape[0], :] = v.astype(BF16)

        def qkv_group(p):
            keys = [(m, 2 * p + b) for m in range(3) for b in range(2 * G)]
            nsplit = 6 if (p == 0 and lhs_split is not None) else 0
            part = [_dot(lhs_split[0], w_head(m, h, 0, KS)) for m, h in keys[:nsplit]]
            full = [_dot(lhs_split[1], w_head(m, h, KS, D)) + part[i]
                    for i, (m, h) in enumerate(keys[:nsplit])]
            full += [_dot(lhs, w_head(m, h)) for m, h in keys[nsplit:]]
            for m in range(3):
                for t in range(G):
                    i = 2 * G * m + 2 * t
                    stash(p + t, m, jnp.concatenate([full[i], full[i + 1]], axis=0))

        def operand(p, m):
            parts = [opnd[p, m, 0:64, :], pltpu.bitcast(early[s, m * NP + p], BF16)]
            if m > 0:
                parts.append(zpad)
            return jnp.concatenate(parts, axis=0)

        def scores(p):
            sc_ = _dot_nt(operand(p, 0), operand(p, 1))
            f = fill[...]
            if pins.get(p):
                f = jnp.concatenate([f[0:8] + pltpu.bitcast(pin_zero(pins[p]), F32), f[8:]], axis=0)
            sc_ = jnp.where(f == 0.0, sc_, f)
            mx = jnp.max(sc_, axis=-1, keepdims=True)
            e = jnp.exp2((sc_ - mx) * (SCALE * LOG2E))
            stash(p, 3, e)
            probs[p] = pl.reciprocal(jnp.sum(e, axis=-1, keepdims=True), approx=True)

        oe = []

        def pv(p):
            o = _dot(opnd[p, 3], operand(p, 2)) * probs[p]
            res = []
            for b in range(2):
                rows, erows = o[32 * b:32 * b + 32], o[64 + 8 * b:72 + 8 * b]
                oe.append(erows)
                if extra is not None:
                    rows = jnp.concatenate([rows, erows, extra[2 * p + b]], axis=0)
                res.append(rows)
            pins.setdefault(p + G, []).append(o)
            return res

        os_ = []
        for p in range(0, NP, G):
            qkv_group(p)
            if p >= G:
                for t in range(G):
                    os_ += pv(p - G + t)
            for t in range(G):
                scores(p + t)
        oa = jnp.concatenate(os_, axis=1).astype(BF16)
        acc, ob = [], []
        for n in range(7):
            acc.append(_dot(oa, wblk(wo, n, 0, KA)))
            if n == 2:
                for t in range(G):
                    ob += pv(NP - G + t)
        ob = jnp.concatenate(ob, axis=1).astype(BF16)
        res = [_dot(ob, wblk(wo, n, KA, H * DH)) + acc[n] for n in range(7)]
        res.append(_dot(ob, wblk(wo, 7, KA, H * DH)) + _dot(oa, wblk(wo, 7, 0, KA)))
        return res, oe

    def make_lhs(mem, s):
        return jnp.concatenate([mem, hj[s].reshape(NJ, D)], axis=0)

    cp_o1 = pltpu.make_async_copy(outv.at[0:OUT_SPLIT], out_hbm.at[0:OUT_SPLIT], sem_out.at[0])
    cp_o2 = pltpu.make_async_copy(outv.at[OUT_SPLIT:NSEG], out_hbm.at[OUT_SPLIT:NSEG],
                                  sem_out.at[1])

    def split_lhs(lhs):
        return lhs.astype(BF16), (lhs[:, :KS].astype(BF16), lhs[:, KS:].astype(BF16))

    def step(i, carry):
        @pl.when(i == NIT - 1)
        def _():
            cp_o1.start()

        prev = pend[...]
        for u in range(UNROLL):
            a = 2 * (UNROLL * i + u)
            pins = post_pair(jnp.maximum(a - 2, 0) if u == 0 else a - 2, prev[M:])
            lhs_a = make_lhs(prev[0:M], a)
            lhs_a = (lhs_a.astype(BF16), None) if u == 0 else split_lhs(lhs_a)
            res_a, oe_a = segment(a, *lhs_a, None,
                                  {k: [v] for k, v in zip((3, 7, 11, 15), pins[:4])})
            res_a = jnp.concatenate(res_a, axis=1)
            pins = pins[4:] + post(a, 0, 3, res_a[M:])
            res_b, _ = segment(a + 1, *split_lhs(make_lhs(res_a[0:M], a + 1)), oe_a,
                               {k: [v] for k, v in zip((3, 7, 11, 15), pins)})
            prev = jnp.concatenate(res_b, axis=1)
        pend[...] = prev
        return carry

    with jax.named_scope("main_loop"):
        jax.lax.fori_loop(0, NIT, step, 0)
    post_pair(NSEG - 2, pend[M:, :])
    cp_o2.start()

    def max_all(v):
        return jnp.max(jnp.max(v, axis=0, keepdims=True), axis=1, keepdims=True)

    def decode(k):
        kb = pltpu.bitcast(jnp.broadcast_to(k, (8, 128)), jnp.int32)
        code = (kb >> 11) & 0xFFFF
        hi = jnp.where(code >= 0x8000, code & 0x7FFF, code ^ 0xFFFF)
        tok = jnp.clip((LAST - (kb & LAST))[0, 0], 0, LAST)
        return tok, pltpu.bitcast(hi << 16, F32)[:, 0:1]

    kv = keys[...]
    k1 = max_all(kv)
    k2 = max_all(jnp.where(kv == k1, 0.0, kv))
    i1, r1 = decode(k1)
    i2, r2 = decode(k2)
    g1, g2 = i1 >> 3, i2 >> 3

    def rows_of(ref):
        return jnp.concatenate([ref[g1 >> 2, pl.ds(g1 & 3, 1)], ref[g2 >> 2, pl.ds(g2 & 3, 1)]],
                               axis=0).astype(F32)

    x1, h2 = rows_of(x1v), rows_of(h2v)
    for cp in cp_ffn:
        cp.wait()
    hl = h2.reshape(16, D).astype(BF16)
    act = []
    for j in range(FF // 128):
        gt = _rb(_dot(hl, wblk(wg, j)))
        up = _rb(_dot(hl, wblk(wu, j)))
        act.append((_rb(gt * jax.nn.sigmoid(gt)) * up).astype(BF16))
    act = jnp.concatenate(act, axis=1)
    y = jnp.concatenate([_dot(act, wblk(wd, n)) for n in range(8)], axis=1).reshape(2, 8, D)
    rowi = jax.lax.broadcasted_iota(jnp.int32, (2, 8, 1), 1)
    gsel = jax.lax.broadcasted_iota(jnp.int32, (2, 8, 1), 0)
    tokp = jnp.where(gsel == 0, g1, g2) * 8 + rowi
    gate = _rb(jax.nn.sigmoid(jnp.where(tokp == i1, r1[None], r2[None])))
    upd = jnp.where((tokp == i1) | (tokp == i2), _rb(_rb(y) * gate), 0.0)
    patch[...] = (x1 + _rb(mod_vec(5) * _rb(h2 + upd))).astype(BF16)
    cp_o1.wait()
    cp_o2.wait()
    cp1 = pltpu.make_async_copy(patch.at[0], out_hbm.at[g1 >> 2, g1 & 3], sem_out.at[0])
    cp1.start()

    @pl.when(g1 != g2)
    def _():
        cp2 = pltpu.make_async_copy(patch.at[1], out_hbm.at[g2 >> 2, g2 & 3], sem_out.at[1])
        cp2.start()
        cp2.wait()

    cp1.wait()


@jax.jit
def pallas_adaLN_cond__memory_aug_recurrent_mem_tr__moe_arch_mod__prompt_kernel(
    A_x: jax.Array,
    A_mem0: jax.Array,
    A_Wq: jax.Array,
    A_Wk: jax.Array,
    A_Wv: jax.Array,
    A_Wo: jax.Array,
    A_seg_len,
    B_x: jax.Array,
    B_w_r: jax.Array,
    B_w_gate: jax.Array,
    B_w_up: jax.Array,
    B_w_down: jax.Array,
    c: jax.Array,
    w_mod: jax.Array,
):
    assert A_x.shape == (1, NSEG * SEG, D)
    any_spec = pl.BlockSpec(memory_space=pl.ANY)
    out = pl.pallas_call(
        _kernel,
        out_shape=jax.ShapeDtypeStruct((NSEG, 4, 8, D), BF16),
        in_specs=[any_spec] * 12,
        out_specs=any_spec,
        scratch_shapes=[
            pltpu.VMEM((H, D // 2, DH), U32),
            pltpu.VMEM((H, D // 2, DH), U32),
            pltpu.VMEM((H, D // 2, DH), U32),
            pltpu.VMEM((H * DH // 2, D), U32),
            pltpu.VMEM((D // 2, FF), U32),
            pltpu.VMEM((D // 2, FF), U32),
            pltpu.VMEM((FF // 2, D), U32),
            pltpu.VMEM((D // 2, 6 * D), U32),
            pltpu.VMEM((NSEG, 4, 8, D), BF16),
            pltpu.VMEM((NSEG, 4, 8, D), BF16),
            pltpu.VMEM((NSEG, 4, 8, D), BF16),
            pltpu.VMEM((NSEG, 4, 8, D), BF16),
            pltpu.VMEM((NSEG, 3 * NP, 8, DH), U32),
            pltpu.VMEM((NE, D), BF16),
            pltpu.VMEM((NSEG, 3, 8, D), F32),
            pltpu.VMEM((M + SEG + M, D), F32),
            pltpu.VMEM((8, 6 * D), F32),
            pltpu.VMEM((80, 128), F32),
            pltpu.VMEM((SEG, 128), F32),
            pltpu.VMEM((2, 8, D), BF16),
            pltpu.VMEM((8, 128), U32),
            pltpu.VMEM((NP, 4, 80, DH), BF16),
            pltpu.VMEM((3, NE, 2 * DH), F32),
            pltpu.VMEM((M, D), BF16),
            pltpu.VMEM((D,), BF16),
            pltpu.VMEM((1, D), BF16),
            pltpu.SemaphoreType.DMA((16 + NP,)),
            pltpu.SemaphoreType.DMA((2,)),
        ],
        compiler_params=pltpu.CompilerParams(vmem_limit_bytes=120 * 1024 * 1024),
    )(
        A_x.reshape(NSEG, 4, 8, D),
        A_mem0.reshape(M, D),
        A_Wq.reshape(D // 2, 2, H, DH),
        A_Wk.reshape(D // 2, 2, H, DH),
        A_Wv.reshape(D // 2, 2, H, DH),
        A_Wo.reshape(H * DH, D),
        B_w_r,
        B_w_gate,
        B_w_up,
        B_w_down,
        c,
        w_mod,
    )
    return out.reshape(1, NSEG * SEG, D)
```

```python
import jax
import jax.numpy as jnp
import jax.experimental.pallas as pl
import jax.experimental.pallas.tpu as pltpu

F32 = jnp.float32
BF16 = jnp.bfloat16
U32 = jnp.uint32

D = 1024
H = 32
DH = 128
NP = H // 2
M = 8
SEG = 32
NSEG = 64
FF = 3584
NJ = SEG - M
NE = NSEG * M
EPS = 1e-5
SCALE = DH ** (-0.5)
NEG = -1000000000.0
LOG2E = 1.4426950408889634
KQ = 256
FIRST = 7
UNROLL = 2
NIT = NSEG // (2 * UNROLL)
OUT_SPLIT = NSEG - 2 * UNROLL - 2


def _rb(x):
    return x.astype(BF16).astype(F32)


def _layernorm(xf):
    m = jnp.mean(xf, axis=-1, keepdims=True)
    d = xf - m
    v = jnp.mean(d * d, axis=-1, keepdims=True)
    return d * jax.lax.rsqrt(v + EPS)


def _dot(a, b):
    return jnp.dot(a, b, preferred_element_type=F32)


def _dot_nt(a, b):
    return jax.lax.dot_general(a, b, (((1,), (1,)), ((), ())), preferred_element_type=F32)


def _kernel(x_hbm, mem0_hbm, wq_hbm, wk_hbm, wv_hbm, wo_hbm, wr_hbm, wg_hbm, wu_hbm, wd_hbm,
            c_hbm, wm_hbm,
            out_hbm,
            wq, wk, wv, wo, wg, wu, wd, wm, xv, x1v, h2v, outv, early, he, hj, pend,
            mod, fill, keys, patch, zero, opnd, acc0, mem0_ref, wr_ref, c_ref,
            sem, sem_out):
    w_u32 = [w.bitcast(U32) for w in (wq_hbm, wk_hbm, wv_hbm)]
    wqkv = (wq, wk, wv)
    wo_hbm, wg_hbm, wu_hbm, wd_hbm, wm_hbm = [
        w.bitcast(U32) for w in (wo_hbm, wg_hbm, wu_hbm, wd_hbm, wm_hbm)]

    def wblk(w, j, lo=None, hi=None):
        rows = slice(None) if lo is None else slice(lo // 2, hi // 2)
        return pltpu.bitcast(w[rows, j * 128:(j + 1) * 128], BF16)

    def wm_copy(lo, n, k):
        return pltpu.make_async_copy(wm_hbm.at[:, pl.ds(lo, n)], wm.at[:, pl.ds(lo, n)], sem.at[k])

    def w_copies(m, p, k):
        return [pltpu.make_async_copy(w_u32[m].at[:, par, p, :], wqkv[m].at[2 * p + par], sem.at[k])
                for par in range(2)]

    def xj_copy(p, k):
        segs = pl.ds(4 * p, 4)
        return pltpu.make_async_copy(x_hbm.at[segs, 0:3], xv.at[segs, 0:3], sem.at[k])

    def group_copies(p, last=False):
        k = 16 + p
        return (w_copies(1, p, k) + w_copies(2, p, k) + ([] if last else w_copies(0, p + 1, k))
                + [xj_copy(p, k)])

    cp_c = pltpu.make_async_copy(c_hbm, c_ref, sem.at[5])
    cp_xe = pltpu.make_async_copy(x_hbm.at[:, 3], xv.at[:, 3], sem.at[0])
    cp_w0 = w_copies(0, 0, 6) + w_copies(1, 0, 6) + w_copies(2, 0, 6)
    cp_wm1 = [[wm_copy(j * KQ, KQ, 1 + j), wm_copy(D + j * KQ, KQ, 1 + j)] for j in range(D // KQ)]
    cp_q1 = w_copies(0, 1, 7) + [xj_copy(0, 7)]
    cp_late = [wm_copy(2 * D, 4 * D, 9), pltpu.make_async_copy(wo_hbm, wo, sem.at[10]),
               pltpu.make_async_copy(mem0_hbm, mem0_ref, sem.at[14]),
               pltpu.make_async_copy(wr_hbm, wr_ref, sem.at[15])]
    cp_ffn = [pltpu.make_async_copy(wg_hbm, wg, sem.at[11]),
              pltpu.make_async_copy(wu_hbm, wu, sem.at[12]),
              pltpu.make_async_copy(wd_hbm, wd, sem.at[13])]

    for cp in [cp_c, cp_xe] + cp_w0 + sum(cp_wm1, []) + cp_q1:
        cp.start()
    for p in range(1, FIRST):
        for cp in group_copies(p):
            cp.start()

    ri = jax.lax.broadcasted_iota(jnp.int32, (80, 128), 0)
    ci = jax.lax.broadcasted_iota(jnp.int32, (80, 128), 1)

    def head_of(i):
        return jnp.where(i < 64, i >> 5, (i - 64) >> 3)

    def pos_of(i):
        return jnp.where(i < 64, i & 31, 32 + (i & 7))

    same = (head_of(ri) == head_of(ci)) & (ci < 80)
    allowed = (pos_of(ri) < M) | (pos_of(ri) >= pos_of(ci))
    fill[...] = jnp.where(same, jnp.where(allowed, 0.0, NEG / SCALE), -jnp.inf).astype(F32)
    keys[...] = jnp.zeros(keys.shape, F32)
    pend[M:, :] = jnp.zeros((SEG + M, D), F32)
    zero[...] = jnp.zeros(zero.shape, U32)

    def pin_zero(vals):
        acc = None
        for v in vals:
            v = pltpu.bitcast(v, U32)
            for r in range(0, v.shape[0], 8):
                acc = v[r:r + 8] if acc is None else acc | v[r:r + 8]
        return acc & zero[...]

    cp_xe.wait()
    cp_c.wait()
    cf = c_ref[...].astype(F32)
    sc = _rb(cf * jax.nn.sigmoid(cf))
    sc = jnp.broadcast_to(sc, (16, D)).astype(BF16)

    def mod_cols(lo, hi):
        for j in range(lo, hi):
            v = _rb(_dot(sc, wblk(wm, j))[0:8])
            if j // 8 in (1, 4):
                v = _rb(1.0 + v)
            mod[:, j * 128:(j + 1) * 128] = v

    def mod_vec(k):
        return mod[:, k * D:(k + 1) * D]

    def affine1(n):
        return _rb(n * mod_vec(1)) + mod_vec(0)

    def ne_body(i, carry):
        n = _layernorm(xv[pl.ds(i * 16, 16), 3].astype(F32))
        he[pl.ds(pl.multiple_of(i * 128, 128), 128), :] = n.reshape(128, D).astype(BF16)
        return carry

    jax.lax.fori_loop(0, NSEG // 16, ne_body, 0)

    def w_head(m, h, lo=0, hi=D):
        return pltpu.bitcast(wqkv[m][h, lo // 2:hi // 2, :], BF16)

    def relayout(m, p):
        w = wqkv[m]
        e = w[2 * p]
        o = w[2 * p + 1]
        w[2 * p] = (e & U32(0xFFFF)) | (o << 16)
        w[2 * p + 1] = (e >> 16) | (o & U32(0xFFFF0000))

    def store_early(m, p, row0, r1, r2):
        ns = r1.shape[0] // 8
        r12 = jnp.concatenate([r1.reshape(ns, 8, DH), r2.reshape(ns, 8, DH)], axis=1)
        early[row0 // 8:row0 // 8 + ns, m * NP + p] = pltpu.bitcast(
            r12.reshape(16 * ns, DH).astype(BF16), U32).reshape(ns, 8, DH)

    for cp in cp_w0:
        cp.wait()
    for m in range(3):
        relayout(m, 0)
    for j in range(D // KQ):
        for cp in cp_wm1[j]:
            cp.wait()
        lo, hi = j * KQ, (j + 1) * KQ
        mod_cols(lo // 128, hi // 128)
        mod_cols((D + lo) // 128, (D + hi) // 128)
        for c in range(2):
            rows = slice(c * 256, (c + 1) * 256)
            n = he[rows, lo:hi].astype(F32).reshape(32, 8, KQ)
            h = (_rb(n * mod[:, D + lo:D + hi]) + mod[:, lo:hi]).reshape(256, KQ)
            he[rows, lo:hi] = h.astype(BF16)
            hb = h.astype(BF16)
            for m in range(3):
                w2 = jnp.concatenate([w_head(m, 0, lo, hi), w_head(m, 1, lo, hi)], axis=1)
                r = _dot(hb, w2)
                if j > 0:
                    r = r + acc0[m, rows, :]
                if hi < D:
                    acc0[m, rows, :] = r
                else:
                    store_early(m, 0, c * 256, r[:, :DH], r[:, DH:])

    def early_proj(m, p, pins=None, rows=256, between=None):
        relayout(m, p)
        for c in range(NE // rows):
            hc = he[c * rows:(c + 1) * rows, :]
            r12 = []
            for b in range(2):
                wv_ = wqkv[m][2 * p + b]
                if pins and 2 * c + b in pins:
                    wv_ = jnp.concatenate([wv_[0:8] | pin_zero(pins[2 * c + b]), wv_[8:]], axis=0)
                r12.append(_dot(hc, pltpu.bitcast(wv_, BF16)))
                if between is not None:
                    between()
            store_early(m, p, c * rows, *r12)

    def make_hj(s):
        h = affine1(_rb(_layernorm(xv[s, 0:3].astype(F32))))
        hj[s] = h
        return [h[g, :, 0:128] for g in range(3)]

    for cp in cp_q1:
        cp.wait()
    pins = sum([make_hj(s) for s in range(4)], [])
    early_proj(0, 1, {i: pins[2 * i - 4:2 * i - 2] for i in range(2, 8)}, rows=128)

    def pro_body(p, carry):
        @pl.when(p == 4)
        def _():
            for pp in range(FIRST, NP):
                for cp in group_copies(pp, pp == NP - 1):
                    cp.start()
            for cp in cp_late:
                cp.start()

        for cp in group_copies(p):
            cp.wait()
        pins = sum([make_hj(p * 4 + t) for t in range(4)], [])
        early_proj(1, p, {2: pins[0:2], 3: pins[2:4]})
        early_proj(2, p, {i: pins[4 + i:5 + i] for i in range(4)})
        early_proj(0, p + 1, {i: pins[8 + i:9 + i] for i in range(4)})
        return carry

    with jax.named_scope("prologue_loop"):
        jax.lax.fori_loop(1, NP - 1, pro_body, 0)

    for cp in cp_ffn:
        cp.start()
    for cp in group_copies(NP - 1, True) + cp_late:
        cp.wait()
    pend[0:M, :] = mem0_ref[...].astype(F32)
    todo = list(range(16, 48))

    def one_mod_col():
        j = todo.pop(0)
        mod_cols(j, j + 1)

    pins = sum([make_hj(s) for s in range(NSEG - 4, NSEG)], [])
    early_proj(1, NP - 1, {4 + 2 * i: pins[i:i + 1] for i in range(6)}, rows=64, between=one_mod_col)
    early_proj(2, NP - 1, {4 + 2 * i: pins[6 + i:7 + i] for i in range(6)}, rows=64,
               between=one_mod_col)
    assert not todo

    wr = jnp.broadcast_to(wr_ref[...].astype(F32).reshape(1, D), (8, D))

    lane8 = jax.lax.broadcasted_iota(jnp.int32, (8, 128), 1)
    sub8 = jax.lax.broadcasted_iota(jnp.int32, (8, 128), 0)
    LAST = NSEG * SEG - 1

    def post(s, g0, g1, attn):
        attn = attn.reshape(g1 - g0, 8, D)
        x1 = _rb(xv[s, g0:g1].astype(F32) + _rb(mod_vec(2) * _rb(attn)))
        n = _rb(_layernorm(x1))
        h2 = _rb(_rb(n * mod_vec(4)) + mod_vec(3))
        r = _rb(jnp.sum(h2 * wr, axis=-1, keepdims=True)) + 0.0
        x1v[s, g0:g1] = x1.astype(BF16)
        h2v[s, g0:g1] = h2.astype(BF16)
        outv[s, g0:g1] = (x1 + _rb(mod_vec(5) * h2)).astype(BF16)
        pins = []
        for g in range(g0, g1):
            bits = pltpu.bitcast(jnp.broadcast_to(r[g - g0], (8, 128)), jnp.int32)
            hi = jax.lax.shift_right_logical(bits, 16)
            code = jnp.where(bits < 0, hi ^ 0xFFFF, hi | 0x8000)
            key = (code << 11) | (LAST - (s * SEG + g * 8) - sub8) | 0x40000000
            rows = slice(g * 8, (g + 1) * 8)
            knew = jnp.where(lane8 == s, pltpu.bitcast(key, F32), keys[rows, :])
            keys[rows, :] = knew
            pins.append(knew)
        return pins

    def post_pair(a, rows):
        return post(a + 1, 0, 4, rows[0:SEG]) + post(a, 3, 4, rows[SEG:])

    zpad = jnp.zeros((48, DH), BF16)
    G = 4
    KA = (NP - G) * 2 * DH
    KS = D - 128

    def segment(s, lhs, lhs_split, extra, pins):
        probs = {}

        def stash(p, m, v):
            opnd[p, m, 0:v.shape[0], :] = v.astype(BF16)

        def qkv_group(p):
            keys = [(m, 2 * p + b) for m in range(3) for b in range(2 * G)]
            nsplit = 6 if (p == 0 and lhs_split is not None) else 0
            part = [_dot(lhs_split[0], w_head(m, h, 0, KS)) for m, h in keys[:nsplit]]
            full = [_dot(lhs_split[1], w_head(m, h, KS, D)) + part[i]
                    for i, (m, h) in enumerate(keys[:nsplit])]
            full += [_dot(lhs, w_head(m, h)) for m, h in keys[nsplit:]]
            for m in range(3):
                for t in range(G):
                    i = 2 * G * m + 2 * t
                    stash(p + t, m, jnp.concatenate([full[i], full[i + 1]], axis=0))

        def operand(p, m):
            parts = [opnd[p, m, 0:64, :], pltpu.bitcast(early[s, m * NP + p], BF16)]
            if m > 0:
                parts.append(zpad)
            return jnp.concatenate(parts, axis=0)

        def scores(p):
            sc_ = _dot_nt(operand(p, 0), operand(p, 1))
            f = fill[...]
            if pins.get(p):
                f = jnp.concatenate([f[0:8] + pltpu.bitcast(pin_zero(pins[p]), F32), f[8:]], axis=0)
            sc_ = jnp.where(f == 0.0, sc_, f)
            mx = jnp.max(sc_, axis=-1, keepdims=True)
            e = jnp.exp2((sc_ - mx) * (SCALE * LOG2E))
            stash(p, 3, e)
            probs[p] = pl.reciprocal(jnp.sum(e, axis=-1, keepdims=True), approx=True)

        oe = []

        def pv(p):
            o = _dot(opnd[p, 3], operand(p, 2)) * probs[p]
            res = []
            for b in range(2):
                rows, erows = o[32 * b:32 * b + 32], o[64 + 8 * b:72 + 8 * b]
                oe.append(erows)
                if extra is not None:
                    rows = jnp.concatenate([rows, erows, extra[2 * p + b]], axis=0)
                res.append(rows)
            pins.setdefault(p + G, []).append(o)
            return res

        os_ = []
        for p in range(0, NP, G):
            qkv_group(p)
            if p >= G:
                for t in range(G):
                    os_ += pv(p - G + t)
            for t in range(G):
                scores(p + t)
        oa = jnp.concatenate(os_, axis=1).astype(BF16)
        acc, ob = [], []
        for n in range(7):
            acc.append(_dot(oa, wblk(wo, n, 0, KA)))
            if n == 2:
                for t in range(G):
                    ob += pv(NP - G + t)
        ob = jnp.concatenate(ob, axis=1).astype(BF16)
        res = [_dot(ob, wblk(wo, n, KA, H * DH)) + acc[n] for n in range(7)]
        res.append(_dot(ob, wblk(wo, 7, KA, H * DH)) + _dot(oa, wblk(wo, 7, 0, KA)))
        return res, oe

    def make_lhs(mem, s):
        return jnp.concatenate([mem, hj[s].reshape(NJ, D)], axis=0)

    cp_o1 = pltpu.make_async_copy(outv.at[0:OUT_SPLIT], out_hbm.at[0:OUT_SPLIT], sem_out.at[0])
    cp_o2 = pltpu.make_async_copy(outv.at[OUT_SPLIT:NSEG], out_hbm.at[OUT_SPLIT:NSEG],
                                  sem_out.at[1])

    def split_lhs(lhs):
        return lhs.astype(BF16), (lhs[:, :KS].astype(BF16), lhs[:, KS:].astype(BF16))

    def step(i, carry):
        @pl.when(i == NIT - 1)
        def _():
            cp_o1.start()

        prev = pend[...]
        for u in range(UNROLL):
            a = 2 * (UNROLL * i + u)
            pins = post_pair(jnp.maximum(a - 2, 0) if u == 0 else a - 2, prev[M:])
            lhs_a = make_lhs(prev[0:M], a)
            lhs_a = (lhs_a.astype(BF16), None) if u == 0 else split_lhs(lhs_a)
            res_a, oe_a = segment(a, *lhs_a, None,
                                  {k: [v] for k, v in zip((3, 7, 11, 15), pins[:4])})
            res_a = jnp.concatenate(res_a, axis=1)
            pins = pins[4:] + post(a, 0, 3, res_a[M:])
            res_b, _ = segment(a + 1, *split_lhs(make_lhs(res_a[0:M], a + 1)), oe_a,
                               {k: [v] for k, v in zip((3, 7, 11, 15), pins)})
            prev = jnp.concatenate(res_b, axis=1)
        pend[...] = prev
        return carry

    with jax.named_scope("main_loop"):
        jax.lax.fori_loop(0, NIT, step, 0)
    post_pair(NSEG - 2, pend[M:, :])
    cp_o2.start()

    def max_all(v):
        return jnp.max(jnp.max(v, axis=0, keepdims=True), axis=1, keepdims=True)

    def decode(k):
        kb = pltpu.bitcast(jnp.broadcast_to(k, (8, 128)), jnp.int32)
        code = (kb >> 11) & 0xFFFF
        hi = jnp.where(code >= 0x8000, code & 0x7FFF, code ^ 0xFFFF)
        tok = jnp.clip((LAST - (kb & LAST))[0, 0], 0, LAST)
        return tok, pltpu.bitcast(hi << 16, F32)[:, 0:1]

    kv = keys[...]
    k1 = max_all(kv)
    k2 = max_all(jnp.where(kv == k1, 0.0, kv))
    i1, r1 = decode(k1)
    i2, r2 = decode(k2)
    g1, g2 = i1 >> 3, i2 >> 3

    def rows_of(ref):
        return jnp.concatenate([ref[g1 >> 2, pl.ds(g1 & 3, 1)], ref[g2 >> 2, pl.ds(g2 & 3, 1)]],
                               axis=0).astype(F32)

    x1, h2 = rows_of(x1v), rows_of(h2v)
    for cp in cp_ffn:
        cp.wait()
    hl = h2.reshape(16, D).astype(BF16)
    act = []
    for j in range(FF // 128):
        gt = _rb(_dot(hl, wblk(wg, j)))
        up = _rb(_dot(hl, wblk(wu, j)))
        act.append((_rb(gt * jax.nn.sigmoid(gt)) * up).astype(BF16))
    act = jnp.concatenate(act, axis=1)
    y = jnp.concatenate([_dot(act, wblk(wd, n)) for n in range(8)], axis=1).reshape(2, 8, D)
    rowi = jax.lax.broadcasted_iota(jnp.int32, (2, 8, 1), 1)
    gsel = jax.lax.broadcasted_iota(jnp.int32, (2, 8, 1), 0)
    tokp = jnp.where(gsel == 0, g1, g2) * 8 + rowi
    gate = _rb(jax.nn.sigmoid(jnp.where(tokp == i1, r1[None], r2[None])))
    upd = jnp.where((tokp == i1) | (tokp == i2), _rb(_rb(y) * gate), 0.0)
    patch[...] = (x1 + _rb(mod_vec(5) * _rb(h2 + upd))).astype(BF16)
    cp_o1.wait()
    cp_o2.wait()
    cp1 = pltpu.make_async_copy(patch.at[0], out_hbm.at[g1 >> 2, g1 & 3], sem_out.at[0])
    cp1.start()

    @pl.when(g1 != g2)
    def _():
        cp2 = pltpu.make_async_copy(patch.at[1], out_hbm.at[g2 >> 2, g2 & 3], sem_out.at[1])
        cp2.start()
        cp2.wait()

    cp1.wait()


@jax.jit
def pallas_adaLN_cond__memory_aug_recurrent_mem_tr__moe_arch_mod__prompt_kernel(
    A_x: jax.Array,
    A_mem0: jax.Array,
    A_Wq: jax.Array,
    A_Wk: jax.Array,
    A_Wv: jax.Array,
    A_Wo: jax.Array,
    A_seg_len,
    B_x: jax.Array,
    B_w_r: jax.Array,
    B_w_gate: jax.Array,
    B_w_up: jax.Array,
    B_w_down: jax.Array,
    c: jax.Array,
    w_mod: jax.Array,
):
    assert A_x.shape == (1, NSEG * SEG, D)
    any_spec = pl.BlockSpec(memory_space=pl.ANY)
    out = pl.pallas_call(
        _kernel,
        out_shape=jax.ShapeDtypeStruct((NSEG, 4, 8, D), BF16),
        in_specs=[any_spec] * 12,
        out_specs=any_spec,
        scratch_shapes=[
            pltpu.VMEM((H, D // 2, DH), U32),
            pltpu.VMEM((H, D // 2, DH), U32),
            pltpu.VMEM((H, D // 2, DH), U32),
            pltpu.VMEM((H * DH // 2, D), U32),
            pltpu.VMEM((D // 2, FF), U32),
            pltpu.VMEM((D // 2, FF), U32),
            pltpu.VMEM((FF // 2, D), U32),
            pltpu.VMEM((D // 2, 6 * D), U32),
            pltpu.VMEM((NSEG, 4, 8, D), BF16),
            pltpu.VMEM((NSEG, 4, 8, D), BF16),
            pltpu.VMEM((NSEG, 4, 8, D), BF16),
            pltpu.VMEM((NSEG, 4, 8, D), BF16),
            pltpu.VMEM((NSEG, 3 * NP, 8, DH), U32),
            pltpu.VMEM((NE, D), BF16),
            pltpu.VMEM((NSEG, 3, 8, D), F32),
            pltpu.VMEM((M + SEG + M, D), F32),
            pltpu.VMEM((8, 6 * D), F32),
            pltpu.VMEM((80, 128), F32),
            pltpu.VMEM((SEG, 128), F32),
            pltpu.VMEM((2, 8, D), BF16),
            pltpu.VMEM((8, 128), U32),
            pltpu.VMEM((NP, 4, 80, DH), BF16),
            pltpu.VMEM((3, NE, 2 * DH), F32),
            pltpu.VMEM((M, D), BF16),
            pltpu.VMEM((D,), BF16),
            pltpu.VMEM((1, D), BF16),
            pltpu.SemaphoreType.DMA((16 + NP,)),
            pltpu.SemaphoreType.DMA((2,)),
        ],
        compiler_params=pltpu.CompilerParams(vmem_limit_bytes=120 * 1024 * 1024),
    )(
        A_x.reshape(NSEG, 4, 8, D),
        A_mem0.reshape(M, D),
        A_Wq.reshape(D // 2, 2, H, DH),
        A_Wk.reshape(D // 2, 2, H, DH),
        A_Wv.reshape(D // 2, 2, H, DH),
        A_Wo.reshape(H * DH, D),
        B_w_r,
        B_w_gate,
        B_w_up,
        B_w_down,
        c,
        w_mod,
    )
    return out.reshape(1, NSEG * SEG, D)
```

```python
import jax
import jax.numpy as jnp
import jax.experimental.pallas as pl
import jax.experimental.pallas.tpu as pltpu

F32 = jnp.float32
BF16 = jnp.bfloat16
U32 = jnp.uint32

D = 1024
H = 32
DH = 128
NP = H // 2
M = 8
SEG = 32
NSEG = 64
FF = 3584
NJ = SEG - M
NE = NSEG * M
EPS = 1e-5
SCALE = DH ** (-0.5)
NEG = -1000000000.0
LOG2E = 1.4426950408889634
KQ = 256
FIRST = 7
UNROLL = 2
NIT = NSEG // (2 * UNROLL)
OUT_SPLIT = NSEG - 2 * UNROLL - 2


def _rb(x):
    return x.astype(BF16).astype(F32)


def _layernorm(xf):
    m = jnp.mean(xf, axis=-1, keepdims=True)
    d = xf - m
    v = jnp.mean(d * d, axis=-1, keepdims=True)
    return d * jax.lax.rsqrt(v + EPS)


def _dot(a, b):
    return jnp.dot(a, b, preferred_element_type=F32)


def _dot_nt(a, b):
    return jax.lax.dot_general(a, b, (((1,), (1,)), ((), ())), preferred_element_type=F32)


def _kernel(x_hbm, mem0_hbm, wq_hbm, wk_hbm, wv_hbm, wo_hbm, wr_hbm, wg_hbm, wu_hbm, wd_hbm,
            c_hbm, wm_hbm,
            out_hbm,
            wq, wk, wv, wo, wg, wu, wd, wm, xv, x1v, h2v, outv, early, he, hj, pend,
            mod, fill, keys, patch, zero, opnd, acc0, mem0_ref, wr_ref, c_ref,
            sem, sem_out):
    w_u32 = [w.bitcast(U32) for w in (wq_hbm, wk_hbm, wv_hbm)]
    wqkv = (wq, wk, wv)
    wo_hbm, wg_hbm, wu_hbm, wd_hbm, wm_hbm = [
        w.bitcast(U32) for w in (wo_hbm, wg_hbm, wu_hbm, wd_hbm, wm_hbm)]

    def wblk(w, j, lo=None, hi=None):
        rows = slice(None) if lo is None else slice(lo // 2, hi // 2)
        return pltpu.bitcast(w[rows, j * 128:(j + 1) * 128], BF16)

    def wm_copy(lo, n, k):
        return pltpu.make_async_copy(wm_hbm.at[:, pl.ds(lo, n)], wm.at[:, pl.ds(lo, n)], sem.at[k])

    def w_copies(m, p, k):
        return [pltpu.make_async_copy(w_u32[m].at[:, par, p, :], wqkv[m].at[2 * p + par], sem.at[k])
                for par in range(2)]

    def xj_copy(p, k):
        segs = pl.ds(4 * p, 4)
        return pltpu.make_async_copy(x_hbm.at[segs, 0:3], xv.at[segs, 0:3], sem.at[k])

    def group_copies(p, last=False):
        k = 16 + p
        return (w_copies(1, p, k) + w_copies(2, p, k) + ([] if last else w_copies(0, p + 1, k))
                + [xj_copy(p, k)])

    cp_c = pltpu.make_async_copy(c_hbm, c_ref, sem.at[5])
    cp_xe = pltpu.make_async_copy(x_hbm.at[:, 3], xv.at[:, 3], sem.at[0])
    cp_w0 = w_copies(0, 0, 6) + w_copies(1, 0, 6) + w_copies(2, 0, 6)
    cp_wm1 = [[wm_copy(j * KQ, KQ, 1 + j), wm_copy(D + j * KQ, KQ, 1 + j)] for j in range(D // KQ)]
    cp_q1 = w_copies(0, 1, 7) + [xj_copy(0, 7)]
    cp_late = [wm_copy(2 * D, 4 * D, 9), pltpu.make_async_copy(wo_hbm, wo, sem.at[10]),
               pltpu.make_async_copy(mem0_hbm, mem0_ref, sem.at[14]),
               pltpu.make_async_copy(wr_hbm, wr_ref, sem.at[15])]
    cp_ffn = [pltpu.make_async_copy(wg_hbm, wg, sem.at[11]),
              pltpu.make_async_copy(wu_hbm, wu, sem.at[12]),
              pltpu.make_async_copy(wd_hbm, wd, sem.at[13])]

    for cp in [cp_c, cp_xe] + cp_w0 + sum(cp_wm1, []) + cp_q1:
        cp.start()
    for p in range(1, FIRST):
        for cp in group_copies(p):
            cp.start()

    ri = jax.lax.broadcasted_iota(jnp.int32, (80, 128), 0)
    ci = jax.lax.broadcasted_iota(jnp.int32, (80, 128), 1)

    def head_of(i):
        return jnp.where(i < 64, i >> 5, (i - 64) >> 3)

    def pos_of(i):
        return jnp.where(i < 64, i & 31, 32 + (i & 7))

    same = (head_of(ri) == head_of(ci)) & (ci < 80)
    allowed = (pos_of(ri) < M) | (pos_of(ri) >= pos_of(ci))
    fill[...] = jnp.where(same, jnp.where(allowed, 0.0, NEG / SCALE), -jnp.inf).astype(F32)
    keys[...] = jnp.zeros(keys.shape, F32)
    pend[M:, :] = jnp.zeros((SEG + M, D), F32)
    zero[...] = jnp.zeros(zero.shape, U32)

    def pin_zero(vals):
        acc = None
        for v in vals:
            v = pltpu.bitcast(v, U32)
            for r in range(0, v.shape[0], 8):
                acc = v[r:r + 8] if acc is None else acc | v[r:r + 8]
        return acc & zero[...]

    cp_xe.wait()
    cp_c.wait()
    cf = c_ref[...].astype(F32)
    sc = _rb(cf * jax.nn.sigmoid(cf))
    sc = jnp.broadcast_to(sc, (16, D)).astype(BF16)

    def mod_cols(lo, hi):
        for j in range(lo, hi):
            v = _rb(_dot(sc, wblk(wm, j))[0:8])
            if j // 8 in (1, 4):
                v = _rb(1.0 + v)
            mod[:, j * 128:(j + 1) * 128] = v

    def mod_vec(k):
        return mod[:, k * D:(k + 1) * D]

    def affine1(n):
        return _rb(n * mod_vec(1)) + mod_vec(0)

    def ne_body(i, carry):
        n = _layernorm(xv[pl.ds(i * 16, 16), 3].astype(F32))
        he[pl.ds(pl.multiple_of(i * 128, 128), 128), :] = n.reshape(128, D).astype(BF16)
        return carry

    jax.lax.fori_loop(0, NSEG // 16, ne_body, 0)

    def w_head(m, h, lo=0, hi=D):
        return pltpu.bitcast(wqkv[m][h, lo // 2:hi // 2, :], BF16)

    def relayout(m, p):
        w = wqkv[m]
        e = w[2 * p]
        o = w[2 * p + 1]
        w[2 * p] = (e & U32(0xFFFF)) | (o << 16)
        w[2 * p + 1] = (e >> 16) | (o & U32(0xFFFF0000))

    def store_early(m, p, row0, r1, r2):
        ns = r1.shape[0] // 8
        r12 = jnp.concatenate([r1.reshape(ns, 8, DH), r2.reshape(ns, 8, DH)], axis=1)
        early[row0 // 8:row0 // 8 + ns, m * NP + p] = pltpu.bitcast(
            r12.reshape(16 * ns, DH).astype(BF16), U32).reshape(ns, 8, DH)

    for cp in cp_w0:
        cp.wait()
    for m in range(3):
        relayout(m, 0)
    for j in range(D // KQ):
        for cp in cp_wm1[j]:
            cp.wait()
        lo, hi = j * KQ, (j + 1) * KQ
        mod_cols(lo // 128, hi // 128)
        mod_cols((D + lo) // 128, (D + hi) // 128)
        for c in range(2):
            rows = slice(c * 256, (c + 1) * 256)
            n = he[rows, lo:hi].astype(F32).reshape(32, 8, KQ)
            h = (_rb(n * mod[:, D + lo:D + hi]) + mod[:, lo:hi]).reshape(256, KQ)
            he[rows, lo:hi] = h.astype(BF16)
            hb = h.astype(BF16)
            for m in range(3):
                w2 = jnp.concatenate([w_head(m, 0, lo, hi), w_head(m, 1, lo, hi)], axis=1)
                r = _dot(hb, w2)
                if j > 0:
                    r = r + acc0[m, rows, :]
                if hi < D:
                    acc0[m, rows, :] = r
                else:
                    store_early(m, 0, c * 256, r[:, :DH], r[:, DH:])

    def early_proj(m, p, pins=None, rows=256, between=None):
        relayout(m, p)
        for c in range(NE // rows):
            hc = he[c * rows:(c + 1) * rows, :]
            r12 = []
            for b in range(2):
                wv_ = wqkv[m][2 * p + b]
                if pins and 2 * c + b in pins:
                    wv_ = jnp.concatenate([wv_[0:8] | pin_zero(pins[2 * c + b]), wv_[8:]], axis=0)
                r12.append(_dot(hc, pltpu.bitcast(wv_, BF16)))
                if between is not None:
                    between()
            store_early(m, p, c * rows, *r12)

    def make_hj(s):
        h = affine1(_rb(_layernorm(xv[s, 0:3].astype(F32))))
        hj[s] = h
        return [h[g, :, 0:128] for g in range(3)]

    for cp in cp_q1:
        cp.wait()
    pins = sum([make_hj(s) for s in range(4)], [])
    early_proj(0, 1, {i: pins[2 * i - 4:2 * i - 2] for i in range(2, 8)}, rows=128)

    def pro_body(p, carry):
        @pl.when(p == 4)
        def _():
            for pp in range(FIRST, NP):
                for cp in group_copies(pp, pp == NP - 1):
                    cp.start()
            for cp in cp_late:
                cp.start()

        for cp in group_copies(p):
            cp.wait()
        pins = sum([make_hj(p * 4 + t) for t in range(4)], [])
        early_proj(1, p, {2: pins[0:2], 3: pins[2:4]})
        early_proj(2, p, {i: pins[4 + i:5 + i] for i in range(4)})
        early_proj(0, p + 1, {i: pins[8 + i:9 + i] for i in range(4)})
        return carry

    with jax.named_scope("prologue_loop"):
        jax.lax.fori_loop(1, NP - 1, pro_body, 0)

    for cp in cp_ffn:
        cp.start()
    for cp in group_copies(NP - 1, True) + cp_late:
        cp.wait()
    pend[0:M, :] = mem0_ref[...].astype(F32)
    todo = list(range(16, 48))

    def one_mod_col():
        j = todo.pop(0)
        mod_cols(j, j + 1)

    pins = sum([make_hj(s) for s in range(NSEG - 4, NSEG)], [])
    early_proj(1, NP - 1, {4 + 2 * i: pins[i:i + 1] for i in range(6)}, rows=64, between=one_mod_col)
    early_proj(2, NP - 1, {4 + 2 * i: pins[6 + i:7 + i] for i in range(6)}, rows=64,
               between=one_mod_col)
    assert not todo

    wr = jnp.broadcast_to(wr_ref[...].astype(F32).reshape(1, D), (8, D))

    lane8 = jax.lax.broadcasted_iota(jnp.int32, (8, 128), 1)
    sub8 = jax.lax.broadcasted_iota(jnp.int32, (8, 128), 0)
    LAST = NSEG * SEG - 1

    def post(s, g0, g1, attn, record=True):
        attn = attn.reshape(g1 - g0, 8, D)
        x1 = _rb(xv[s, g0:g1].astype(F32) + _rb(mod_vec(2) * _rb(attn)))
        n = _rb(_layernorm(x1))
        h2 = _rb(_rb(n * mod_vec(4)) + mod_vec(3))
        r = _rb(jnp.sum(h2 * wr, axis=-1, keepdims=True)) + 0.0
        x1v[s, g0:g1] = x1.astype(BF16)
        h2v[s, g0:g1] = h2.astype(BF16)
        outv[s, g0:g1] = (x1 + _rb(mod_vec(5) * h2)).astype(BF16)
        pins = []
        for g in range(g0, g1):
            bits = pltpu.bitcast(jnp.broadcast_to(r[g - g0], (8, 128)), jnp.int32)
            hi = jax.lax.shift_right_logical(bits, 16)
            code = jnp.where(bits < 0, hi ^ 0xFFFF, hi | 0x8000)
            key = (code << 11) | (LAST - (s * SEG + g * 8) - sub8) | 0x40000000
            key = pltpu.bitcast(key, F32)
            if record:
                rows = slice(g * 8, (g + 1) * 8)
                keys[rows, :] = jnp.where(lane8 == s, key, keys[rows, :])
            pins.append(key)
        return pins

    def post_pair(a, rows, record=True):
        return post(a + 1, 0, 4, rows[0:SEG], record) + post(a, 3, 4, rows[SEG:], record)

    zpad = jnp.zeros((48, DH), BF16)
    G = 4
    KA = (NP - G) * 2 * DH
    KS = D - 128

    def segment(s, lhs, lhs_split, extra, pins):
        probs = {}

        def stash(p, m, v):
            opnd[p, m, 0:v.shape[0], :] = v.astype(BF16)

        def qkv_group(p):
            keys = [(m, 2 * p + b) for m in range(3) for b in range(2 * G)]
            nsplit = 6 if (p == 0 and lhs_split is not None) else 0
            part = [_dot(lhs_split[0], w_head(m, h, 0, KS)) for m, h in keys[:nsplit]]
            full = [_dot(lhs_split[1], w_head(m, h, KS, D)) + part[i]
                    for i, (m, h) in enumerate(keys[:nsplit])]
            full += [_dot(lhs, w_head(m, h)) for m, h in keys[nsplit:]]
            for m in range(3):
                for t in range(G):
                    i = 2 * G * m + 2 * t
                    stash(p + t, m, jnp.concatenate([full[i], full[i + 1]], axis=0))

        def operand(p, m):
            parts = [opnd[p, m, 0:64, :], pltpu.bitcast(early[s, m * NP + p], BF16)]
            if m > 0:
                parts.append(zpad)
            return jnp.concatenate(parts, axis=0)

        def scores(p):
            sc_ = _dot_nt(operand(p, 0), operand(p, 1))
            f = fill[...]
            if pins.get(p):
                f = jnp.concatenate([f[0:8] + pltpu.bitcast(pin_zero(pins[p]), F32), f[8:]], axis=0)
            sc_ = jnp.where(f == 0.0, sc_, f)
            mx = jnp.max(sc_, axis=-1, keepdims=True)
            e = jnp.exp2((sc_ - mx) * (SCALE * LOG2E))
            stash(p, 3, e)
            probs[p] = pl.reciprocal(jnp.sum(e, axis=-1, keepdims=True), approx=True)

        oe = []

        def pv(p):
            o = _dot(opnd[p, 3], operand(p, 2)) * probs[p]
            res = []
            for b in range(2):
                rows, erows = o[32 * b:32 * b + 32], o[64 + 8 * b:72 + 8 * b]
                oe.append(erows)
                if extra is not None:
                    rows = jnp.concatenate([rows, erows, extra[2 * p + b]], axis=0)
                res.append(rows)
            pins.setdefault(p + G, []).append(o)
            return res

        os_ = []
        for p in range(0, NP, G):
            qkv_group(p)
            if p >= G:
                for t in range(G):
                    os_ += pv(p - G + t)
            for t in range(G):
                scores(p + t)
        oa = jnp.concatenate(os_, axis=1).astype(BF16)
        acc, ob = [], []
        for n in range(7):
            acc.append(_dot(oa, wblk(wo, n, 0, KA)))
            if n == 2:
                for t in range(G):
                    ob += pv(NP - G + t)
        ob = jnp.concatenate(ob, axis=1).astype(BF16)
        res = [_dot(ob, wblk(wo, n, KA, H * DH)) + acc[n] for n in range(7)]
        res.append(_dot(ob, wblk(wo, 7, KA, H * DH)) + _dot(oa, wblk(wo, 7, 0, KA)))
        return res, oe

    def make_lhs(mem, s):
        return jnp.concatenate([mem, hj[s].reshape(NJ, D)], axis=0)

    cp_o1 = pltpu.make_async_copy(outv.at[0:OUT_SPLIT], out_hbm.at[0:OUT_SPLIT], sem_out.at[0])
    cp_o2 = pltpu.make_async_copy(outv.at[OUT_SPLIT:NSEG], out_hbm.at[OUT_SPLIT:NSEG],
                                  sem_out.at[1])

    def split_lhs(lhs):
        return lhs.astype(BF16), (lhs[:, :KS].astype(BF16), lhs[:, KS:].astype(BF16))

    def step(i, carry):
        @pl.when(i == NIT - 1)
        def _():
            cp_o1.start()

        prev = pend[...]
        for u in range(UNROLL):
            a = 2 * (UNROLL * i + u)
            pins = post_pair(jnp.maximum(a - 2, 0) if u == 0 else a - 2, prev[M:])
            lhs_a = make_lhs(prev[0:M], a)
            lhs_a = (lhs_a.astype(BF16), None) if u == 0 else split_lhs(lhs_a)
            res_a, oe_a = segment(a, *lhs_a, None,
                                  {k: [v] for k, v in zip((3, 7, 11, 15), pins[:4])})
            res_a = jnp.concatenate(res_a, axis=1)
            pins = pins[4:] + post(a, 0, 3, res_a[M:])
            res_b, _ = segment(a + 1, *split_lhs(make_lhs(res_a[0:M], a + 1)), oe_a,
                               {k: [v] for k, v in zip((3, 7, 11, 15), pins)})
            prev = jnp.concatenate(res_b, axis=1)
        pend[...] = prev
        return carry

    with jax.named_scope("main_loop"):
        jax.lax.fori_loop(0, NIT, step, 0)
    for cp in cp_ffn:
        cp.wait()
    last_keys = post_pair(NSEG - 2, pend[M:, :], record=False)
    cp_o2.start()

    def max_all(v):
        return jnp.max(jnp.max(v, axis=0, keepdims=True), axis=1, keepdims=True)

    def decode(k):
        kb = pltpu.bitcast(jnp.broadcast_to(k, (8, 128)), jnp.int32)
        code = (kb >> 11) & 0xFFFF
        hi = jnp.where(code >= 0x8000, code & 0x7FFF, code ^ 0xFFFF)
        tok = jnp.clip((LAST - (kb & LAST))[0, 0], 0, LAST)
        return tok, pltpu.bitcast(hi << 16, F32)[:, 0:1]

    kv = keys[...]
    o1 = max_all(kv)
    o2 = max_all(jnp.where(kv == o1, 0.0, kv))
    kv = jnp.concatenate(last_keys + [jnp.where(sub8 < 4, o1, o2)], axis=0)
    k1 = jnp.max(kv, axis=0, keepdims=True)
    k2 = jnp.max(jnp.where(kv == k1, 0.0, kv), axis=0, keepdims=True)
    i1, r1 = decode(k1)
    i2, r2 = decode(k2)
    g1, g2 = i1 >> 3, i2 >> 3

    def rows_of(ref):
        return jnp.concatenate([ref[g1 >> 2, pl.ds(g1 & 3, 1)], ref[g2 >> 2, pl.ds(g2 & 3, 1)]],
                               axis=0).astype(F32)

    x1, h2 = rows_of(x1v), rows_of(h2v)
    hl = h2.reshape(16, D).astype(BF16)
    act = []
    for j in range(FF // 128):
        gt = _rb(_dot(hl, wblk(wg, j)))
        up = _rb(_dot(hl, wblk(wu, j)))
        act.append((_rb(gt * jax.nn.sigmoid(gt)) * up).astype(BF16))
    act = jnp.concatenate(act, axis=1)
    y = jnp.concatenate([_dot(act, wblk(wd, n)) for n in range(8)], axis=1).reshape(2, 8, D)
    rowi = jax.lax.broadcasted_iota(jnp.int32, (2, 8, 1), 1)
    gsel = jax.lax.broadcasted_iota(jnp.int32, (2, 8, 1), 0)
    tokp = jnp.where(gsel == 0, g1, g2) * 8 + rowi
    gate = _rb(jax.nn.sigmoid(jnp.where(tokp == i1, r1[None], r2[None])))
    upd = jnp.where((tokp == i1) | (tokp == i2), _rb(_rb(y) * gate), 0.0)
    patch[...] = (x1 + _rb(mod_vec(5) * _rb(h2 + upd))).astype(BF16)
    cp_o1.wait()
    cp_o2.wait()
    cp1 = pltpu.make_async_copy(patch.at[0], out_hbm.at[g1 >> 2, g1 & 3], sem_out.at[0])
    cp1.start()

    @pl.when(g1 != g2)
    def _():
        cp2 = pltpu.make_async_copy(patch.at[1], out_hbm.at[g2 >> 2, g2 & 3], sem_out.at[1])
        cp2.start()
        cp2.wait()

    cp1.wait()


@jax.jit
def pallas_adaLN_cond__memory_aug_recurrent_mem_tr__moe_arch_mod__prompt_kernel(
    A_x: jax.Array,
    A_mem0: jax.Array,
    A_Wq: jax.Array,
    A_Wk: jax.Array,
    A_Wv: jax.Array,
    A_Wo: jax.Array,
    A_seg_len,
    B_x: jax.Array,
    B_w_r: jax.Array,
    B_w_gate: jax.Array,
    B_w_up: jax.Array,
    B_w_down: jax.Array,
    c: jax.Array,
    w_mod: jax.Array,
):
    assert A_x.shape == (1, NSEG * SEG, D)
    any_spec = pl.BlockSpec(memory_space=pl.ANY)
    out = pl.pallas_call(
        _kernel,
        out_shape=jax.ShapeDtypeStruct((NSEG, 4, 8, D), BF16),
        in_specs=[any_spec] * 12,
        out_specs=any_spec,
        scratch_shapes=[
            pltpu.VMEM((H, D // 2, DH), U32),
            pltpu.VMEM((H, D // 2, DH), U32),
            pltpu.VMEM((H, D // 2, DH), U32),
            pltpu.VMEM((H * DH // 2, D), U32),
            pltpu.VMEM((D // 2, FF), U32),
            pltpu.VMEM((D // 2, FF), U32),
            pltpu.VMEM((FF // 2, D), U32),
            pltpu.VMEM((D // 2, 6 * D), U32),
            pltpu.VMEM((NSEG, 4, 8, D), BF16),
            pltpu.VMEM((NSEG, 4, 8, D), BF16),
            pltpu.VMEM((NSEG, 4, 8, D), BF16),
            pltpu.VMEM((NSEG, 4, 8, D), BF16),
            pltpu.VMEM((NSEG, 3 * NP, 8, DH), U32),
            pltpu.VMEM((NE, D), BF16),
            pltpu.VMEM((NSEG, 3, 8, D), F32),
            pltpu.VMEM((M + SEG + M, D), F32),
            pltpu.VMEM((8, 6 * D), F32),
            pltpu.VMEM((80, 128), F32),
            pltpu.VMEM((SEG, 128), F32),
            pltpu.VMEM((2, 8, D), BF16),
            pltpu.VMEM((8, 128), U32),
            pltpu.VMEM((NP, 4, 80, DH), BF16),
            pltpu.VMEM((3, NE, 2 * DH), F32),
            pltpu.VMEM((M, D), BF16),
            pltpu.VMEM((D,), BF16),
            pltpu.VMEM((1, D), BF16),
            pltpu.SemaphoreType.DMA((16 + NP,)),
            pltpu.SemaphoreType.DMA((2,)),
        ],
        compiler_params=pltpu.CompilerParams(vmem_limit_bytes=120 * 1024 * 1024,
                                             disable_bounds_checks=True,
                                             disable_semaphore_checks=True),
    )(
        A_x.reshape(NSEG, 4, 8, D),
        A_mem0.reshape(M, D),
        A_Wq.reshape(D // 2, 2, H, DH),
        A_Wk.reshape(D // 2, 2, H, DH),
        A_Wv.reshape(D // 2, 2, H, DH),
        A_Wo.reshape(H * DH, D),
        B_w_r,
        B_w_gate,
        B_w_up,
        B_w_down,
        c,
        w_mod,
    )
    return out.reshape(1, NSEG * SEG, D)
```

```python
import jax
import jax.numpy as jnp
import jax.experimental.pallas as pl
import jax.experimental.pallas.tpu as pltpu

F32 = jnp.float32
BF16 = jnp.bfloat16
U32 = jnp.uint32

D = 1024
H = 32
DH = 128
NP = H // 2
M = 8
SEG = 32
NSEG = 64
FF = 3584
NJ = SEG - M
NE = NSEG * M
EPS = 1e-5
SCALE = DH ** (-0.5)
NEG = -1000000000.0
LOG2E = 1.4426950408889634
KQ = 256
FIRST = 7
UNROLL = 2
NIT = NSEG // (2 * UNROLL)
OUT_SPLIT = NSEG - 2 * UNROLL - 2


def _rb(x):
    return x.astype(BF16).astype(F32)


def _layernorm(xf):
    m = jnp.mean(xf, axis=-1, keepdims=True)
    d = xf - m
    v = jnp.mean(d * d, axis=-1, keepdims=True)
    return d * jax.lax.rsqrt(v + EPS)


def _dot(a, b):
    return jnp.dot(a, b, preferred_element_type=F32)


def _dot_nt(a, b):
    return jax.lax.dot_general(a, b, (((1,), (1,)), ((), ())), preferred_element_type=F32)


def _kernel(x_hbm, mem0_hbm, wq_hbm, wk_hbm, wv_hbm, wo_hbm, wr_hbm, wg_hbm, wu_hbm, wd_hbm,
            c_hbm, wm_hbm,
            out_hbm,
            wq, wk, wv, wo, wg, wu, wd, wm, xv, x1v, h2v, outv, early, he, hj, pend,
            mod, fill, keys, patch, zero, opnd, acc0, mem0_ref, wr_ref, c_ref,
            sem, sem_out):
    w_u32 = [w.bitcast(U32) for w in (wq_hbm, wk_hbm, wv_hbm)]
    wqkv = (wq, wk, wv)
    wo_hbm, wg_hbm, wu_hbm, wd_hbm, wm_hbm = [
        w.bitcast(U32) for w in (wo_hbm, wg_hbm, wu_hbm, wd_hbm, wm_hbm)]

    def wblk(w, j, lo=None, hi=None):
        rows = slice(None) if lo is None else slice(lo // 2, hi // 2)
        return pltpu.bitcast(w[rows, j * 128:(j + 1) * 128], BF16)

    def wm_copy(lo, n, k):
        return pltpu.make_async_copy(wm_hbm.at[:, pl.ds(lo, n)], wm.at[:, pl.ds(lo, n)], sem.at[k])

    def w_copies(m, p, k):
        return [pltpu.make_async_copy(w_u32[m].at[:, par, p, :], wqkv[m].at[2 * p + par], sem.at[k])
                for par in range(2)]

    def xj_copy(p, k):
        segs = pl.ds(4 * p, 4)
        return pltpu.make_async_copy(x_hbm.at[segs, 0:3], xv.at[segs, 0:3], sem.at[k])

    def group_copies(p, last=False):
        k = 16 + p
        return (w_copies(1, p, k) + w_copies(2, p, k) + ([] if last else w_copies(0, p + 1, k))
                + [xj_copy(p, k)])

    cp_c = pltpu.make_async_copy(c_hbm, c_ref, sem.at[5])
    cp_xe = pltpu.make_async_copy(x_hbm.at[:, 3], xv.at[:, 3], sem.at[0])
    cp_w0 = w_copies(0, 0, 6) + w_copies(1, 0, 6) + w_copies(2, 0, 6)
    cp_wm1 = [[wm_copy(j * KQ, KQ, 1 + j), wm_copy(D + j * KQ, KQ, 1 + j)] for j in range(D // KQ)]
    cp_q1 = w_copies(0, 1, 7) + [xj_copy(0, 7)]
    cp_late = [wm_copy(2 * D, 4 * D, 9), pltpu.make_async_copy(wo_hbm, wo.at[:, 0:D], sem.at[10]),
               pltpu.make_async_copy(mem0_hbm, mem0_ref, sem.at[14]),
               pltpu.make_async_copy(wr_hbm, wr_ref, sem.at[15])]
    cp_ffn = [pltpu.make_async_copy(wg_hbm, wg.at[:, 0:FF], sem.at[11]),
              pltpu.make_async_copy(wu_hbm, wu.at[:, 0:FF], sem.at[12]),
              pltpu.make_async_copy(wd_hbm, wd.at[:, 0:D], sem.at[13])]

    for cp in [cp_c, cp_xe] + cp_w0 + sum(cp_wm1, []) + cp_q1:
        cp.start()
    for p in range(1, FIRST):
        for cp in group_copies(p):
            cp.start()

    ri = jax.lax.broadcasted_iota(jnp.int32, (80, 128), 0)
    ci = jax.lax.broadcasted_iota(jnp.int32, (80, 128), 1)

    def head_of(i):
        return jnp.where(i < 64, i >> 5, (i - 64) >> 3)

    def pos_of(i):
        return jnp.where(i < 64, i & 31, 32 + (i & 7))

    same = (head_of(ri) == head_of(ci)) & (ci < 80)
    allowed = (pos_of(ri) < M) | (pos_of(ri) >= pos_of(ci))
    fill[...] = jnp.where(same, jnp.where(allowed, 0.0, NEG / SCALE), -jnp.inf).astype(F32)
    keys[...] = jnp.zeros(keys.shape, F32)
    pend[M:, :] = jnp.zeros((SEG + M, D), F32)
    zero[...] = jnp.zeros(zero.shape, U32)

    def pin_zero(vals):
        acc = None
        for v in vals:
            v = pltpu.bitcast(v, U32)
            for r in range(0, v.shape[0], 8):
                acc = v[r:r + 8] if acc is None else acc | v[r:r + 8]
        return acc & zero[...]

    cp_xe.wait()
    cp_c.wait()
    cf = c_ref[...].astype(F32)
    sc = _rb(cf * jax.nn.sigmoid(cf))
    sc = jnp.broadcast_to(sc, (16, D)).astype(BF16)

    def mod_cols(lo, hi):
        for j in range(lo, hi):
            v = _rb(_dot(sc, wblk(wm, j))[0:8])
            if j // 8 in (1, 4):
                v = _rb(1.0 + v)
            mod[:, j * 128:(j + 1) * 128] = v

    def mod_vec(k):
        return mod[:, k * D:(k + 1) * D]

    def affine1(n):
        return _rb(n * mod_vec(1)) + mod_vec(0)

    def ne_body(i, carry):
        n = _layernorm(xv[pl.ds(i * 16, 16), 3].astype(F32))
        he[pl.ds(pl.multiple_of(i * 128, 128), 128), :] = n.reshape(128, D).astype(BF16)
        return carry

    jax.lax.fori_loop(0, NSEG // 16, ne_body, 0)

    def w_head(m, h, lo=0, hi=D):
        return pltpu.bitcast(wqkv[m][h, lo // 2:hi // 2, :], BF16)

    def relayout(m, p):
        w = wqkv[m]
        e = w[2 * p]
        o = w[2 * p + 1]
        w[2 * p] = (e & U32(0xFFFF)) | (o << 16)
        w[2 * p + 1] = (e >> 16) | (o & U32(0xFFFF0000))

    def store_early(m, p, row0, r1, r2):
        ns = r1.shape[0] // 8
        r12 = jnp.concatenate([r1.reshape(ns, 8, DH), r2.reshape(ns, 8, DH)], axis=1)
        early[row0 // 8:row0 // 8 + ns, m * NP + p] = pltpu.bitcast(
            r12.reshape(16 * ns, DH).astype(BF16), U32).reshape(ns, 8, DH)

    for cp in cp_w0:
        cp.wait()
    for m in range(3):
        relayout(m, 0)
    for j in range(D // KQ):
        for cp in cp_wm1[j]:
            cp.wait()
        lo, hi = j * KQ, (j + 1) * KQ
        mod_cols(lo // 128, hi // 128)
        mod_cols((D + lo) // 128, (D + hi) // 128)
        for c in range(2):
            rows = slice(c * 256, (c + 1) * 256)
            n = he[rows, lo:hi].astype(F32).reshape(32, 8, KQ)
            h = (_rb(n * mod[:, D + lo:D + hi]) + mod[:, lo:hi]).reshape(256, KQ)
            he[rows, lo:hi] = h.astype(BF16)
            hb = h.astype(BF16)
            for m in range(3):
                w2 = jnp.concatenate([w_head(m, 0, lo, hi), w_head(m, 1, lo, hi)], axis=1)
                r = _dot(hb, w2)
                if j > 0:
                    r = r + acc0[m, rows, :]
                if hi < D:
                    acc0[m, rows, :] = r
                else:
                    store_early(m, 0, c * 256, r[:, :DH], r[:, DH:])

    def early_proj(m, p, pins=None, rows=256, between=None):
        relayout(m, p)
        for c in range(NE // rows):
            hc = he[c * rows:(c + 1) * rows, :]
            r12 = []
            for b in range(2):
                wv_ = wqkv[m][2 * p + b]
                if pins and 2 * c + b in pins:
                    wv_ = jnp.concatenate([wv_[0:8] | pin_zero(pins[2 * c + b]), wv_[8:]], axis=0)
                r12.append(_dot(hc, pltpu.bitcast(wv_, BF16)))
                if between is not None:
                    between()
            store_early(m, p, c * rows, *r12)

    def make_hj(s):
        h = affine1(_rb(_layernorm(xv[s, 0:3].astype(F32))))
        hj[s] = h
        return [h[g, :, 0:128] for g in range(3)]

    for cp in cp_q1:
        cp.wait()
    pins = sum([make_hj(s) for s in range(4)], [])
    early_proj(0, 1, {i: pins[2 * i - 4:2 * i - 2] for i in range(2, 8)}, rows=128)

    def pro_body(p, carry):
        @pl.when(p == 4)
        def _():
            for pp in range(FIRST, NP):
                for cp in group_copies(pp, pp == NP - 1):
                    cp.start()
            for cp in cp_late:
                cp.start()

        for cp in group_copies(p):
            cp.wait()
        pins = sum([make_hj(p * 4 + t) for t in range(4)], [])
        early_proj(1, p, {2: pins[0:2], 3: pins[2:4]})
        early_proj(2, p, {i: pins[4 + i:5 + i] for i in range(4)})
        early_proj(0, p + 1, {i: pins[8 + i:9 + i] for i in range(4)})
        return carry

    with jax.named_scope("prologue_loop"):
        jax.lax.fori_loop(1, NP - 1, pro_body, 0)

    for cp in cp_ffn:
        cp.start()
    for cp in group_copies(NP - 1, True) + cp_late:
        cp.wait()
    pend[0:M, :] = mem0_ref[...].astype(F32)
    todo = list(range(16, 48))

    def one_mod_col():
        j = todo.pop(0)
        mod_cols(j, j + 1)

    pins = sum([make_hj(s) for s in range(NSEG - 4, NSEG)], [])
    early_proj(1, NP - 1, {4 + 2 * i: pins[i:i + 1] for i in range(6)}, rows=64, between=one_mod_col)
    early_proj(2, NP - 1, {4 + 2 * i: pins[6 + i:7 + i] for i in range(6)}, rows=64,
               between=one_mod_col)
    assert not todo

    wr = jnp.broadcast_to(wr_ref[...].astype(F32).reshape(1, D), (8, D))

    lane8 = jax.lax.broadcasted_iota(jnp.int32, (8, 128), 1)
    sub8 = jax.lax.broadcasted_iota(jnp.int32, (8, 128), 0)
    LAST = NSEG * SEG - 1

    def post(s, g0, g1, attn, record=True):
        attn = attn.reshape(g1 - g0, 8, D)
        x1 = _rb(xv[s, g0:g1].astype(F32) + _rb(mod_vec(2) * _rb(attn)))
        n = _rb(_layernorm(x1))
        h2 = _rb(_rb(n * mod_vec(4)) + mod_vec(3))
        r = _rb(jnp.sum(h2 * wr, axis=-1, keepdims=True)) + 0.0
        x1v[s, g0:g1] = x1.astype(BF16)
        h2v[s, g0:g1] = h2.astype(BF16)
        outv[s, g0:g1] = (x1 + _rb(mod_vec(5) * h2)).astype(BF16)
        pins = []
        for g in range(g0, g1):
            bits = pltpu.bitcast(jnp.broadcast_to(r[g - g0], (8, 128)), jnp.int32)
            hi = jax.lax.shift_right_logical(bits, 16)
            code = jnp.where(bits < 0, hi ^ 0xFFFF, hi | 0x8000)
            key = (code << 11) | (LAST - (s * SEG + g * 8) - sub8) | 0x40000000
            key = pltpu.bitcast(key, F32)
            if record:
                rows = slice(g * 8, (g + 1) * 8)
                keys[rows, :] = jnp.where(lane8 == s, key, keys[rows, :])
            pins.append(key)
        return pins

    def post_pair(a, rows, record=True):
        return post(a + 1, 0, 4, rows[0:SEG], record) + post(a, 3, 4, rows[SEG:], record)

    zpad = jnp.zeros((48, DH), BF16)
    G = 4
    KA = (NP - G) * 2 * DH
    KS = D - 128

    def segment(s, lhs, lhs_split, extra, pins):
        probs = {}

        def stash(p, m, v):
            opnd[p, m, 0:v.shape[0], :] = v.astype(BF16)

        def qkv_group(p):
            keys = [(m, 2 * p + b) for m in range(3) for b in range(2 * G)]
            nsplit = 6 if (p == 0 and lhs_split is not None) else 0
            part = [_dot(lhs_split[0], w_head(m, h, 0, KS)) for m, h in keys[:nsplit]]
            full = [_dot(lhs_split[1], w_head(m, h, KS, D)) + part[i]
                    for i, (m, h) in enumerate(keys[:nsplit])]
            full += [_dot(lhs, w_head(m, h)) for m, h in keys[nsplit:]]
            for m in range(3):
                for t in range(G):
                    i = 2 * G * m + 2 * t
                    stash(p + t, m, jnp.concatenate([full[i], full[i + 1]], axis=0))

        def operand(p, m):
            parts = [opnd[p, m, 0:64, :], pltpu.bitcast(early[s, m * NP + p], BF16)]
            if m > 0:
                parts.append(zpad)
            return jnp.concatenate(parts, axis=0)

        def scores(p):
            sc_ = _dot_nt(operand(p, 0), operand(p, 1))
            f = fill[...]
            if pins.get(p):
                f = jnp.concatenate([f[0:8] + pltpu.bitcast(pin_zero(pins[p]), F32), f[8:]], axis=0)
            sc_ = jnp.where(f == 0.0, sc_, f)
            mx = jnp.max(sc_, axis=-1, keepdims=True)
            e = jnp.exp2((sc_ - mx) * (SCALE * LOG2E))
            stash(p, 3, e)
            probs[p] = pl.reciprocal(jnp.sum(e, axis=-1, keepdims=True), approx=True)

        oe = []

        def pv(p):
            o = _dot(opnd[p, 3], operand(p, 2)) * probs[p]
            res = []
            for b in range(2):
                rows, erows = o[32 * b:32 * b + 32], o[64 + 8 * b:72 + 8 * b]
                oe.append(erows)
                if extra is not None:
                    rows = jnp.concatenate([rows, erows, extra[2 * p + b]], axis=0)
                res.append(rows)
            pins.setdefault(p + G, []).append(o)
            return res

        os_ = []
        for p in range(0, NP, G):
            qkv_group(p)
            if p >= G:
                for t in range(G):
                    os_ += pv(p - G + t)
            for t in range(G):
                scores(p + t)
        oa = jnp.concatenate(os_, axis=1).astype(BF16)
        acc, ob = [], []
        for n in range(7):
            acc.append(_dot(oa, wblk(wo, n, 0, KA)))
            if n == 2:
                for t in range(G):
                    ob += pv(NP - G + t)
        ob = jnp.concatenate(ob, axis=1).astype(BF16)
        res = [_dot(ob, wblk(wo, n, KA, H * DH)) + acc[n] for n in range(7)]
        res.append(_dot(ob, wblk(wo, 7, KA, H * DH)) + _dot(oa, wblk(wo, 7, 0, KA)))
        return res, oe

    def make_lhs(mem, s):
        return jnp.concatenate([mem, hj[s].reshape(NJ, D)], axis=0)

    cp_o1 = pltpu.make_async_copy(outv.at[0:OUT_SPLIT], out_hbm.at[0:OUT_SPLIT], sem_out.at[0])
    cp_o2 = pltpu.make_async_copy(outv.at[OUT_SPLIT:NSEG], out_hbm.at[OUT_SPLIT:NSEG],
                                  sem_out.at[1])

    def split_lhs(lhs):
        return lhs.astype(BF16), (lhs[:, :KS].astype(BF16), lhs[:, KS:].astype(BF16))

    def step(i, carry):
        @pl.when(i == NIT - 1)
        def _():
            cp_o1.start()

        prev = pend[...]
        for u in range(UNROLL):
            a = 2 * (UNROLL * i + u)
            pins = post_pair(jnp.maximum(a - 2, 0) if u == 0 else a - 2, prev[M:])
            lhs_a = make_lhs(prev[0:M], a)
            lhs_a = (lhs_a.astype(BF16), None) if u == 0 else split_lhs(lhs_a)
            res_a, oe_a = segment(a, *lhs_a, None,
                                  {k: [v] for k, v in zip((3, 7, 11, 15), pins[:4])})
            res_a = jnp.concatenate(res_a, axis=1)
            pins = pins[4:] + post(a, 0, 3, res_a[M:])
            res_b, _ = segment(a + 1, *split_lhs(make_lhs(res_a[0:M], a + 1)), oe_a,
                               {k: [v] for k, v in zip((3, 7, 11, 15), pins)})
            prev = jnp.concatenate(res_b, axis=1)
        pend[...] = prev
        return carry

    with jax.named_scope("main_loop"):
        jax.lax.fori_loop(0, NIT, step, 0)
    for cp in cp_ffn:
        cp.wait()
    last_keys = post_pair(NSEG - 2, pend[M:, :], record=False)
    cp_o2.start()

    def max_all(v):
        return jnp.max(jnp.max(v, axis=0, keepdims=True), axis=1, keepdims=True)

    def decode(k):
        kb = pltpu.bitcast(jnp.broadcast_to(k, (8, 128)), jnp.int32)
        code = (kb >> 11) & 0xFFFF
        hi = jnp.where(code >= 0x8000, code & 0x7FFF, code ^ 0xFFFF)
        tok = jnp.clip((LAST - (kb & LAST))[0, 0], 0, LAST)
        return tok, pltpu.bitcast(hi << 16, F32)[:, 0:1]

    kv = keys[...]
    o1 = max_all(kv)
    o2 = max_all(jnp.where(kv == o1, 0.0, kv))
    kv = jnp.concatenate(last_keys + [jnp.where(sub8 < 4, o1, o2)], axis=0)
    k1 = jnp.max(kv, axis=0, keepdims=True)
    k2 = jnp.max(jnp.where(kv == k1, 0.0, kv), axis=0, keepdims=True)
    i1, r1 = decode(k1)
    i2, r2 = decode(k2)
    g1, g2 = i1 >> 3, i2 >> 3

    def rows_of(ref):
        return jnp.concatenate([ref[g1 >> 2, pl.ds(g1 & 3, 1)], ref[g2 >> 2, pl.ds(g2 & 3, 1)]],
                               axis=0).astype(F32)

    x1, h2 = rows_of(x1v), rows_of(h2v)
    hl = h2.reshape(16, D).astype(BF16)
    act = []
    for j in range(FF // 128):
        gt = _rb(_dot(hl, wblk(wg, j)))
        up = _rb(_dot(hl, wblk(wu, j)))
        act.append((_rb(gt * jax.nn.sigmoid(gt)) * up).astype(BF16))
    act = jnp.concatenate(act, axis=1)
    y = jnp.concatenate([_dot(act, wblk(wd, n)) for n in range(8)], axis=1).reshape(2, 8, D)
    rowi = jax.lax.broadcasted_iota(jnp.int32, (2, 8, 1), 1)
    gsel = jax.lax.broadcasted_iota(jnp.int32, (2, 8, 1), 0)
    tokp = jnp.where(gsel == 0, g1, g2) * 8 + rowi
    gate = _rb(jax.nn.sigmoid(jnp.where(tokp == i1, r1[None], r2[None])))
    upd = jnp.where((tokp == i1) | (tokp == i2), _rb(_rb(y) * gate), 0.0)
    patch[...] = (x1 + _rb(mod_vec(5) * _rb(h2 + upd))).astype(BF16)
    cp_o1.wait()
    cp_o2.wait()
    cp1 = pltpu.make_async_copy(patch.at[0], out_hbm.at[g1 >> 2, g1 & 3], sem_out.at[0])
    cp1.start()

    @pl.when(g1 != g2)
    def _():
        cp2 = pltpu.make_async_copy(patch.at[1], out_hbm.at[g2 >> 2, g2 & 3], sem_out.at[1])
        cp2.start()
        cp2.wait()

    cp1.wait()


@jax.jit
def pallas_adaLN_cond__memory_aug_recurrent_mem_tr__moe_arch_mod__prompt_kernel(
    A_x: jax.Array,
    A_mem0: jax.Array,
    A_Wq: jax.Array,
    A_Wk: jax.Array,
    A_Wv: jax.Array,
    A_Wo: jax.Array,
    A_seg_len,
    B_x: jax.Array,
    B_w_r: jax.Array,
    B_w_gate: jax.Array,
    B_w_up: jax.Array,
    B_w_down: jax.Array,
    c: jax.Array,
    w_mod: jax.Array,
):
    assert A_x.shape == (1, NSEG * SEG, D)
    any_spec = pl.BlockSpec(memory_space=pl.ANY)
    out = pl.pallas_call(
        _kernel,
        out_shape=jax.ShapeDtypeStruct((NSEG, 4, 8, D), BF16),
        in_specs=[any_spec] * 12,
        out_specs=any_spec,
        scratch_shapes=[
            pltpu.VMEM((H, D // 2, DH), U32),
            pltpu.VMEM((H, D // 2, DH), U32),
            pltpu.VMEM((H, D // 2, DH), U32),
            pltpu.VMEM((H * DH // 2, D + 128), U32),
            pltpu.VMEM((D // 2, FF + 128), U32),
            pltpu.VMEM((D // 2, FF + 128), U32),
            pltpu.VMEM((FF // 2, D + 128), U32),
            pltpu.VMEM((D // 2, 6 * D + 128), U32),
            pltpu.VMEM((NSEG, 4, 8, D), BF16),
            pltpu.VMEM((NSEG, 4, 8, D), BF16),
            pltpu.VMEM((NSEG, 4, 8, D), BF16),
            pltpu.VMEM((NSEG, 4, 8, D), BF16),
            pltpu.VMEM((NSEG, 3 * NP, 8, DH), U32),
            pltpu.VMEM((NE, D), BF16),
            pltpu.VMEM((NSEG, 3, 8, D), F32),
            pltpu.VMEM((M + SEG + M, D), F32),
            pltpu.VMEM((8, 6 * D), F32),
            pltpu.VMEM((80, 128), F32),
            pltpu.VMEM((SEG, 128), F32),
            pltpu.VMEM((2, 8, D), BF16),
            pltpu.VMEM((8, 128), U32),
            pltpu.VMEM((NP, 4, 80, DH), BF16),
            pltpu.VMEM((3, NE, 2 * DH), F32),
            pltpu.VMEM((M, D), BF16),
            pltpu.VMEM((D,), BF16),
            pltpu.VMEM((1, D), BF16),
            pltpu.SemaphoreType.DMA((16 + NP,)),
            pltpu.SemaphoreType.DMA((2,)),
        ],
        compiler_params=pltpu.CompilerParams(vmem_limit_bytes=120 * 1024 * 1024,
                                             disable_bounds_checks=True,
                                             disable_semaphore_checks=True),
    )(
        A_x.reshape(NSEG, 4, 8, D),
        A_mem0.reshape(M, D),
        A_Wq.reshape(D // 2, 2, H, DH),
        A_Wk.reshape(D // 2, 2, H, DH),
        A_Wv.reshape(D // 2, 2, H, DH),
        A_Wo.reshape(H * DH, D),
        B_w_r,
        B_w_gate,
        B_w_up,
        B_w_down,
        c,
        w_mod,
    )
    return out.reshape(1, NSEG * SEG, D)
```

```python
import jax
import jax.numpy as jnp
import jax.experimental.pallas as pl
import jax.experimental.pallas.tpu as pltpu

F32 = jnp.float32
BF16 = jnp.bfloat16
U32 = jnp.uint32

D = 1024
H = 32
DH = 128
NP = H // 2
M = 8
SEG = 32
NSEG = 64
FF = 3584
NJ = SEG - M
NE = NSEG * M
EPS = 1e-5
SCALE = DH ** (-0.5)
NEG = -1000000000.0
LOG2E = 1.4426950408889634
KQ = 256
FIRST = 7
UNROLL = 2
NIT = NSEG // (2 * UNROLL)
OUT_SPLIT = NSEG - 2 * UNROLL - 2


def _rb(x):
    return x.astype(BF16).astype(F32)


def _layernorm(xf):
    m = jnp.mean(xf, axis=-1, keepdims=True)
    d = xf - m
    v = jnp.mean(d * d, axis=-1, keepdims=True)
    return d * jax.lax.rsqrt(v + EPS)


def _dot(a, b):
    return jnp.dot(a, b, preferred_element_type=F32)


def _dot_nt(a, b):
    return jax.lax.dot_general(a, b, (((1,), (1,)), ((), ())), preferred_element_type=F32)


def _kernel(x_hbm, mem0_hbm, wq_hbm, wk_hbm, wv_hbm, wo_hbm, wr_hbm, wg_hbm, wu_hbm, wd_hbm,
            c_hbm, wm_hbm,
            out_hbm,
            wq, wk, wv, wo, wg, wu, wd, wm, xv, x1v, h2v, outv, early, he, hj, pend,
            mod, fill, keys, patch, zero, opnd, acc0, mem0_ref, wr_ref, c_ref,
            sem, sem_out):
    w_u32 = [w.bitcast(U32) for w in (wq_hbm, wk_hbm, wv_hbm)]
    wqkv = (wq, wk, wv)
    wo_hbm, wg_hbm, wu_hbm, wd_hbm, wm_hbm = [
        w.bitcast(U32) for w in (wo_hbm, wg_hbm, wu_hbm, wd_hbm, wm_hbm)]

    def wblk(w, j, lo=None, hi=None):
        rows = slice(None) if lo is None else slice(lo // 2, hi // 2)
        return pltpu.bitcast(w[rows, j * 128:(j + 1) * 128], BF16)

    def wm_copy(lo, n, k):
        return pltpu.make_async_copy(wm_hbm.at[:, pl.ds(lo, n)], wm.at[:, pl.ds(lo, n)], sem.at[k])

    def w_copies(m, p, k):
        return [pltpu.make_async_copy(w_u32[m].at[:, par, p, :], wqkv[m].at[2 * p + par], sem.at[k])
                for par in range(2)]

    def xj_copy(p, k):
        segs = pl.ds(4 * p, 4)
        return pltpu.make_async_copy(x_hbm.at[segs, 0:3], xv.at[segs, 0:3], sem.at[k])

    def group_copies(p, last=False):
        k = 16 + p
        return (w_copies(1, p, k) + w_copies(2, p, k) + ([] if last else w_copies(0, p + 1, k))
                + [xj_copy(p, k)])

    cp_c = pltpu.make_async_copy(c_hbm, c_ref, sem.at[5])
    cp_xe = pltpu.make_async_copy(x_hbm.at[:, 3], xv.at[:, 3], sem.at[0])
    cp_w0 = w_copies(0, 0, 6) + w_copies(1, 0, 6) + w_copies(2, 0, 6)
    cp_wm1 = [[wm_copy(j * KQ, KQ, 1 + j), wm_copy(D + j * KQ, KQ, 1 + j)] for j in range(D // KQ)]
    cp_q1 = w_copies(0, 1, 7) + [xj_copy(0, 7)]
    cp_late = [wm_copy(2 * D, 4 * D, 9), pltpu.make_async_copy(wo_hbm, wo.at[:, 0:D], sem.at[10]),
               pltpu.make_async_copy(mem0_hbm, mem0_ref, sem.at[14]),
               pltpu.make_async_copy(wr_hbm, wr_ref, sem.at[15])]
    cp_ffn = [pltpu.make_async_copy(wg_hbm, wg.at[:, 0:FF], sem.at[11]),
              pltpu.make_async_copy(wu_hbm, wu.at[:, 0:FF], sem.at[12]),
              pltpu.make_async_copy(wd_hbm, wd.at[:, 0:D], sem.at[13])]

    for cp in [cp_c, cp_xe] + cp_w0 + sum(cp_wm1, []) + cp_q1:
        cp.start()
    for p in range(1, FIRST):
        for cp in group_copies(p):
            cp.start()

    ri = jax.lax.broadcasted_iota(jnp.int32, (80, 128), 0)
    ci = jax.lax.broadcasted_iota(jnp.int32, (80, 128), 1)

    def head_of(i):
        return jnp.where(i < 64, i >> 5, (i - 64) >> 3)

    def pos_of(i):
        return jnp.where(i < 64, i & 31, 32 + (i & 7))

    same = (head_of(ri) == head_of(ci)) & (ci < 80)
    allowed = (pos_of(ri) < M) | (pos_of(ri) >= pos_of(ci))
    fill[...] = jnp.where(same, jnp.where(allowed, 0.0, NEG / SCALE), -jnp.inf).astype(F32)
    keys[...] = jnp.zeros(keys.shape, F32)
    pend[M:, :] = jnp.zeros((SEG + M, D), F32)
    zero[...] = jnp.zeros(zero.shape, U32)

    def pin_zero(vals):
        acc = None
        for v in vals:
            v = pltpu.bitcast(v, U32)
            for r in range(0, v.shape[0], 8):
                acc = v[r:r + 8] if acc is None else acc | v[r:r + 8]
        return acc & zero[...]

    cp_xe.wait()
    cp_c.wait()
    cf = c_ref[...].astype(F32)
    sc = _rb(cf * jax.nn.sigmoid(cf))
    sc = jnp.broadcast_to(sc, (16, D)).astype(BF16)

    def mod_cols(lo, hi):
        for j in range(lo, hi):
            v = _rb(_dot(sc, wblk(wm, j))[0:8])
            if j // 8 in (1, 4):
                v = _rb(1.0 + v)
            mod[:, j * 128:(j + 1) * 128] = v

    def mod_vec(k):
        return mod[:, k * D:(k + 1) * D]

    def affine1(n):
        return _rb(n * mod_vec(1)) + mod_vec(0)

    def ne_body(i, carry):
        n = _layernorm(xv[pl.ds(i * 16, 16), 3].astype(F32))
        he[pl.ds(pl.multiple_of(i * 128, 128), 128), :] = n.reshape(128, D).astype(BF16)
        return carry

    jax.lax.fori_loop(0, NSEG // 16, ne_body, 0)

    def w_head(m, h, lo=0, hi=D):
        return pltpu.bitcast(wqkv[m][h, lo // 2:hi // 2, :], BF16)

    def relayout(m, p):
        w = wqkv[m]
        e = w[2 * p]
        o = w[2 * p + 1]
        w[2 * p] = (e & U32(0xFFFF)) | (o << 16)
        w[2 * p + 1] = (e >> 16) | (o & U32(0xFFFF0000))

    def store_early(m, p, row0, r1, r2):
        ns = r1.shape[0] // 8
        r12 = jnp.concatenate([r1.reshape(ns, 8, DH), r2.reshape(ns, 8, DH)], axis=1)
        early[row0 // 8:row0 // 8 + ns, m * NP + p] = pltpu.bitcast(
            r12.reshape(16 * ns, DH).astype(BF16), U32).reshape(ns, 8, DH)

    for cp in cp_w0:
        cp.wait()
    for m in range(3):
        relayout(m, 0)
    for j in range(D // KQ):
        for cp in cp_wm1[j]:
            cp.wait()
        lo, hi = j * KQ, (j + 1) * KQ
        mod_cols(lo // 128, hi // 128)
        mod_cols((D + lo) // 128, (D + hi) // 128)
        for c in range(2):
            rows = slice(c * 256, (c + 1) * 256)
            n = he[rows, lo:hi].astype(F32).reshape(32, 8, KQ)
            h = (_rb(n * mod[:, D + lo:D + hi]) + mod[:, lo:hi]).reshape(256, KQ)
            he[rows, lo:hi] = h.astype(BF16)
            hb = h.astype(BF16)
            for m in range(3):
                w2 = jnp.concatenate([w_head(m, 0, lo, hi), w_head(m, 1, lo, hi)], axis=1)
                r = _dot(hb, w2)
                if j > 0:
                    r = r + acc0[m, rows, :]
                if hi < D:
                    acc0[m, rows, :] = r
                else:
                    store_early(m, 0, c * 256, r[:, :DH], r[:, DH:])

    def early_proj(m, p, pins=None, rows=256, between=None):
        relayout(m, p)
        for c in range(NE // rows):
            hc = he[c * rows:(c + 1) * rows, :]
            r12 = []
            for b in range(2):
                wv_ = wqkv[m][2 * p + b]
                if pins and 2 * c + b in pins:
                    wv_ = jnp.concatenate([wv_[0:8] | pin_zero(pins[2 * c + b]), wv_[8:]], axis=0)
                r12.append(_dot(hc, pltpu.bitcast(wv_, BF16)))
                if between is not None:
                    between()
            store_early(m, p, c * rows, *r12)

    def make_hj(s):
        h = affine1(_rb(_layernorm(xv[s, 0:3].astype(F32))))
        hj[s] = h
        return [h[g, :, 0:128] for g in range(3)]

    for cp in cp_q1:
        cp.wait()
    pins = sum([make_hj(s) for s in range(4)], [])
    early_proj(0, 1, {i: pins[2 * i - 4:2 * i - 2] for i in range(2, 8)}, rows=128)

    def pro_body(p, carry):
        @pl.when(p == 4)
        def _():
            for pp in range(FIRST, NP):
                for cp in group_copies(pp, pp == NP - 1):
                    cp.start()
            for cp in cp_late:
                cp.start()

        for cp in group_copies(p):
            cp.wait()
        pins = sum([make_hj(p * 4 + t) for t in range(4)], [])
        early_proj(1, p, {2: pins[0:2], 3: pins[2:4]})
        early_proj(2, p, {i: pins[4 + i:5 + i] for i in range(4)})
        early_proj(0, p + 1, {i: pins[8 + i:9 + i] for i in range(4)})
        return carry

    with jax.named_scope("prologue_loop"):
        jax.lax.fori_loop(1, NP - 1, pro_body, 0)

    for cp in cp_ffn:
        cp.start()
    for cp in group_copies(NP - 1, True) + cp_late:
        cp.wait()
    pend[0:M, :] = mem0_ref[...].astype(F32)
    todo = list(range(16, 48))

    def one_mod_col():
        j = todo.pop(0)
        mod_cols(j, j + 1)

    pins = sum([make_hj(s) for s in range(NSEG - 4, NSEG)], [])
    early_proj(1, NP - 1, {4 + 2 * i: pins[i:i + 1] for i in range(6)}, rows=64, between=one_mod_col)
    early_proj(2, NP - 1, {4 + 2 * i: pins[6 + i:7 + i] for i in range(6)}, rows=64,
               between=one_mod_col)
    assert not todo

    wr = jnp.broadcast_to(wr_ref[...].astype(F32).reshape(1, D), (8, D))

    lane8 = jax.lax.broadcasted_iota(jnp.int32, (8, 128), 1)
    sub8 = jax.lax.broadcasted_iota(jnp.int32, (8, 128), 0)
    LAST = NSEG * SEG - 1

    def post(s, g0, g1, attn, record=True):
        attn = attn.reshape(g1 - g0, 8, D)
        x1 = _rb(xv[s, g0:g1].astype(F32) + _rb(mod_vec(2) * _rb(attn)))
        n = _rb(_layernorm(x1))
        h2 = _rb(_rb(n * mod_vec(4)) + mod_vec(3))
        r = _rb(jnp.sum(h2 * wr, axis=-1, keepdims=True)) + 0.0
        x1v[s, g0:g1] = x1.astype(BF16)
        h2v[s, g0:g1] = h2.astype(BF16)
        outv[s, g0:g1] = (x1 + _rb(mod_vec(5) * h2)).astype(BF16)
        pins = []
        for g in range(g0, g1):
            bits = pltpu.bitcast(jnp.broadcast_to(r[g - g0], (8, 128)), jnp.int32)
            hi = jax.lax.shift_right_logical(bits, 16)
            code = jnp.where(bits < 0, hi ^ 0xFFFF, hi | 0x8000)
            key = (code << 11) | (LAST - (s * SEG + g * 8) - sub8) | 0x40000000
            key = pltpu.bitcast(key, F32)
            if record:
                rows = slice(g * 8, (g + 1) * 8)
                keys[rows, :] = jnp.where(lane8 == s, key, keys[rows, :])
            pins.append(key)
        return pins

    def post_pair(a, rows, record=True):
        return post(a + 1, 0, 4, rows[0:SEG], record) + post(a, 3, 4, rows[SEG:], record)

    zpad = jnp.zeros((48, DH), BF16)
    G = 4
    KA = (NP - G) * 2 * DH
    KS = D - 128

    def segment(s, lhs, lhs_split, extra, pins):
        scales = {}

        def stash(p, m, v):
            opnd[p, m, 0:v.shape[0], :] = v.astype(BF16)

        def qkv_group(p):
            keys = [(m, 2 * p + b) for m in range(3) for b in range(2 * G)]
            nsplit = 6 if (p == 0 and lhs_split is not None) else 0
            part = [_dot(lhs_split[0], w_head(m, h, 0, KS)) for m, h in keys[:nsplit]]
            full = [_dot(lhs_split[1], w_head(m, h, KS, D)) + part[i]
                    for i, (m, h) in enumerate(keys[:nsplit])]
            full += [_dot(lhs, w_head(m, h)) for m, h in keys[nsplit:]]
            for m in range(3):
                for t in range(G):
                    i = 2 * G * m + 2 * t
                    stash(p + t, m, jnp.concatenate([full[i], full[i + 1]], axis=0))

        def operand(p, m):
            parts = [opnd[p, m, 0:64, :], pltpu.bitcast(early[s, m * NP + p], BF16)]
            if m > 0:
                parts.append(zpad)
            return jnp.concatenate(parts, axis=0)

        def scores(p):
            sc_ = _dot_nt(operand(p, 0), operand(p, 1))
            f = fill[...]
            if pins.get(p):
                f = jnp.concatenate([f[0:8] + pltpu.bitcast(pin_zero(pins[p]), F32), f[8:]], axis=0)
            sc_ = jnp.where(f == 0.0, sc_, f)
            mx = jnp.max(sc_, axis=-1, keepdims=True)
            e = jnp.exp2((sc_ - mx) * (SCALE * LOG2E))
            inv = pl.reciprocal(jnp.sum(e, axis=-1, keepdims=True), approx=True)
            if p // G == NP // G - 2:
                stash(p, 3, e * inv)
            else:
                stash(p, 3, e)
                scales[p] = inv

        oe = []

        def pv(p):
            o = _dot(opnd[p, 3], operand(p, 2))
            if p in scales:
                o = o * scales[p]
                pins.setdefault(p + G, []).append(o)
            res = []
            for b in range(2):
                rows, erows = o[32 * b:32 * b + 32], o[64 + 8 * b:72 + 8 * b]
                oe.append(erows)
                if extra is not None:
                    rows = jnp.concatenate([rows, erows, extra[2 * p + b]], axis=0)
                res.append(rows)
            return res

        os_ = []
        for p in range(0, NP, G):
            qkv_group(p)
            if p >= G:
                for t in range(G):
                    os_ += pv(p - G + t)
            for t in range(G):
                scores(p + t)
        oa = jnp.concatenate(os_, axis=1).astype(BF16)
        acc, ob = [], []
        for n in range(7):
            acc.append(_dot(oa, wblk(wo, n, 0, KA)))
            if n == 1:
                for t in range(G):
                    ob += pv(NP - G + t)
        ob = jnp.concatenate(ob, axis=1).astype(BF16)
        res = [_dot(ob, wblk(wo, n, KA, H * DH)) + acc[n] for n in range(7)]
        res.append(_dot(ob, wblk(wo, 7, KA, H * DH)) + _dot(oa, wblk(wo, 7, 0, KA)))
        return res, oe

    def make_lhs(mem, s):
        return jnp.concatenate([mem, hj[s].reshape(NJ, D)], axis=0)

    cp_o1 = pltpu.make_async_copy(outv.at[0:OUT_SPLIT], out_hbm.at[0:OUT_SPLIT], sem_out.at[0])
    cp_o2 = pltpu.make_async_copy(outv.at[OUT_SPLIT:NSEG], out_hbm.at[OUT_SPLIT:NSEG],
                                  sem_out.at[1])

    def split_lhs(lhs):
        return lhs.astype(BF16), (lhs[:, :KS].astype(BF16), lhs[:, KS:].astype(BF16))

    def step(i, carry):
        @pl.when(i == NIT - 1)
        def _():
            cp_o1.start()

        prev = pend[...]
        for u in range(UNROLL):
            a = 2 * (UNROLL * i + u)
            pins = post_pair(jnp.maximum(a - 2, 0) if u == 0 else a - 2, prev[M:])
            lhs_a = make_lhs(prev[0:M], a)
            lhs_a = (lhs_a.astype(BF16), None) if u == 0 else split_lhs(lhs_a)
            res_a, oe_a = segment(a, *lhs_a, None,
                                  {k: [v] for k, v in zip((3, 7, 11, 15), pins[:4])})
            res_a = jnp.concatenate(res_a, axis=1)
            pins = pins[4:] + post(a, 0, 3, res_a[M:])
            res_b, _ = segment(a + 1, *split_lhs(make_lhs(res_a[0:M], a + 1)), oe_a,
                               {k: [v] for k, v in zip((3, 7, 11, 15), pins)})
            prev = jnp.concatenate(res_b, axis=1)
        pend[...] = prev
        return carry

    with jax.named_scope("main_loop"):
        jax.lax.fori_loop(0, NIT, step, 0)
    for cp in cp_ffn:
        cp.wait()
    last_keys = post_pair(NSEG - 2, pend[M:, :], record=False)
    cp_o2.start()

    def max_all(v):
        return jnp.max(jnp.max(v, axis=0, keepdims=True), axis=1, keepdims=True)

    def decode(k):
        kb = pltpu.bitcast(jnp.broadcast_to(k, (8, 128)), jnp.int32)
        code = (kb >> 11) & 0xFFFF
        hi = jnp.where(code >= 0x8000, code & 0x7FFF, code ^ 0xFFFF)
        tok = jnp.clip((LAST - (kb & LAST))[0, 0], 0, LAST)
        return tok, pltpu.bitcast(hi << 16, F32)[:, 0:1]

    kv = keys[...]
    o1 = max_all(kv)
    o2 = max_all(jnp.where(kv == o1, 0.0, kv))
    kv = jnp.concatenate(last_keys + [jnp.where(sub8 < 4, o1, o2)], axis=0)
    k1 = jnp.max(kv, axis=0, keepdims=True)
    k2 = jnp.max(jnp.where(kv == k1, 0.0, kv), axis=0, keepdims=True)
    i1, r1 = decode(k1)
    i2, r2 = decode(k2)
    g1, g2 = i1 >> 3, i2 >> 3

    def rows_of(ref):
        return jnp.concatenate([ref[g1 >> 2, pl.ds(g1 & 3, 1)], ref[g2 >> 2, pl.ds(g2 & 3, 1)]],
                               axis=0).astype(F32)

    x1, h2 = rows_of(x1v), rows_of(h2v)
    hl = h2.reshape(16, D).astype(BF16)
    act = []
    for j in range(FF // 128):
        gt = _rb(_dot(hl, wblk(wg, j)))
        up = _rb(_dot(hl, wblk(wu, j)))
        act.append((_rb(gt * jax.nn.sigmoid(gt)) * up).astype(BF16))
    act = jnp.concatenate(act, axis=1)
    y = jnp.concatenate([_dot(act, wblk(wd, n)) for n in range(8)], axis=1).reshape(2, 8, D)
    rowi = jax.lax.broadcasted_iota(jnp.int32, (2, 8, 1), 1)
    gsel = jax.lax.broadcasted_iota(jnp.int32, (2, 8, 1), 0)
    tokp = jnp.where(gsel == 0, g1, g2) * 8 + rowi
    gate = _rb(jax.nn.sigmoid(jnp.where(tokp == i1, r1[None], r2[None])))
    upd = jnp.where((tokp == i1) | (tokp == i2), _rb(_rb(y) * gate), 0.0)
    patch[...] = (x1 + _rb(mod_vec(5) * _rb(h2 + upd))).astype(BF16)
    cp_o1.wait()
    cp_o2.wait()
    cp1 = pltpu.make_async_copy(patch.at[0], out_hbm.at[g1 >> 2, g1 & 3], sem_out.at[0])
    cp1.start()

    @pl.when(g1 != g2)
    def _():
        cp2 = pltpu.make_async_copy(patch.at[1], out_hbm.at[g2 >> 2, g2 & 3], sem_out.at[1])
        cp2.start()
        cp2.wait()

    cp1.wait()


@jax.jit
def pallas_adaLN_cond__memory_aug_recurrent_mem_tr__moe_arch_mod__prompt_kernel(
    A_x: jax.Array,
    A_mem0: jax.Array,
    A_Wq: jax.Array,
    A_Wk: jax.Array,
    A_Wv: jax.Array,
    A_Wo: jax.Array,
    A_seg_len,
    B_x: jax.Array,
    B_w_r: jax.Array,
    B_w_gate: jax.Array,
    B_w_up: jax.Array,
    B_w_down: jax.Array,
    c: jax.Array,
    w_mod: jax.Array,
):
    assert A_x.shape == (1, NSEG * SEG, D)
    any_spec = pl.BlockSpec(memory_space=pl.ANY)
    out = pl.pallas_call(
        _kernel,
        out_shape=jax.ShapeDtypeStruct((NSEG, 4, 8, D), BF16),
        in_specs=[any_spec] * 12,
        out_specs=any_spec,
        scratch_shapes=[
            pltpu.VMEM((H, D // 2, DH), U32),
            pltpu.VMEM((H, D // 2, DH), U32),
            pltpu.VMEM((H, D // 2, DH), U32),
            pltpu.VMEM((H * DH // 2, D + 128), U32),
            pltpu.VMEM((D // 2, FF + 128), U32),
            pltpu.VMEM((D // 2, FF + 128), U32),
            pltpu.VMEM((FF // 2, D + 128), U32),
            pltpu.VMEM((D // 2, 6 * D + 128), U32),
            pltpu.VMEM((NSEG, 4, 8, D), BF16),
            pltpu.VMEM((NSEG, 4, 8, D), BF16),
            pltpu.VMEM((NSEG, 4, 8, D), BF16),
            pltpu.VMEM((NSEG, 4, 8, D), BF16),
            pltpu.VMEM((NSEG, 3 * NP, 8, DH), U32),
            pltpu.VMEM((NE, D), BF16),
            pltpu.VMEM((NSEG, 3, 8, D), F32),
            pltpu.VMEM((M + SEG + M, D), F32),
            pltpu.VMEM((8, 6 * D), F32),
            pltpu.VMEM((80, 128), F32),
            pltpu.VMEM((SEG, 128), F32),
            pltpu.VMEM((2, 8, D), BF16),
            pltpu.VMEM((8, 128), U32),
            pltpu.VMEM((NP, 4, 80, DH), BF16),
            pltpu.VMEM((3, NE, 2 * DH), F32),
            pltpu.VMEM((M, D), BF16),
            pltpu.VMEM((D,), BF16),
            pltpu.VMEM((1, D), BF16),
            pltpu.SemaphoreType.DMA((16 + NP,)),
            pltpu.SemaphoreType.DMA((2,)),
        ],
        compiler_params=pltpu.CompilerParams(vmem_limit_bytes=120 * 1024 * 1024,
                                             disable_bounds_checks=True,
                                             disable_semaphore_checks=True),
    )(
        A_x.reshape(NSEG, 4, 8, D),
        A_mem0.reshape(M, D),
        A_Wq.reshape(D // 2, 2, H, DH),
        A_Wk.reshape(D // 2, 2, H, DH),
        A_Wv.reshape(D // 2, 2, H, DH),
        A_Wo.reshape(H * DH, D),
        B_w_r,
        B_w_gate,
        B_w_up,
        B_w_down,
        c,
        w_mod,
    )
    return out.reshape(1, NSEG * SEG, D)
```

```python
import jax
import jax.numpy as jnp
import jax.experimental.pallas as pl
import jax.experimental.pallas.tpu as pltpu

F32 = jnp.float32
BF16 = jnp.bfloat16
U32 = jnp.uint32

D = 1024
H = 32
DH = 128
NP = H // 2
M = 8
SEG = 32
NSEG = 64
FF = 3584
NJ = SEG - M
NE = NSEG * M
EPS = 1.0013580322265625e-05
SCALE = DH ** (-0.5)
NEG = -1000000000.0
LOG2E = 1.4426950408889634
KQ = 256
FIRST = 7
UNROLL = 2
NIT = NSEG // (2 * UNROLL)
OUT_SPLIT = NSEG - 2 * UNROLL - 2


def _rb(x):
    return x.astype(BF16).astype(F32)


def _layernorm(xf):
    m = jnp.mean(xf, axis=-1, keepdims=True)
    d = xf - m
    v = jnp.mean(d * d, axis=-1, keepdims=True)
    std = _rb(jnp.sqrt(_rb(_rb(v) + EPS)))
    return _rb(xf - _rb(m)) * (1.0 / std)


def _sigmoid(x):
    return _rb(1.0 / _rb(1.0 + _rb(jnp.exp(-x))))


def _dot(a, b):
    return jnp.dot(a, b, preferred_element_type=F32)


def _dot_nt(a, b):
    return jax.lax.dot_general(a, b, (((1,), (1,)), ((), ())), preferred_element_type=F32)


def _kernel(x_hbm, mem0_hbm, wq_hbm, wk_hbm, wv_hbm, wo_hbm, wr_hbm, wg_hbm, wu_hbm, wd_hbm,
            c_hbm, wm_hbm,
            out_hbm,
            wq, wk, wv, wo, wg, wu, wd, wm, xv, x1v, h2v, outv, early, he, hj, pend,
            mod, fill, keys, patch, zero, opnd, acc0, mem0_ref, wr_ref, c_ref,
            sem, sem_out):
    w_u32 = [w.bitcast(U32) for w in (wq_hbm, wk_hbm, wv_hbm)]
    wqkv = (wq, wk, wv)
    wo_hbm, wg_hbm, wu_hbm, wd_hbm, wm_hbm = [
        w.bitcast(U32) for w in (wo_hbm, wg_hbm, wu_hbm, wd_hbm, wm_hbm)]

    def wblk(w, j, lo=None, hi=None):
        rows = slice(None) if lo is None else slice(lo // 2, hi // 2)
        return pltpu.bitcast(w[rows, j * 128:(j + 1) * 128], BF16)

    def wm_copy(lo, n, k):
        return pltpu.make_async_copy(wm_hbm.at[:, pl.ds(lo, n)], wm.at[:, pl.ds(lo, n)], sem.at[k])

    def w_copies(m, p, k):
        return [pltpu.make_async_copy(w_u32[m].at[:, par, p, :], wqkv[m].at[2 * p + par], sem.at[k])
                for par in range(2)]

    def xj_copy(p, k):
        segs = pl.ds(4 * p, 4)
        return pltpu.make_async_copy(x_hbm.at[segs, 0:3], xv.at[segs, 0:3], sem.at[k])

    def group_copies(p, last=False):
        k = 16 + p
        return (w_copies(1, p, k) + w_copies(2, p, k) + ([] if last else w_copies(0, p + 1, k))
                + [xj_copy(p, k)])

    cp_c = pltpu.make_async_copy(c_hbm, c_ref, sem.at[5])
    cp_xe = pltpu.make_async_copy(x_hbm.at[:, 3], xv.at[:, 3], sem.at[0])
    cp_w0 = w_copies(0, 0, 6) + w_copies(1, 0, 6) + w_copies(2, 0, 6)
    cp_wm1 = [[wm_copy(j * KQ, KQ, 1 + j), wm_copy(D + j * KQ, KQ, 1 + j)] for j in range(D // KQ)]
    cp_q1 = w_copies(0, 1, 7) + [xj_copy(0, 7)]
    cp_late = [wm_copy(2 * D, 4 * D, 9), pltpu.make_async_copy(wo_hbm, wo.at[:, 0:D], sem.at[10]),
               pltpu.make_async_copy(mem0_hbm, mem0_ref, sem.at[14]),
               pltpu.make_async_copy(wr_hbm, wr_ref, sem.at[15])]
    cp_ffn = [pltpu.make_async_copy(wg_hbm, wg.at[:, 0:FF], sem.at[11]),
              pltpu.make_async_copy(wu_hbm, wu.at[:, 0:FF], sem.at[12]),
              pltpu.make_async_copy(wd_hbm, wd.at[:, 0:D], sem.at[13])]

    for cp in [cp_c, cp_xe] + cp_w0 + sum(cp_wm1, []) + cp_q1:
        cp.start()
    for p in range(1, FIRST):
        for cp in group_copies(p):
            cp.start()

    ri = jax.lax.broadcasted_iota(jnp.int32, (80, 128), 0)
    ci = jax.lax.broadcasted_iota(jnp.int32, (80, 128), 1)

    def head_of(i):
        return jnp.where(i < 64, i >> 5, (i - 64) >> 3)

    def pos_of(i):
        return jnp.where(i < 64, i & 31, 32 + (i & 7))

    same = (head_of(ri) == head_of(ci)) & (ci < 80)
    allowed = (pos_of(ri) < M) | (pos_of(ri) >= pos_of(ci))
    fill[...] = jnp.where(same, jnp.where(allowed, 0.0, NEG / SCALE), -jnp.inf).astype(F32)
    keys[...] = jnp.zeros(keys.shape, F32)
    pend[M:, :] = jnp.zeros((SEG + M, D), F32)
    zero[...] = jnp.zeros(zero.shape, U32)

    def pin_zero(vals):
        acc = None
        for v in vals:
            v = pltpu.bitcast(v, U32)
            for r in range(0, v.shape[0], 8):
                acc = v[r:r + 8] if acc is None else acc | v[r:r + 8]
        return acc & zero[...]

    cp_xe.wait()
    cp_c.wait()
    cf = c_ref[...].astype(F32)
    sc = _rb(cf * _sigmoid(cf))
    sc = jnp.broadcast_to(sc, (16, D)).astype(BF16)

    def mod_cols(lo, hi):
        for j in range(lo, hi):
            v = _rb(_dot(sc, wblk(wm, j))[0:8])
            if j // 8 in (1, 4):
                v = _rb(1.0 + v)
            mod[:, j * 128:(j + 1) * 128] = v

    def mod_vec(k):
        return mod[:, k * D:(k + 1) * D]

    def affine1(n):
        return _rb(n * mod_vec(1)) + mod_vec(0)

    def ne_body(i, carry):
        n = _layernorm(xv[pl.ds(i * 16, 16), 3].astype(F32))
        he[pl.ds(pl.multiple_of(i * 128, 128), 128), :] = n.reshape(128, D).astype(BF16)
        return carry

    jax.lax.fori_loop(0, NSEG // 16, ne_body, 0)

    def w_head(m, h, lo=0, hi=D):
        return pltpu.bitcast(wqkv[m][h, lo // 2:hi // 2, :], BF16)

    def relayout(m, p):
        w = wqkv[m]
        e = w[2 * p]
        o = w[2 * p + 1]
        w[2 * p] = (e & U32(0xFFFF)) | (o << 16)
        w[2 * p + 1] = (e >> 16) | (o & U32(0xFFFF0000))

    def store_early(m, p, row0, r1, r2):
        ns = r1.shape[0] // 8
        r12 = jnp.concatenate([r1.reshape(ns, 8, DH), r2.reshape(ns, 8, DH)], axis=1)
        early[row0 // 8:row0 // 8 + ns, m * NP + p] = pltpu.bitcast(
            r12.reshape(16 * ns, DH).astype(BF16), U32).reshape(ns, 8, DH)

    for cp in cp_w0:
        cp.wait()
    for m in range(3):
        relayout(m, 0)
    for j in range(D // KQ):
        for cp in cp_wm1[j]:
            cp.wait()
        lo, hi = j * KQ, (j + 1) * KQ
        mod_cols(lo // 128, hi // 128)
        mod_cols((D + lo) // 128, (D + hi) // 128)
        for c in range(2):
            rows = slice(c * 256, (c + 1) * 256)
            n = he[rows, lo:hi].astype(F32).reshape(32, 8, KQ)
            h = (_rb(n * mod[:, D + lo:D + hi]) + mod[:, lo:hi]).reshape(256, KQ)
            he[rows, lo:hi] = h.astype(BF16)
            hb = h.astype(BF16)
            for m in range(3):
                w2 = jnp.concatenate([w_head(m, 0, lo, hi), w_head(m, 1, lo, hi)], axis=1)
                r = _dot(hb, w2)
                if j > 0:
                    r = r + acc0[m, rows, :]
                if hi < D:
                    acc0[m, rows, :] = r
                else:
                    store_early(m, 0, c * 256, r[:, :DH], r[:, DH:])

    def early_proj(m, p, pins=None, rows=256, between=None):
        relayout(m, p)
        for c in range(NE // rows):
            hc = he[c * rows:(c + 1) * rows, :]
            r12 = []
            for b in range(2):
                wv_ = wqkv[m][2 * p + b]
                if pins and 2 * c + b in pins:
                    wv_ = jnp.concatenate([wv_[0:8] | pin_zero(pins[2 * c + b]), wv_[8:]], axis=0)
                r12.append(_dot(hc, pltpu.bitcast(wv_, BF16)))
                if between is not None:
                    between()
            store_early(m, p, c * rows, *r12)

    def make_hj(s):
        h = affine1(_rb(_layernorm(xv[s, 0:3].astype(F32))))
        hj[s] = h
        return [h[g, :, 0:128] for g in range(3)]

    for cp in cp_q1:
        cp.wait()
    pins = sum([make_hj(s) for s in range(4)], [])
    early_proj(0, 1, {i: pins[2 * i - 4:2 * i - 2] for i in range(2, 8)}, rows=128)

    def pro_body(p, carry):
        @pl.when(p == 4)
        def _():
            for pp in range(FIRST, NP):
                for cp in group_copies(pp, pp == NP - 1):
                    cp.start()
            for cp in cp_late:
                cp.start()

        for cp in group_copies(p):
            cp.wait()
        pins = sum([make_hj(p * 4 + t) for t in range(4)], [])
        early_proj(1, p, {2: pins[0:2], 3: pins[2:4]})
        early_proj(2, p, {i: pins[4 + i:5 + i] for i in range(4)})
        early_proj(0, p + 1, {i: pins[8 + i:9 + i] for i in range(4)})
        return carry

    with jax.named_scope("prologue_loop"):
        jax.lax.fori_loop(1, NP - 1, pro_body, 0)

    for cp in cp_ffn:
        cp.start()
    for cp in group_copies(NP - 1, True) + cp_late:
        cp.wait()
    pend[0:M, :] = mem0_ref[...].astype(F32)
    todo = list(range(16, 48))

    def one_mod_col():
        j = todo.pop(0)
        mod_cols(j, j + 1)

    pins = sum([make_hj(s) for s in range(NSEG - 4, NSEG)], [])
    early_proj(1, NP - 1, {4 + 2 * i: pins[i:i + 1] for i in range(6)}, rows=64, between=one_mod_col)
    early_proj(2, NP - 1, {4 + 2 * i: pins[6 + i:7 + i] for i in range(6)}, rows=64,
               between=one_mod_col)
    assert not todo

    wr = jnp.broadcast_to(wr_ref[...].astype(F32).reshape(1, D), (8, D))

    lane8 = jax.lax.broadcasted_iota(jnp.int32, (8, 128), 1)
    sub8 = jax.lax.broadcasted_iota(jnp.int32, (8, 128), 0)
    LAST = NSEG * SEG - 1

    def post(s, g0, g1, attn, record=True):
        attn = attn.reshape(g1 - g0, 8, D)
        x1 = _rb(xv[s, g0:g1].astype(F32) + _rb(mod_vec(2) * _rb(attn)))
        n = _rb(_layernorm(x1))
        h2 = _rb(_rb(n * mod_vec(4)) + mod_vec(3))
        r = _rb(jnp.sum(h2 * wr, axis=-1, keepdims=True)) + 0.0
        x1v[s, g0:g1] = x1.astype(BF16)
        h2v[s, g0:g1] = h2.astype(BF16)
        outv[s, g0:g1] = (x1 + _rb(mod_vec(5) * h2)).astype(BF16)
        pins = []
        for g in range(g0, g1):
            bits = pltpu.bitcast(jnp.broadcast_to(r[g - g0], (8, 128)), jnp.int32)
            hi = jax.lax.shift_right_logical(bits, 16)
            code = jnp.where(bits < 0, hi ^ 0xFFFF, hi | 0x8000)
            key = (code << 11) | (LAST - (s * SEG + g * 8) - sub8) | 0x40000000
            key = pltpu.bitcast(key, F32)
            if record:
                rows = slice(g * 8, (g + 1) * 8)
                keys[rows, :] = jnp.where(lane8 == s, key, keys[rows, :])
            pins.append(key)
        return pins

    def post_pair(a, rows, record=True):
        return post(a + 1, 0, 4, rows[0:SEG], record) + post(a, 3, 4, rows[SEG:], record)

    zpad = jnp.zeros((48, DH), BF16)
    G = 4
    KA = (NP - G) * 2 * DH
    KS = D - 128

    def segment(s, lhs, lhs_split, extra, pins):
        scales = {}

        def stash(p, m, v):
            opnd[p, m, 0:v.shape[0], :] = v.astype(BF16)

        def qkv_group(p):
            keys = [(m, 2 * p + b) for m in range(3) for b in range(2 * G)]
            nsplit = 6 if (p == 0 and lhs_split is not None) else 0
            part = [_dot(lhs_split[0], w_head(m, h, 0, KS)) for m, h in keys[:nsplit]]
            full = [_dot(lhs_split[1], w_head(m, h, KS, D)) + part[i]
                    for i, (m, h) in enumerate(keys[:nsplit])]
            full += [_dot(lhs, w_head(m, h)) for m, h in keys[nsplit:]]
            for m in range(3):
                for t in range(G):
                    i = 2 * G * m + 2 * t
                    stash(p + t, m, jnp.concatenate([full[i], full[i + 1]], axis=0))

        def operand(p, m):
            parts = [opnd[p, m, 0:64, :], pltpu.bitcast(early[s, m * NP + p], BF16)]
            if m > 0:
                parts.append(zpad)
            return jnp.concatenate(parts, axis=0)

        def scores(p):
            sc_ = _dot_nt(operand(p, 0), operand(p, 1))
            f = fill[...]
            if pins.get(p):
                f = jnp.concatenate([f[0:8] + pltpu.bitcast(pin_zero(pins[p]), F32), f[8:]], axis=0)
            sc_ = jnp.where(f == 0.0, sc_, f)
            mx = jnp.max(sc_, axis=-1, keepdims=True)
            e = jnp.exp2((sc_ - mx) * (SCALE * LOG2E))
            inv = pl.reciprocal(jnp.sum(e, axis=-1, keepdims=True), approx=True)
            if p // G == NP // G - 2:
                stash(p, 3, e * inv)
            else:
                stash(p, 3, e)
                scales[p] = inv

        oe = []

        def pv(p):
            o = _dot(opnd[p, 3], operand(p, 2))
            if p in scales:
                o = o * scales[p]
                pins.setdefault(p + G, []).append(o)
            res = []
            for b in range(2):
                rows, erows = o[32 * b:32 * b + 32], o[64 + 8 * b:72 + 8 * b]
                oe.append(erows)
                if extra is not None:
                    rows = jnp.concatenate([rows, erows, extra[2 * p + b]], axis=0)
                res.append(rows)
            return res

        os_ = []
        for p in range(0, NP, G):
            qkv_group(p)
            if p >= G:
                for t in range(G):
                    os_ += pv(p - G + t)
            for t in range(G):
                scores(p + t)
        oa = jnp.concatenate(os_, axis=1).astype(BF16)
        acc, ob = [], []
        for n in range(7):
            acc.append(_dot(oa, wblk(wo, n, 0, KA)))
            if n == 1:
                for t in range(G):
                    ob += pv(NP - G + t)
        ob = jnp.concatenate(ob, axis=1).astype(BF16)
        res = [_dot(ob, wblk(wo, n, KA, H * DH)) + acc[n] for n in range(7)]
        res.append(_dot(ob, wblk(wo, 7, KA, H * DH)) + _dot(oa, wblk(wo, 7, 0, KA)))
        return res, oe

    def make_lhs(mem, s):
        return jnp.concatenate([mem, hj[s].reshape(NJ, D)], axis=0)

    cp_o1 = pltpu.make_async_copy(outv.at[0:OUT_SPLIT], out_hbm.at[0:OUT_SPLIT], sem_out.at[0])
    cp_o2 = pltpu.make_async_copy(outv.at[OUT_SPLIT:NSEG], out_hbm.at[OUT_SPLIT:NSEG],
                                  sem_out.at[1])

    def split_lhs(lhs):
        return lhs.astype(BF16), (lhs[:, :KS].astype(BF16), lhs[:, KS:].astype(BF16))

    def step(i, carry):
        @pl.when(i == NIT - 1)
        def _():
            cp_o1.start()

        prev = pend[...]
        for u in range(UNROLL):
            a = 2 * (UNROLL * i + u)
            pins = post_pair(jnp.maximum(a - 2, 0) if u == 0 else a - 2, prev[M:])
            lhs_a = make_lhs(prev[0:M], a)
            lhs_a = (lhs_a.astype(BF16), None) if u == 0 else split_lhs(lhs_a)
            res_a, oe_a = segment(a, *lhs_a, None,
                                  {k: [v] for k, v in zip((3, 7, 11, 15), pins[:4])})
            res_a = jnp.concatenate(res_a, axis=1)
            pins = pins[4:] + post(a, 0, 3, res_a[M:])
            res_b, _ = segment(a + 1, *split_lhs(make_lhs(res_a[0:M], a + 1)), oe_a,
                               {k: [v] for k, v in zip((3, 7, 11, 15), pins)})
            prev = jnp.concatenate(res_b, axis=1)
        pend[...] = prev
        return carry

    with jax.named_scope("main_loop"):
        jax.lax.fori_loop(0, NIT, step, 0)
    for cp in cp_ffn:
        cp.wait()
    last_keys = post_pair(NSEG - 2, pend[M:, :], record=False)
    cp_o2.start()

    def max_all(v):
        return jnp.max(jnp.max(v, axis=0, keepdims=True), axis=1, keepdims=True)

    def decode(k):
        kb = pltpu.bitcast(jnp.broadcast_to(k, (8, 128)), jnp.int32)
        code = (kb >> 11) & 0xFFFF
        hi = jnp.where(code >= 0x8000, code & 0x7FFF, code ^ 0xFFFF)
        tok = jnp.clip((LAST - (kb & LAST))[0, 0], 0, LAST)
        return tok, pltpu.bitcast(hi << 16, F32)[:, 0:1]

    kv = keys[...]
    o1 = max_all(kv)
    o2 = max_all(jnp.where(kv == o1, 0.0, kv))
    kv = jnp.concatenate(last_keys + [jnp.where(sub8 < 4, o1, o2)], axis=0)
    k1 = jnp.max(kv, axis=0, keepdims=True)
    k2 = jnp.max(jnp.where(kv == k1, 0.0, kv), axis=0, keepdims=True)
    i1, r1 = decode(k1)
    i2, r2 = decode(k2)
    g1, g2 = i1 >> 3, i2 >> 3

    def rows_of(ref):
        return jnp.concatenate([ref[g1 >> 2, pl.ds(g1 & 3, 1)], ref[g2 >> 2, pl.ds(g2 & 3, 1)]],
                               axis=0).astype(F32)

    x1, h2 = rows_of(x1v), rows_of(h2v)
    hl = h2.reshape(16, D).astype(BF16)
    act = []
    for j in range(FF // 128):
        gt = _rb(_dot(hl, wblk(wg, j)))
        up = _rb(_dot(hl, wblk(wu, j)))
        act.append((_rb(gt * _sigmoid(gt)) * up).astype(BF16))
    act = jnp.concatenate(act, axis=1)
    y = jnp.concatenate([_dot(act, wblk(wd, n)) for n in range(8)], axis=1).reshape(2, 8, D)
    rowi = jax.lax.broadcasted_iota(jnp.int32, (2, 8, 1), 1)
    gsel = jax.lax.broadcasted_iota(jnp.int32, (2, 8, 1), 0)
    tokp = jnp.where(gsel == 0, g1, g2) * 8 + rowi
    gate = _sigmoid(jnp.where(tokp == i1, r1[None], r2[None]))
    upd = jnp.where((tokp == i1) | (tokp == i2), _rb(_rb(y) * gate), 0.0)
    patch[...] = (x1 + _rb(mod_vec(5) * _rb(h2 + upd))).astype(BF16)
    cp_o1.wait()
    cp_o2.wait()
    cp1 = pltpu.make_async_copy(patch.at[0], out_hbm.at[g1 >> 2, g1 & 3], sem_out.at[0])
    cp1.start()

    @pl.when(g1 != g2)
    def _():
        cp2 = pltpu.make_async_copy(patch.at[1], out_hbm.at[g2 >> 2, g2 & 3], sem_out.at[1])
        cp2.start()
        cp2.wait()

    cp1.wait()


@jax.jit
def pallas_adaLN_cond__memory_aug_recurrent_mem_tr__moe_arch_mod__prompt_kernel(
    A_x: jax.Array,
    A_mem0: jax.Array,
    A_Wq: jax.Array,
    A_Wk: jax.Array,
    A_Wv: jax.Array,
    A_Wo: jax.Array,
    A_seg_len,
    B_x: jax.Array,
    B_w_r: jax.Array,
    B_w_gate: jax.Array,
    B_w_up: jax.Array,
    B_w_down: jax.Array,
    c: jax.Array,
    w_mod: jax.Array,
):
    assert A_x.shape == (1, NSEG * SEG, D)
    any_spec = pl.BlockSpec(memory_space=pl.ANY)
    out = pl.pallas_call(
        _kernel,
        out_shape=jax.ShapeDtypeStruct((NSEG, 4, 8, D), BF16),
        in_specs=[any_spec] * 12,
        out_specs=any_spec,
        scratch_shapes=[
            pltpu.VMEM((H, D // 2, DH), U32),
            pltpu.VMEM((H, D // 2, DH), U32),
            pltpu.VMEM((H, D // 2, DH), U32),
            pltpu.VMEM((H * DH // 2, D + 128), U32),
            pltpu.VMEM((D // 2, FF + 128), U32),
            pltpu.VMEM((D // 2, FF + 128), U32),
            pltpu.VMEM((FF // 2, D + 128), U32),
            pltpu.VMEM((D // 2, 6 * D + 128), U32),
            pltpu.VMEM((NSEG, 4, 8, D), BF16),
            pltpu.VMEM((NSEG, 4, 8, D), BF16),
            pltpu.VMEM((NSEG, 4, 8, D), BF16),
            pltpu.VMEM((NSEG, 4, 8, D), BF16),
            pltpu.VMEM((NSEG, 3 * NP, 8, DH), U32),
            pltpu.VMEM((NE, D), BF16),
            pltpu.VMEM((NSEG, 3, 8, D), F32),
            pltpu.VMEM((M + SEG + M, D), F32),
            pltpu.VMEM((8, 6 * D), F32),
            pltpu.VMEM((80, 128), F32),
            pltpu.VMEM((SEG, 128), F32),
            pltpu.VMEM((2, 8, D), BF16),
            pltpu.VMEM((8, 128), U32),
            pltpu.VMEM((NP, 4, 80, DH), BF16),
            pltpu.VMEM((3, NE, 2 * DH), F32),
            pltpu.VMEM((M, D), BF16),
            pltpu.VMEM((D,), BF16),
            pltpu.VMEM((1, D), BF16),
            pltpu.SemaphoreType.DMA((16 + NP,)),
            pltpu.SemaphoreType.DMA((2,)),
        ],
        compiler_params=pltpu.CompilerParams(vmem_limit_bytes=120 * 1024 * 1024,
                                             disable_bounds_checks=True,
                                             disable_semaphore_checks=True),
    )(
        A_x.reshape(NSEG, 4, 8, D),
        A_mem0.reshape(M, D),
        A_Wq.reshape(D // 2, 2, H, DH),
        A_Wk.reshape(D // 2, 2, H, DH),
        A_Wv.reshape(D // 2, 2, H, DH),
        A_Wo.reshape(H * DH, D),
        B_w_r,
        B_w_gate,
        B_w_up,
        B_w_down,
        c,
        w_mod,
    )
    return out.reshape(1, NSEG * SEG, D)
```

```python
import jax
import jax.numpy as jnp
import jax.experimental.pallas as pl
import jax.experimental.pallas.tpu as pltpu

F32 = jnp.float32
BF16 = jnp.bfloat16
U32 = jnp.uint32

D = 1024
H = 32
DH = 128
NP = H // 2
M = 8
SEG = 32
NSEG = 64
FF = 3584
NJ = SEG - M
NE = NSEG * M
EPS = 1.0013580322265625e-05
SCALE = DH ** (-0.5)
NEG = -1000000000.0
LOG2E = 1.4426950408889634
KQ = 256
FIRST = 7
UNROLL = 2
NIT = NSEG // (2 * UNROLL)
OUT_SPLIT = NSEG - 2 * UNROLL - 2


def _rb(x):
    return x.astype(BF16).astype(F32)


def _layernorm(xf):
    m = jnp.mean(xf, axis=-1, keepdims=True)
    d = xf - m
    v = jnp.mean(d * d, axis=-1, keepdims=True)
    std = _rb(jnp.sqrt(_rb(_rb(v) + EPS)))
    return _rb(xf - _rb(m)) * (1.0 / std)


def _sigmoid(x):
    return _rb(1.0 / _rb(1.0 + _rb(jnp.exp(-x))))


def _dot(a, b):
    return jnp.dot(a, b, preferred_element_type=F32)


def _dot_nt(a, b):
    return jax.lax.dot_general(a, b, (((1,), (1,)), ((), ())), preferred_element_type=F32)


def _kernel(x_hbm, mem0_hbm, wq_hbm, wk_hbm, wv_hbm, wo_hbm, wr_hbm, wg_hbm, wu_hbm, wd_hbm,
            c_hbm, wm_hbm,
            out_hbm,
            wq, wk, wv, wo, wg, wu, wd, wm, xv, x1v, h2v, outv, early, he, hj, pend,
            mod, fill, keys, patch, zero, opnd, acc0, mem0_ref, wr_ref, c_ref,
            sem, sem_out):
    w_u32 = [w.bitcast(U32) for w in (wq_hbm, wk_hbm, wv_hbm)]
    wqkv = (wq, wk, wv)
    wo_hbm, wg_hbm, wu_hbm, wd_hbm, wm_hbm = [
        w.bitcast(U32) for w in (wo_hbm, wg_hbm, wu_hbm, wd_hbm, wm_hbm)]

    def wblk(w, j, lo=None, hi=None):
        rows = slice(None) if lo is None else slice(lo // 2, hi // 2)
        return pltpu.bitcast(w[rows, j * 128:(j + 1) * 128], BF16)

    def wm_copy(lo, n, k):
        return pltpu.make_async_copy(wm_hbm.at[:, pl.ds(lo, n)], wm.at[:, pl.ds(lo, n)], sem.at[k])

    def w_copies(m, p, k):
        return [pltpu.make_async_copy(w_u32[m].at[:, par, p, :], wqkv[m].at[2 * p + par], sem.at[k])
                for par in range(2)]

    def xj_copy(p, k):
        segs = pl.ds(4 * p, 4)
        return pltpu.make_async_copy(x_hbm.at[segs, 0:3], xv.at[segs, 0:3], sem.at[k])

    def group_copies(p, last=False):
        k = 16 + p
        return (w_copies(1, p, k) + w_copies(2, p, k) + ([] if last else w_copies(0, p + 1, k))
                + [xj_copy(p, k)])

    cp_c = pltpu.make_async_copy(c_hbm, c_ref, sem.at[5])
    cp_xe = pltpu.make_async_copy(x_hbm.at[:, 3], xv.at[:, 3], sem.at[0])
    cp_w0 = w_copies(0, 0, 6) + w_copies(1, 0, 6) + w_copies(2, 0, 6)
    cp_wm1 = [[wm_copy(j * KQ, KQ, 1 + j), wm_copy(D + j * KQ, KQ, 1 + j)] for j in range(D // KQ)]
    cp_q1 = w_copies(0, 1, 7) + [xj_copy(0, 7)]
    cp_late = [wm_copy(2 * D, 4 * D, 9), pltpu.make_async_copy(wo_hbm, wo.at[:, 0:D], sem.at[10]),
               pltpu.make_async_copy(mem0_hbm, mem0_ref, sem.at[14]),
               pltpu.make_async_copy(wr_hbm, wr_ref, sem.at[15])]
    cp_ffn = [pltpu.make_async_copy(wg_hbm, wg.at[:, 0:FF], sem.at[11]),
              pltpu.make_async_copy(wu_hbm, wu.at[:, 0:FF], sem.at[12]),
              pltpu.make_async_copy(wd_hbm, wd.at[:, 0:D], sem.at[13])]

    for cp in [cp_c, cp_xe] + cp_w0 + sum(cp_wm1, []) + cp_q1:
        cp.start()
    for p in range(1, FIRST):
        for cp in group_copies(p):
            cp.start()

    ri = jax.lax.broadcasted_iota(jnp.int32, (80, 128), 0)
    ci = jax.lax.broadcasted_iota(jnp.int32, (80, 128), 1)

    def head_of(i):
        return jnp.where(i < 64, i >> 5, (i - 64) >> 3)

    def pos_of(i):
        return jnp.where(i < 64, i & 31, 32 + (i & 7))

    same = (head_of(ri) == head_of(ci)) & (ci < 80)
    allowed = (pos_of(ri) < M) | (pos_of(ri) >= pos_of(ci))
    fill[...] = jnp.where(same, jnp.where(allowed, 0.0, NEG / SCALE), -jnp.inf).astype(F32)
    keys[...] = jnp.zeros(keys.shape, F32)
    pend[M:, :] = jnp.zeros((SEG + M, D), F32)
    zero[...] = jnp.zeros(zero.shape, U32)

    def pin_zero(vals):
        acc = None
        for v in vals:
            v = pltpu.bitcast(v, U32)
            for r in range(0, v.shape[0], 8):
                acc = v[r:r + 8] if acc is None else acc | v[r:r + 8]
        return acc & zero[...]

    cp_xe.wait()
    cp_c.wait()
    cf = c_ref[...].astype(F32)
    sc = _rb(cf * _sigmoid(cf))
    sc = jnp.broadcast_to(sc, (16, D)).astype(BF16)

    def mod_cols(lo, hi):
        for j in range(lo, hi):
            v = _rb(_dot(sc, wblk(wm, j))[0:8])
            if j // 8 in (1, 4):
                v = _rb(1.0 + v)
            mod[:, j * 128:(j + 1) * 128] = v

    def mod_vec(k):
        return mod[:, k * D:(k + 1) * D]

    def affine1(n):
        return _rb(n * mod_vec(1)) + mod_vec(0)

    def ne_body(i, carry):
        n = _layernorm(xv[pl.ds(i * 16, 16), 3].astype(F32))
        he[pl.ds(pl.multiple_of(i * 128, 128), 128), :] = n.reshape(128, D).astype(BF16)
        return carry

    jax.lax.fori_loop(0, NSEG // 16, ne_body, 0)

    def w_head(m, h, lo=0, hi=D):
        return pltpu.bitcast(wqkv[m][h, lo // 2:hi // 2, :], BF16)

    def relayout(m, p):
        w = wqkv[m]
        e = w[2 * p]
        o = w[2 * p + 1]
        w[2 * p] = (e & U32(0xFFFF)) | (o << 16)
        w[2 * p + 1] = (e >> 16) | (o & U32(0xFFFF0000))

    def store_early(m, p, row0, r1, r2):
        ns = r1.shape[0] // 8
        r12 = jnp.concatenate([r1.reshape(ns, 8, DH), r2.reshape(ns, 8, DH)], axis=1)
        early[row0 // 8:row0 // 8 + ns, m * NP + p] = pltpu.bitcast(
            r12.reshape(16 * ns, DH).astype(BF16), U32).reshape(ns, 8, DH)

    for cp in cp_w0:
        cp.wait()
    for m in range(3):
        relayout(m, 0)
    for j in range(D // KQ):
        for cp in cp_wm1[j]:
            cp.wait()
        lo, hi = j * KQ, (j + 1) * KQ
        mod_cols(lo // 128, hi // 128)
        mod_cols((D + lo) // 128, (D + hi) // 128)
        for c in range(2):
            rows = slice(c * 256, (c + 1) * 256)
            n = he[rows, lo:hi].astype(F32).reshape(32, 8, KQ)
            h = (_rb(n * mod[:, D + lo:D + hi]) + mod[:, lo:hi]).reshape(256, KQ)
            he[rows, lo:hi] = h.astype(BF16)
            hb = h.astype(BF16)
            for m in range(3):
                w2 = jnp.concatenate([w_head(m, 0, lo, hi), w_head(m, 1, lo, hi)], axis=1)
                r = _dot(hb, w2)
                if j > 0:
                    r = r + acc0[m, rows, :]
                if hi < D:
                    acc0[m, rows, :] = r
                else:
                    store_early(m, 0, c * 256, r[:, :DH], r[:, DH:])

    def early_proj(m, p, pins=None, rows=256, between=None):
        relayout(m, p)
        for c in range(NE // rows):
            hc = he[c * rows:(c + 1) * rows, :]
            r12 = []
            for b in range(2):
                wv_ = wqkv[m][2 * p + b]
                if pins and 2 * c + b in pins:
                    wv_ = jnp.concatenate([wv_[0:8] | pin_zero(pins[2 * c + b]), wv_[8:]], axis=0)
                r12.append(_dot(hc, pltpu.bitcast(wv_, BF16)))
                if between is not None:
                    between()
            store_early(m, p, c * rows, *r12)

    def make_hj(s):
        h = affine1(_rb(_layernorm(xv[s, 0:3].astype(F32))))
        hj[s] = h
        return [h[g, :, 0:128] for g in range(3)]

    for cp in cp_q1:
        cp.wait()
    pins = sum([make_hj(s) for s in range(4)], [])
    early_proj(0, 1, {i: pins[2 * i - 4:2 * i - 2] for i in range(2, 8)}, rows=128)

    def pro_body(p, carry):
        @pl.when(p == 4)
        def _():
            for pp in range(FIRST, NP):
                for cp in group_copies(pp, pp == NP - 1):
                    cp.start()
            for cp in cp_late:
                cp.start()

        for cp in group_copies(p):
            cp.wait()
        pins = sum([make_hj(p * 4 + t) for t in range(4)], [])
        early_proj(1, p, {2: pins[0:2], 3: pins[2:4]})
        early_proj(2, p, {i: pins[4 + i:5 + i] for i in range(4)})
        early_proj(0, p + 1, {i: pins[8 + i:9 + i] for i in range(4)})
        return carry

    jax.lax.fori_loop(1, NP - 1, pro_body, 0)

    for cp in cp_ffn:
        cp.start()
    for cp in group_copies(NP - 1, True) + cp_late:
        cp.wait()
    pend[0:M, :] = mem0_ref[...].astype(F32)
    todo = list(range(16, 48))

    def one_mod_col():
        j = todo.pop(0)
        mod_cols(j, j + 1)

    pins = sum([make_hj(s) for s in range(NSEG - 4, NSEG)], [])
    early_proj(1, NP - 1, {4 + 2 * i: pins[i:i + 1] for i in range(6)}, rows=64, between=one_mod_col)
    early_proj(2, NP - 1, {4 + 2 * i: pins[6 + i:7 + i] for i in range(6)}, rows=64,
               between=one_mod_col)
    assert not todo

    wr = jnp.broadcast_to(wr_ref[...].astype(F32).reshape(1, D), (8, D))

    lane8 = jax.lax.broadcasted_iota(jnp.int32, (8, 128), 1)
    sub8 = jax.lax.broadcasted_iota(jnp.int32, (8, 128), 0)
    LAST = NSEG * SEG - 1

    def post(s, g0, g1, attn, record=True):
        attn = attn.reshape(g1 - g0, 8, D)
        x1 = _rb(xv[s, g0:g1].astype(F32) + _rb(mod_vec(2) * _rb(attn)))
        n = _rb(_layernorm(x1))
        h2 = _rb(_rb(n * mod_vec(4)) + mod_vec(3))
        r = _rb(jnp.sum(h2 * wr, axis=-1, keepdims=True)) + 0.0
        x1v[s, g0:g1] = x1.astype(BF16)
        h2v[s, g0:g1] = h2.astype(BF16)
        outv[s, g0:g1] = (x1 + _rb(mod_vec(5) * h2)).astype(BF16)
        pins = []
        for g in range(g0, g1):
            bits = pltpu.bitcast(jnp.broadcast_to(r[g - g0], (8, 128)), jnp.int32)
            hi = jax.lax.shift_right_logical(bits, 16)
            code = jnp.where(bits < 0, hi ^ 0xFFFF, hi | 0x8000)
            key = (code << 11) | (LAST - (s * SEG + g * 8) - sub8) | 0x40000000
            key = pltpu.bitcast(key, F32)
            if record:
                rows = slice(g * 8, (g + 1) * 8)
                keys[rows, :] = jnp.where(lane8 == s, key, keys[rows, :])
            pins.append(key)
        return pins

    def post_pair(a, rows, record=True):
        return post(a + 1, 0, 4, rows[0:SEG], record) + post(a, 3, 4, rows[SEG:], record)

    zpad = jnp.zeros((48, DH), BF16)
    G = 4
    KA = (NP - G) * 2 * DH
    KS = D - 128

    def segment(s, lhs, lhs_split, extra, pins):
        scales = {}

        def stash(p, m, v):
            opnd[p, m, 0:v.shape[0], :] = v.astype(BF16)

        def qkv_group(p):
            keys = [(m, 2 * p + b) for m in range(3) for b in range(2 * G)]
            nsplit = 6 if (p == 0 and lhs_split is not None) else 0
            part = [_dot(lhs_split[0], w_head(m, h, 0, KS)) for m, h in keys[:nsplit]]
            full = [_dot(lhs_split[1], w_head(m, h, KS, D)) + part[i]
                    for i, (m, h) in enumerate(keys[:nsplit])]
            full += [_dot(lhs, w_head(m, h)) for m, h in keys[nsplit:]]
            for m in range(3):
                for t in range(G):
                    i = 2 * G * m + 2 * t
                    stash(p + t, m, jnp.concatenate([full[i], full[i + 1]], axis=0))

        def operand(p, m):
            parts = [opnd[p, m, 0:64, :], pltpu.bitcast(early[s, m * NP + p], BF16)]
            if m > 0:
                parts.append(zpad)
            return jnp.concatenate(parts, axis=0)

        def scores(p):
            sc_ = _dot_nt(operand(p, 0), operand(p, 1))
            f = fill[...]
            if pins.get(p):
                f = jnp.concatenate([f[0:8] + pltpu.bitcast(pin_zero(pins[p]), F32), f[8:]], axis=0)
            sc_ = jnp.where(f == 0.0, sc_, f)
            mx = jnp.max(sc_, axis=-1, keepdims=True)
            e = jnp.exp2((sc_ - mx) * (SCALE * LOG2E))
            inv = pl.reciprocal(jnp.sum(e, axis=-1, keepdims=True), approx=True)
            if p // G == NP // G - 2:
                stash(p, 3, e * inv)
            else:
                stash(p, 3, e)
                scales[p] = inv

        oe = []

        def pv(p):
            o = _dot(opnd[p, 3], operand(p, 2))
            if p in scales:
                o = o * scales[p]
                pins.setdefault(p + G, []).append(o)
            res = []
            for b in range(2):
                rows, erows = o[32 * b:32 * b + 32], o[64 + 8 * b:72 + 8 * b]
                oe.append(erows)
                if extra is not None:
                    rows = jnp.concatenate([rows, erows, extra[2 * p + b]], axis=0)
                res.append(rows)
            return res

        os_ = []
        for p in range(0, NP, G):
            qkv_group(p)
            if p >= G:
                for t in range(G):
                    os_ += pv(p - G + t)
            for t in range(G):
                scores(p + t)
        oa = jnp.concatenate(os_, axis=1).astype(BF16)
        acc, ob = [], []
        for n in range(7):
            acc.append(_dot(oa, wblk(wo, n, 0, KA)))
            if n == 1:
                for t in range(G):
                    ob += pv(NP - G + t)
        ob = jnp.concatenate(ob, axis=1).astype(BF16)
        res = [_dot(ob, wblk(wo, n, KA, H * DH)) + acc[n] for n in range(7)]
        res.append(_dot(ob, wblk(wo, 7, KA, H * DH)) + _dot(oa, wblk(wo, 7, 0, KA)))
        return res, oe

    def make_lhs(mem, s):
        return jnp.concatenate([mem, hj[s].reshape(NJ, D)], axis=0)

    cp_o1 = pltpu.make_async_copy(outv.at[0:OUT_SPLIT], out_hbm.at[0:OUT_SPLIT], sem_out.at[0])
    cp_o2 = pltpu.make_async_copy(outv.at[OUT_SPLIT:NSEG], out_hbm.at[OUT_SPLIT:NSEG],
                                  sem_out.at[1])

    def split_lhs(lhs):
        return lhs.astype(BF16), (lhs[:, :KS].astype(BF16), lhs[:, KS:].astype(BF16))

    def step(i, carry):
        @pl.when(i == NIT - 1)
        def _():
            cp_o1.start()

        prev = pend[...]
        for u in range(UNROLL):
            a = 2 * (UNROLL * i + u)
            pins = post_pair(jnp.maximum(a - 2, 0) if u == 0 else a - 2, prev[M:])
            lhs_a = make_lhs(prev[0:M], a)
            lhs_a = (lhs_a.astype(BF16), None) if u == 0 else split_lhs(lhs_a)
            res_a, oe_a = segment(a, *lhs_a, None,
                                  {k: [v] for k, v in zip((3, 7, 11, 15), pins[:4])})
            res_a = jnp.concatenate(res_a, axis=1)
            pins = pins[4:] + post(a, 0, 3, res_a[M:])
            res_b, _ = segment(a + 1, *split_lhs(make_lhs(res_a[0:M], a + 1)), oe_a,
                               {k: [v] for k, v in zip((3, 7, 11, 15), pins)})
            prev = jnp.concatenate(res_b, axis=1)
        pend[...] = prev
        return carry

    jax.lax.fori_loop(0, NIT, step, 0)
    for cp in cp_ffn:
        cp.wait()
    last_keys = post_pair(NSEG - 2, pend[M:, :], record=False)
    cp_o2.start()

    def max_all(v):
        return jnp.max(jnp.max(v, axis=0, keepdims=True), axis=1, keepdims=True)

    def decode(k):
        kb = pltpu.bitcast(jnp.broadcast_to(k, (8, 128)), jnp.int32)
        code = (kb >> 11) & 0xFFFF
        hi = jnp.where(code >= 0x8000, code & 0x7FFF, code ^ 0xFFFF)
        tok = jnp.clip((LAST - (kb & LAST))[0, 0], 0, LAST)
        return tok, pltpu.bitcast(hi << 16, F32)[:, 0:1]

    kv = keys[...]
    o1 = max_all(kv)
    o2 = max_all(jnp.where(kv == o1, 0.0, kv))
    kv = jnp.concatenate(last_keys + [jnp.where(sub8 < 4, o1, o2)], axis=0)
    k1 = jnp.max(kv, axis=0, keepdims=True)
    k2 = jnp.max(jnp.where(kv == k1, 0.0, kv), axis=0, keepdims=True)
    i1, r1 = decode(k1)
    i2, r2 = decode(k2)
    g1, g2 = i1 >> 3, i2 >> 3

    def rows_of(ref):
        return jnp.concatenate([ref[g1 >> 2, pl.ds(g1 & 3, 1)], ref[g2 >> 2, pl.ds(g2 & 3, 1)]],
                               axis=0).astype(F32)

    x1, h2 = rows_of(x1v), rows_of(h2v)
    hl = h2.reshape(16, D).astype(BF16)
    act = []
    for j in range(FF // 128):
        gt = _rb(_dot(hl, wblk(wg, j)))
        up = _rb(_dot(hl, wblk(wu, j)))
        act.append((_rb(gt * _sigmoid(gt)) * up).astype(BF16))
    act = jnp.concatenate(act, axis=1)
    y = jnp.concatenate([_dot(act, wblk(wd, n)) for n in range(8)], axis=1).reshape(2, 8, D)
    rowi = jax.lax.broadcasted_iota(jnp.int32, (2, 8, 1), 1)
    gsel = jax.lax.broadcasted_iota(jnp.int32, (2, 8, 1), 0)
    tokp = jnp.where(gsel == 0, g1, g2) * 8 + rowi
    gate = _sigmoid(jnp.where(tokp == i1, r1[None], r2[None]))
    upd = jnp.where((tokp == i1) | (tokp == i2), _rb(_rb(y) * gate), 0.0)
    patch[...] = (x1 + _rb(mod_vec(5) * _rb(h2 + upd))).astype(BF16)
    cp_o1.wait()
    cp_o2.wait()
    cp1 = pltpu.make_async_copy(patch.at[0], out_hbm.at[g1 >> 2, g1 & 3], sem_out.at[0])
    cp1.start()

    @pl.when(g1 != g2)
    def _():
        cp2 = pltpu.make_async_copy(patch.at[1], out_hbm.at[g2 >> 2, g2 & 3], sem_out.at[1])
        cp2.start()
        cp2.wait()

    cp1.wait()


@jax.jit
def pallas_adaLN_cond__memory_aug_recurrent_mem_tr__moe_arch_mod__prompt_kernel(
    A_x: jax.Array,
    A_mem0: jax.Array,
    A_Wq: jax.Array,
    A_Wk: jax.Array,
    A_Wv: jax.Array,
    A_Wo: jax.Array,
    A_seg_len,
    B_x: jax.Array,
    B_w_r: jax.Array,
    B_w_gate: jax.Array,
    B_w_up: jax.Array,
    B_w_down: jax.Array,
    c: jax.Array,
    w_mod: jax.Array,
):
    assert A_x.shape == (1, NSEG * SEG, D)
    any_spec = pl.BlockSpec(memory_space=pl.ANY)
    out = pl.pallas_call(
        _kernel,
        out_shape=jax.ShapeDtypeStruct((NSEG, 4, 8, D), BF16),
        in_specs=[any_spec] * 12,
        out_specs=any_spec,
        scratch_shapes=[
            pltpu.VMEM((H, D // 2, DH), U32),
            pltpu.VMEM((H, D // 2, DH), U32),
            pltpu.VMEM((H, D // 2, DH), U32),
            pltpu.VMEM((H * DH // 2, D + 128), U32),
            pltpu.VMEM((D // 2, FF + 128), U32),
            pltpu.VMEM((D // 2, FF + 128), U32),
            pltpu.VMEM((FF // 2, D + 128), U32),
            pltpu.VMEM((D // 2, 6 * D + 128), U32),
            pltpu.VMEM((NSEG, 4, 8, D), BF16),
            pltpu.VMEM((NSEG, 4, 8, D), BF16),
            pltpu.VMEM((NSEG, 4, 8, D), BF16),
            pltpu.VMEM((NSEG, 4, 8, D), BF16),
            pltpu.VMEM((NSEG, 3 * NP, 8, DH), U32),
            pltpu.VMEM((NE, D), BF16),
            pltpu.VMEM((NSEG, 3, 8, D), F32),
            pltpu.VMEM((M + SEG + M, D), F32),
            pltpu.VMEM((8, 6 * D), F32),
            pltpu.VMEM((80, 128), F32),
            pltpu.VMEM((SEG, 128), F32),
            pltpu.VMEM((2, 8, D), BF16),
            pltpu.VMEM((8, 128), U32),
            pltpu.VMEM((NP, 4, 80, DH), BF16),
            pltpu.VMEM((3, NE, 2 * DH), F32),
            pltpu.VMEM((M, D), BF16),
            pltpu.VMEM((D,), BF16),
            pltpu.VMEM((1, D), BF16),
            pltpu.SemaphoreType.DMA((16 + NP,)),
            pltpu.SemaphoreType.DMA((2,)),
        ],
        compiler_params=pltpu.CompilerParams(vmem_limit_bytes=120 * 1024 * 1024,
                                             disable_bounds_checks=True,
                                             disable_semaphore_checks=True),
    )(
        A_x.reshape(NSEG, 4, 8, D),
        A_mem0.reshape(M, D),
        A_Wq.reshape(D // 2, 2, H, DH),
        A_Wk.reshape(D // 2, 2, H, DH),
        A_Wv.reshape(D // 2, 2, H, DH),
        A_Wo.reshape(H * DH, D),
        B_w_r,
        B_w_gate,
        B_w_up,
        B_w_down,
        c,
        w_mod,
    )
    return out.reshape(1, NSEG * SEG, D)
```

```python
import jax
import jax.numpy as jnp
import jax.experimental.pallas as pl
import jax.experimental.pallas.tpu as pltpu

F32 = jnp.float32
BF16 = jnp.bfloat16
U32 = jnp.uint32

D = 1024
H = 32
DH = 128
NP = H // 2
M = 8
SEG = 32
NSEG = 64
FF = 3584
NJ = SEG - M
NE = NSEG * M
EPS = 1.0013580322265625e-05
SCALE = DH ** (-0.5)
NEG = -1000000000.0
LOG2E = 1.4426950408889634
KQ = 256
MC = 512
NC = 4 * D // MC
MB = MC // 128
AHEAD = 6
UNROLL = 2
NIT = NSEG // (2 * UNROLL)
OUT_SPLIT = NSEG - 2 * UNROLL - 2


def _rb(x):
    return x.astype(BF16).astype(F32)


def _layernorm(xf):
    m = jnp.mean(xf, axis=-1, keepdims=True)
    d = xf - m
    v = jnp.mean(d * d, axis=-1, keepdims=True)
    std = _rb(jnp.sqrt(_rb(_rb(v) + EPS)))
    return _rb(xf - _rb(m)) * (1.0 / std)


def _sigmoid(x):
    return _rb(1.0 / _rb(1.0 + _rb(jnp.exp(-x))))


def _dot(a, b):
    return jnp.dot(a, b, preferred_element_type=F32)


def _dot_nt(a, b):
    return jax.lax.dot_general(a, b, (((1,), (1,)), ((), ())), preferred_element_type=F32)


def _kernel(x_hbm, mem0_hbm, wq_hbm, wk_hbm, wv_hbm, wo_hbm, wr_hbm, wg_hbm, wu_hbm, wd_hbm,
            c_hbm, wm_hbm,
            out_hbm,
            wq, wk, wv, wo, wg, wu, wd, wm, wm2, cb, mod2, xv, x1v, h2v, outv, early, he, hj, pend,
            mod, fill, keys, patch, zero, opnd, acc0, mem0_ref, wr_ref, c_ref,
            sem, sem_out):
    w_u32 = [w.bitcast(U32) for w in (wq_hbm, wk_hbm, wv_hbm)]
    wqkv = (wq, wk, wv)
    wo_hbm, wg_hbm, wu_hbm, wd_hbm, wm_hbm = [
        w.bitcast(U32) for w in (wo_hbm, wg_hbm, wu_hbm, wd_hbm, wm_hbm)]

    def wblk(w, j):
        return pltpu.bitcast(w[:, j * 128:(j + 1) * 128], BF16)

    def wo_blk(n, lo, hi):
        return pltpu.bitcast(wo[n, lo // 2:hi // 2, :], BF16)

    def wm_copy(lo, n, k):
        return pltpu.make_async_copy(wm_hbm.at[:, pl.ds(lo, n)], wm.at[:, pl.ds(lo, n)], sem.at[k])

    def w_copies(m, p, k):
        return [pltpu.make_async_copy(w_u32[m].at[:, par, p, :], wqkv[m].at[2 * p + par], sem.at[k])
                for par in range(2)]

    def xj_copy(p, k):
        segs = pl.ds(4 * p, 4)
        return pltpu.make_async_copy(x_hbm.at[segs, 0:3], xv.at[segs, 0:3], sem.at[k])

    def group_copies(p, last=False):
        k = 16 + p
        return (w_copies(1, p, k) + w_copies(2, p, k) + ([] if last else w_copies(0, p + 1, k))
                + [xj_copy(p, k)])

    cp_c = pltpu.make_async_copy(c_hbm, c_ref, sem.at[5])
    cp_xe = pltpu.make_async_copy(x_hbm.at[:, 3], xv.at[:, 3], sem.at[0])
    cp_w0 = w_copies(0, 0, 6) + w_copies(1, 0, 6) + w_copies(2, 0, 6)
    cp_wm1 = [[wm_copy(j * KQ, KQ, 1 + j), wm_copy(D + j * KQ, KQ, 1 + j)] for j in range(D // KQ)]
    cp_q1 = w_copies(0, 1, 7) + [xj_copy(0, 7)]
    def col_copy(src, first, dst, j, k):
        lo = (first + j) * 128
        if not isinstance(j, int):
            lo = pl.multiple_of(lo, 128)
        return pltpu.make_async_copy(src.at[:, pl.ds(lo, 128)], dst.at[j], sem.at[k])

    def wm2_copies(t):
        return [col_copy(wm_hbm, 2 * D // 128, wm2, t * MB + j, 16 + NP + t) for j in range(MB)]

    cp_small = [pltpu.make_async_copy(mem0_hbm, mem0_ref, sem.at[14]),
                pltpu.make_async_copy(wr_hbm, wr_ref, sem.at[15])]
    cp_ffn = [pltpu.make_async_copy(wg_hbm, wg.at[:, 0:FF], sem.at[11]),
              pltpu.make_async_copy(wu_hbm, wu.at[:, 0:FF], sem.at[12]),
              pltpu.make_async_copy(wd_hbm, wd.at[:, 0:D], sem.at[13])]

    for cp in [cp_c, cp_xe] + cp_w0 + sum(cp_wm1, []) + cp_q1:
        cp.start()
    for p in range(1, AHEAD + 1):
        for cp in group_copies(p):
            cp.start()
    for cp in cp_small:
        cp.start()

    ri = jax.lax.broadcasted_iota(jnp.int32, (80, 128), 0)
    ci = jax.lax.broadcasted_iota(jnp.int32, (80, 128), 1)

    def head_of(i):
        return jnp.where(i < 64, i >> 5, (i - 64) >> 3)

    def pos_of(i):
        return jnp.where(i < 64, i & 31, 32 + (i & 7))

    same = (head_of(ri) == head_of(ci)) & (ci < 80)
    allowed = (pos_of(ri) < M) | (pos_of(ri) >= pos_of(ci))
    fill[...] = jnp.where(same, jnp.where(allowed, 0.0, NEG / SCALE), -jnp.inf).astype(F32)
    keys[...] = jnp.zeros(keys.shape, F32)
    pend[M:, :] = jnp.zeros((SEG + M, D), F32)
    zero[...] = jnp.zeros(zero.shape, U32)
    wm2[NC * MB:] = jnp.zeros((MB, D // 2, 128), U32)

    def pin_zero(vals):
        acc = None
        for v in vals:
            v = pltpu.bitcast(v, U32)
            for r in range(0, v.shape[0], 8):
                acc = v[r:r + 8] if acc is None else acc | v[r:r + 8]
        return acc & zero[...]

    cp_xe.wait()
    cp_c.wait()
    cf = c_ref[...].astype(F32)
    sc = _rb(cf * _sigmoid(cf))
    cb[...] = jnp.broadcast_to(sc, (128, D)).T
    sc = jnp.broadcast_to(sc, (16, D)).astype(BF16)

    def mod_cols(lo, hi):
        for j in range(lo, hi):
            v = _rb(_dot(sc, wblk(wm, j))[0:8])
            if j // 8 == 1:
                v = _rb(1.0 + v)
            mod[:, j * 128:(j + 1) * 128] = v

    def mod_vec(k):
        if k < 2:
            return mod[:, k * D:(k + 1) * D]
        t = (k - 2) * D // MC
        return jnp.concatenate([mod2[t + i] for i in range(D // MC)], axis=1)

    def mod2_block(t, j):
        acc = None
        for r in range(0, D // 2, 8):
            w = wm2[t * MB + j, r:r + 8, :]
            term = (pltpu.bitcast(w << 16, F32) * cb[pl.ds(2 * r, 8, stride=2), :]
                    + pltpu.bitcast(w & U32(0xFFFF0000), F32) * cb[pl.ds(2 * r + 1, 8, stride=2), :])
            acc = term if acc is None else acc + term
        v = _rb(jnp.broadcast_to(jnp.sum(acc, axis=0, keepdims=True), (8, 128)))
        is_scale = (t >= 2 * D // MC) & (t < 3 * D // MC)
        v = jnp.where(is_scale, _rb(1.0 + v), v)
        mod2[t, :, j * 128:(j + 1) * 128] = v
        return v

    def affine1(n):
        return _rb(n * mod_vec(1)) + mod_vec(0)

    def ne_body(i, carry):
        n = _layernorm(xv[pl.ds(i * 16, 16), 3].astype(F32))
        he[pl.ds(pl.multiple_of(i * 128, 128), 128), :] = n.reshape(128, D).astype(BF16)
        return carry

    jax.lax.fori_loop(0, NSEG // 16, ne_body, 0)

    def w_head(m, h, lo=0, hi=D):
        return pltpu.bitcast(wqkv[m][h, lo // 2:hi // 2, :], BF16)

    def relayout(m, p):
        w = wqkv[m]
        e = w[2 * p]
        o = w[2 * p + 1]
        w[2 * p] = (e & U32(0xFFFF)) | (o << 16)
        w[2 * p + 1] = (e >> 16) | (o & U32(0xFFFF0000))

    def store_early(m, p, row0, r1, r2):
        ns = r1.shape[0] // 8
        r12 = jnp.concatenate([r1.reshape(ns, 8, DH), r2.reshape(ns, 8, DH)], axis=1)
        early[row0 // 8:row0 // 8 + ns, m * NP + p] = pltpu.bitcast(
            r12.reshape(16 * ns, DH).astype(BF16), U32).reshape(ns, 8, DH)

    for cp in cp_w0:
        cp.wait()
    for m in range(3):
        relayout(m, 0)
    for j in range(D // KQ):
        for cp in cp_wm1[j]:
            cp.wait()
        lo, hi = j * KQ, (j + 1) * KQ
        mod_cols(lo // 128, hi // 128)
        mod_cols((D + lo) // 128, (D + hi) // 128)
        for c in range(2):
            rows = slice(c * 256, (c + 1) * 256)
            n = he[rows, lo:hi].astype(F32).reshape(32, 8, KQ)
            h = (_rb(n * mod[:, D + lo:D + hi]) + mod[:, lo:hi]).reshape(256, KQ)
            he[rows, lo:hi] = h.astype(BF16)
            hb = h.astype(BF16)
            for m in range(3):
                w2 = jnp.concatenate([w_head(m, 0, lo, hi), w_head(m, 1, lo, hi)], axis=1)
                r = _dot(hb, w2)
                if j > 0:
                    r = r + acc0[m, rows, :]
                if hi < D:
                    acc0[m, rows, :] = r
                else:
                    store_early(m, 0, c * 256, r[:, :DH], r[:, DH:])

    def early_proj(m, p, pins=None, rows=256):
        relayout(m, p)
        for c in range(NE // rows):
            hc = he[c * rows:(c + 1) * rows, :]
            r12 = []
            for b in range(2):
                wv_ = wqkv[m][2 * p + b]
                if pins and 2 * c + b in pins:
                    wv_ = jnp.concatenate([wv_[0:8] | pin_zero(pins[2 * c + b]), wv_[8:]], axis=0)
                r12.append(_dot(hc, pltpu.bitcast(wv_, BF16)))
            store_early(m, p, c * rows, *r12)

    def make_hj(s):
        h = affine1(_rb(_layernorm(xv[s, 0:3].astype(F32))))
        hj[s] = h
        return [h[g, :, 0:128] for g in range(3)]

    for cp in cp_q1:
        cp.wait()
    pins = sum([make_hj(s) for s in range(4)], [])
    early_proj(0, 1, {i: pins[2 * i - 4:2 * i - 2] for i in range(2, 8)}, rows=128)

    P2 = NP - 1 - NC

    def pro_body(p, carry):
        @pl.when(p >= P2)
        def _():
            for cp in wm2_copies(p - P2):
                cp.wait()

        for cp in group_copies(p):
            cp.wait()

        pins = sum([make_hj(p * 4 + t) for t in range(4)], [])
        t = jnp.where(p >= P2, p - P2, NC)
        mv = [mod2_block(t, j) for j in range(MC // 128)]
        early_proj(1, p, {1: mv[0:1], 2: pins[0:2], 3: pins[2:4]})
        early_proj(2, p, {i: pins[4 + i:5 + i] + (mv[1:2] if i == 2 else []) for i in range(4)})
        early_proj(0, p + 1, {i: pins[8 + i:9 + i] + (mv[2 + i // 3:3 + i // 3] if i in (0, 3) else [])
                              for i in range(4)})

        def start_if(cond, cps):
            for cp in cps:
                pl.when(cond)(cp.start)

        nxt = jnp.minimum(p + AHEAD, NP - 2)
        start_if(nxt == p + AHEAD, group_copies(nxt))
        start_if(p + AHEAD == NP - 1, group_copies(NP - 1, True))
        start_if(p <= NC, wm2_copies(jnp.minimum(p - 1, NC - 1)))
        start_if((p >= 5) & (p < 13), [col_copy(wo_hbm, 0, wo, jnp.clip(p - 5, 0, 7), 10)])
        return carry

    jax.lax.fori_loop(1, NP - 1, pro_body, 0)

    for cp in cp_ffn:
        cp.start()
    for cp in (group_copies(NP - 1, True) + cp_small
               + [col_copy(wo_hbm, 0, wo, n, 10) for n in range(8)]):
        cp.wait()
    pend[0:M, :] = mem0_ref[...].astype(F32)
    pins = sum([make_hj(s) for s in range(NSEG - 4, NSEG)], [])
    early_proj(1, NP - 1, {2: pins[0:2], 3: pins[2:4]})
    early_proj(2, NP - 1, {i: pins[4 + 2 * i:6 + 2 * i] for i in range(4)})

    wr = jnp.broadcast_to(wr_ref[...].astype(F32).reshape(1, D), (8, D))

    lane8 = jax.lax.broadcasted_iota(jnp.int32, (8, 128), 1)
    sub8 = jax.lax.broadcasted_iota(jnp.int32, (8, 128), 0)
    LAST = NSEG * SEG - 1

    def post(s, g0, g1, attn, record=True):
        attn = attn.reshape(g1 - g0, 8, D)
        x1 = _rb(xv[s, g0:g1].astype(F32) + _rb(mod_vec(2) * _rb(attn)))
        n = _rb(_layernorm(x1))
        h2 = _rb(_rb(n * mod_vec(4)) + mod_vec(3))
        r = _rb(jnp.sum(h2 * wr, axis=-1, keepdims=True)) + 0.0
        x1v[s, g0:g1] = x1.astype(BF16)
        h2v[s, g0:g1] = h2.astype(BF16)
        outv[s, g0:g1] = (x1 + _rb(mod_vec(5) * h2)).astype(BF16)
        pins = []
        for g in range(g0, g1):
            bits = pltpu.bitcast(jnp.broadcast_to(r[g - g0], (8, 128)), jnp.int32)
            hi = jax.lax.shift_right_logical(bits, 16)
            code = jnp.where(bits < 0, hi ^ 0xFFFF, hi | 0x8000)
            key = (code << 11) | (LAST - (s * SEG + g * 8) - sub8) | 0x40000000
            key = pltpu.bitcast(key, F32)
            if record:
                rows = slice(g * 8, (g + 1) * 8)
                keys[rows, :] = jnp.where(lane8 == s, key, keys[rows, :])
            pins.append(key)
        return pins

    def post_pair(a, rows, record=True):
        return post(a + 1, 0, 4, rows[0:SEG], record) + post(a, 3, 4, rows[SEG:], record)

    zpad = jnp.zeros((48, DH), BF16)
    G = 4
    KA = (NP - G) * 2 * DH
    KS = D - 128

    def segment(s, lhs, lhs_split, extra, pins):
        scales = {}

        def stash(p, m, v):
            opnd[p, m, 0:v.shape[0], :] = v.astype(BF16)

        def qkv_group(p):
            keys = [(m, 2 * p + b) for m in range(3) for b in range(2 * G)]
            nsplit = 6 if (p == 0 and lhs_split is not None) else 0
            part = [_dot(lhs_split[0], w_head(m, h, 0, KS)) for m, h in keys[:nsplit]]
            full = [_dot(lhs_split[1], w_head(m, h, KS, D)) + part[i]
                    for i, (m, h) in enumerate(keys[:nsplit])]
            full += [_dot(lhs, w_head(m, h)) for m, h in keys[nsplit:]]
            for m in range(3):
                for t in range(G):
                    i = 2 * G * m + 2 * t
                    stash(p + t, m, jnp.concatenate([full[i], full[i + 1]], axis=0))

        def operand(p, m):
            parts = [opnd[p, m, 0:64, :], pltpu.bitcast(early[s, m * NP + p], BF16)]
            if m > 0:
                parts.append(zpad)
            return jnp.concatenate(parts, axis=0)

        def scores(p):
            sc_ = _dot_nt(operand(p, 0), operand(p, 1))
            f = fill[...]
            if pins.get(p):
                f = jnp.concatenate([f[0:8] + pltpu.bitcast(pin_zero(pins[p]), F32), f[8:]], axis=0)
            sc_ = jnp.where(f == 0.0, sc_, f)
            mx = jnp.max(sc_, axis=-1, keepdims=True)
            e = jnp.exp2((sc_ - mx) * (SCALE * LOG2E))
            inv = pl.reciprocal(jnp.sum(e, axis=-1, keepdims=True), approx=True)
            if p // G == NP // G - 2:
                stash(p, 3, e * inv)
            else:
                stash(p, 3, e)
                scales[p] = inv

        oe = []

        def pv(p):
            o = _dot(opnd[p, 3], operand(p, 2))
            if p in scales:
                o = o * scales[p]
                pins.setdefault(p + G, []).append(o)
            res = []
            for b in range(2):
                rows, erows = o[32 * b:32 * b + 32], o[64 + 8 * b:72 + 8 * b]
                oe.append(erows)
                if extra is not None:
                    rows = jnp.concatenate([rows, erows, extra[2 * p + b]], axis=0)
                res.append(rows)
            return res

        os_ = []
        for p in range(0, NP, G):
            qkv_group(p)
            if p >= G:
                for t in range(G):
                    os_ += pv(p - G + t)
            for t in range(G):
                scores(p + t)
        oa = jnp.concatenate(os_, axis=1).astype(BF16)
        acc, ob = [], []
        for n in range(7):
            acc.append(_dot(oa, wo_blk(n, 0, KA)))
            if n == 1:
                for t in range(G):
                    ob += pv(NP - G + t)
        ob = jnp.concatenate(ob, axis=1).astype(BF16)
        res = [_dot(ob, wo_blk(n, KA, H * DH)) + acc[n] for n in range(7)]
        res.append(_dot(ob, wo_blk(7, KA, H * DH)) + _dot(oa, wo_blk(7, 0, KA)))
        return res, oe

    def make_lhs(mem, s):
        return jnp.concatenate([mem, hj[s].reshape(NJ, D)], axis=0)

    cp_o1 = pltpu.make_async_copy(outv.at[0:OUT_SPLIT], out_hbm.at[0:OUT_SPLIT], sem_out.at[0])
    cp_o2 = pltpu.make_async_copy(outv.at[OUT_SPLIT:NSEG], out_hbm.at[OUT_SPLIT:NSEG],
                                  sem_out.at[1])

    def split_lhs(lhs):
        return lhs.astype(BF16), (lhs[:, :KS].astype(BF16), lhs[:, KS:].astype(BF16))

    def step(i, carry):
        @pl.when(i == NIT - 1)
        def _():
            cp_o1.start()

        prev = pend[...]
        for u in range(UNROLL):
            a = 2 * (UNROLL * i + u)
            pins = post_pair(jnp.maximum(a - 2, 0) if u == 0 else a - 2, prev[M:])
            lhs_a = make_lhs(prev[0:M], a)
            lhs_a = (lhs_a.astype(BF16), None) if u == 0 else split_lhs(lhs_a)
            res_a, oe_a = segment(a, *lhs_a, None,
                                  {k: [v] for k, v in zip((3, 7, 11, 15), pins[:4])})
            res_a = jnp.concatenate(res_a, axis=1)
            pins = pins[4:] + post(a, 0, 3, res_a[M:])
            res_b, _ = segment(a + 1, *split_lhs(make_lhs(res_a[0:M], a + 1)), oe_a,
                               {k: [v] for k, v in zip((3, 7, 11, 15), pins)})
            prev = jnp.concatenate(res_b, axis=1)
        pend[...] = prev
        return carry

    jax.lax.fori_loop(0, NIT, step, 0)
    for cp in cp_ffn:
        cp.wait()
    last_keys = post_pair(NSEG - 2, pend[M:, :], record=False)
    cp_o2.start()

    def max_all(v):
        return jnp.max(jnp.max(v, axis=0, keepdims=True), axis=1, keepdims=True)

    def decode(k):
        kb = pltpu.bitcast(jnp.broadcast_to(k, (8, 128)), jnp.int32)
        code = (kb >> 11) & 0xFFFF
        hi = jnp.where(code >= 0x8000, code & 0x7FFF, code ^ 0xFFFF)
        tok = jnp.clip((LAST - (kb & LAST))[0, 0], 0, LAST)
        return tok, pltpu.bitcast(hi << 16, F32)[:, 0:1]

    kv = keys[...]
    o1 = max_all(kv)
    o2 = max_all(jnp.where(kv == o1, 0.0, kv))
    kv = jnp.concatenate(last_keys + [jnp.where(sub8 < 4, o1, o2)], axis=0)
    k1 = jnp.max(kv, axis=0, keepdims=True)
    k2 = jnp.max(jnp.where(kv == k1, 0.0, kv), axis=0, keepdims=True)
    i1, r1 = decode(k1)
    i2, r2 = decode(k2)
    g1, g2 = i1 >> 3, i2 >> 3

    def rows_of(ref):
        return jnp.concatenate([ref[g1 >> 2, pl.ds(g1 & 3, 1)], ref[g2 >> 2, pl.ds(g2 & 3, 1)]],
                               axis=0).astype(F32)

    x1, h2 = rows_of(x1v), rows_of(h2v)
    hl = h2.reshape(16, D).astype(BF16)
    act = []
    for j in range(FF // 128):
        gt = _rb(_dot(hl, wblk(wg, j)))
        up = _rb(_dot(hl, wblk(wu, j)))
        act.append((_rb(gt * _sigmoid(gt)) * up).astype(BF16))
    act = jnp.concatenate(act, axis=1)
    y = jnp.concatenate([_dot(act, wblk(wd, n)) for n in range(8)], axis=1).reshape(2, 8, D)
    rowi = jax.lax.broadcasted_iota(jnp.int32, (2, 8, 1), 1)
    gsel = jax.lax.broadcasted_iota(jnp.int32, (2, 8, 1), 0)
    tokp = jnp.where(gsel == 0, g1, g2) * 8 + rowi
    gate = _sigmoid(jnp.where(tokp == i1, r1[None], r2[None]))
    upd = jnp.where((tokp == i1) | (tokp == i2), _rb(_rb(y) * gate), 0.0)
    patch[...] = (x1 + _rb(mod_vec(5) * _rb(h2 + upd))).astype(BF16)
    cp_o1.wait()
    cp_o2.wait()
    cp1 = pltpu.make_async_copy(patch.at[0], out_hbm.at[g1 >> 2, g1 & 3], sem_out.at[0])
    cp1.start()

    @pl.when(g1 != g2)
    def _():
        cp2 = pltpu.make_async_copy(patch.at[1], out_hbm.at[g2 >> 2, g2 & 3], sem_out.at[1])
        cp2.start()
        cp2.wait()

    cp1.wait()


@jax.jit
def pallas_adaLN_cond__memory_aug_recurrent_mem_tr__moe_arch_mod__prompt_kernel(
    A_x: jax.Array,
    A_mem0: jax.Array,
    A_Wq: jax.Array,
    A_Wk: jax.Array,
    A_Wv: jax.Array,
    A_Wo: jax.Array,
    A_seg_len,
    B_x: jax.Array,
    B_w_r: jax.Array,
    B_w_gate: jax.Array,
    B_w_up: jax.Array,
    B_w_down: jax.Array,
    c: jax.Array,
    w_mod: jax.Array,
):
    assert A_x.shape == (1, NSEG * SEG, D)
    any_spec = pl.BlockSpec(memory_space=pl.ANY)
    out = pl.pallas_call(
        _kernel,
        out_shape=jax.ShapeDtypeStruct((NSEG, 4, 8, D), BF16),
        in_specs=[any_spec] * 12,
        out_specs=any_spec,
        scratch_shapes=[
            pltpu.VMEM((H, D // 2, DH), U32),
            pltpu.VMEM((H, D // 2, DH), U32),
            pltpu.VMEM((H, D // 2, DH), U32),
            pltpu.VMEM((8, H * DH // 2, 128), U32),
            pltpu.VMEM((D // 2, FF + 128), U32),
            pltpu.VMEM((D // 2, FF + 128), U32),
            pltpu.VMEM((FF // 2, D + 128), U32),
            pltpu.VMEM((D // 2, 2 * D + 128), U32),
            pltpu.VMEM(((NC + 1) * MB, D // 2, 128), U32),
            pltpu.VMEM((D, 128), F32),
            pltpu.VMEM((NC + 1, 8, MC), F32),
            pltpu.VMEM((NSEG, 4, 8, D), BF16),
            pltpu.VMEM((NSEG, 4, 8, D), BF16),
            pltpu.VMEM((NSEG, 4, 8, D), BF16),
            pltpu.VMEM((NSEG, 4, 8, D), BF16),
            pltpu.VMEM((NSEG, 3 * NP, 8, DH), U32),
            pltpu.VMEM((NE, D), BF16),
            pltpu.VMEM((NSEG, 3, 8, D), F32),
            pltpu.VMEM((M + SEG + M, D), F32),
            pltpu.VMEM((8, 2 * D), F32),
            pltpu.VMEM((80, 128), F32),
            pltpu.VMEM((SEG, 128), F32),
            pltpu.VMEM((2, 8, D), BF16),
            pltpu.VMEM((8, 128), U32),
            pltpu.VMEM((NP, 4, 80, DH), BF16),
            pltpu.VMEM((3, NE, 2 * DH), F32),
            pltpu.VMEM((M, D), BF16),
            pltpu.VMEM((D,), BF16),
            pltpu.VMEM((1, D), BF16),
            pltpu.SemaphoreType.DMA((16 + NP + NC,)),
            pltpu.SemaphoreType.DMA((2,)),
        ],
        compiler_params=pltpu.CompilerParams(vmem_limit_bytes=120 * 1024 * 1024,
                                             disable_bounds_checks=True,
                                             disable_semaphore_checks=True),
    )(
        A_x.reshape(NSEG, 4, 8, D),
        A_mem0.reshape(M, D),
        A_Wq.reshape(D // 2, 2, H, DH),
        A_Wk.reshape(D // 2, 2, H, DH),
        A_Wv.reshape(D // 2, 2, H, DH),
        A_Wo.reshape(H * DH, D),
        B_w_r,
        B_w_gate,
        B_w_up,
        B_w_down,
        c,
        w_mod,
    )
    return out.reshape(1, NSEG * SEG, D)
```

```python
import jax
import jax.numpy as jnp
import jax.experimental.pallas as pl
import jax.experimental.pallas.tpu as pltpu

F32 = jnp.float32
BF16 = jnp.bfloat16
U32 = jnp.uint32

D = 1024
H = 32
DH = 128
NP = H // 2
M = 8
SEG = 32
NSEG = 64
FF = 3584
NJ = SEG - M
NE = NSEG * M
EPS = 1.0013580322265625e-05
SCALE = DH ** (-0.5)
NEG = -1000000000.0
LOG2E = 1.4426950408889634
KQ = 256
NG = 8
UNROLL = 2
NIT = NSEG // (2 * UNROLL)
OUT_SPLIT = NSEG - 2 * UNROLL - 2


def _rb(x):
    return x.astype(BF16).astype(F32)


def _layernorm(xf):
    m = jnp.mean(xf, axis=-1, keepdims=True)
    d = xf - m
    v = jnp.mean(d * d, axis=-1, keepdims=True)
    std = _rb(jnp.sqrt(_rb(_rb(v) + EPS)))
    return _rb(xf - _rb(m)) * (1.0 / std)


def _sigmoid(x):
    return _rb(1.0 / _rb(1.0 + _rb(jnp.exp(-x))))


def _dot(a, b):
    return jnp.dot(a, b, preferred_element_type=F32)


def _dot_nt(a, b):
    return jax.lax.dot_general(a, b, (((1,), (1,)), ((), ())), preferred_element_type=F32)


def _kernel(x_hbm, mem0_hbm, wq_hbm, wk_hbm, wv_hbm, wo_hbm, wr_hbm, wg_hbm, wu_hbm, wd_hbm,
            c_hbm, wm_hbm,
            out_hbm,
            wq, wk, wv, wo, wg, wu, wd, wm, cb, xv, x1v, h2v, outv, early, he, hj, pend,
            mod, fill, keys, patch, zero, opnd, acc0, mem0_ref, wr_ref, c_ref,
            sem, sem_out):
    w_u32 = [w.bitcast(U32) for w in (wq_hbm, wk_hbm, wv_hbm)]
    wqkv = (wq, wk, wv)
    wo_hbm, wg_hbm, wu_hbm, wd_hbm, wm_hbm = [
        w.bitcast(U32) for w in (wo_hbm, wg_hbm, wu_hbm, wd_hbm, wm_hbm)]

    def wblk(w, j):
        return pltpu.bitcast(w[:, j * 128:(j + 1) * 128], BF16)

    def wo_blk(n, lo, hi):
        return pltpu.bitcast(wo[n, lo // 2:hi // 2, :], BF16)

    def w_copies(m, p, k):
        return [pltpu.make_async_copy(w_u32[m].at[:, par, p, :], wqkv[m].at[2 * p + par], sem.at[k])
                for par in range(2)]

    def col_copy(src, dst, j, k):
        lo = j * 128 if isinstance(j, int) else pl.multiple_of(j * 128, 128)
        return pltpu.make_async_copy(src.at[:, pl.ds(lo, 128)], dst.at[j], sem.at[k])

    def units(g):
        return [(0, 2 * g), (1, 2 * g), (2, NG + g), (0, 2 * g + 1), (1, 2 * g + 1)]

    def group_copies(g):
        segs = pl.ds(8 * g, 8)
        return (sum([w_copies(m, p, 16 + g) for m, p in units(g)], [])
                + [pltpu.make_async_copy(x_hbm.at[segs, 0:3], xv.at[segs, 0:3], sem.at[16 + g])])

    def wm1_blocks(j):
        return [2 * j, 2 * j + 1, 8 + 2 * j, 8 + 2 * j + 1]

    def wm1_copies(j):
        return [col_copy(wm_hbm, wm, b, 1 + j) for b in wm1_blocks(j)]

    def wm2_copies(t):
        return [col_copy(wm_hbm, wm, 16 + 8 * t + b, 16 + NG + t) for b in range(8)]

    def v2_copies(i):
        return w_copies(2, 4 + 2 * i, 8 + i) + w_copies(2, 5 + 2 * i, 8 + i)

    cp_c = pltpu.make_async_copy(c_hbm, c_ref, sem.at[5])
    cp_xe = pltpu.make_async_copy(x_hbm.at[:, 3], xv.at[:, 3], sem.at[0])
    cp_v0 = w_copies(2, 0, 6) + w_copies(2, 1, 6) + w_copies(2, 2, 6)
    cp_v3 = w_copies(2, 3, 7)
    cp_small = [pltpu.make_async_copy(mem0_hbm, mem0_ref, sem.at[14]),
                pltpu.make_async_copy(wr_hbm, wr_ref, sem.at[15])]
    cp_ffn = [pltpu.make_async_copy(wg_hbm, wg.at[:, 0:FF], sem.at[11]),
              pltpu.make_async_copy(wu_hbm, wu.at[:, 0:FF], sem.at[12]),
              pltpu.make_async_copy(wd_hbm, wd.at[:, 0:D], sem.at[13])]

    for cp in ([cp_c, cp_xe] + cp_v0 + sum([wm1_copies(j) for j in range(D // KQ)], []) + cp_v3
               + v2_copies(0) + v2_copies(1) + group_copies(0) + group_copies(1) + cp_small):
        cp.start()

    ri = jax.lax.broadcasted_iota(jnp.int32, (80, 128), 0)
    ci = jax.lax.broadcasted_iota(jnp.int32, (80, 128), 1)

    def head_of(i):
        return jnp.where(i < 64, i >> 5, (i - 64) >> 3)

    def pos_of(i):
        return jnp.where(i < 64, i & 31, 32 + (i & 7))

    same = (head_of(ri) == head_of(ci)) & (ci < 80)
    allowed = (pos_of(ri) < M) | (pos_of(ri) >= pos_of(ci))
    fill[...] = jnp.where(same, jnp.where(allowed, 0.0, NEG / SCALE), -jnp.inf).astype(F32)
    keys[...] = jnp.zeros(keys.shape, F32)
    pend[M:, :] = jnp.zeros((SEG + M, D), F32)
    zero[...] = jnp.zeros(zero.shape, U32)

    def pin_zero(vals):
        acc = None
        for v in vals:
            v = pltpu.bitcast(v, U32)
            for r in range(0, v.shape[0], 8):
                acc = v[r:r + 8] if acc is None else acc | v[r:r + 8]
        return acc & zero[...]

    cp_xe.wait()
    cp_c.wait()
    cf = c_ref[...].astype(F32)
    sc = _rb(cf * _sigmoid(cf))
    cb[...] = jnp.broadcast_to(sc, (128, D)).T
    sc = jnp.broadcast_to(sc, (16, D)).astype(BF16)

    def mod_vec(k):
        return jnp.concatenate([mod[8 * k + b] for b in range(8)], axis=1)

    def mod_block_vpu(src, dst, is_scale):
        acc = None
        for r in range(0, D // 2, 8):
            w = wm[src, r:r + 8, :]
            term = (pltpu.bitcast(w << 16, F32) * cb[pl.ds(2 * r, 8, stride=2), :]
                    + pltpu.bitcast(w & U32(0xFFFF0000), F32) * cb[pl.ds(2 * r + 1, 8, stride=2), :])
            acc = term if acc is None else acc + term
        v = _rb(jnp.broadcast_to(jnp.sum(acc, axis=0, keepdims=True), (8, 128)))
        v = jnp.where(is_scale, _rb(1.0 + v), v)
        mod[dst] = v
        return v

    def ne_body(i, carry):
        n = _layernorm(xv[pl.ds(i * 16, 16), 3].astype(F32)).reshape(128, D).astype(BF16)
        for j in range(D // KQ):
            he[j, pl.ds(pl.multiple_of(i * 128, 128), 128), :] = n[:, j * KQ:(j + 1) * KQ]
        return carry

    jax.lax.fori_loop(0, NSEG // 16, ne_body, 0)

    def w_head(m, h, lo=0, hi=D):
        return pltpu.bitcast(wqkv[m][h, lo // 2:hi // 2, :], BF16)

    def relayout(m, p):
        w = wqkv[m]
        e = w[2 * p]
        o = w[2 * p + 1]
        w[2 * p] = (e & U32(0xFFFF)) | (o << 16)
        w[2 * p + 1] = (e >> 16) | (o & U32(0xFFFF0000))

    def store_early(m, p, row0, r1, r2):
        ns = r1.shape[0] // 8
        r12 = jnp.concatenate([r1.reshape(ns, 8, DH), r2.reshape(ns, 8, DH)], axis=1)
        v = pltpu.bitcast(r12.reshape(16 * ns, DH).astype(BF16), U32)
        early[row0 // 8:row0 // 8 + ns, m * NP + p] = v.reshape(ns, 8, DH)
        return v

    for cp in cp_v0:
        cp.wait()

    def relayout_body(p, carry):
        relayout(2, p)
        return carry

    jax.lax.fori_loop(0, 3, relayout_body, 0)

    def chunk_body(j, carry):
        for cp in wm1_copies(j):
            cp.wait()
        mv = [_rb(_dot(sc, pltpu.bitcast(wm[b], BF16))[0:8]) for b in wm1_blocks(j)]
        mv = mv[0:2] + [_rb(1.0 + v) for v in mv[2:4]]
        for b, v in zip(wm1_blocks(j), mv):
            mod[b] = v
        shift = jnp.concatenate(mv[0:2], axis=1)
        scale = jnp.concatenate(mv[2:4], axis=1)
        krows = pl.ds(pl.multiple_of(j * (KQ // 2), KQ // 2), KQ // 2)
        for c in range(2):
            rows = slice(c * 256, (c + 1) * 256)
            n = he[j, rows, :].astype(F32).reshape(32, 8, KQ)
            h = (_rb(n * scale) + shift).reshape(256, KQ)
            he[j, rows, :] = h.astype(BF16)
            hb = h.astype(BF16)
            for p in range(3):
                w2 = jnp.concatenate([wv[2 * p, krows, :], wv[2 * p + 1, krows, :]], axis=1)
                acc0[p, rows, :] = (_dot(hb, pltpu.bitcast(w2, BF16))
                                    + jnp.where(j > 0, acc0[p, rows, :], 0.0))
        return carry

    jax.lax.fori_loop(0, D // KQ, chunk_body, 0)

    def early_proj(m, p, pins=None):
        relayout(m, p)
        for c in range(2):
            rows = slice(c * 256, (c + 1) * 256)
            hc = jnp.concatenate([he[j, rows, :] for j in range(D // KQ)], axis=1)
            r12 = []
            for b in range(2):
                wv_ = wqkv[m][2 * p + b]
                if pins and pins.get(2 * c + b):
                    wv_ = jnp.concatenate([wv_[0:8] | pin_zero(pins[2 * c + b]), wv_[8:]], axis=0)
                r12.append(_dot(hc, pltpu.bitcast(wv_, BF16)))
            store_early(m, p, c * 256, *r12)

    for cp in group_copies(2) + wm2_copies(0):
        cp.start()
    for cp in cp_v3:
        cp.wait()
    fin = [store_early(2, p, 0, acc0[p, :, 0:DH], acc0[p, :, DH:2 * DH]) for p in range(3)]
    early_proj(2, 3, {i + 1: [fin[i]] for i in range(3)})

    def v2_body(i, carry):
        for cp in v2_copies(i):
            cp.wait()
        early_proj(2, 4 + 2 * i)
        early_proj(2, 5 + 2 * i)
        return carry

    jax.lax.fori_loop(0, 2, v2_body, 0)

    def make_hj(s):
        n = _rb(_layernorm(xv[s, 0:3].astype(F32)))
        h = _rb(n * mod_vec(1)) + mod_vec(0)
        hj[s] = h
        return [h[g, :, 0:128] for g in range(3)]

    def pro_body(g, carry):
        late = g >= NG - 4

        @pl.when(late)
        def _():
            for cp in wm2_copies(g - (NG - 4)):
                cp.wait()

        for cp in group_copies(g):
            cp.wait()
        lnp = sum([make_hj(g * 8 + t) for t in range(8)], [])
        first = 16 + 8 * (g - (NG - 4))
        mv = [mod_block_vpu(jnp.where(late, first + b, b), jnp.where(late, first + b, 48 + b),
                            g == NG - 2) for b in range(8)]
        sites = {i: [] for i in range(20)}
        for i, v in zip(sorted(list(range(2, 20)) + [3, 7, 11, 15, 18, 19]), lnp):
            sites[i].append(v)
        for i, v in zip((1, 4, 6, 8, 10, 12, 14, 16), mv):
            sites[i].append(v)
        for u, (m, p) in enumerate(units(g)):
            early_proj(m, p, {i: sites[4 * u + i] for i in range(4)})

        def start_if(cond, cps):
            for cp in cps:
                pl.when(cond)(cp.start)

        start_if(g + 3 < NG, group_copies(jnp.minimum(g + 3, NG - 1)))
        start_if(g < 3, wm2_copies(jnp.minimum(g + 1, 3)))
        n0 = 2 * jnp.clip(g - 2, 0, 3)
        start_if((g >= 2) & (g < 6), [col_copy(wo_hbm, wo, n0 + b, 10) for b in range(2)])
        return carry

    jax.lax.fori_loop(0, NG, pro_body, 0)

    for cp in cp_ffn:
        cp.start()
    for cp in cp_small + [col_copy(wo_hbm, wo, n, 10) for n in range(8)]:
        cp.wait()
    pend[0:M, :] = mem0_ref[...].astype(F32)

    wr = jnp.broadcast_to(wr_ref[...].astype(F32).reshape(1, D), (8, D))

    lane8 = jax.lax.broadcasted_iota(jnp.int32, (8, 128), 1)
    sub8 = jax.lax.broadcasted_iota(jnp.int32, (8, 128), 0)
    LAST = NSEG * SEG - 1

    def post(s, g0, g1, attn, record=True):
        attn = attn.reshape(g1 - g0, 8, D)
        x1 = _rb(xv[s, g0:g1].astype(F32) + _rb(mod_vec(2) * _rb(attn)))
        n = _rb(_layernorm(x1))
        h2 = _rb(_rb(n * mod_vec(4)) + mod_vec(3))
        r = _rb(jnp.sum(h2 * wr, axis=-1, keepdims=True)) + 0.0
        x1v[s, g0:g1] = x1.astype(BF16)
        h2v[s, g0:g1] = h2.astype(BF16)
        outv[s, g0:g1] = (x1 + _rb(mod_vec(5) * h2)).astype(BF16)
        pins = []
        for g in range(g0, g1):
            bits = pltpu.bitcast(jnp.broadcast_to(r[g - g0], (8, 128)), jnp.int32)
            hi = jax.lax.shift_right_logical(bits, 16)
            code = jnp.where(bits < 0, hi ^ 0xFFFF, hi | 0x8000)
            key = (code << 11) | (LAST - (s * SEG + g * 8) - sub8) | 0x40000000
            key = pltpu.bitcast(key, F32)
            if record:
                rows = slice(g * 8, (g + 1) * 8)
                keys[rows, :] = jnp.where(lane8 == s, key, keys[rows, :])
            pins.append(key)
        return pins

    def post_pair(a, rows, record=True):
        return post(a + 1, 0, 4, rows[0:SEG], record) + post(a, 3, 4, rows[SEG:], record)

    zpad = jnp.zeros((48, DH), BF16)
    G = 4
    KA = (NP - G) * 2 * DH
    KS = D - 128

    def segment(s, lhs, lhs_split, extra, pins):
        scales = {}

        def stash(p, m, v):
            opnd[p, m, 0:v.shape[0], :] = v.astype(BF16)

        def qkv_group(p):
            keys = [(m, 2 * p + b) for m in range(3) for b in range(2 * G)]
            nsplit = 6 if (p == 0 and lhs_split is not None) else 0
            part = [_dot(lhs_split[0], w_head(m, h, 0, KS)) for m, h in keys[:nsplit]]
            full = [_dot(lhs_split[1], w_head(m, h, KS, D)) + part[i]
                    for i, (m, h) in enumerate(keys[:nsplit])]
            full += [_dot(lhs, w_head(m, h)) for m, h in keys[nsplit:]]
            for m in range(3):
                for t in range(G):
                    i = 2 * G * m + 2 * t
                    stash(p + t, m, jnp.concatenate([full[i], full[i + 1]], axis=0))

        def operand(p, m):
            parts = [opnd[p, m, 0:64, :], pltpu.bitcast(early[s, m * NP + p], BF16)]
            if m > 0:
                parts.append(zpad)
            return jnp.concatenate(parts, axis=0)

        def scores(p):
            sc_ = _dot_nt(operand(p, 0), operand(p, 1))
            f = fill[...]
            if pins.get(p):
                f = jnp.concatenate([f[0:8] + pltpu.bitcast(pin_zero(pins[p]), F32), f[8:]], axis=0)
            sc_ = jnp.where(f == 0.0, sc_, f)
            mx = jnp.max(sc_, axis=-1, keepdims=True)
            e = jnp.exp2((sc_ - mx) * (SCALE * LOG2E))
            inv = pl.reciprocal(jnp.sum(e, axis=-1, keepdims=True), approx=True)
            if p // G == NP // G - 2:
                stash(p, 3, e * inv)
            else:
                stash(p, 3, e)
                scales[p] = inv

        oe = []

        def pv(p):
            o = _dot(opnd[p, 3], operand(p, 2))
            if p in scales:
                o = o * scales[p]
                pins.setdefault(p + G, []).append(o)
            res = []
            for b in range(2):
                rows, erows = o[32 * b:32 * b + 32], o[64 + 8 * b:72 + 8 * b]
                oe.append(erows)
                if extra is not None:
                    rows = jnp.concatenate([rows, erows, extra[2 * p + b]], axis=0)
                res.append(rows)
            return res

        os_ = []
        for p in range(0, NP, G):
            qkv_group(p)
            if p >= G:
                for t in range(G):
                    os_ += pv(p - G + t)
            for t in range(G):
                scores(p + t)
        oa = jnp.concatenate(os_, axis=1).astype(BF16)
        acc, ob = [], []
        for n in range(7):
            acc.append(_dot(oa, wo_blk(n, 0, KA)))
            if n == 1:
                for t in range(G):
                    ob += pv(NP - G + t)
        ob = jnp.concatenate(ob, axis=1).astype(BF16)
        res = [_dot(ob, wo_blk(n, KA, H * DH)) + acc[n] for n in range(7)]
        res.append(_dot(ob, wo_blk(7, KA, H * DH)) + _dot(oa, wo_blk(7, 0, KA)))
        return res, oe

    def make_lhs(mem, s):
        return jnp.concatenate([mem, hj[s].reshape(NJ, D)], axis=0)

    cp_o1 = pltpu.make_async_copy(outv.at[0:OUT_SPLIT], out_hbm.at[0:OUT_SPLIT], sem_out.at[0])
    cp_o2 = pltpu.make_async_copy(outv.at[OUT_SPLIT:NSEG], out_hbm.at[OUT_SPLIT:NSEG],
                                  sem_out.at[1])

    def split_lhs(lhs):
        return lhs.astype(BF16), (lhs[:, :KS].astype(BF16), lhs[:, KS:].astype(BF16))

    def step(i, carry):
        @pl.when(i == NIT - 1)
        def _():
            cp_o1.start()

        prev = pend[...]
        for u in range(UNROLL):
            a = 2 * (UNROLL * i + u)
            pins = post_pair(jnp.maximum(a - 2, 0) if u == 0 else a - 2, prev[M:])
            lhs_a = make_lhs(prev[0:M], a)
            lhs_a = (lhs_a.astype(BF16), None) if u == 0 else split_lhs(lhs_a)
            res_a, oe_a = segment(a, *lhs_a, None,
                                  {k: [v] for k, v in zip((3, 7, 11, 15), pins[:4])})
            res_a = jnp.concatenate(res_a, axis=1)
            pins = pins[4:] + post(a, 0, 3, res_a[M:])
            res_b, _ = segment(a + 1, *split_lhs(make_lhs(res_a[0:M], a + 1)), oe_a,
                               {k: [v] for k, v in zip((3, 7, 11, 15), pins)})
            prev = jnp.concatenate(res_b, axis=1)
        pend[...] = prev
        return carry

    jax.lax.fori_loop(0, NIT, step, 0)
    for cp in cp_ffn:
        cp.wait()
    last_keys = post_pair(NSEG - 2, pend[M:, :], record=False)
    cp_o2.start()

    def max_all(v):
        return jnp.max(jnp.max(v, axis=0, keepdims=True), axis=1, keepdims=True)

    def decode(k):
        kb = pltpu.bitcast(jnp.broadcast_to(k, (8, 128)), jnp.int32)
        code = (kb >> 11) & 0xFFFF
        hi = jnp.where(code >= 0x8000, code & 0x7FFF, code ^ 0xFFFF)
        tok = jnp.clip((LAST - (kb & LAST))[0, 0], 0, LAST)
        return tok, pltpu.bitcast(hi << 16, F32)[:, 0:1]

    kv = keys[...]
    o1 = max_all(kv)
    o2 = max_all(jnp.where(kv == o1, 0.0, kv))
    kv = jnp.concatenate(last_keys + [jnp.where(sub8 < 4, o1, o2)], axis=0)
    k1 = jnp.max(kv, axis=0, keepdims=True)
    k2 = jnp.max(jnp.where(kv == k1, 0.0, kv), axis=0, keepdims=True)
    i1, r1 = decode(k1)
    i2, r2 = decode(k2)
    g1, g2 = i1 >> 3, i2 >> 3

    def rows_of(ref):
        return jnp.concatenate([ref[g1 >> 2, pl.ds(g1 & 3, 1)], ref[g2 >> 2, pl.ds(g2 & 3, 1)]],
                               axis=0).astype(F32)

    x1, h2 = rows_of(x1v), rows_of(h2v)
    hl = h2.reshape(16, D).astype(BF16)
    act = []
    for j in range(FF // 128):
        gt = _rb(_dot(hl, wblk(wg, j)))
        up = _rb(_dot(hl, wblk(wu, j)))
        act.append((_rb(gt * _sigmoid(gt)) * up).astype(BF16))
    act = jnp.concatenate(act, axis=1)
    y = jnp.concatenate([_dot(act, wblk(wd, n)) for n in range(8)], axis=1).reshape(2, 8, D)
    rowi = jax.lax.broadcasted_iota(jnp.int32, (2, 8, 1), 1)
    gsel = jax.lax.broadcasted_iota(jnp.int32, (2, 8, 1), 0)
    tokp = jnp.where(gsel == 0, g1, g2) * 8 + rowi
    gate = _sigmoid(jnp.where(tokp == i1, r1[None], r2[None]))
    upd = jnp.where((tokp == i1) | (tokp == i2), _rb(_rb(y) * gate), 0.0)
    patch[...] = (x1 + _rb(mod_vec(5) * _rb(h2 + upd))).astype(BF16)
    cp_o1.wait()
    cp_o2.wait()
    cp1 = pltpu.make_async_copy(patch.at[0], out_hbm.at[g1 >> 2, g1 & 3], sem_out.at[0])
    cp1.start()

    @pl.when(g1 != g2)
    def _():
        cp2 = pltpu.make_async_copy(patch.at[1], out_hbm.at[g2 >> 2, g2 & 3], sem_out.at[1])
        cp2.start()
        cp2.wait()

    cp1.wait()


@jax.jit
def pallas_adaLN_cond__memory_aug_recurrent_mem_tr__moe_arch_mod__prompt_kernel(
    A_x: jax.Array,
    A_mem0: jax.Array,
    A_Wq: jax.Array,
    A_Wk: jax.Array,
    A_Wv: jax.Array,
    A_Wo: jax.Array,
    A_seg_len,
    B_x: jax.Array,
    B_w_r: jax.Array,
    B_w_gate: jax.Array,
    B_w_up: jax.Array,
    B_w_down: jax.Array,
    c: jax.Array,
    w_mod: jax.Array,
):
    assert A_x.shape == (1, NSEG * SEG, D)
    any_spec = pl.BlockSpec(memory_space=pl.ANY)
    out = pl.pallas_call(
        _kernel,
        out_shape=jax.ShapeDtypeStruct((NSEG, 4, 8, D), BF16),
        in_specs=[any_spec] * 12,
        out_specs=any_spec,
        scratch_shapes=[
            pltpu.VMEM((H, D // 2, DH), U32),
            pltpu.VMEM((H, D // 2, DH), U32),
            pltpu.VMEM((H, D // 2, DH), U32),
            pltpu.VMEM((8, H * DH // 2, 128), U32),
            pltpu.VMEM((D // 2, FF + 128), U32),
            pltpu.VMEM((D // 2, FF + 128), U32),
            pltpu.VMEM((FF // 2, D + 128), U32),
            pltpu.VMEM((48, D // 2, 128), U32),
            pltpu.VMEM((D, 128), F32),
            pltpu.VMEM((NSEG, 4, 8, D), BF16),
            pltpu.VMEM((NSEG, 4, 8, D), BF16),
            pltpu.VMEM((NSEG, 4, 8, D), BF16),
            pltpu.VMEM((NSEG, 4, 8, D), BF16),
            pltpu.VMEM((NSEG, 3 * NP, 8, DH), U32),
            pltpu.VMEM((D // KQ, NE, KQ), BF16),
            pltpu.VMEM((NSEG, 3, 8, D), F32),
            pltpu.VMEM((M + SEG + M, D), F32),
            pltpu.VMEM((48 + 8, 8, 128), F32),
            pltpu.VMEM((80, 128), F32),
            pltpu.VMEM((SEG, 128), F32),
            pltpu.VMEM((2, 8, D), BF16),
            pltpu.VMEM((8, 128), U32),
            pltpu.VMEM((NP, 4, 80, DH), BF16),
            pltpu.VMEM((3, NE, 2 * DH), F32),
            pltpu.VMEM((M, D), BF16),
            pltpu.VMEM((D,), BF16),
            pltpu.VMEM((1, D), BF16),
            pltpu.SemaphoreType.DMA((16 + NG + 4,)),
            pltpu.SemaphoreType.DMA((2,)),
        ],
        compiler_params=pltpu.CompilerParams(vmem_limit_bytes=120 * 1024 * 1024,
                                             disable_bounds_checks=True,
                                             disable_semaphore_checks=True),
    )(
        A_x.reshape(NSEG, 4, 8, D),
        A_mem0.reshape(M, D),
        A_Wq.reshape(D // 2, 2, H, DH),
        A_Wk.reshape(D // 2, 2, H, DH),
        A_Wv.reshape(D // 2, 2, H, DH),
        A_Wo.reshape(H * DH, D),
        B_w_r,
        B_w_gate,
        B_w_up,
        B_w_down,
        c,
        w_mod,
    )
    return out.reshape(1, NSEG * SEG, D)
```

```python
import jax
import jax.numpy as jnp
import jax.experimental.pallas as pl
import jax.experimental.pallas.tpu as pltpu

F32 = jnp.float32
BF16 = jnp.bfloat16
U32 = jnp.uint32

D = 1024
H = 32
DH = 128
NP = H // 2
M = 8
SEG = 32
NSEG = 64
FF = 3584
NJ = SEG - M
NE = NSEG * M
EPS = 1.0013580322265625e-05
SCALE = DH ** (-0.5)
NEG = -1000000000.0
LOG2E = 1.4426950408889634
KQ = 256
NG = 8
UNROLL = 2
NIT = NSEG // (2 * UNROLL)
OUT_SPLIT = NSEG - 2 * UNROLL - 2


def _rb(x):
    return x.astype(BF16).astype(F32)


def _layernorm(xf):
    m = jnp.mean(xf, axis=-1, keepdims=True)
    d = xf - m
    v = jnp.mean(d * d, axis=-1, keepdims=True)
    std = _rb(jnp.sqrt(_rb(_rb(v) + EPS)))
    return _rb(xf - _rb(m)) * (1.0 / std)


def _sigmoid(x):
    return _rb(1.0 / _rb(1.0 + _rb(jnp.exp(-x))))


def _dot(a, b):
    return jnp.dot(a, b, preferred_element_type=F32)


def _dot_nt(a, b):
    return jax.lax.dot_general(a, b, (((1,), (1,)), ((), ())), preferred_element_type=F32)


def _kernel(x_hbm, mem0_hbm, wq_hbm, wk_hbm, wv_hbm, wo_hbm, wr_hbm, wg_hbm, wu_hbm, wd_hbm,
            c_hbm, wm_hbm,
            out_hbm,
            wq, wk, wv, wo, wg, wu, wd, wm, cb, xv, x1v, h2v, outv, early, he, hj, pend,
            mod, fill, keys, patch, zero, opnd, acc0, mem0_ref, wr_ref, c_ref,
            sem, sem_out):
    w_u32 = [w.bitcast(U32) for w in (wq_hbm, wk_hbm, wv_hbm)]
    wqkv = (wq, wk, wv)
    wo_hbm, wg_hbm, wu_hbm, wd_hbm, wm_hbm = [
        w.bitcast(U32) for w in (wo_hbm, wg_hbm, wu_hbm, wd_hbm, wm_hbm)]

    def wblk(w, j):
        return pltpu.bitcast(w[:, j * 128:(j + 1) * 128], BF16)

    def wo_blk(n, lo, hi):
        return pltpu.bitcast(wo[n, lo // 2:hi // 2, :], BF16)

    def w_copies(m, p, k):
        return [pltpu.make_async_copy(w_u32[m].at[:, par, p, :], wqkv[m].at[2 * p + par], sem.at[k])
                for par in range(2)]

    def col_copy(src, dst, j, k):
        lo = j * 128 if isinstance(j, int) else pl.multiple_of(j * 128, 128)
        return pltpu.make_async_copy(src.at[:, pl.ds(lo, 128)], dst.at[j], sem.at[k])

    def units(g):
        return [(0, 2 * g), (1, 2 * g), (2, NG + g), (0, 2 * g + 1), (1, 2 * g + 1)]

    def group_copies(g):
        segs = pl.ds(8 * g, 8)
        return (sum([w_copies(m, p, 16 + g) for m, p in units(g)], [])
                + [pltpu.make_async_copy(x_hbm.at[segs, 0:3], xv.at[segs, 0:3], sem.at[16 + g])])

    def wm1_blocks(j):
        return [2 * j, 2 * j + 1, 8 + 2 * j, 8 + 2 * j + 1]

    def wm1_copies(j):
        return [col_copy(wm_hbm, wm, b, 1 + j) for b in wm1_blocks(j)]

    def wm2_copies(t):
        return [col_copy(wm_hbm, wm, 16 + 8 * t + b, 16 + NG + t) for b in range(8)]

    cp_c = pltpu.make_async_copy(c_hbm, c_ref, sem.at[5])
    cp_xe = pltpu.make_async_copy(x_hbm.at[:, 3], xv.at[:, 3], sem.at[0])
    cp_v0 = w_copies(2, 0, 6) + w_copies(2, 1, 6) + w_copies(2, 2, 6)
    cp_v3 = w_copies(2, 3, 7) + w_copies(2, 4, 7)
    cp_v5 = w_copies(2, 5, 8) + w_copies(2, 6, 8) + w_copies(2, 7, 8)
    cp_small = [pltpu.make_async_copy(mem0_hbm, mem0_ref, sem.at[14]),
                pltpu.make_async_copy(wr_hbm, wr_ref, sem.at[15])]
    cp_ffn = [pltpu.make_async_copy(wg_hbm, wg.at[:, 0:FF], sem.at[11]),
              pltpu.make_async_copy(wu_hbm, wu.at[:, 0:FF], sem.at[12]),
              pltpu.make_async_copy(wd_hbm, wd.at[:, 0:D], sem.at[13])]

    for cp in ([cp_c, cp_xe] + cp_v0 + sum([wm1_copies(j) for j in range(D // KQ)], []) + cp_v3
               + cp_v5 + group_copies(0) + group_copies(1) + cp_small):
        cp.start()

    ri = jax.lax.broadcasted_iota(jnp.int32, (80, 128), 0)
    ci = jax.lax.broadcasted_iota(jnp.int32, (80, 128), 1)

    def head_of(i):
        return jnp.where(i < 64, i >> 5, (i - 64) >> 3)

    def pos_of(i):
        return jnp.where(i < 64, i & 31, 32 + (i & 7))

    same = (head_of(ri) == head_of(ci)) & (ci < 80)
    allowed = (pos_of(ri) < M) | (pos_of(ri) >= pos_of(ci))
    fill[...] = jnp.where(same, jnp.where(allowed, 0.0, NEG / SCALE), -jnp.inf).astype(F32)
    keys[...] = jnp.zeros(keys.shape, F32)
    pend[M:, :] = jnp.zeros((SEG + M, D), F32)
    zero[...] = jnp.zeros(zero.shape, U32)

    def pin_zero(vals):
        acc = None
        for v in vals:
            v = pltpu.bitcast(v, U32)
            for r in range(0, v.shape[0], 8):
                acc = v[r:r + 8] if acc is None else acc | v[r:r + 8]
        return acc & zero[...]

    cp_xe.wait()
    cp_c.wait()
    cf = c_ref[...].astype(F32)
    sc = _rb(cf * _sigmoid(cf))
    cb[...] = jnp.broadcast_to(sc, (128, D)).T
    sc = jnp.broadcast_to(sc, (16, D)).astype(BF16)

    def mod_vec(k):
        return jnp.concatenate([mod[8 * k + b] for b in range(8)], axis=1)

    def mod_block_vpu(src, dst, is_scale):
        acc = None
        for r in range(0, D // 2, 8):
            w = wm[src, r:r + 8, :]
            term = (pltpu.bitcast(w << 16, F32) * cb[pl.ds(2 * r, 8, stride=2), :]
                    + pltpu.bitcast(w & U32(0xFFFF0000), F32) * cb[pl.ds(2 * r + 1, 8, stride=2), :])
            acc = term if acc is None else acc + term
        v = _rb(jnp.broadcast_to(jnp.sum(acc, axis=0, keepdims=True), (8, 128)))
        v = jnp.where(is_scale, _rb(1.0 + v), v)
        mod[dst] = v
        return v

    def ne_body(i, carry):
        n = _layernorm(xv[pl.ds(i * 16, 16), 3].astype(F32)).reshape(128, D).astype(BF16)
        for j in range(D // KQ):
            he[j, pl.ds(pl.multiple_of(i * 128, 128), 128), :] = n[:, j * KQ:(j + 1) * KQ]
        return carry

    jax.lax.fori_loop(0, NSEG // 16, ne_body, 0)

    def w_head(m, h, lo=0, hi=D):
        return pltpu.bitcast(wqkv[m][h, lo // 2:hi // 2, :], BF16)

    def relayout(m, p):
        w = wqkv[m]
        e = w[2 * p]
        o = w[2 * p + 1]
        w[2 * p] = (e & U32(0xFFFF)) | (o << 16)
        w[2 * p + 1] = (e >> 16) | (o & U32(0xFFFF0000))

    def store_early(m, p, row0, r1, r2):
        ns = r1.shape[0] // 8
        r12 = jnp.concatenate([r1.reshape(ns, 8, DH), r2.reshape(ns, 8, DH)], axis=1)
        v = pltpu.bitcast(r12.reshape(16 * ns, DH).astype(BF16), U32)
        early[row0 // 8:row0 // 8 + ns, m * NP + p] = v.reshape(ns, 8, DH)
        return v

    for cp in cp_v0:
        cp.wait()

    def relayout_body(p, carry):
        relayout(2, p)
        return carry

    jax.lax.fori_loop(0, 3, relayout_body, 0)

    def chunk_body(j, carry):
        for cp in wm1_copies(j):
            cp.wait()
        mv = [_rb(_dot(sc, pltpu.bitcast(wm[b], BF16))[0:8]) for b in wm1_blocks(j)]
        mv = mv[0:2] + [_rb(1.0 + v) for v in mv[2:4]]
        for b, v in zip(wm1_blocks(j), mv):
            mod[b] = v
        shift = jnp.concatenate(mv[0:2], axis=1)
        scale = jnp.concatenate(mv[2:4], axis=1)
        krows = pl.ds(pl.multiple_of(j * (KQ // 2), KQ // 2), KQ // 2)
        for c in range(2):
            rows = slice(c * 256, (c + 1) * 256)
            n = he[j, rows, :].astype(F32).reshape(32, 8, KQ)
            h = (_rb(n * scale) + shift).reshape(256, KQ)
            he[j, rows, :] = h.astype(BF16)
            hb = h.astype(BF16)
            for p in range(3):
                w2 = jnp.concatenate([wv[2 * p, krows, :], wv[2 * p + 1, krows, :]], axis=1)
                acc0[p, rows, :] = (_dot(hb, pltpu.bitcast(w2, BF16))
                                    + jnp.where(j > 0, acc0[p, rows, :], 0.0))
        return carry

    jax.lax.fori_loop(0, D // KQ, chunk_body, 0)

    def early_proj(m, p, pins=None):
        relayout(m, p)
        for c in range(2):
            rows = slice(c * 256, (c + 1) * 256)
            hc = jnp.concatenate([he[j, rows, :] for j in range(D // KQ)], axis=1)
            r12 = []
            for b in range(2):
                wv_ = wqkv[m][2 * p + b]
                if pins and pins.get(2 * c + b):
                    wv_ = jnp.concatenate([wv_[0:8] | pin_zero(pins[2 * c + b]), wv_[8:]], axis=0)
                r12.append(_dot(hc, pltpu.bitcast(wv_, BF16)))
            store_early(m, p, c * 256, *r12)

    for cp in group_copies(2) + wm2_copies(0):
        cp.start()
    for cp in cp_v3:
        cp.wait()
    fin = [store_early(2, p, 0, acc0[p, :, 0:DH], acc0[p, :, DH:2 * DH]) for p in range(3)]
    early_proj(2, 3, {i + 1: [fin[i]] for i in range(3)})

    early_proj(2, 4)
    for cp in cp_v5:
        cp.wait()
    for p in range(5, 8):
        early_proj(2, p)

    def make_hj(s):
        n = _rb(_layernorm(xv[s, 0:3].astype(F32)))
        h = _rb(n * mod_vec(1)) + mod_vec(0)
        hj[s] = h
        return [h[g, :, 0:128] for g in range(3)]

    def pro_body(g, carry):
        late = g >= NG - 4

        @pl.when(late)
        def _():
            for cp in wm2_copies(g - (NG - 4)):
                cp.wait()

        for cp in group_copies(g):
            cp.wait()
        lnp = sum([make_hj(g * 8 + t) for t in range(8)], [])
        first = 16 + 8 * (g - (NG - 4))
        mv = [mod_block_vpu(jnp.where(late, first + b, b), jnp.where(late, first + b, 48 + b),
                            g == NG - 2) for b in range(8)]
        sites = {i: [] for i in range(20)}
        for i, v in zip(sorted(list(range(2, 20)) + [3, 7, 11, 15, 18, 19]), lnp):
            sites[i].append(v)
        for i, v in zip((1, 4, 6, 8, 10, 12, 14, 16), mv):
            sites[i].append(v)
        for u, (m, p) in enumerate(units(g)):
            early_proj(m, p, {i: sites[4 * u + i] for i in range(4)})

        def start_if(cond, cps):
            for cp in cps:
                pl.when(cond)(cp.start)

        start_if(g + 3 < NG, group_copies(jnp.minimum(g + 3, NG - 1)))
        start_if(g < 3, wm2_copies(jnp.minimum(g + 1, 3)))
        n0 = 2 * jnp.clip(g - 2, 0, 3)
        start_if((g >= 2) & (g < 6), [col_copy(wo_hbm, wo, n0 + b, 10) for b in range(2)])
        return carry

    jax.lax.fori_loop(0, NG, pro_body, 0)

    for cp in cp_ffn:
        cp.start()
    for cp in cp_small + [col_copy(wo_hbm, wo, n, 10) for n in range(8)]:
        cp.wait()
    pend[0:M, :] = mem0_ref[...].astype(F32)

    wr = jnp.broadcast_to(wr_ref[...].astype(F32).reshape(1, D), (8, D))

    lane8 = jax.lax.broadcasted_iota(jnp.int32, (8, 128), 1)
    sub8 = jax.lax.broadcasted_iota(jnp.int32, (8, 128), 0)
    LAST = NSEG * SEG - 1

    def post(s, g0, g1, attn, record=True):
        attn = attn.reshape(g1 - g0, 8, D)
        x1 = _rb(xv[s, g0:g1].astype(F32) + _rb(mod_vec(2) * _rb(attn)))
        n = _rb(_layernorm(x1))
        h2 = _rb(_rb(n * mod_vec(4)) + mod_vec(3))
        r = _rb(jnp.sum(h2 * wr, axis=-1, keepdims=True)) + 0.0
        x1v[s, g0:g1] = x1.astype(BF16)
        h2v[s, g0:g1] = h2.astype(BF16)
        outv[s, g0:g1] = (x1 + _rb(mod_vec(5) * h2)).astype(BF16)
        pins = []
        for g in range(g0, g1):
            bits = pltpu.bitcast(jnp.broadcast_to(r[g - g0], (8, 128)), jnp.int32)
            hi = jax.lax.shift_right_logical(bits, 16)
            code = jnp.where(bits < 0, hi ^ 0xFFFF, hi | 0x8000)
            key = (code << 11) | (LAST - (s * SEG + g * 8) - sub8) | 0x40000000
            key = pltpu.bitcast(key, F32)
            if record:
                rows = slice(g * 8, (g + 1) * 8)
                keys[rows, :] = jnp.where(lane8 == s, key, keys[rows, :])
            pins.append(key)
        return pins

    def post_pair(a, rows, record=True):
        return post(a + 1, 0, 4, rows[0:SEG], record) + post(a, 3, 4, rows[SEG:], record)

    zpad = jnp.zeros((48, DH), BF16)
    G = 4
    KA = (NP - G) * 2 * DH
    KS = D - 128

    def segment(s, lhs, lhs_split, extra, pins):
        scales = {}

        def stash(p, m, v):
            opnd[p, m, 0:v.shape[0], :] = v.astype(BF16)

        def qkv_group(p):
            keys = [(m, 2 * p + b) for m in range(3) for b in range(2 * G)]
            nsplit = 6 if (p == 0 and lhs_split is not None) else 0
            part = [_dot(lhs_split[0], w_head(m, h, 0, KS)) for m, h in keys[:nsplit]]
            full = [_dot(lhs_split[1], w_head(m, h, KS, D)) + part[i]
                    for i, (m, h) in enumerate(keys[:nsplit])]
            full += [_dot(lhs, w_head(m, h)) for m, h in keys[nsplit:]]
            for m in range(3):
                for t in range(G):
                    i = 2 * G * m + 2 * t
                    stash(p + t, m, jnp.concatenate([full[i], full[i + 1]], axis=0))

        def operand(p, m):
            parts = [opnd[p, m, 0:64, :], pltpu.bitcast(early[s, m * NP + p], BF16)]
            if m > 0:
                parts.append(zpad)
            return jnp.concatenate(parts, axis=0)

        def scores(p):
            sc_ = _dot_nt(operand(p, 0), operand(p, 1))
            f = fill[...]
            if pins.get(p):
                f = jnp.concatenate([f[0:8] + pltpu.bitcast(pin_zero(pins[p]), F32), f[8:]], axis=0)
            sc_ = jnp.where(f == 0.0, sc_, f)
            mx = jnp.max(sc_, axis=-1, keepdims=True)
            e = jnp.exp2((sc_ - mx) * (SCALE * LOG2E))
            inv = pl.reciprocal(jnp.sum(e, axis=-1, keepdims=True), approx=True)
            if p // G == NP // G - 2:
                stash(p, 3, e * inv)
            else:
                stash(p, 3, e)
                scales[p] = inv

        oe = []

        def pv(p):
            o = _dot(opnd[p, 3], operand(p, 2))
            if p in scales:
                o = o * scales[p]
                pins.setdefault(p + G, []).append(o)
            res = []
            for b in range(2):
                rows, erows = o[32 * b:32 * b + 32], o[64 + 8 * b:72 + 8 * b]
                oe.append(erows)
                if extra is not None:
                    rows = jnp.concatenate([rows, erows, extra[2 * p + b]], axis=0)
                res.append(rows)
            return res

        os_ = []
        for p in range(0, NP, G):
            qkv_group(p)
            if p >= G:
                for t in range(G):
                    os_ += pv(p - G + t)
            for t in range(G):
                scores(p + t)
        oa = jnp.concatenate(os_, axis=1).astype(BF16)
        acc, ob = [], []
        for n in range(7):
            acc.append(_dot(oa, wo_blk(n, 0, KA)))
            if n == 1:
                for t in range(G):
                    ob += pv(NP - G + t)
        ob = jnp.concatenate(ob, axis=1).astype(BF16)
        res = [_dot(ob, wo_blk(n, KA, H * DH)) + acc[n] for n in range(7)]
        res.append(_dot(ob, wo_blk(7, KA, H * DH)) + _dot(oa, wo_blk(7, 0, KA)))
        return res, oe

    def make_lhs(mem, s):
        return jnp.concatenate([mem, hj[s].reshape(NJ, D)], axis=0)

    cp_o1 = pltpu.make_async_copy(outv.at[0:OUT_SPLIT], out_hbm.at[0:OUT_SPLIT], sem_out.at[0])
    cp_o2 = pltpu.make_async_copy(outv.at[OUT_SPLIT:NSEG], out_hbm.at[OUT_SPLIT:NSEG],
                                  sem_out.at[1])

    def split_lhs(lhs):
        return lhs.astype(BF16), (lhs[:, :KS].astype(BF16), lhs[:, KS:].astype(BF16))

    def step(i, carry):
        @pl.when(i == NIT - 1)
        def _():
            cp_o1.start()

        prev = pend[...]
        for u in range(UNROLL):
            a = 2 * (UNROLL * i + u)
            pins = post_pair(jnp.maximum(a - 2, 0) if u == 0 else a - 2, prev[M:])
            lhs_a = make_lhs(prev[0:M], a)
            lhs_a = (lhs_a.astype(BF16), None) if u == 0 else split_lhs(lhs_a)
            res_a, oe_a = segment(a, *lhs_a, None,
                                  {k: [v] for k, v in zip((3, 7, 11, 15), pins[:4])})
            res_a = jnp.concatenate(res_a, axis=1)
            pins = pins[4:] + post(a, 0, 3, res_a[M:])
            res_b, _ = segment(a + 1, *split_lhs(make_lhs(res_a[0:M], a + 1)), oe_a,
                               {k: [v] for k, v in zip((3, 7, 11, 15), pins)})
            prev = jnp.concatenate(res_b, axis=1)
        pend[...] = prev
        return carry

    jax.lax.fori_loop(0, NIT, step, 0)
    for cp in cp_ffn:
        cp.wait()
    last_keys = post_pair(NSEG - 2, pend[M:, :], record=False)
    cp_o2.start()

    def max_all(v):
        return jnp.max(jnp.max(v, axis=0, keepdims=True), axis=1, keepdims=True)

    def decode(k):
        kb = pltpu.bitcast(jnp.broadcast_to(k, (8, 128)), jnp.int32)
        code = (kb >> 11) & 0xFFFF
        hi = jnp.where(code >= 0x8000, code & 0x7FFF, code ^ 0xFFFF)
        tok = jnp.clip((LAST - (kb & LAST))[0, 0], 0, LAST)
        return tok, pltpu.bitcast(hi << 16, F32)[:, 0:1]

    kv = keys[...]
    o1 = max_all(kv)
    o2 = max_all(jnp.where(kv == o1, 0.0, kv))
    kv = jnp.concatenate(last_keys + [jnp.where(sub8 < 4, o1, o2)], axis=0)
    k1 = jnp.max(kv, axis=0, keepdims=True)
    k2 = jnp.max(jnp.where(kv == k1, 0.0, kv), axis=0, keepdims=True)
    i1, r1 = decode(k1)
    i2, r2 = decode(k2)
    g1, g2 = i1 >> 3, i2 >> 3

    def rows_of(ref):
        return jnp.concatenate([ref[g1 >> 2, pl.ds(g1 & 3, 1)], ref[g2 >> 2, pl.ds(g2 & 3, 1)]],
                               axis=0).astype(F32)

    x1, h2 = rows_of(x1v), rows_of(h2v)
    hl = h2.reshape(16, D).astype(BF16)
    act = []
    for j in range(FF // 128):
        gt = _rb(_dot(hl, wblk(wg, j)))
        up = _rb(_dot(hl, wblk(wu, j)))
        act.append((_rb(gt * _sigmoid(gt)) * up).astype(BF16))
    act = jnp.concatenate(act, axis=1)
    y = jnp.concatenate([_dot(act, wblk(wd, n)) for n in range(8)], axis=1).reshape(2, 8, D)
    rowi = jax.lax.broadcasted_iota(jnp.int32, (2, 8, 1), 1)
    gsel = jax.lax.broadcasted_iota(jnp.int32, (2, 8, 1), 0)
    tokp = jnp.where(gsel == 0, g1, g2) * 8 + rowi
    gate = _sigmoid(jnp.where(tokp == i1, r1[None], r2[None]))
    upd = jnp.where((tokp == i1) | (tokp == i2), _rb(_rb(y) * gate), 0.0)
    patch[...] = (x1 + _rb(mod_vec(5) * _rb(h2 + upd))).astype(BF16)
    cp_o1.wait()
    cp_o2.wait()
    cp1 = pltpu.make_async_copy(patch.at[0], out_hbm.at[g1 >> 2, g1 & 3], sem_out.at[0])
    cp1.start()

    @pl.when(g1 != g2)
    def _():
        cp2 = pltpu.make_async_copy(patch.at[1], out_hbm.at[g2 >> 2, g2 & 3], sem_out.at[1])
        cp2.start()
        cp2.wait()

    cp1.wait()


@jax.jit
def pallas_adaLN_cond__memory_aug_recurrent_mem_tr__moe_arch_mod__prompt_kernel(
    A_x: jax.Array,
    A_mem0: jax.Array,
    A_Wq: jax.Array,
    A_Wk: jax.Array,
    A_Wv: jax.Array,
    A_Wo: jax.Array,
    A_seg_len,
    B_x: jax.Array,
    B_w_r: jax.Array,
    B_w_gate: jax.Array,
    B_w_up: jax.Array,
    B_w_down: jax.Array,
    c: jax.Array,
    w_mod: jax.Array,
):
    assert A_x.shape == (1, NSEG * SEG, D)
    any_spec = pl.BlockSpec(memory_space=pl.ANY)
    out = pl.pallas_call(
        _kernel,
        out_shape=jax.ShapeDtypeStruct((NSEG, 4, 8, D), BF16),
        in_specs=[any_spec] * 12,
        out_specs=any_spec,
        scratch_shapes=[
            pltpu.VMEM((H, D // 2, DH), U32),
            pltpu.VMEM((H, D // 2, DH), U32),
            pltpu.VMEM((H, D // 2, DH), U32),
            pltpu.VMEM((8, H * DH // 2, 128), U32),
            pltpu.VMEM((D // 2, FF + 128), U32),
            pltpu.VMEM((D // 2, FF + 128), U32),
            pltpu.VMEM((FF // 2, D + 128), U32),
            pltpu.VMEM((48, D // 2, 128), U32),
            pltpu.VMEM((D, 128), F32),
            pltpu.VMEM((NSEG, 4, 8, D), BF16),
            pltpu.VMEM((NSEG, 4, 8, D), BF16),
            pltpu.VMEM((NSEG, 4, 8, D), BF16),
            pltpu.VMEM((NSEG, 4, 8, D), BF16),
            pltpu.VMEM((NSEG, 3 * NP, 8, DH), U32),
            pltpu.VMEM((D // KQ, NE, KQ), BF16),
            pltpu.VMEM((NSEG, 3, 8, D), F32),
            pltpu.VMEM((M + SEG + M, D), F32),
            pltpu.VMEM((48 + 8, 8, 128), F32),
            pltpu.VMEM((80, 128), F32),
            pltpu.VMEM((SEG, 128), F32),
            pltpu.VMEM((2, 8, D), BF16),
            pltpu.VMEM((8, 128), U32),
            pltpu.VMEM((NP, 4, 80, DH), BF16),
            pltpu.VMEM((3, NE, 2 * DH), F32),
            pltpu.VMEM((M, D), BF16),
            pltpu.VMEM((D,), BF16),
            pltpu.VMEM((1, D), BF16),
            pltpu.SemaphoreType.DMA((16 + NG + 4,)),
            pltpu.SemaphoreType.DMA((2,)),
        ],
        compiler_params=pltpu.CompilerParams(vmem_limit_bytes=120 * 1024 * 1024,
                                             disable_bounds_checks=True,
                                             disable_semaphore_checks=True),
    )(
        A_x.reshape(NSEG, 4, 8, D),
        A_mem0.reshape(M, D),
        A_Wq.reshape(D // 2, 2, H, DH),
        A_Wk.reshape(D // 2, 2, H, DH),
        A_Wv.reshape(D // 2, 2, H, DH),
        A_Wo.reshape(H * DH, D),
        B_w_r,
        B_w_gate,
        B_w_up,
        B_w_down,
        c,
        w_mod,
    )
    return out.reshape(1, NSEG * SEG, D)
```

```python
import jax
import jax.numpy as jnp
import jax.experimental.pallas as pl
import jax.experimental.pallas.tpu as pltpu

F32 = jnp.float32
BF16 = jnp.bfloat16
U32 = jnp.uint32

D = 1024
H = 32
DH = 128
NP = H // 2
M = 8
SEG = 32
NSEG = 64
FF = 3584
NJ = SEG - M
NE = NSEG * M
EPS = 1.0013580322265625e-05
SCALE = DH ** (-0.5)
NEG = -1000000000.0
LOG2E = 1.4426950408889634
KQ = 256
NG = 8
UNROLL = 2
NIT = NSEG // (2 * UNROLL)
OUT_SPLIT = NSEG - 2 * UNROLL - 2


def _rb(x):
    return x.astype(BF16).astype(F32)


def _layernorm(xf):
    m = jnp.mean(xf, axis=-1, keepdims=True)
    d = xf - m
    v = jnp.mean(d * d, axis=-1, keepdims=True)
    std = _rb(jnp.sqrt(_rb(_rb(v) + EPS)))
    return _rb(xf - _rb(m)) * (1.0 / std)


def _sigmoid(x):
    return _rb(1.0 / _rb(1.0 + _rb(jnp.exp(-x))))


def _dot(a, b):
    return jnp.dot(a, b, preferred_element_type=F32)


def _dot_nt(a, b):
    return jax.lax.dot_general(a, b, (((1,), (1,)), ((), ())), preferred_element_type=F32)


def _kernel(x_hbm, mem0_hbm, wq_hbm, wk_hbm, wv_hbm, wo_hbm, wr_hbm, wg_hbm, wu_hbm, wd_hbm,
            c_hbm, wm_hbm,
            out_hbm,
            wq, wk, wv, wo, wg, wu, wd, wm, cb, xv, x1v, h2v, outv, early, he, hj, pend,
            mod, fill, keys, patch, zero, opnd, acc0, mem0_ref, wr_ref, c_ref,
            sem, sem_out):
    w_u32 = [w.bitcast(U32) for w in (wq_hbm, wk_hbm, wv_hbm)]
    wqkv = (wq, wk, wv)
    wo_hbm, wg_hbm, wu_hbm, wd_hbm, wm_hbm = [
        w.bitcast(U32) for w in (wo_hbm, wg_hbm, wu_hbm, wd_hbm, wm_hbm)]

    def wblk(w, j):
        return pltpu.bitcast(w[:, j * 128:(j + 1) * 128], BF16)

    def wo_blk(n, lo, hi):
        return pltpu.bitcast(wo[n, lo // 2:hi // 2, :], BF16)

    def w_copies(m, p, k):
        return [pltpu.make_async_copy(w_u32[m].at[:, par, p, :], wqkv[m].at[2 * p + par], sem.at[k])
                for par in range(2)]

    def col_copy(src, dst, j, k):
        lo = j * 128 if isinstance(j, int) else pl.multiple_of(j * 128, 128)
        return pltpu.make_async_copy(src.at[:, pl.ds(lo, 128)], dst.at[j], sem.at[k])

    def units(g):
        return [(0, 2 * g), (1, 2 * g), (2, NG + g), (0, 2 * g + 1), (1, 2 * g + 1)]

    def group_copies(g):
        segs = pl.ds(8 * g, 8)
        return (sum([w_copies(m, p, 16 + g) for m, p in units(g)], [])
                + [pltpu.make_async_copy(x_hbm.at[segs, 0:3], xv.at[segs, 0:3], sem.at[16 + g])])

    def wm1_blocks(j):
        return [2 * j, 2 * j + 1, 8 + 2 * j, 8 + 2 * j + 1]

    def wm1_copies(j):
        return [col_copy(wm_hbm, wm, b, 1 + j) for b in wm1_blocks(j)]

    def wm2_copies(t):
        return [col_copy(wm_hbm, wm, 16 + 8 * t + b, 16 + NG + t) for b in range(8)]

    cp_c = pltpu.make_async_copy(c_hbm, c_ref, sem.at[5])
    cp_xe = pltpu.make_async_copy(x_hbm.at[:, 3], xv.at[:, 3], sem.at[0])
    cp_v0 = w_copies(2, 0, 6) + w_copies(2, 1, 6) + w_copies(2, 2, 6)
    cp_v3 = w_copies(2, 3, 7) + w_copies(2, 4, 7)
    cp_v5 = w_copies(2, 5, 8) + w_copies(2, 6, 8) + w_copies(2, 7, 8)
    cp_small = [pltpu.make_async_copy(mem0_hbm, mem0_ref, sem.at[14]),
                pltpu.make_async_copy(wr_hbm, wr_ref, sem.at[15])]
    cp_ffn = [pltpu.make_async_copy(wg_hbm, wg.at[:, 0:FF], sem.at[11]),
              pltpu.make_async_copy(wu_hbm, wu.at[:, 0:FF], sem.at[12]),
              pltpu.make_async_copy(wd_hbm, wd.at[:, 0:D], sem.at[13])]

    for cp in ([cp_c, cp_xe] + cp_v0 + sum([wm1_copies(j) for j in range(D // KQ)], []) + cp_v3
               + cp_v5 + group_copies(0) + group_copies(1) + cp_small):
        cp.start()

    ri = jax.lax.broadcasted_iota(jnp.int32, (80, 128), 0)
    ci = jax.lax.broadcasted_iota(jnp.int32, (80, 128), 1)

    def head_of(i):
        return jnp.where(i < 64, i >> 5, (i - 64) >> 3)

    def pos_of(i):
        return jnp.where(i < 64, i & 31, 32 + (i & 7))

    same = (head_of(ri) == head_of(ci)) & (ci < 80)
    allowed = (pos_of(ri) < M) | (pos_of(ri) >= pos_of(ci))
    fill[...] = jnp.where(same, jnp.where(allowed, 0.0, NEG / SCALE), -jnp.inf).astype(F32)
    keys[...] = jnp.zeros(keys.shape, F32)
    pend[M:, :] = jnp.zeros((SEG + M, D), F32)
    zero[...] = jnp.zeros(zero.shape, U32)

    def pin_zero(vals):
        acc = None
        for v in vals:
            v = pltpu.bitcast(v, U32)
            for r in range(0, v.shape[0], 8):
                acc = v[r:r + 8] if acc is None else acc | v[r:r + 8]
        return acc & zero[...]

    cp_xe.wait()
    cp_c.wait()
    cf = c_ref[...].astype(F32)
    sc = _rb(cf * _sigmoid(cf))
    cb[0:D, :] = jnp.broadcast_to(sc, (128, D)).T
    cb[D:, :] = jnp.zeros((32, 128), F32)
    sc = jnp.broadcast_to(sc, (16, D)).astype(BF16)

    def mod_vec(k):
        return jnp.concatenate([mod[8 * k + b] for b in range(8)], axis=1)

    def mod_block_vpu(src, dst, is_scale):
        acc = None
        for r in range(0, D // 2, 8):
            w = wm[src, r:r + 8, :]
            term = (pltpu.bitcast(w << 16, F32) * cb[pl.ds(2 * r, 8, stride=2), :]
                    + pltpu.bitcast(w & U32(0xFFFF0000), F32) * cb[pl.ds(2 * r + 1, 8, stride=2), :])
            acc = term if acc is None else acc + term
        v = _rb(jnp.broadcast_to(jnp.sum(acc, axis=0, keepdims=True), (8, 128)))
        v = jnp.where(is_scale, _rb(1.0 + v), v)
        mod[dst] = v
        return v

    def ne_body(i, carry):
        n = _layernorm(xv[pl.ds(i * 16, 16), 3].astype(F32)).reshape(128, D).astype(BF16)
        for j in range(D // KQ):
            he[j, pl.ds(pl.multiple_of(i * 128, 128), 128), :] = n[:, j * KQ:(j + 1) * KQ]
        return carry

    jax.lax.fori_loop(0, NSEG // 16, ne_body, 0)

    def w_head(m, h, lo=0, hi=D):
        return pltpu.bitcast(wqkv[m][h, lo // 2:hi // 2, :], BF16)

    def relayout(m, p):
        w = wqkv[m]
        e = w[2 * p]
        o = w[2 * p + 1]
        w[2 * p] = (e & U32(0xFFFF)) | (o << 16)
        w[2 * p + 1] = (e >> 16) | (o & U32(0xFFFF0000))

    def store_early(m, p, row0, r1, r2):
        ns = r1.shape[0] // 8
        r12 = jnp.concatenate([r1.reshape(ns, 8, DH), r2.reshape(ns, 8, DH)], axis=1)
        v = pltpu.bitcast(r12.reshape(16 * ns, DH).astype(BF16), U32)
        early[row0 // 8:row0 // 8 + ns, m * NP + p] = v.reshape(ns, 8, DH)
        return v

    for cp in cp_v0:
        cp.wait()

    def relayout_body(p, carry):
        relayout(2, p)
        return carry

    jax.lax.fori_loop(0, 3, relayout_body, 0)

    def chunk_body(j, carry):
        for cp in wm1_copies(j):
            cp.wait()
        mv = [_rb(_dot(sc, pltpu.bitcast(wm[b], BF16))[0:8]) for b in wm1_blocks(j)]
        mv = mv[0:2] + [_rb(1.0 + v) for v in mv[2:4]]
        for b, v in zip(wm1_blocks(j), mv):
            mod[b] = v
        shift = jnp.concatenate(mv[0:2], axis=1)
        scale = jnp.concatenate(mv[2:4], axis=1)
        krows = pl.ds(pl.multiple_of(j * (KQ // 2), KQ // 2), KQ // 2)
        for c in range(2):
            rows = slice(c * 256, (c + 1) * 256)
            n = he[j, rows, :].astype(F32).reshape(32, 8, KQ)
            h = (_rb(n * scale) + shift).reshape(256, KQ)
            he[j, rows, :] = h.astype(BF16)
            hb = h.astype(BF16)
            for p in range(3):
                w2 = jnp.concatenate([wv[2 * p, krows, :], wv[2 * p + 1, krows, :]], axis=1)
                acc0[p, rows, :] = (_dot(hb, pltpu.bitcast(w2, BF16))
                                    + jnp.where(j > 0, acc0[p, rows, :], 0.0))
        return carry

    jax.lax.fori_loop(0, D // KQ, chunk_body, 0)

    def early_proj(m, p, pins=None):
        relayout(m, p)
        for c in range(2):
            rows = slice(c * 256, (c + 1) * 256)
            hc = jnp.concatenate([he[j, rows, :] for j in range(D // KQ)], axis=1)
            r12 = []
            for b in range(2):
                wv_ = wqkv[m][2 * p + b]
                if pins and pins.get(2 * c + b):
                    wv_ = jnp.concatenate([wv_[0:8] | pin_zero(pins[2 * c + b]), wv_[8:]], axis=0)
                r12.append(_dot(hc, pltpu.bitcast(wv_, BF16)))
            store_early(m, p, c * 256, *r12)

    for cp in group_copies(2) + wm2_copies(0):
        cp.start()
    for cp in cp_v3:
        cp.wait()
    fin = [store_early(2, p, 0, acc0[p, :, 0:DH], acc0[p, :, DH:2 * DH]) for p in range(3)]
    early_proj(2, 3, {i + 1: [fin[i]] for i in range(3)})

    early_proj(2, 4)
    for cp in cp_v5:
        cp.wait()
    for p in range(5, 8):
        early_proj(2, p)

    def make_hj(s):
        n = _rb(_layernorm(xv[s, 0:3].astype(F32)))
        h = _rb(n * mod_vec(1)) + mod_vec(0)
        hj[s] = h
        return [h[g, :, 0:128] for g in range(3)]

    def pro_body(g, carry):
        late = g >= NG - 4

        @pl.when(late)
        def _():
            for cp in wm2_copies(g - (NG - 4)):
                cp.wait()

        for cp in group_copies(g):
            cp.wait()
        lnp = sum([make_hj(g * 8 + t) for t in range(8)], [])
        first = 16 + 8 * (g - (NG - 4))
        mv = [mod_block_vpu(jnp.where(late, first + b, b), jnp.where(late, first + b, 48 + b),
                            g == NG - 2) for b in range(8)]
        sites = {i: [] for i in range(20)}
        for i, v in zip(sorted(list(range(2, 20)) + [3, 7, 11, 15, 18, 19]), lnp):
            sites[i].append(v)
        for i, v in zip((1, 4, 6, 8, 10, 12, 14, 16), mv):
            sites[i].append(v)
        for u, (m, p) in enumerate(units(g)):
            early_proj(m, p, {i: sites[4 * u + i] for i in range(4)})

        def start_if(cond, cps):
            for cp in cps:
                pl.when(cond)(cp.start)

        start_if(g + 3 < NG, group_copies(jnp.minimum(g + 3, NG - 1)))
        start_if(g < 3, wm2_copies(jnp.minimum(g + 1, 3)))
        n0 = 2 * jnp.clip(g - 2, 0, 3)
        start_if((g >= 2) & (g < 6), [col_copy(wo_hbm, wo, n0 + b, 10) for b in range(2)])
        return carry

    jax.lax.fori_loop(0, NG, pro_body, 0)

    for cp in cp_ffn:
        cp.start()
    for cp in cp_small + [col_copy(wo_hbm, wo, n, 10) for n in range(8)]:
        cp.wait()
    pend[0:M, :] = mem0_ref[...].astype(F32)

    wr = jnp.broadcast_to(wr_ref[...].astype(F32).reshape(1, D), (8, D))

    lane8 = jax.lax.broadcasted_iota(jnp.int32, (8, 128), 1)
    sub8 = jax.lax.broadcasted_iota(jnp.int32, (8, 128), 0)
    LAST = NSEG * SEG - 1

    def post(s, g0, g1, attn, record=True):
        attn = attn.reshape(g1 - g0, 8, D)
        x1 = _rb(xv[s, g0:g1].astype(F32) + _rb(mod_vec(2) * _rb(attn)))
        n = _rb(_layernorm(x1))
        h2 = _rb(_rb(n * mod_vec(4)) + mod_vec(3))
        r = _rb(jnp.sum(h2 * wr, axis=-1, keepdims=True)) + 0.0
        x1v[s, g0:g1] = x1.astype(BF16)
        h2v[s, g0:g1] = h2.astype(BF16)
        outv[s, g0:g1] = (x1 + _rb(mod_vec(5) * h2)).astype(BF16)
        pins = []
        for g in range(g0, g1):
            bits = pltpu.bitcast(jnp.broadcast_to(r[g - g0], (8, 128)), jnp.int32)
            hi = jax.lax.shift_right_logical(bits, 16)
            code = jnp.where(bits < 0, hi ^ 0xFFFF, hi | 0x8000)
            key = (code << 11) | (LAST - (s * SEG + g * 8) - sub8) | 0x40000000
            key = pltpu.bitcast(key, F32)
            if record:
                rows = slice(g * 8, (g + 1) * 8)
                keys[rows, :] = jnp.where(lane8 == s, key, keys[rows, :])
            pins.append(key)
        return pins

    def post_pair(a, rows, record=True):
        return post(a + 1, 0, 4, rows[0:SEG], record) + post(a, 3, 4, rows[SEG:], record)

    zpad = jnp.zeros((48, DH), BF16)
    G = 4
    KA = (NP - G) * 2 * DH
    KS = D - 128

    def segment(s, lhs, lhs_split, extra, pins):
        scales = {}

        def stash(p, m, v):
            opnd[p, m, 0:v.shape[0], :] = v.astype(BF16)

        def qkv_group(p):
            keys = [(m, 2 * p + b) for m in range(3) for b in range(2 * G)]
            nsplit = 6 if (p == 0 and lhs_split is not None) else 0
            part = [_dot(lhs_split[0], w_head(m, h, 0, KS)) for m, h in keys[:nsplit]]
            full = [_dot(lhs_split[1], w_head(m, h, KS, D)) + part[i]
                    for i, (m, h) in enumerate(keys[:nsplit])]
            full += [_dot(lhs, w_head(m, h)) for m, h in keys[nsplit:]]
            for m in range(3):
                for t in range(G):
                    i = 2 * G * m + 2 * t
                    stash(p + t, m, jnp.concatenate([full[i], full[i + 1]], axis=0))

        def operand(p, m):
            parts = [opnd[p, m, 0:64, :], pltpu.bitcast(early[s, m * NP + p], BF16)]
            if m > 0:
                parts.append(zpad)
            return jnp.concatenate(parts, axis=0)

        def scores(p):
            sc_ = _dot_nt(operand(p, 0), operand(p, 1))
            f = fill[...]
            if pins.get(p):
                f = jnp.concatenate([f[0:8] + pltpu.bitcast(pin_zero(pins[p]), F32), f[8:]], axis=0)
            sc_ = jnp.where(f == 0.0, sc_, f)
            mx = jnp.max(sc_, axis=-1, keepdims=True)
            e = jnp.exp2((sc_ - mx) * (SCALE * LOG2E))
            inv = pl.reciprocal(jnp.sum(e, axis=-1, keepdims=True), approx=True)
            if p // G == NP // G - 2:
                stash(p, 3, e * inv)
            else:
                stash(p, 3, e)
                scales[p] = inv

        oe = []

        def pv(p):
            o = _dot(opnd[p, 3], operand(p, 2))
            if p in scales:
                o = o * scales[p]
                pins.setdefault(p + G, []).append(o)
            res = []
            for b in range(2):
                rows, erows = o[32 * b:32 * b + 32], o[64 + 8 * b:72 + 8 * b]
                oe.append(erows)
                if extra is not None:
                    rows = jnp.concatenate([rows, erows, extra[2 * p + b]], axis=0)
                res.append(rows)
            return res

        os_ = []
        for p in range(0, NP, G):
            qkv_group(p)
            if p >= G:
                for t in range(G):
                    os_ += pv(p - G + t)
            for t in range(G):
                scores(p + t)
        oa = jnp.concatenate(os_, axis=1).astype(BF16)
        acc, ob = [], []
        for n in range(7):
            acc.append(_dot(oa, wo_blk(n, 0, KA)))
            if n == 1:
                for t in range(G):
                    ob += pv(NP - G + t)
        ob = jnp.concatenate(ob, axis=1).astype(BF16)
        res = [_dot(ob, wo_blk(n, KA, H * DH)) + acc[n] for n in range(7)]
        res.append(_dot(ob, wo_blk(7, KA, H * DH)) + _dot(oa, wo_blk(7, 0, KA)))
        return res, oe

    def make_lhs(mem, s):
        return jnp.concatenate([mem, hj[s].reshape(NJ, D)], axis=0)

    cp_o1 = pltpu.make_async_copy(outv.at[0:OUT_SPLIT], out_hbm.at[0:OUT_SPLIT], sem_out.at[0])
    cp_o2 = pltpu.make_async_copy(outv.at[OUT_SPLIT:NSEG], out_hbm.at[OUT_SPLIT:NSEG],
                                  sem_out.at[1])

    def split_lhs(lhs):
        return lhs.astype(BF16), (lhs[:, :KS].astype(BF16), lhs[:, KS:].astype(BF16))

    def step(i, carry):
        @pl.when(i == NIT - 1)
        def _():
            cp_o1.start()

        prev = pend[...]
        for u in range(UNROLL):
            a = 2 * (UNROLL * i + u)
            pins = post_pair(jnp.maximum(a - 2, 0) if u == 0 else a - 2, prev[M:])
            lhs_a = make_lhs(prev[0:M], a)
            lhs_a = (lhs_a.astype(BF16), None) if u == 0 else split_lhs(lhs_a)
            res_a, oe_a = segment(a, *lhs_a, None,
                                  {k: [v] for k, v in zip((2, 6, 10, 14), pins[:4])})
            res_a = jnp.concatenate(res_a, axis=1)
            pins = pins[4:] + post(a, 0, 3, res_a[M:])
            res_b, _ = segment(a + 1, *split_lhs(make_lhs(res_a[0:M], a + 1)), oe_a,
                               {k: [v] for k, v in zip((2, 6, 10, 14), pins)})
            prev = jnp.concatenate(res_b, axis=1)
        pend[...] = prev
        return carry

    jax.lax.fori_loop(0, NIT, step, 0)
    for cp in cp_ffn:
        cp.wait()
    last_keys = post_pair(NSEG - 2, pend[M:, :], record=False)
    cp_o2.start()

    def max_all(v):
        return jnp.max(jnp.max(v, axis=0, keepdims=True), axis=1, keepdims=True)

    def decode(k):
        kb = pltpu.bitcast(jnp.broadcast_to(k, (8, 128)), jnp.int32)
        code = (kb >> 11) & 0xFFFF
        hi = jnp.where(code >= 0x8000, code & 0x7FFF, code ^ 0xFFFF)
        tok = jnp.clip((LAST - (kb & LAST))[0, 0], 0, LAST)
        return tok, pltpu.bitcast(hi << 16, F32)[:, 0:1]

    kv = keys[...]
    o1 = max_all(kv)
    o2 = max_all(jnp.where(kv == o1, 0.0, kv))
    kv = jnp.concatenate(last_keys + [jnp.where(sub8 < 4, o1, o2)], axis=0)
    k1 = jnp.max(kv, axis=0, keepdims=True)
    k2 = jnp.max(jnp.where(kv == k1, 0.0, kv), axis=0, keepdims=True)
    i1, r1 = decode(k1)
    i2, r2 = decode(k2)
    g1, g2 = i1 >> 3, i2 >> 3

    def rows_of(ref):
        return jnp.concatenate([ref[g1 >> 2, pl.ds(g1 & 3, 1)], ref[g2 >> 2, pl.ds(g2 & 3, 1)]],
                               axis=0).astype(F32)

    x1, h2 = rows_of(x1v), rows_of(h2v)
    hl = h2.reshape(16, D).astype(BF16)
    act = []
    for j in range(FF // 128):
        gt = _rb(_dot(hl, wblk(wg, j)))
        up = _rb(_dot(hl, wblk(wu, j)))
        act.append((_rb(gt * _sigmoid(gt)) * up).astype(BF16))
    act = jnp.concatenate(act, axis=1)
    y = jnp.concatenate([_dot(act, wblk(wd, n)) for n in range(8)], axis=1).reshape(2, 8, D)
    rowi = jax.lax.broadcasted_iota(jnp.int32, (2, 8, 1), 1)
    gsel = jax.lax.broadcasted_iota(jnp.int32, (2, 8, 1), 0)
    tokp = jnp.where(gsel == 0, g1, g2) * 8 + rowi
    gate = _sigmoid(jnp.where(tokp == i1, r1[None], r2[None]))
    upd = jnp.where((tokp == i1) | (tokp == i2), _rb(_rb(y) * gate), 0.0)
    patch[...] = (x1 + _rb(mod_vec(5) * _rb(h2 + upd))).astype(BF16)
    cp_o1.wait()
    cp_o2.wait()
    cp1 = pltpu.make_async_copy(patch.at[0], out_hbm.at[g1 >> 2, g1 & 3], sem_out.at[0])
    cp1.start()

    @pl.when(g1 != g2)
    def _():
        cp2 = pltpu.make_async_copy(patch.at[1], out_hbm.at[g2 >> 2, g2 & 3], sem_out.at[1])
        cp2.start()
        cp2.wait()

    cp1.wait()


@jax.jit
def pallas_adaLN_cond__memory_aug_recurrent_mem_tr__moe_arch_mod__prompt_kernel(
    A_x: jax.Array,
    A_mem0: jax.Array,
    A_Wq: jax.Array,
    A_Wk: jax.Array,
    A_Wv: jax.Array,
    A_Wo: jax.Array,
    A_seg_len,
    B_x: jax.Array,
    B_w_r: jax.Array,
    B_w_gate: jax.Array,
    B_w_up: jax.Array,
    B_w_down: jax.Array,
    c: jax.Array,
    w_mod: jax.Array,
):
    assert A_x.shape == (1, NSEG * SEG, D)
    any_spec = pl.BlockSpec(memory_space=pl.ANY)
    out = pl.pallas_call(
        _kernel,
        out_shape=jax.ShapeDtypeStruct((NSEG, 4, 8, D), BF16),
        in_specs=[any_spec] * 12,
        out_specs=any_spec,
        scratch_shapes=[
            pltpu.VMEM((H, D // 2, DH), U32),
            pltpu.VMEM((H, D // 2, DH), U32),
            pltpu.VMEM((H, D // 2, DH), U32),
            pltpu.VMEM((8, H * DH // 2, 128), U32),
            pltpu.VMEM((D // 2, FF + 128), U32),
            pltpu.VMEM((D // 2, FF + 128), U32),
            pltpu.VMEM((FF // 2, D + 128), U32),
            pltpu.VMEM((48, D // 2, 128), U32),
            pltpu.VMEM((D + 32, 128), F32),
            pltpu.VMEM((NSEG, 4, 8, D), BF16),
            pltpu.VMEM((NSEG, 4, 8, D), BF16),
            pltpu.VMEM((NSEG, 4, 8, D), BF16),
            pltpu.VMEM((NSEG, 4, 8, D), BF16),
            pltpu.VMEM((NSEG, 3 * NP, 8, DH), U32),
            pltpu.VMEM((D // KQ, NE, KQ), BF16),
            pltpu.VMEM((NSEG, 3, 8, D), F32),
            pltpu.VMEM((M + SEG + M, D), F32),
            pltpu.VMEM((48 + 8, 8, 128), F32),
            pltpu.VMEM((80, 128), F32),
            pltpu.VMEM((SEG, 128), F32),
            pltpu.VMEM((2, 8, D), BF16),
            pltpu.VMEM((8, 128), U32),
            pltpu.VMEM((NP, 4, 80, DH), BF16),
            pltpu.VMEM((3, NE, 2 * DH), F32),
            pltpu.VMEM((M, D), BF16),
            pltpu.VMEM((D,), BF16),
            pltpu.VMEM((1, D), BF16),
            pltpu.SemaphoreType.DMA((16 + NG + 4,)),
            pltpu.SemaphoreType.DMA((2,)),
        ],
        compiler_params=pltpu.CompilerParams(vmem_limit_bytes=120 * 1024 * 1024,
                                             disable_bounds_checks=True,
                                             disable_semaphore_checks=True),
    )(
        A_x.reshape(NSEG, 4, 8, D),
        A_mem0.reshape(M, D),
        A_Wq.reshape(D // 2, 2, H, DH),
        A_Wk.reshape(D // 2, 2, H, DH),
        A_Wv.reshape(D // 2, 2, H, DH),
        A_Wo.reshape(H * DH, D),
        B_w_r,
        B_w_gate,
        B_w_up,
        B_w_down,
        c,
        w_mod,
    )
    return out.reshape(1, NSEG * SEG, D)
```

```python
import jax
import jax.numpy as jnp
import jax.experimental.pallas as pl
import jax.experimental.pallas.tpu as pltpu

F32 = jnp.float32
BF16 = jnp.bfloat16
U32 = jnp.uint32

D = 1024
H = 32
DH = 128
NP = H // 2
M = 8
SEG = 32
NSEG = 64
FF = 3584
NJ = SEG - M
NE = NSEG * M
EPS = 1.0013580322265625e-05
SCALE = DH ** (-0.5)
NEG = -1000000000.0
LOG2E = 1.4426950408889634
KQ = 128
NK = D // KQ
MB = 11
NG = 4
UNROLL = 2
NIT = NSEG // (2 * UNROLL)
OUT_SPLIT = NSEG - 2 * UNROLL - 2


def _rb(x):
    return x.astype(BF16).astype(F32)


def _layernorm(xf):
    m = jnp.mean(xf, axis=-1, keepdims=True)
    d = xf - m
    v = jnp.mean(d * d, axis=-1, keepdims=True)
    std = _rb(jnp.sqrt(_rb(_rb(v) + EPS)))
    return _rb(xf - _rb(m)) * (1.0 / std)


def _sigmoid(x):
    return _rb(1.0 / _rb(1.0 + _rb(jnp.exp(-x))))


def _dot(a, b):
    return jnp.dot(a, b, preferred_element_type=F32)


def _dot_nt(a, b):
    return jax.lax.dot_general(a, b, (((1,), (1,)), ((), ())), preferred_element_type=F32)


def _kernel(x_hbm, mem0_hbm, wq_hbm, wk_hbm, wv_hbm, wo_hbm, wr_hbm, wg_hbm, wu_hbm, wd_hbm,
            c_hbm, wm_hbm,
            out_hbm,
            wq, wk, wv, wo, wg, wu, wd, wm, cb, xv, x1v, h2v, outv, early, hn, he, hj, pend,
            mod, fill, keys, patch, zero, opnd, acc0, mem0_ref, wr_ref, c_ref,
            sem, sem_out):
    w_u32 = [w.bitcast(U32) for w in (wq_hbm, wk_hbm, wv_hbm)]
    wqkv = (wq, wk, wv)
    wo_hbm, wg_hbm, wu_hbm, wd_hbm, wm_hbm = [
        w.bitcast(U32) for w in (wo_hbm, wg_hbm, wu_hbm, wd_hbm, wm_hbm)]

    def wblk(w, j):
        return pltpu.bitcast(w[:, j * 128:(j + 1) * 128], BF16)

    def wo_blk(n, lo, hi):
        return pltpu.bitcast(wo[n, lo // 2:hi // 2, :], BF16)

    def w_copies(m, p, k):
        return [pltpu.make_async_copy(w_u32[m].at[:, par, p, :], wqkv[m].at[2 * p + par], sem.at[k])
                for par in range(2)]

    def col_copy(src, dst, j, k):
        lo = j * 128 if isinstance(j, int) else pl.multiple_of(j * 128, 128)
        return pltpu.make_async_copy(src.at[:, pl.ds(lo, 128)], dst.at[j], sem.at[k])

    def units(g):
        return [(m, 4 * g + t) for t in range(4) for m in range(2)]

    def xj_copy(g):
        segs = pl.ds(16 * g, 16)
        return pltpu.make_async_copy(x_hbm.at[segs, 0:3], xv.at[segs, 0:3], sem.at[16 + g])

    def qk_copies(g):
        return sum([w_copies(m, p, 16 + g) for m, p in units(g)], [])

    def wm1_copies(j):
        return [col_copy(wm_hbm, wm, j, 1 + j), col_copy(wm_hbm, wm, 8 + j, 1 + j)]

    def wv_copies(j):
        lo = j * (KQ // 2) if isinstance(j, int) else pl.multiple_of(j * (KQ // 2), KQ // 2)
        rows = pl.ds(lo, KQ // 2)
        return [pltpu.make_async_copy(w_u32[2].at[rows, par, p, :], wv.at[2 * p + par, rows],
                                      sem.at[24 + j]) for p in range(NP) for par in range(2)]

    def wm2_copies(lo, n, t):
        return [col_copy(wm_hbm, wm, lo + b, 20 + t) for b in range(n)]

    def wait_if(cond, cps):
        for cp in cps:
            pl.when(cond)(cp.wait)

    def start_if(cond, cps):
        for cp in cps:
            pl.when(cond)(cp.start)

    def start_if_below(i, n, cps):
        for k in range(0, len(cps), 4):
            start_if(i < n if k % 8 == 0 else i + 1 <= n, cps[k:k + 4])

    cp_c = pltpu.make_async_copy(c_hbm, c_ref, sem.at[9])
    cp_xe = pltpu.make_async_copy(x_hbm.at[:, 3], xv.at[:, 3], sem.at[0])
    cp_wo = [col_copy(wo_hbm, wo, n, 10) for n in range(8)]
    cp_small = [pltpu.make_async_copy(mem0_hbm, mem0_ref, sem.at[14]),
                pltpu.make_async_copy(wr_hbm, wr_ref, sem.at[15])]
    cp_ffn = [pltpu.make_async_copy(wg_hbm, wg.at[:, 0:FF], sem.at[11]),
              pltpu.make_async_copy(wu_hbm, wu.at[:, 0:FF], sem.at[12]),
              pltpu.make_async_copy(wd_hbm, wd.at[:, 0:D], sem.at[13])]

    for cp in ([cp_c, cp_xe] + wm1_copies(0) + wv_copies(0) + wm1_copies(1) + wm1_copies(2)
               + wv_copies(1) + cp_small):
        cp.start()

    ri = jax.lax.broadcasted_iota(jnp.int32, (80, 128), 0)
    ci = jax.lax.broadcasted_iota(jnp.int32, (80, 128), 1)

    def head_of(i):
        return jnp.where(i < 64, i >> 5, (i - 64) >> 3)

    def pos_of(i):
        return jnp.where(i < 64, i & 31, 32 + (i & 7))

    same = (head_of(ri) == head_of(ci)) & (ci < 80)
    allowed = (pos_of(ri) < M) | (pos_of(ri) >= pos_of(ci))
    fill[...] = jnp.where(same, jnp.where(allowed, 0.0, NEG / SCALE), -jnp.inf).astype(F32)
    keys[...] = jnp.zeros(keys.shape, F32)
    pend[M:, :] = jnp.zeros((SEG + M, D), F32)
    zero[...] = jnp.zeros(zero.shape, U32)

    def pin_zero(vals):
        acc = None
        for v in vals:
            v = pltpu.bitcast(v, U32)
            for r in range(0, v.shape[0], 8):
                acc = v[r:r + 8] if acc is None else acc | v[r:r + 8]
        return acc & zero[...]

    cp_c.wait()
    cf = c_ref[...].astype(F32)
    sc = _rb(cf * _sigmoid(cf))
    cb[0:D, :] = jnp.broadcast_to(sc, (128, D)).T
    cb[D:, :] = jnp.zeros((32, 128), F32)

    def mod_vec(k):
        return jnp.concatenate([mod[8 * k + b] for b in range(8)], axis=1)

    def mod_block_vpu(src, dst, is_scale, after=None):
        acc = None if after is None else pltpu.bitcast(pin_zero([after]), F32)
        for r in range(0, D // 2, 8):
            w = wm[src, r:r + 8, :]
            t0 = pltpu.bitcast(w << 16, F32) * cb[pl.ds(2 * r, 8, stride=2), :]
            t1 = pltpu.bitcast(w & U32(0xFFFF0000), F32) * cb[pl.ds(2 * r + 1, 8, stride=2), :]
            if after is not None:
                acc = (acc + t0) + t1
            else:
                acc = t0 + t1 if acc is None else acc + (t0 + t1)
        v = _rb(jnp.broadcast_to(jnp.sum(acc, axis=0, keepdims=True), (8, 128)))
        v = jnp.where(is_scale, _rb(1.0 + v), v)
        mod[dst] = v
        return v

    def ne_body(i, carry):
        n = _layernorm(xv[pl.ds(i * 16, 16), 3].astype(F32)).reshape(128, D).astype(BF16)
        for j in range(NK):
            hn[j, pl.ds(pl.multiple_of(i * 128, 128), 128), :] = n[:, j * KQ:(j + 1) * KQ]
        return carry

    cp_xe.wait()
    jax.lax.fori_loop(0, NSEG // 16, ne_body, 0)

    def w_head(m, h, lo=0, hi=D):
        return pltpu.bitcast(wqkv[m][h, lo // 2:hi // 2, :], BF16)

    def relayout(m, p, rows=slice(None)):
        w = wqkv[m]
        e = w[2 * p, rows, :]
        o = w[2 * p + 1, rows, :]
        w[2 * p, rows, :] = (e & U32(0xFFFF)) | (o << 16)
        w[2 * p + 1, rows, :] = (e >> 16) | (o & U32(0xFFFF0000))

    def store_early(m, p, row0, r1, r2):
        ns = r1.shape[0] // 8
        r12 = jnp.concatenate([r1.reshape(ns, 8, DH), r2.reshape(ns, 8, DH)], axis=1)
        v = pltpu.bitcast(r12.reshape(16 * ns, DH).astype(BF16), U32)
        early[row0 // 8:row0 // 8 + ns, m * NP + p] = v.reshape(ns, 8, DH)
        return v

    def modulate(j, shift, scale):
        n = hn[j].astype(F32).reshape(NSEG, 8, KQ)
        h = (_rb(n * scale) + shift).reshape(NE, KQ)
        he[j] = h.astype(BF16)
        return h

    def chunk_body(j, carry):
        @pl.when(j <= 1)
        def _():
            for cp in wm1_copies(j):
                cp.wait()
            modulate(j, mod_block_vpu(j, j, False), mod_block_vpu(8 + j, 8 + j, True))

        nxt = jnp.where(j >= 1, jnp.minimum(j + 1, NK - 1), 0)
        wait_if(nxt == j + 1, wm1_copies(nxt))
        for cp in wv_copies(j):
            cp.wait()
        krows = pl.ds(pl.multiple_of(j * (KQ // 2), KQ // 2), KQ // 2)
        hb = [he[j, c * 256:(c + 1) * 256, :] for c in range(2)]
        pins = {}
        for c in range(2):
            rows = slice(c * 256, (c + 1) * 256)
            for q in range(NP // 2):
                i = 8 * c + q
                if c == 0:
                    relayout(2, 2 * q, krows)
                    relayout(2, 2 * q + 1, krows)
                w4 = [wv[4 * q + b, krows, :] for b in range(4)]
                if i in pins:
                    w4[0] = jnp.concatenate([w4[0][0:8] | pin_zero(pins[i]), w4[0][8:]], axis=0)
                r = _dot(hb[c], pltpu.bitcast(jnp.concatenate(w4, axis=1), BF16))
                acc0[q, rows, :] = r + jnp.where(j > 0, acc0[q, rows, :], 0.0)
                if i == 7:
                    shift = mod_block_vpu(nxt, nxt, False, r[0:8, 0:128])
                if i == 9:
                    scale = mod_block_vpu(8 + nxt, 8 + nxt, True, r[0:8, 0:128])
                    h = modulate(nxt, shift, scale)
                    pins = {13: [h[0:256]], 15: [h[256:512]]}
        pr = 1 + (j >> 1)
        t = jnp.maximum(j - 5, 0)
        start_if(j + 4 < NK, wm1_copies(jnp.minimum(j + 4, NK - 1)))
        start_if_below(j, NK - 3, wv_copies(jnp.minimum(j + 3, NK - 1)))
        start_if((j & 1) == 0, w_copies(0, pr, 16 + (pr >> 2)))
        start_if((j & 1) == 1, w_copies(1, pr, 16 + (pr >> 2)))
        start_if_below(4, j, [xj_copy(t)] + w_copies(0, 5 + t, 17) + w_copies(1, 5 + t, 17)
                       + wm2_copies(16 + 4 * t, 4, 0))
        return carry

    for cp in wm1_copies(3) + wv_copies(2) + w_copies(0, 0, 16) + w_copies(1, 0, 16):
        cp.start()
    jax.lax.fori_loop(0, NK, chunk_body, 0)

    def early_proj(m, p, pins=None):
        relayout(m, p)
        for c in range(2):
            rows = slice(c * 256, (c + 1) * 256)
            hc = jnp.concatenate([he[j, rows, :] for j in range(NK)], axis=1)
            r12 = []
            for b in range(2):
                halves = []
                for k in range(2):
                    wh = wqkv[m][2 * p + b, k * 256:(k + 1) * 256, :]
                    if pins.get(4 * c + 2 * b + k):
                        wh = jnp.concatenate(
                            [wh[0:8] | pin_zero(pins[4 * c + 2 * b + k]), wh[8:]], axis=0)
                    halves.append(wh)
                r12.append(_dot(hc, pltpu.bitcast(jnp.concatenate(halves, axis=0), BF16)))
            store_early(m, p, c * 256, *r12)

    def make_hj(s):
        n = _rb(_layernorm(xv[s, 0:3].astype(F32)))
        h = _rb(n * mod_vec(1)) + mod_vec(0)
        hj[s] = h
        return [h[g, :, 0:128] for g in range(3)]

    def pro_body(g, carry):
        wait_if(g == 1, wm2_copies(16, 12, 0))
        tb = jnp.maximum(g - 2, 0)
        wait_if(g >= 2, wm2_copies(28 + 10 * tb, 10, 1 + tb))
        for cp in qk_copies(g) + [xj_copy(g)]:
            cp.wait()
        lnp = sum([make_hj(g * 16 + t) for t in range(16)], [])
        mv = []
        for b in range(MB):
            blk = 16 + MB * (g - 1) + b
            live = (g > 0) & (blk < 48)
            mv.append(mod_block_vpu(jnp.where(live, blk, b), jnp.where(live, blk, 48 + b),
                                    (blk >= 32) & (blk < 40)))
        fin = [store_early(2, 4 * g + t, 0, acc0[2 * g + t // 2, :, (t % 2) * 256:(t % 2) * 256 + DH],
                           acc0[2 * g + t // 2, :, (t % 2) * 256 + DH:(t % 2) * 256 + 2 * DH])
               for t in range(4)]
        sites = {i: [] for i in range(64)}
        twice = [3, 4, 6, 7, 10, 11, 12, 14, 15, 18, 19, 20, 22, 23, 26, 27, 30, 31]
        for i, v in zip(sorted(list(range(2, 32)) + twice), lnp):
            sites[2 * i].append(v)
        for i, v in zip(range(1, 31, 2), mv + fin):
            sites[2 * i + 1].append(v)
        for u, (m, p) in enumerate(units(g)):
            early_proj(m, p, {i: sites[8 * u + i] for i in range(8)})
        gn = jnp.minimum(g, 1)
        start_if_below(g, 2, qk_copies(gn + 2))
        start_if(g == 1, [xj_copy(3)])
        start_if_below(g, 2, wm2_copies(28 + 10 * gn, 10, 1 + gn))
        start_if(g == 0, cp_wo[:1])
        start_if(g == 1, cp_wo[1:])
        return carry

    jax.lax.fori_loop(0, NG, pro_body, 0)

    for cp in cp_ffn:
        cp.start()
    for cp in cp_small + cp_wo:
        cp.wait()
    pend[0:M, :] = mem0_ref[...].astype(F32)

    wr = jnp.broadcast_to(wr_ref[...].astype(F32).reshape(1, D), (8, D))

    lane8 = jax.lax.broadcasted_iota(jnp.int32, (8, 128), 1)
    sub8 = jax.lax.broadcasted_iota(jnp.int32, (8, 128), 0)
    LAST = NSEG * SEG - 1

    def post(s, g0, g1, attn, record=True):
        attn = attn.reshape(g1 - g0, 8, D)
        x1 = _rb(xv[s, g0:g1].astype(F32) + _rb(mod_vec(2) * _rb(attn)))
        n = _rb(_layernorm(x1))
        h2 = _rb(_rb(n * mod_vec(4)) + mod_vec(3))
        r = _rb(jnp.sum(h2 * wr, axis=-1, keepdims=True)) + 0.0
        x1v[s, g0:g1] = x1.astype(BF16)
        h2v[s, g0:g1] = h2.astype(BF16)
        outv[s, g0:g1] = (x1 + _rb(mod_vec(5) * h2)).astype(BF16)
        pins = []
        for g in range(g0, g1):
            bits = pltpu.bitcast(jnp.broadcast_to(r[g - g0], (8, 128)), jnp.int32)
            hi = jax.lax.shift_right_logical(bits, 16)
            code = jnp.where(bits < 0, hi ^ 0xFFFF, hi | 0x8000)
            key = (code << 11) | (LAST - (s * SEG + g * 8) - sub8) | 0x40000000
            key = pltpu.bitcast(key, F32)
            if record:
                rows = slice(g * 8, (g + 1) * 8)
                keys[rows, :] = jnp.where(lane8 == s, key, keys[rows, :])
            pins.append(key)
        return pins

    def post_pair(a, rows, record=True):
        return post(a + 1, 0, 4, rows[0:SEG], record) + post(a, 3, 4, rows[SEG:], record)

    zpad = jnp.zeros((48, DH), BF16)
    G = 4
    KA = (NP - G) * 2 * DH
    KS = D - 128

    def segment(s, lhs, lhs_split, extra, pins):
        scales = {}

        def stash(p, m, v):
            opnd[p, m, 0:v.shape[0], :] = v.astype(BF16)

        def qkv_group(p):
            keys = [(m, 2 * p + b) for m in range(3) for b in range(2 * G)]
            nsplit = 6 if (p == 0 and lhs_split is not None) else 0
            part = [_dot(lhs_split[0], w_head(m, h, 0, KS)) for m, h in keys[:nsplit]]
            full = [_dot(lhs_split[1], w_head(m, h, KS, D)) + part[i]
                    for i, (m, h) in enumerate(keys[:nsplit])]
            full += [_dot(lhs, w_head(m, h)) for m, h in keys[nsplit:]]
            for m in range(3):
                for t in range(G):
                    i = 2 * G * m + 2 * t
                    stash(p + t, m, jnp.concatenate([full[i], full[i + 1]], axis=0))

        def operand(p, m):
            parts = [opnd[p, m, 0:64, :], pltpu.bitcast(early[s, m * NP + p], BF16)]
            if m > 0:
                parts.append(zpad)
            return jnp.concatenate(parts, axis=0)

        def scores(p):
            sc_ = _dot_nt(operand(p, 0), operand(p, 1))
            f = fill[...]
            if pins.get(p):
                f = jnp.concatenate([f[0:8] + pltpu.bitcast(pin_zero(pins[p]), F32), f[8:]], axis=0)
            sc_ = jnp.where(f == 0.0, sc_, f)
            mx = jnp.max(sc_, axis=-1, keepdims=True)
            e = jnp.exp2((sc_ - mx) * (SCALE * LOG2E))
            inv = pl.reciprocal(jnp.sum(e, axis=-1, keepdims=True), approx=True)
            if p // G == NP // G - 2:
                stash(p, 3, e * inv)
            else:
                stash(p, 3, e)
                scales[p] = inv

        oe = []

        def pv(p):
            o = _dot(opnd[p, 3], operand(p, 2))
            if p in scales:
                o = o * scales[p]
                pins.setdefault(p + G, []).append(o)
            res = []
            for b in range(2):
                rows, erows = o[32 * b:32 * b + 32], o[64 + 8 * b:72 + 8 * b]
                oe.append(erows)
                if extra is not None:
                    rows = jnp.concatenate([rows, erows, extra[2 * p + b]], axis=0)
                res.append(rows)
            return res

        os_ = []
        for p in range(0, NP, G):
            qkv_group(p)
            if p >= G:
                for t in range(G):
                    os_ += pv(p - G + t)
            for t in range(G):
                scores(p + t)
        oa = jnp.concatenate(os_, axis=1).astype(BF16)
        acc, ob = [], []
        for n in range(7):
            acc.append(_dot(oa, wo_blk(n, 0, KA)))
            if n == 1:
                for t in range(G):
                    ob += pv(NP - G + t)
        ob = jnp.concatenate(ob, axis=1).astype(BF16)
        res = [_dot(ob, wo_blk(n, KA, H * DH)) + acc[n] for n in range(7)]
        res.append(_dot(ob, wo_blk(7, KA, H * DH)) + _dot(oa, wo_blk(7, 0, KA)))
        return res, oe

    def make_lhs(mem, s):
        return jnp.concatenate([mem, hj[s].reshape(NJ, D)], axis=0)

    cp_o1 = pltpu.make_async_copy(outv.at[0:OUT_SPLIT], out_hbm.at[0:OUT_SPLIT], sem_out.at[0])
    cp_o2 = pltpu.make_async_copy(outv.at[OUT_SPLIT:NSEG], out_hbm.at[OUT_SPLIT:NSEG],
                                  sem_out.at[1])

    def split_lhs(lhs):
        return lhs.astype(BF16), (lhs[:, :KS].astype(BF16), lhs[:, KS:].astype(BF16))

    def step(i, carry):
        @pl.when(i == NIT - 1)
        def _():
            cp_o1.start()

        prev = pend[...]
        for u in range(UNROLL):
            a = 2 * (UNROLL * i + u)
            pins = post_pair(jnp.maximum(a - 2, 0) if u == 0 else a - 2, prev[M:])
            lhs_a = make_lhs(prev[0:M], a)
            lhs_a = (lhs_a.astype(BF16), None) if u == 0 else split_lhs(lhs_a)
            res_a, oe_a = segment(a, *lhs_a, None,
                                  {k: [v] for k, v in zip((2, 6, 10, 14), pins[:4])})
            res_a = jnp.concatenate(res_a, axis=1)
            pins = pins[4:] + post(a, 0, 3, res_a[M:])
            res_b, _ = segment(a + 1, *split_lhs(make_lhs(res_a[0:M], a + 1)), oe_a,
                               {k: [v] for k, v in zip((2, 6, 10, 14), pins)})
            prev = jnp.concatenate(res_b, axis=1)
        pend[...] = prev
        return carry

    jax.lax.fori_loop(0, NIT, step, 0)
    for cp in cp_ffn:
        cp.wait()
    last_keys = post_pair(NSEG - 2, pend[M:, :], record=False)
    cp_o2.start()

    def max_all(v):
        return jnp.max(jnp.max(v, axis=0, keepdims=True), axis=1, keepdims=True)

    def decode(k):
        kb = pltpu.bitcast(jnp.broadcast_to(k, (8, 128)), jnp.int32)
        code = (kb >> 11) & 0xFFFF
        hi = jnp.where(code >= 0x8000, code & 0x7FFF, code ^ 0xFFFF)
        tok = jnp.clip((LAST - (kb & LAST))[0, 0], 0, LAST)
        return tok, pltpu.bitcast(hi << 16, F32)[:, 0:1]

    kv = keys[...]
    o1 = max_all(kv)
    o2 = max_all(jnp.where(kv == o1, 0.0, kv))
    kv = jnp.concatenate(last_keys + [jnp.where(sub8 < 4, o1, o2)], axis=0)
    k1 = jnp.max(kv, axis=0, keepdims=True)
    k2 = jnp.max(jnp.where(kv == k1, 0.0, kv), axis=0, keepdims=True)
    i1, r1 = decode(k1)
    i2, r2 = decode(k2)
    g1, g2 = i1 >> 3, i2 >> 3

    def rows_of(ref):
        return jnp.concatenate([ref[g1 >> 2, pl.ds(g1 & 3, 1)], ref[g2 >> 2, pl.ds(g2 & 3, 1)]],
                               axis=0).astype(F32)

    x1, h2 = rows_of(x1v), rows_of(h2v)
    hl = h2.reshape(16, D).astype(BF16)
    act = []
    for j in range(FF // 128):
        gt = _rb(_dot(hl, wblk(wg, j)))
        up = _rb(_dot(hl, wblk(wu, j)))
        act.append((_rb(gt * _sigmoid(gt)) * up).astype(BF16))
    act = jnp.concatenate(act, axis=1)
    y = jnp.concatenate([_dot(act, wblk(wd, n)) for n in range(8)], axis=1).reshape(2, 8, D)
    rowi = jax.lax.broadcasted_iota(jnp.int32, (2, 8, 1), 1)
    gsel = jax.lax.broadcasted_iota(jnp.int32, (2, 8, 1), 0)
    tokp = jnp.where(gsel == 0, g1, g2) * 8 + rowi
    gate = _sigmoid(jnp.where(tokp == i1, r1[None], r2[None]))
    upd = jnp.where((tokp == i1) | (tokp == i2), _rb(_rb(y) * gate), 0.0)
    patch[...] = (x1 + _rb(mod_vec(5) * _rb(h2 + upd))).astype(BF16)
    cp_o1.wait()
    cp_o2.wait()
    cp1 = pltpu.make_async_copy(patch.at[0], out_hbm.at[g1 >> 2, g1 & 3], sem_out.at[0])
    cp1.start()

    @pl.when(g1 != g2)
    def _():
        cp2 = pltpu.make_async_copy(patch.at[1], out_hbm.at[g2 >> 2, g2 & 3], sem_out.at[1])
        cp2.start()
        cp2.wait()

    cp1.wait()


@jax.jit
def pallas_adaLN_cond__memory_aug_recurrent_mem_tr__moe_arch_mod__prompt_kernel(
    A_x: jax.Array,
    A_mem0: jax.Array,
    A_Wq: jax.Array,
    A_Wk: jax.Array,
    A_Wv: jax.Array,
    A_Wo: jax.Array,
    A_seg_len,
    B_x: jax.Array,
    B_w_r: jax.Array,
    B_w_gate: jax.Array,
    B_w_up: jax.Array,
    B_w_down: jax.Array,
    c: jax.Array,
    w_mod: jax.Array,
):
    assert A_x.shape == (1, NSEG * SEG, D)
    any_spec = pl.BlockSpec(memory_space=pl.ANY)
    out = pl.pallas_call(
        _kernel,
        out_shape=jax.ShapeDtypeStruct((NSEG, 4, 8, D), BF16),
        in_specs=[any_spec] * 12,
        out_specs=any_spec,
        scratch_shapes=[
            pltpu.VMEM((H, D // 2, DH), U32),
            pltpu.VMEM((H, D // 2, DH), U32),
            pltpu.VMEM((H, D // 2, DH), U32),
            pltpu.VMEM((8, H * DH // 2, 128), U32),
            pltpu.VMEM((D // 2, FF + 128), U32),
            pltpu.VMEM((D // 2, FF + 128), U32),
            pltpu.VMEM((FF // 2, D + 128), U32),
            pltpu.VMEM((48, D // 2, 128), U32),
            pltpu.VMEM((D + 32, 128), F32),
            pltpu.VMEM((NSEG, 4, 8, D), BF16),
            pltpu.VMEM((NSEG, 4, 8, D), BF16),
            pltpu.VMEM((NSEG, 4, 8, D), BF16),
            pltpu.VMEM((NSEG, 4, 8, D), BF16),
            pltpu.VMEM((NSEG, 3 * NP, 8, DH), U32),
            pltpu.VMEM((NK, NE, KQ), BF16),
            pltpu.VMEM((NK, NE, KQ), BF16),
            pltpu.VMEM((NSEG, 3, 8, D), F32),
            pltpu.VMEM((M + SEG + M, D), F32),
            pltpu.VMEM((48 + 16, 8, 128), F32),
            pltpu.VMEM((80, 128), F32),
            pltpu.VMEM((SEG, 128), F32),
            pltpu.VMEM((2, 8, D), BF16),
            pltpu.VMEM((8, 128), U32),
            pltpu.VMEM((NP, 4, 80, DH), BF16),
            pltpu.VMEM((NP // 2, NE, 4 * DH), F32),
            pltpu.VMEM((M, D), BF16),
            pltpu.VMEM((D,), BF16),
            pltpu.VMEM((1, D), BF16),
            pltpu.SemaphoreType.DMA((24 + NK,)),
            pltpu.SemaphoreType.DMA((2,)),
        ],
        compiler_params=pltpu.CompilerParams(vmem_limit_bytes=124 * 1024 * 1024,
                                             disable_bounds_checks=True,
                                             disable_semaphore_checks=True),
    )(
        A_x.reshape(NSEG, 4, 8, D),
        A_mem0.reshape(M, D),
        A_Wq.reshape(D // 2, 2, H, DH),
        A_Wk.reshape(D // 2, 2, H, DH),
        A_Wv.reshape(D // 2, 2, H, DH),
        A_Wo.reshape(H * DH, D),
        B_w_r,
        B_w_gate,
        B_w_up,
        B_w_down,
        c,
        w_mod,
    )
    return out.reshape(1, NSEG * SEG, D)
```

```python
import jax
import jax.numpy as jnp
import jax.experimental.pallas as pl
import jax.experimental.pallas.tpu as pltpu

F32 = jnp.float32
BF16 = jnp.bfloat16
U32 = jnp.uint32

D = 1024
H = 32
DH = 128
NP = H // 2
M = 8
SEG = 32
NSEG = 64
FF = 3584
NJ = SEG - M
NE = NSEG * M
EPS = 1.0013580322265625e-05
SCALE = DH ** (-0.5)
NEG = -1000000000.0
LOG2E = 1.4426950408889634
KQ = 128
NK = D // KQ
MB = 11
NG = 4
UNROLL = 2
NIT = NSEG // (2 * UNROLL)
OUT_SPLIT = NSEG - 2 * UNROLL - 2


def _rb(x):
    return x.astype(BF16).astype(F32)


def _layernorm(xf):
    m = jnp.mean(xf, axis=-1, keepdims=True)
    d = xf - m
    v = jnp.mean(d * d, axis=-1, keepdims=True)
    std = _rb(jnp.sqrt(_rb(_rb(v) + EPS)))
    return _rb(xf - _rb(m)) * (1.0 / std)


def _sigmoid(x):
    return _rb(1.0 / _rb(1.0 + _rb(jnp.exp(-x))))


def _dot(a, b):
    return jnp.dot(a, b, preferred_element_type=F32)


def _dot_nt(a, b):
    return jax.lax.dot_general(a, b, (((1,), (1,)), ((), ())), preferred_element_type=F32)


def _kernel(x_hbm, mem0_hbm, wq_hbm, wk_hbm, wv_hbm, wo_hbm, wr_hbm, wg_hbm, wu_hbm, wd_hbm,
            c_hbm, wm_hbm,
            out_hbm,
            wq, wk, wv, wo, wg, wu, wd, wm, cb, xv, x1v, h2v, outv, early, hn, he, hj, pend,
            mod, fill, keys, patch, zero, opnd, acc0, mem0_ref, wr_ref, c_ref,
            sem, sem_out):
    w_u32 = [w.bitcast(U32) for w in (wq_hbm, wk_hbm, wv_hbm)]
    wqkv = (wq, wk, wv)
    wo_hbm, wg_hbm, wu_hbm, wd_hbm, wm_hbm = [
        w.bitcast(U32) for w in (wo_hbm, wg_hbm, wu_hbm, wd_hbm, wm_hbm)]

    def wblk(w, j):
        return pltpu.bitcast(w[:, j * 128:(j + 1) * 128], BF16)

    def wo_blk(n, lo, hi):
        return pltpu.bitcast(wo[n, lo // 2:hi // 2, :], BF16)

    def w_copies(m, p, k):
        return [pltpu.make_async_copy(w_u32[m].at[:, par, p, :], wqkv[m].at[2 * p + par], sem.at[k])
                for par in range(2)]

    def col_copy(src, dst, j, k):
        lo = j * 128 if isinstance(j, int) else pl.multiple_of(j * 128, 128)
        return pltpu.make_async_copy(src.at[:, pl.ds(lo, 128)], dst.at[j], sem.at[k])

    def units(g):
        return [(m, 4 * g + t) for t in range(4) for m in range(2)]

    def xj_copy(g):
        segs = pl.ds(16 * g, 16)
        return pltpu.make_async_copy(x_hbm.at[segs, 0:3], xv.at[segs, 0:3], sem.at[16 + g])

    def qk_copies(g):
        return sum([w_copies(m, p, 16 + g) for m, p in units(g)], [])

    def wm1_copies(j):
        return [col_copy(wm_hbm, wm, j, 1 + j), col_copy(wm_hbm, wm, 8 + j, 1 + j)]

    def wv_copies(j):
        lo = j * (KQ // 2) if isinstance(j, int) else pl.multiple_of(j * (KQ // 2), KQ // 2)
        rows = pl.ds(lo, KQ // 2)
        return [pltpu.make_async_copy(w_u32[2].at[rows, par, p, :], wv.at[2 * p + par, rows],
                                      sem.at[24 + j]) for p in range(NP) for par in range(2)]

    def wm2_copies(lo, n, t):
        return [col_copy(wm_hbm, wm, lo + b, 20 + t) for b in range(n)]

    def wait_if(cond, cps):
        for cp in cps:
            pl.when(cond)(cp.wait)

    def start_if(cond, cps):
        for cp in cps:
            pl.when(cond)(cp.start)

    def start_if_below(i, n, cps):
        for k in range(0, len(cps), 4):
            start_if(i < n if k % 8 == 0 else i + 1 <= n, cps[k:k + 4])

    cp_c = pltpu.make_async_copy(c_hbm, c_ref, sem.at[9])
    cp_xe = pltpu.make_async_copy(x_hbm.at[:, 3], xv.at[:, 3], sem.at[0])
    cp_wo = [col_copy(wo_hbm, wo, n, 10) for n in range(8)]
    cp_small = [pltpu.make_async_copy(mem0_hbm, mem0_ref, sem.at[14]),
                pltpu.make_async_copy(wr_hbm, wr_ref, sem.at[15])]
    cp_ffn = [pltpu.make_async_copy(wg_hbm, wg.at[:, 0:FF], sem.at[11]),
              pltpu.make_async_copy(wu_hbm, wu.at[:, 0:FF], sem.at[12]),
              pltpu.make_async_copy(wd_hbm, wd.at[:, 0:D], sem.at[13])]

    for cp in ([cp_c, cp_xe] + wm1_copies(0) + wv_copies(0) + wm1_copies(1) + wm1_copies(2)
               + wv_copies(1) + cp_small):
        cp.start()

    ri = jax.lax.broadcasted_iota(jnp.int32, (80, 128), 0)
    ci = jax.lax.broadcasted_iota(jnp.int32, (80, 128), 1)

    def head_of(i):
        return jnp.where(i < 64, i >> 5, (i - 64) >> 3)

    def pos_of(i):
        return jnp.where(i < 64, i & 31, 32 + (i & 7))

    same = (head_of(ri) == head_of(ci)) & (ci < 80)
    allowed = (pos_of(ri) < M) | (pos_of(ri) >= pos_of(ci))
    fill[...] = jnp.where(same, jnp.where(allowed, 0.0, NEG / SCALE), -jnp.inf).astype(F32)
    keys[...] = jnp.zeros(keys.shape, F32)
    pend[M:, :] = jnp.zeros((SEG + M, D), F32)
    zero[...] = jnp.zeros(zero.shape, U32)

    def pin_zero(vals):
        acc = None
        for v in vals:
            v = pltpu.bitcast(v, U32)
            for r in range(0, v.shape[0], 8):
                acc = v[r:r + 8] if acc is None else acc | v[r:r + 8]
        return acc & zero[...]

    cp_c.wait()
    cf = c_ref[...].astype(F32)
    sc = _rb(cf * _sigmoid(cf))
    cb[0:D, :] = jnp.broadcast_to(sc, (128, D)).T
    cb[D:, :] = jnp.zeros((32, 128), F32)

    def mod_vec(k):
        return jnp.concatenate([mod[8 * k + b] for b in range(8)], axis=1)

    def mod_block_vpu(src, dst, is_scale, after=None):
        acc = None if after is None else pltpu.bitcast(pin_zero([after]), F32)
        for r in range(0, D // 2, 8):
            w = wm[src, r:r + 8, :]
            t0 = pltpu.bitcast(w << 16, F32) * cb[pl.ds(2 * r, 8, stride=2), :]
            t1 = pltpu.bitcast(w & U32(0xFFFF0000), F32) * cb[pl.ds(2 * r + 1, 8, stride=2), :]
            if after is not None:
                acc = (acc + t0) + t1
            else:
                acc = t0 + t1 if acc is None else acc + (t0 + t1)
        v = _rb(jnp.broadcast_to(jnp.sum(acc, axis=0, keepdims=True), (8, 128)))
        v = jnp.where(is_scale, _rb(1.0 + v), v)
        mod[dst] = v
        return v

    def ne_body(i, carry):
        n = _layernorm(xv[pl.ds(i * 16, 16), 3].astype(F32)).reshape(128, D).astype(BF16)
        for j in range(NK):
            hn[j, pl.ds(pl.multiple_of(i * 128, 128), 128), :] = n[:, j * KQ:(j + 1) * KQ]
        return carry

    cp_xe.wait()
    jax.lax.fori_loop(0, NSEG // 16, ne_body, 0)

    def w_head(m, h, lo=0, hi=D):
        return pltpu.bitcast(wqkv[m][h, lo // 2:hi // 2, :], BF16)

    def relayout(m, p, rows=slice(None)):
        w = wqkv[m]
        e = w[2 * p, rows, :]
        o = w[2 * p + 1, rows, :]
        w[2 * p, rows, :] = (e & U32(0xFFFF)) | (o << 16)
        w[2 * p + 1, rows, :] = (e >> 16) | (o & U32(0xFFFF0000))

    def store_early(m, p, row0, r1, r2):
        ns = r1.shape[0] // 8
        r12 = jnp.concatenate([r1.reshape(ns, 8, DH), r2.reshape(ns, 8, DH)], axis=1)
        v = pltpu.bitcast(r12.reshape(16 * ns, DH).astype(BF16), U32)
        early[row0 // 8:row0 // 8 + ns, m * NP + p] = v.reshape(ns, 8, DH)
        return v

    def modulate(j, shift, scale):
        n = hn[j].astype(F32).reshape(NSEG, 8, KQ)
        h = (_rb(n * scale) + shift).reshape(NE, KQ)
        he[j] = h.astype(BF16)
        return h

    def chunk_body(j, carry):
        @pl.when(j <= 1)
        def _():
            for cp in wm1_copies(j):
                cp.wait()
            modulate(j, mod_block_vpu(j, j, False), mod_block_vpu(8 + j, 8 + j, True))

        nxt = jnp.where(j >= 1, jnp.minimum(j + 1, NK - 1), 0)
        wait_if(nxt == j + 1, wm1_copies(nxt))
        for cp in wv_copies(j):
            cp.wait()
        krows = pl.ds(pl.multiple_of(j * (KQ // 2), KQ // 2), KQ // 2)
        hb = [he[j, c * 256:(c + 1) * 256, :] for c in range(2)]
        pins = {}
        for c in range(2):
            rows = slice(c * 256, (c + 1) * 256)
            for q in range(NP // 2):
                i = 8 * c + q
                if c == 0:
                    relayout(2, 2 * q, krows)
                    relayout(2, 2 * q + 1, krows)
                w4 = [wv[4 * q + b, krows, :] for b in range(4)]
                if i in pins:
                    w4[0] = jnp.concatenate([w4[0][0:8] | pin_zero(pins[i]), w4[0][8:]], axis=0)
                r = _dot(hb[c], pltpu.bitcast(jnp.concatenate(w4, axis=1), BF16))
                for b in range(4):
                    acc0[4 * q + b, rows, :] = (r[:, b * DH:(b + 1) * DH]
                                                + jnp.where(j > 0, acc0[4 * q + b, rows, :], 0.0))
                if i == 7:
                    shift = mod_block_vpu(nxt, nxt, False, r[0:8, 0:128])
                if i == 9:
                    scale = mod_block_vpu(8 + nxt, 8 + nxt, True, r[0:8, 0:128])
                    h = modulate(nxt, shift, scale)
                    pins = {13: [h[0:256]], 15: [h[256:512]]}
        pr = 1 + (j >> 1)
        t = jnp.maximum(j - 5, 0)
        start_if(j + 4 < NK, wm1_copies(jnp.minimum(j + 4, NK - 1)))
        start_if_below(j, NK - 3, wv_copies(jnp.minimum(j + 3, NK - 1)))
        start_if((j & 1) == 0, w_copies(0, pr, 16 + (pr >> 2)))
        start_if((j & 1) == 1, w_copies(1, pr, 16 + (pr >> 2)))
        start_if_below(4, j, [xj_copy(t)] + w_copies(0, 5 + t, 17) + w_copies(1, 5 + t, 17)
                       + wm2_copies(16 + 4 * t, 4, 0))
        return carry

    for cp in wm1_copies(3) + wv_copies(2) + w_copies(0, 0, 16) + w_copies(1, 0, 16):
        cp.start()
    jax.lax.fori_loop(0, NK, chunk_body, 0)

    def early_proj(m, p, pins=None):
        relayout(m, p)
        for c in range(2):
            rows = slice(c * 256, (c + 1) * 256)
            hc = jnp.concatenate([he[j, rows, :] for j in range(NK)], axis=1)
            r12 = []
            for b in range(2):
                halves = []
                for k in range(2):
                    wh = wqkv[m][2 * p + b, k * 256:(k + 1) * 256, :]
                    if pins.get(4 * c + 2 * b + k):
                        wh = jnp.concatenate(
                            [wh[0:8] | pin_zero(pins[4 * c + 2 * b + k]), wh[8:]], axis=0)
                    halves.append(wh)
                r12.append(_dot(hc, pltpu.bitcast(jnp.concatenate(halves, axis=0), BF16)))
            store_early(m, p, c * 256, *r12)

    def make_hj(s):
        n = _rb(_layernorm(xv[s, 0:3].astype(F32)))
        h = _rb(n * mod_vec(1)) + mod_vec(0)
        hj[s] = h
        return [h[g, :, 0:128] for g in range(3)]

    def pro_body(g, carry):
        wait_if(g == 1, wm2_copies(16, 12, 0))
        tb = jnp.maximum(g - 2, 0)
        wait_if(g >= 2, wm2_copies(28 + 10 * tb, 10, 1 + tb))
        for cp in qk_copies(g) + [xj_copy(g)]:
            cp.wait()
        lnp = sum([make_hj(g * 16 + t) for t in range(16)], [])
        mv = []
        for b in range(MB):
            blk = 16 + MB * (g - 1) + b
            live = (g > 0) & (blk < 48)
            mv.append(mod_block_vpu(jnp.where(live, blk, b), jnp.where(live, blk, 48 + b),
                                    (blk >= 32) & (blk < 40)))
        fin = [store_early(2, 4 * g + t, 0, acc0[8 * g + 2 * t], acc0[8 * g + 2 * t + 1])
               for t in range(4)]
        sites = {i: [] for i in range(64)}
        twice = [3, 4, 6, 7, 10, 11, 12, 14, 15, 18, 19, 20, 22, 23, 26, 27, 30, 31]
        for i, v in zip(sorted(list(range(2, 32)) + twice), lnp):
            sites[2 * i].append(v)
        for i, v in zip(range(1, 31, 2), mv + fin):
            sites[2 * i + 1].append(v)
        for u, (m, p) in enumerate(units(g)):
            early_proj(m, p, {i: sites[8 * u + i] for i in range(8)})
        gn = jnp.minimum(g, 1)
        start_if_below(g, 2, qk_copies(gn + 2))
        start_if(g == 1, [xj_copy(3)])
        start_if_below(g, 2, wm2_copies(28 + 10 * gn, 10, 1 + gn))
        start_if(g == 0, cp_wo[:1])
        start_if(g == 1, cp_wo[1:])
        return carry

    jax.lax.fori_loop(0, NG, pro_body, 0)

    for cp in cp_ffn:
        cp.start()
    for cp in cp_small + cp_wo:
        cp.wait()
    pend[0:M, :] = mem0_ref[...].astype(F32)

    wr = jnp.broadcast_to(wr_ref[...].astype(F32).reshape(1, D), (8, D))

    lane8 = jax.lax.broadcasted_iota(jnp.int32, (8, 128), 1)
    sub8 = jax.lax.broadcasted_iota(jnp.int32, (8, 128), 0)
    LAST = NSEG * SEG - 1

    def post(s, g0, g1, attn, record=True):
        attn = attn.reshape(g1 - g0, 8, D)
        x1 = _rb(xv[s, g0:g1].astype(F32) + _rb(mod_vec(2) * _rb(attn)))
        n = _rb(_layernorm(x1))
        h2 = _rb(_rb(n * mod_vec(4)) + mod_vec(3))
        r = _rb(jnp.sum(h2 * wr, axis=-1, keepdims=True)) + 0.0
        x1v[s, g0:g1] = x1.astype(BF16)
        h2v[s, g0:g1] = h2.astype(BF16)
        outv[s, g0:g1] = (x1 + _rb(mod_vec(5) * h2)).astype(BF16)
        pins = []
        for g in range(g0, g1):
            bits = pltpu.bitcast(jnp.broadcast_to(r[g - g0], (8, 128)), jnp.int32)
            hi = jax.lax.shift_right_logical(bits, 16)
            code = jnp.where(bits < 0, hi ^ 0xFFFF, hi | 0x8000)
            key = (code << 11) | (LAST - (s * SEG + g * 8) - sub8) | 0x40000000
            key = pltpu.bitcast(key, F32)
            if record:
                rows = slice(g * 8, (g + 1) * 8)
                keys[rows, :] = jnp.where(lane8 == s, key, keys[rows, :])
            pins.append(key)
        return pins

    def post_pair(a, rows, record=True):
        return post(a + 1, 0, 4, rows[0:SEG], record) + post(a, 3, 4, rows[SEG:], record)

    zpad = jnp.zeros((48, DH), BF16)
    G = 4
    KA = (NP - G) * 2 * DH
    KS = D - 128

    def segment(s, lhs, lhs_split, extra, pins):
        scales = {}

        def stash(p, m, v):
            opnd[p, m, 0:v.shape[0], :] = v.astype(BF16)

        def qkv_group(p):
            keys = [(m, 2 * p + b) for m in range(3) for b in range(2 * G)]
            nsplit = 6 if (p == 0 and lhs_split is not None) else 0
            part = [_dot(lhs_split[0], w_head(m, h, 0, KS)) for m, h in keys[:nsplit]]
            full = [_dot(lhs_split[1], w_head(m, h, KS, D)) + part[i]
                    for i, (m, h) in enumerate(keys[:nsplit])]
            full += [_dot(lhs, w_head(m, h)) for m, h in keys[nsplit:]]
            for m in range(3):
                for t in range(G):
                    i = 2 * G * m + 2 * t
                    stash(p + t, m, jnp.concatenate([full[i], full[i + 1]], axis=0))

        def operand(p, m):
            parts = [opnd[p, m, 0:64, :], pltpu.bitcast(early[s, m * NP + p], BF16)]
            if m > 0:
                parts.append(zpad)
            return jnp.concatenate(parts, axis=0)

        def scores(p):
            sc_ = _dot_nt(operand(p, 0), operand(p, 1))
            f = fill[...]
            if pins.get(p):
                f = jnp.concatenate([f[0:8] + pltpu.bitcast(pin_zero(pins[p]), F32), f[8:]], axis=0)
            sc_ = jnp.where(f == 0.0, sc_, f)
            mx = jnp.max(sc_, axis=-1, keepdims=True)
            e = jnp.exp2((sc_ - mx) * (SCALE * LOG2E))
            inv = pl.reciprocal(jnp.sum(e, axis=-1, keepdims=True), approx=True)
            if p // G == NP // G - 2:
                stash(p, 3, e * inv)
            else:
                stash(p, 3, e)
                scales[p] = inv

        oe = []

        def pv(p):
            o = _dot(opnd[p, 3], operand(p, 2))
            if p in scales:
                o = o * scales[p]
                pins.setdefault(p + G, []).append(o)
            res = []
            for b in range(2):
                rows, erows = o[32 * b:32 * b + 32], o[64 + 8 * b:72 + 8 * b]
                oe.append(erows)
                if extra is not None:
                    rows = jnp.concatenate([rows, erows, extra[2 * p + b]], axis=0)
                res.append(rows)
            return res

        os_ = []
        for p in range(0, NP, G):
            qkv_group(p)
            if p >= G:
                for t in range(G):
                    os_ += pv(p - G + t)
            for t in range(G):
                scores(p + t)
        oa = jnp.concatenate(os_, axis=1).astype(BF16)
        acc, ob = [], []
        for n in range(7):
            acc.append(_dot(oa, wo_blk(n, 0, KA)))
            if n == 1:
                for t in range(G):
                    ob += pv(NP - G + t)
        ob = jnp.concatenate(ob, axis=1).astype(BF16)
        res = [_dot(ob, wo_blk(n, KA, H * DH)) + acc[n] for n in range(7)]
        res.append(_dot(ob, wo_blk(7, KA, H * DH)) + _dot(oa, wo_blk(7, 0, KA)))
        return res, oe

    def make_lhs(mem, s):
        return jnp.concatenate([mem, hj[s].reshape(NJ, D)], axis=0)

    cp_o1 = pltpu.make_async_copy(outv.at[0:OUT_SPLIT], out_hbm.at[0:OUT_SPLIT], sem_out.at[0])
    cp_o2 = pltpu.make_async_copy(outv.at[OUT_SPLIT:NSEG], out_hbm.at[OUT_SPLIT:NSEG],
                                  sem_out.at[1])

    def split_lhs(lhs):
        return lhs.astype(BF16), (lhs[:, :KS].astype(BF16), lhs[:, KS:].astype(BF16))

    def step(i, carry):
        @pl.when(i == NIT - 1)
        def _():
            cp_o1.start()

        prev = pend[...]
        for u in range(UNROLL):
            a = 2 * (UNROLL * i + u)
            pins = post_pair(jnp.maximum(a - 2, 0) if u == 0 else a - 2, prev[M:])
            lhs_a = make_lhs(prev[0:M], a)
            lhs_a = (lhs_a.astype(BF16), None) if u == 0 else split_lhs(lhs_a)
            res_a, oe_a = segment(a, *lhs_a, None,
                                  {k: [v] for k, v in zip((2, 6, 10, 14), pins[:4])})
            res_a = jnp.concatenate(res_a, axis=1)
            pins = pins[4:] + post(a, 0, 3, res_a[M:])
            res_b, _ = segment(a + 1, *split_lhs(make_lhs(res_a[0:M], a + 1)), oe_a,
                               {k: [v] for k, v in zip((2, 6, 10, 14), pins)})
            prev = jnp.concatenate(res_b, axis=1)
        pend[...] = prev
        return carry

    jax.lax.fori_loop(0, NIT, step, 0)
    for cp in cp_ffn:
        cp.wait()
    last_keys = post_pair(NSEG - 2, pend[M:, :], record=False)
    cp_o2.start()

    def max_all(v):
        return jnp.max(jnp.max(v, axis=0, keepdims=True), axis=1, keepdims=True)

    def decode(k):
        kb = pltpu.bitcast(jnp.broadcast_to(k, (8, 128)), jnp.int32)
        code = (kb >> 11) & 0xFFFF
        hi = jnp.where(code >= 0x8000, code & 0x7FFF, code ^ 0xFFFF)
        tok = jnp.clip((LAST - (kb & LAST))[0, 0], 0, LAST)
        return tok, pltpu.bitcast(hi << 16, F32)[:, 0:1]

    kv = keys[...]
    o1 = max_all(kv)
    o2 = max_all(jnp.where(kv == o1, 0.0, kv))
    kv = jnp.concatenate(last_keys + [jnp.where(sub8 < 4, o1, o2)], axis=0)
    k1 = jnp.max(kv, axis=0, keepdims=True)
    k2 = jnp.max(jnp.where(kv == k1, 0.0, kv), axis=0, keepdims=True)
    i1, r1 = decode(k1)
    i2, r2 = decode(k2)
    g1, g2 = i1 >> 3, i2 >> 3

    def rows_of(ref):
        return jnp.concatenate([ref[g1 >> 2, pl.ds(g1 & 3, 1)], ref[g2 >> 2, pl.ds(g2 & 3, 1)]],
                               axis=0).astype(F32)

    x1, h2 = rows_of(x1v), rows_of(h2v)
    hl = h2.reshape(16, D).astype(BF16)
    act = []
    for j in range(FF // 128):
        gt = _rb(_dot(hl, wblk(wg, j)))
        up = _rb(_dot(hl, wblk(wu, j)))
        act.append((_rb(gt * _sigmoid(gt)) * up).astype(BF16))
    act = jnp.concatenate(act, axis=1)
    y = jnp.concatenate([_dot(act, wblk(wd, n)) for n in range(8)], axis=1).reshape(2, 8, D)
    rowi = jax.lax.broadcasted_iota(jnp.int32, (2, 8, 1), 1)
    gsel = jax.lax.broadcasted_iota(jnp.int32, (2, 8, 1), 0)
    tokp = jnp.where(gsel == 0, g1, g2) * 8 + rowi
    gate = _sigmoid(jnp.where(tokp == i1, r1[None], r2[None]))
    upd = jnp.where((tokp == i1) | (tokp == i2), _rb(_rb(y) * gate), 0.0)
    patch[...] = (x1 + _rb(mod_vec(5) * _rb(h2 + upd))).astype(BF16)
    cp_o1.wait()
    cp_o2.wait()
    cp1 = pltpu.make_async_copy(patch.at[0], out_hbm.at[g1 >> 2, g1 & 3], sem_out.at[0])
    cp1.start()

    @pl.when(g1 != g2)
    def _():
        cp2 = pltpu.make_async_copy(patch.at[1], out_hbm.at[g2 >> 2, g2 & 3], sem_out.at[1])
        cp2.start()
        cp2.wait()

    cp1.wait()


@jax.jit
def pallas_adaLN_cond__memory_aug_recurrent_mem_tr__moe_arch_mod__prompt_kernel(
    A_x: jax.Array,
    A_mem0: jax.Array,
    A_Wq: jax.Array,
    A_Wk: jax.Array,
    A_Wv: jax.Array,
    A_Wo: jax.Array,
    A_seg_len,
    B_x: jax.Array,
    B_w_r: jax.Array,
    B_w_gate: jax.Array,
    B_w_up: jax.Array,
    B_w_down: jax.Array,
    c: jax.Array,
    w_mod: jax.Array,
):
    assert A_x.shape == (1, NSEG * SEG, D)
    any_spec = pl.BlockSpec(memory_space=pl.ANY)
    out = pl.pallas_call(
        _kernel,
        out_shape=jax.ShapeDtypeStruct((NSEG, 4, 8, D), BF16),
        in_specs=[any_spec] * 12,
        out_specs=any_spec,
        scratch_shapes=[
            pltpu.VMEM((H, D // 2, DH), U32),
            pltpu.VMEM((H, D // 2, DH), U32),
            pltpu.VMEM((H, D // 2, DH), U32),
            pltpu.VMEM((8, H * DH // 2, 128), U32),
            pltpu.VMEM((D // 2, FF + 128), U32),
            pltpu.VMEM((D // 2, FF + 128), U32),
            pltpu.VMEM((FF // 2, D + 128), U32),
            pltpu.VMEM((48, D // 2, 128), U32),
            pltpu.VMEM((D + 32, 128), F32),
            pltpu.VMEM((NSEG, 4, 8, D), BF16),
            pltpu.VMEM((NSEG, 4, 8, D), BF16),
            pltpu.VMEM((NSEG, 4, 8, D), BF16),
            pltpu.VMEM((NSEG, 4, 8, D), BF16),
            pltpu.VMEM((NSEG, 3 * NP, 8, DH), U32),
            pltpu.VMEM((NK, NE, KQ), BF16),
            pltpu.VMEM((NK, NE, KQ), BF16),
            pltpu.VMEM((NSEG, 3, 8, D), F32),
            pltpu.VMEM((M + SEG + M, D), F32),
            pltpu.VMEM((48 + 16, 8, 128), F32),
            pltpu.VMEM((80, 128), F32),
            pltpu.VMEM((SEG, 128), F32),
            pltpu.VMEM((2, 8, D), BF16),
            pltpu.VMEM((8, 128), U32),
            pltpu.VMEM((NP, 4, 80, DH), BF16),
            pltpu.VMEM((H, NE, DH), F32),
            pltpu.VMEM((M, D), BF16),
            pltpu.VMEM((D,), BF16),
            pltpu.VMEM((1, D), BF16),
            pltpu.SemaphoreType.DMA((24 + NK,)),
            pltpu.SemaphoreType.DMA((2,)),
        ],
        compiler_params=pltpu.CompilerParams(vmem_limit_bytes=124 * 1024 * 1024,
                                             disable_bounds_checks=True,
                                             disable_semaphore_checks=True),
    )(
        A_x.reshape(NSEG, 4, 8, D),
        A_mem0.reshape(M, D),
        A_Wq.reshape(D // 2, 2, H, DH),
        A_Wk.reshape(D // 2, 2, H, DH),
        A_Wv.reshape(D // 2, 2, H, DH),
        A_Wo.reshape(H * DH, D),
        B_w_r,
        B_w_gate,
        B_w_up,
        B_w_down,
        c,
        w_mod,
    )
    return out.reshape(1, NSEG * SEG, D)
```

```python
import jax
import jax.numpy as jnp
import jax.experimental.pallas as pl
import jax.experimental.pallas.tpu as pltpu

F32 = jnp.float32
BF16 = jnp.bfloat16
U32 = jnp.uint32

D = 1024
H = 32
DH = 128
NP = H // 2
M = 8
SEG = 32
NSEG = 64
FF = 3584
NJ = SEG - M
NE = NSEG * M
EPS = 1.0013580322265625e-05
SCALE = DH ** (-0.5)
NEG = -1000000000.0
LOG2E = 1.4426950408889634
KQ = 128
NK = D // KQ
MB = 11
NG = 4
UNROLL = 2
NIT = NSEG // (2 * UNROLL)
OUT_SPLIT = NSEG - 2 * UNROLL - 2


def _rb(x):
    return x.astype(BF16).astype(F32)


def _layernorm(xf):
    m = jnp.mean(xf, axis=-1, keepdims=True)
    d = xf - m
    v = jnp.mean(d * d, axis=-1, keepdims=True)
    std = _rb(jnp.sqrt(_rb(_rb(v) + EPS)))
    return _rb(xf - _rb(m)) * (1.0 / std)


def _sigmoid(x):
    return _rb(1.0 / _rb(1.0 + _rb(jnp.exp(-x))))


def _dot(a, b):
    return jnp.dot(a, b, preferred_element_type=F32)


def _dot_nt(a, b):
    return jax.lax.dot_general(a, b, (((1,), (1,)), ((), ())), preferred_element_type=F32)


def _kernel(x_hbm, mem0_hbm, wq_hbm, wk_hbm, wv_hbm, wo_hbm, wr_hbm, wg_hbm, wu_hbm, wd_hbm,
            c_hbm, wm_hbm,
            out_hbm,
            wq, wk, wv, wo, wg, wu, wd, wm, cb, xv, x1v, h2v, outv, early, hn, he, hj, pend,
            mod, fill, keys, patch, zero, opnd, acc0, mem0_ref, wr_ref, c_ref,
            sem, sem_out):
    w_u32 = [w.bitcast(U32) for w in (wq_hbm, wk_hbm, wv_hbm)]
    wqkv = (wq, wk, wv)
    wo_hbm, wg_hbm, wu_hbm, wd_hbm, wm_hbm = [
        w.bitcast(U32) for w in (wo_hbm, wg_hbm, wu_hbm, wd_hbm, wm_hbm)]

    def wblk(w, j):
        return pltpu.bitcast(w[:, j * 128:(j + 1) * 128], BF16)

    def wo_blk(n, lo, hi):
        return pltpu.bitcast(wo[n, lo // 2:hi // 2, :], BF16)

    def w_copies(m, p, k):
        return [pltpu.make_async_copy(w_u32[m].at[:, par, p, :], wqkv[m].at[2 * p + par], sem.at[k])
                for par in range(2)]

    def col_copy(src, dst, j, k):
        lo = j * 128 if isinstance(j, int) else pl.multiple_of(j * 128, 128)
        return pltpu.make_async_copy(src.at[:, pl.ds(lo, 128)], dst.at[j], sem.at[k])

    def units(g):
        return [(m, 4 * g + t) for t in range(4) for m in range(2)]

    def xj_copy(g):
        segs = pl.ds(16 * g, 16)
        return pltpu.make_async_copy(x_hbm.at[segs, 0:3], xv.at[segs, 0:3], sem.at[16 + g])

    def qk_copies(g):
        return sum([w_copies(m, p, 16 + g) for m, p in units(g)], [])

    def wm1_copies(j):
        return [col_copy(wm_hbm, wm, j, 1 + j), col_copy(wm_hbm, wm, 8 + j, 1 + j)]

    def wv_copies(j):
        lo = j * (KQ // 2) if isinstance(j, int) else pl.multiple_of(j * (KQ // 2), KQ // 2)
        rows = pl.ds(lo, KQ // 2)
        return [pltpu.make_async_copy(w_u32[2].at[rows, par, p, :], wv.at[2 * p + par, rows],
                                      sem.at[24 + j]) for p in range(NP) for par in range(2)]

    def wm2_copies(lo, n, t):
        return [col_copy(wm_hbm, wm, lo + b, 20 + t) for b in range(n)]

    def wait_if(cond, cps):
        for cp in cps:
            pl.when(cond)(cp.wait)

    def start_if(cond, cps):
        for cp in cps:
            pl.when(cond)(cp.start)

    def start_if_below(i, n, cps):
        for k in range(0, len(cps), 4):
            start_if(i < n if k % 8 == 0 else i + 1 <= n, cps[k:k + 4])

    cp_c = pltpu.make_async_copy(c_hbm, c_ref, sem.at[9])
    cp_xe = pltpu.make_async_copy(x_hbm.at[:, 3], xv.at[:, 3], sem.at[0])
    cp_wo = [col_copy(wo_hbm, wo, n, 10) for n in range(8)]
    cp_small = [pltpu.make_async_copy(mem0_hbm, mem0_ref, sem.at[14]),
                pltpu.make_async_copy(wr_hbm, wr_ref, sem.at[15])]
    cp_ffn = [pltpu.make_async_copy(wg_hbm, wg.at[:, 0:FF], sem.at[11]),
              pltpu.make_async_copy(wu_hbm, wu.at[:, 0:FF], sem.at[12]),
              pltpu.make_async_copy(wd_hbm, wd.at[:, 0:D], sem.at[13])]

    for cp in ([cp_c, cp_xe] + wm1_copies(0) + wv_copies(0) + wm1_copies(1) + wm1_copies(2)
               + wv_copies(1) + cp_small):
        cp.start()

    ri = jax.lax.broadcasted_iota(jnp.int32, (80, 128), 0)
    ci = jax.lax.broadcasted_iota(jnp.int32, (80, 128), 1)

    def head_of(i):
        return jnp.where(i < 64, i >> 5, (i - 64) >> 3)

    def pos_of(i):
        return jnp.where(i < 64, i & 31, 32 + (i & 7))

    same = (head_of(ri) == head_of(ci)) & (ci < 80)
    allowed = (pos_of(ri) < M) | (pos_of(ri) >= pos_of(ci))
    fill[...] = jnp.where(same, jnp.where(allowed, 0.0, NEG / SCALE), -jnp.inf).astype(F32)
    keys[...] = jnp.zeros(keys.shape, F32)
    pend[M:, :] = jnp.zeros((SEG + M, D), F32)
    zero[...] = jnp.zeros(zero.shape, U32)

    def pin_zero(vals):
        acc = None
        for v in vals:
            v = pltpu.bitcast(v, U32)
            for r in range(0, v.shape[0], 8):
                acc = v[r:r + 8] if acc is None else acc | v[r:r + 8]
        return acc & zero[...]

    cp_c.wait()
    cf = c_ref[...].astype(F32)
    sc = _rb(cf * _sigmoid(cf))
    cb[0:D, :] = jnp.broadcast_to(sc, (128, D)).T
    cb[D:, :] = jnp.zeros((32, 128), F32)

    def mod_vec(k):
        return jnp.concatenate([mod[8 * k + b] for b in range(8)], axis=1)

    def mod_block_vpu(src, dst, is_scale, after=None):
        acc = None if after is None else pltpu.bitcast(pin_zero([after]), F32)
        for r in range(0, D // 2, 8):
            w = wm[src, r:r + 8, :]
            t0 = pltpu.bitcast(w << 16, F32) * cb[pl.ds(2 * r, 8, stride=2), :]
            t1 = pltpu.bitcast(w & U32(0xFFFF0000), F32) * cb[pl.ds(2 * r + 1, 8, stride=2), :]
            if after is not None:
                acc = (acc + t0) + t1
            else:
                acc = t0 + t1 if acc is None else acc + (t0 + t1)
        v = _rb(jnp.broadcast_to(jnp.sum(acc, axis=0, keepdims=True), (8, 128)))
        v = jnp.where(is_scale, _rb(1.0 + v), v)
        mod[dst] = v
        return v

    def ne_body(i, carry):
        n = _layernorm(xv[pl.ds(i * 16, 16), 3].astype(F32)).reshape(128, D).astype(BF16)
        for j in range(NK):
            hn[j, pl.ds(pl.multiple_of(i * 128, 128), 128), :] = n[:, j * KQ:(j + 1) * KQ]
        return carry

    cp_xe.wait()
    jax.lax.fori_loop(0, NSEG // 16, ne_body, 0)

    def w_head(m, h, lo=0, hi=D):
        return pltpu.bitcast(wqkv[m][h, lo // 2:hi // 2, :], BF16)

    def relayout(m, p, rows=slice(None)):
        w = wqkv[m]
        e = w[2 * p, rows, :]
        o = w[2 * p + 1, rows, :]
        w[2 * p, rows, :] = (e & U32(0xFFFF)) | (o << 16)
        w[2 * p + 1, rows, :] = (e >> 16) | (o & U32(0xFFFF0000))

    def store_early(m, p, row0, r1, r2):
        ns = r1.shape[0] // 8
        r12 = jnp.concatenate([r1.reshape(ns, 8, DH), r2.reshape(ns, 8, DH)], axis=1)
        v = pltpu.bitcast(r12.reshape(16 * ns, DH).astype(BF16), U32)
        early[row0 // 8:row0 // 8 + ns, m * NP + p] = v.reshape(ns, 8, DH)
        return v

    def modulate(src, dst, shift, scale):
        n = hn[src].astype(F32).reshape(NSEG, 8, KQ)
        h = (_rb(n * scale) + shift).reshape(NE, KQ)
        he[dst] = h.astype(BF16)
        return h

    def chunk_body(j, carry):
        @pl.when(j <= 1)
        def _():
            for cp in wm1_copies(j):
                cp.wait()
            modulate(j, j, mod_block_vpu(j, j, False), mod_block_vpu(8 + j, 8 + j, True))

        nxt = jnp.where(j >= 1, jnp.minimum(j + 1, NK - 1), 0)
        live = nxt == j + 1
        wait_if(live, wm1_copies(nxt))
        for cp in wv_copies(j):
            cp.wait()
        krows = pl.ds(pl.multiple_of(j * (KQ // 2), KQ // 2), KQ // 2)
        hb = [he[j, c * 256:(c + 1) * 256, :] for c in range(2)]
        pins = {}
        for c in range(2):
            rows = slice(c * 256, (c + 1) * 256)
            for q in range(NP // 2):
                i = 8 * c + q
                if c == 0:
                    relayout(2, 2 * q, krows)
                    relayout(2, 2 * q + 1, krows)
                w4 = [wv[4 * q + b, krows, :] for b in range(4)]
                if i in pins:
                    w4[0] = jnp.concatenate([w4[0][0:8] | pin_zero(pins[i]), w4[0][8:]], axis=0)
                r = _dot(hb[c], pltpu.bitcast(jnp.concatenate(w4, axis=1), BF16))
                for b in range(4):
                    acc0[4 * q + b, rows, :] = (r[:, b * DH:(b + 1) * DH]
                                                + jnp.where(j > 0, acc0[4 * q + b, rows, :], 0.0))
                if i == 7:
                    shift = mod_block_vpu(nxt, jnp.where(live, nxt, 48), False, r[0:8, 0:128])
                if i == 9:
                    scale = mod_block_vpu(8 + nxt, jnp.where(live, 8 + nxt, 49), True,
                                          r[0:8, 0:128])
                    h = modulate(nxt, jnp.where(live, nxt, NK), shift, scale)
                    pins = {13: [h[0:256]], 15: [h[256:512]]}
        pr = 1 + (j >> 1)
        t = jnp.maximum(j - 5, 0)
        start_if(j + 4 < NK, wm1_copies(jnp.minimum(j + 4, NK - 1)))
        start_if_below(j, NK - 3, wv_copies(jnp.minimum(j + 3, NK - 1)))
        start_if((j & 1) == 0, w_copies(0, pr, 16 + (pr >> 2)))
        start_if((j & 1) == 1, w_copies(1, pr, 16 + (pr >> 2)))
        start_if_below(4, j, [xj_copy(t)] + w_copies(0, 5 + t, 17) + w_copies(1, 5 + t, 17)
                       + wm2_copies(16 + 4 * t, 4, 0))
        return carry

    for cp in wm1_copies(3) + wv_copies(2) + w_copies(0, 0, 16) + w_copies(1, 0, 16):
        cp.start()
    jax.lax.fori_loop(0, NK, chunk_body, 0)

    def early_proj(m, p, pins):
        relayout(m, p)
        for c in range(2):
            rows = slice(c * 256, (c + 1) * 256)
            hc = jnp.concatenate([he[j, rows, :] for j in range(NK)], axis=1)
            r12 = []
            for b in range(2):
                halves = []
                for k in range(2):
                    wh = wqkv[m][2 * p + b, k * 256:(k + 1) * 256, :]
                    if pins.get(4 * c + 2 * b + k):
                        wh = jnp.concatenate(
                            [wh[0:8] | pin_zero(pins[4 * c + 2 * b + k]), wh[8:]], axis=0)
                    halves.append(wh)
                r12.append(_dot(hc, pltpu.bitcast(jnp.concatenate(halves, axis=0), BF16)))
            store_early(m, p, c * 256, *r12)

    def make_hj(s):
        n = _rb(_layernorm(xv[s, 0:3].astype(F32)))
        h = _rb(n * mod_vec(1)) + mod_vec(0)
        hj[s] = h
        return [h[g, :, 0:128] for g in range(3)]

    def pro_body(g, carry):
        wait_if(g == 1, wm2_copies(16, 12, 0))
        tb = jnp.maximum(g - 2, 0)
        wait_if(g >= 2, wm2_copies(28 + 10 * tb, 10, 1 + tb))
        for cp in qk_copies(g) + [xj_copy(g)]:
            cp.wait()
        lnp = sum([make_hj(g * 16 + t) for t in range(16)], [])
        mv = []
        for b in range(MB):
            blk = 16 + MB * (g - 1) + b
            live = (g > 0) & (blk < 48)
            mv.append(mod_block_vpu(jnp.where(live, blk, b), jnp.where(live, blk, 48 + b),
                                    (blk >= 32) & (blk < 40)))
        fin = [store_early(2, 4 * g + t, 0, acc0[8 * g + 2 * t], acc0[8 * g + 2 * t + 1])
               for t in range(4)]
        sites = {i: [] for i in range(64)}
        twice = [3, 4, 6, 7, 10, 11, 12, 14, 15, 18, 19, 20, 22, 23, 26, 27, 30, 31]
        for i, v in zip(sorted(list(range(2, 32)) + twice), lnp):
            sites[2 * i].append(v)
        for i, v in zip(range(1, 31, 2), mv + fin):
            sites[2 * i + 1].append(v)
        for u, (m, p) in enumerate(units(g)):
            early_proj(m, p, {i: sites[8 * u + i] for i in range(8)})
        gn = jnp.minimum(g, 1)
        start_if_below(g, 2, qk_copies(gn + 2))
        start_if(g == 1, [xj_copy(3)])
        start_if_below(g, 2, wm2_copies(28 + 10 * gn, 10, 1 + gn))
        start_if(g == 0, cp_wo[:1])
        start_if(g == 1, cp_wo[1:])
        return carry

    jax.lax.fori_loop(0, NG, pro_body, 0)

    for cp in cp_ffn:
        cp.start()
    for cp in cp_small + cp_wo:
        cp.wait()
    pend[0:M, :] = mem0_ref[...].astype(F32)

    wr = jnp.broadcast_to(wr_ref[...].astype(F32).reshape(1, D), (8, D))

    lane8 = jax.lax.broadcasted_iota(jnp.int32, (8, 128), 1)
    sub8 = jax.lax.broadcasted_iota(jnp.int32, (8, 128), 0)
    LAST = NSEG * SEG - 1

    def post(s, g0, g1, attn, record=True):
        attn = attn.reshape(g1 - g0, 8, D)
        x1 = _rb(xv[s, g0:g1].astype(F32) + _rb(mod_vec(2) * _rb(attn)))
        n = _rb(_layernorm(x1))
        h2 = _rb(_rb(n * mod_vec(4)) + mod_vec(3))
        r = _rb(jnp.sum(h2 * wr, axis=-1, keepdims=True)) + 0.0
        x1v[s, g0:g1] = x1.astype(BF16)
        h2v[s, g0:g1] = h2.astype(BF16)
        outv[s, g0:g1] = (x1 + _rb(mod_vec(5) * h2)).astype(BF16)
        pins = []
        for g in range(g0, g1):
            bits = pltpu.bitcast(jnp.broadcast_to(r[g - g0], (8, 128)), jnp.int32)
            hi = jax.lax.shift_right_logical(bits, 16)
            code = jnp.where(bits < 0, hi ^ 0xFFFF, hi | 0x8000)
            key = (code << 11) | (LAST - (s * SEG + g * 8) - sub8) | 0x40000000
            key = pltpu.bitcast(key, F32)
            if record:
                rows = slice(g * 8, (g + 1) * 8)
                keys[rows, :] = jnp.where(lane8 == s, key, keys[rows, :])
            pins.append(key)
        return pins

    def post_pair(a, rows, record=True):
        return post(a + 1, 0, 4, rows[0:SEG], record) + post(a, 3, 4, rows[SEG:], record)

    zpad = jnp.zeros((48, DH), BF16)
    G = 4
    KA = (NP - G) * 2 * DH
    KS = D - 128

    def segment(s, lhs, lhs_split, extra, pins):
        scales = {}

        def stash(p, m, v):
            opnd[p, m, 0:v.shape[0], :] = v.astype(BF16)

        def qkv_group(p):
            keys = [(m, 2 * p + b) for m in range(3) for b in range(2 * G)]
            nsplit = 6 if (p == 0 and lhs_split is not None) else 0
            part = [_dot(lhs_split[0], w_head(m, h, 0, KS)) for m, h in keys[:nsplit]]
            full = [_dot(lhs_split[1], w_head(m, h, KS, D)) + part[i]
                    for i, (m, h) in enumerate(keys[:nsplit])]
            full += [_dot(lhs, w_head(m, h)) for m, h in keys[nsplit:]]
            for m in range(3):
                for t in range(G):
                    i = 2 * G * m + 2 * t
                    stash(p + t, m, jnp.concatenate([full[i], full[i + 1]], axis=0))

        def operand(p, m):
            parts = [opnd[p, m, 0:64, :], pltpu.bitcast(early[s, m * NP + p], BF16)]
            if m > 0:
                parts.append(zpad)
            return jnp.concatenate(parts, axis=0)

        def scores(p):
            sc_ = _dot_nt(operand(p, 0), operand(p, 1))
            f = fill[...]
            if pins.get(p):
                f = jnp.concatenate([f[0:8] + pltpu.bitcast(pin_zero(pins[p]), F32), f[8:]], axis=0)
            sc_ = jnp.where(f == 0.0, sc_, f)
            mx = jnp.max(sc_, axis=-1, keepdims=True)
            e = jnp.exp2((sc_ - mx) * (SCALE * LOG2E))
            inv = pl.reciprocal(jnp.sum(e, axis=-1, keepdims=True), approx=True)
            if p // G == NP // G - 2:
                stash(p, 3, e * inv)
            else:
                stash(p, 3, e)
                scales[p] = inv

        oe = []

        def pv(p):
            o = _dot(opnd[p, 3], operand(p, 2))
            if p in scales:
                o = o * scales[p]
                pins.setdefault(p + G, []).append(o)
            res = []
            for b in range(2):
                rows, erows = o[32 * b:32 * b + 32], o[64 + 8 * b:72 + 8 * b]
                oe.append(erows)
                if extra is not None:
                    rows = jnp.concatenate([rows, erows, extra[2 * p + b]], axis=0)
                res.append(rows)
            return res

        os_ = []
        for p in range(0, NP, G):
            qkv_group(p)
            if p >= G:
                for t in range(G):
                    os_ += pv(p - G + t)
            for t in range(G):
                scores(p + t)
        oa = jnp.concatenate(os_, axis=1).astype(BF16)
        acc, ob = [], []
        for n in range(7):
            acc.append(_dot(oa, wo_blk(n, 0, KA)))
            if n == 1:
                for t in range(G):
                    ob += pv(NP - G + t)
        ob = jnp.concatenate(ob, axis=1).astype(BF16)
        res = [_dot(ob, wo_blk(n, KA, H * DH)) + acc[n] for n in range(7)]
        res.append(_dot(ob, wo_blk(7, KA, H * DH)) + _dot(oa, wo_blk(7, 0, KA)))
        return res, oe

    def make_lhs(mem, s):
        return jnp.concatenate([mem, hj[s].reshape(NJ, D)], axis=0)

    cp_o1 = pltpu.make_async_copy(outv.at[0:OUT_SPLIT], out_hbm.at[0:OUT_SPLIT], sem_out.at[0])
    cp_o2 = pltpu.make_async_copy(outv.at[OUT_SPLIT:NSEG], out_hbm.at[OUT_SPLIT:NSEG],
                                  sem_out.at[1])

    def split_lhs(lhs):
        return lhs.astype(BF16), (lhs[:, :KS].astype(BF16), lhs[:, KS:].astype(BF16))

    def step(i, carry):
        @pl.when(i == NIT - 1)
        def _():
            cp_o1.start()

        prev = pend[...]
        for u in range(UNROLL):
            a = 2 * (UNROLL * i + u)
            pins = post_pair(jnp.maximum(a - 2, 0) if u == 0 else a - 2, prev[M:])
            lhs_a = make_lhs(prev[0:M], a)
            lhs_a = (lhs_a.astype(BF16), None) if u == 0 else split_lhs(lhs_a)
            res_a, oe_a = segment(a, *lhs_a, None,
                                  {k: [v] for k, v in zip((2, 6, 10, 14), pins[:4])})
            res_a = jnp.concatenate(res_a, axis=1)
            pins = pins[4:] + post(a, 0, 3, res_a[M:])
            res_b, _ = segment(a + 1, *split_lhs(make_lhs(res_a[0:M], a + 1)), oe_a,
                               {k: [v] for k, v in zip((2, 6, 10, 14), pins)})
            prev = jnp.concatenate(res_b, axis=1)
        pend[...] = prev
        return carry

    jax.lax.fori_loop(0, NIT, step, 0)
    for cp in cp_ffn:
        cp.wait()
    last_keys = post_pair(NSEG - 2, pend[M:, :], record=False)
    cp_o2.start()

    def max_all(v):
        return jnp.max(jnp.max(v, axis=0, keepdims=True), axis=1, keepdims=True)

    def decode(k):
        kb = pltpu.bitcast(jnp.broadcast_to(k, (8, 128)), jnp.int32)
        code = (kb >> 11) & 0xFFFF
        hi = jnp.where(code >= 0x8000, code & 0x7FFF, code ^ 0xFFFF)
        tok = jnp.clip((LAST - (kb & LAST))[0, 0], 0, LAST)
        return tok, pltpu.bitcast(hi << 16, F32)[:, 0:1]

    kv = keys[...]
    o1 = max_all(kv)
    o2 = max_all(jnp.where(kv == o1, 0.0, kv))
    kv = jnp.concatenate(last_keys + [jnp.where(sub8 < 4, o1, o2)], axis=0)
    k1 = jnp.max(kv, axis=0, keepdims=True)
    k2 = jnp.max(jnp.where(kv == k1, 0.0, kv), axis=0, keepdims=True)
    i1, r1 = decode(k1)
    i2, r2 = decode(k2)
    g1, g2 = i1 >> 3, i2 >> 3

    def rows_of(ref):
        return jnp.concatenate([ref[g1 >> 2, pl.ds(g1 & 3, 1)], ref[g2 >> 2, pl.ds(g2 & 3, 1)]],
                               axis=0).astype(F32)

    x1, h2 = rows_of(x1v), rows_of(h2v)
    hl = h2.reshape(16, D).astype(BF16)
    act = []
    for j in range(FF // 128):
        gt = _rb(_dot(hl, wblk(wg, j)))
        up = _rb(_dot(hl, wblk(wu, j)))
        act.append((_rb(gt * _sigmoid(gt)) * up).astype(BF16))
    act = jnp.concatenate(act, axis=1)
    y = jnp.concatenate([_dot(act, wblk(wd, n)) for n in range(8)], axis=1).reshape(2, 8, D)
    rowi = jax.lax.broadcasted_iota(jnp.int32, (2, 8, 1), 1)
    gsel = jax.lax.broadcasted_iota(jnp.int32, (2, 8, 1), 0)
    tokp = jnp.where(gsel == 0, g1, g2) * 8 + rowi
    gate = _sigmoid(jnp.where(tokp == i1, r1[None], r2[None]))
    upd = jnp.where((tokp == i1) | (tokp == i2), _rb(_rb(y) * gate), 0.0)
    patch[...] = (x1 + _rb(mod_vec(5) * _rb(h2 + upd))).astype(BF16)
    cp_o1.wait()
    cp_o2.wait()
    cp1 = pltpu.make_async_copy(patch.at[0], out_hbm.at[g1 >> 2, g1 & 3], sem_out.at[0])
    cp1.start()

    @pl.when(g1 != g2)
    def _():
        cp2 = pltpu.make_async_copy(patch.at[1], out_hbm.at[g2 >> 2, g2 & 3], sem_out.at[1])
        cp2.start()
        cp2.wait()

    cp1.wait()


@jax.jit
def pallas_adaLN_cond__memory_aug_recurrent_mem_tr__moe_arch_mod__prompt_kernel(
    A_x: jax.Array,
    A_mem0: jax.Array,
    A_Wq: jax.Array,
    A_Wk: jax.Array,
    A_Wv: jax.Array,
    A_Wo: jax.Array,
    A_seg_len,
    B_x: jax.Array,
    B_w_r: jax.Array,
    B_w_gate: jax.Array,
    B_w_up: jax.Array,
    B_w_down: jax.Array,
    c: jax.Array,
    w_mod: jax.Array,
):
    assert A_x.shape == (1, NSEG * SEG, D)
    any_spec = pl.BlockSpec(memory_space=pl.ANY)
    out = pl.pallas_call(
        _kernel,
        out_shape=jax.ShapeDtypeStruct((NSEG, 4, 8, D), BF16),
        in_specs=[any_spec] * 12,
        out_specs=any_spec,
        scratch_shapes=[
            pltpu.VMEM((H, D // 2, DH), U32),
            pltpu.VMEM((H, D // 2, DH), U32),
            pltpu.VMEM((H, D // 2, DH), U32),
            pltpu.VMEM((8, H * DH // 2, 128), U32),
            pltpu.VMEM((D // 2, FF + 128), U32),
            pltpu.VMEM((D // 2, FF + 128), U32),
            pltpu.VMEM((FF // 2, D + 128), U32),
            pltpu.VMEM((48, D // 2, 128), U32),
            pltpu.VMEM((D + 32, 128), F32),
            pltpu.VMEM((NSEG, 4, 8, D), BF16),
            pltpu.VMEM((NSEG, 4, 8, D), BF16),
            pltpu.VMEM((NSEG, 4, 8, D), BF16),
            pltpu.VMEM((NSEG, 4, 8, D), BF16),
            pltpu.VMEM((NSEG, 3 * NP, 8, DH), U32),
            pltpu.VMEM((NK, NE, KQ), BF16),
            pltpu.VMEM((NK + 1, NE, KQ), BF16),
            pltpu.VMEM((NSEG, 3, 8, D), F32),
            pltpu.VMEM((M + SEG + M, D), F32),
            pltpu.VMEM((48 + 16, 8, 128), F32),
            pltpu.VMEM((80, 128), F32),
            pltpu.VMEM((SEG, 128), F32),
            pltpu.VMEM((2, 8, D), BF16),
            pltpu.VMEM((8, 128), U32),
            pltpu.VMEM((NP, 4, 80, DH), BF16),
            pltpu.VMEM((H, NE, DH), F32),
            pltpu.VMEM((M, D), BF16),
            pltpu.VMEM((D,), BF16),
            pltpu.VMEM((1, D), BF16),
            pltpu.SemaphoreType.DMA((24 + NK,)),
            pltpu.SemaphoreType.DMA((2,)),
        ],
        compiler_params=pltpu.CompilerParams(vmem_limit_bytes=124 * 1024 * 1024,
                                             disable_bounds_checks=True,
                                             disable_semaphore_checks=True),
    )(
        A_x.reshape(NSEG, 4, 8, D),
        A_mem0.reshape(M, D),
        A_Wq.reshape(D // 2, 2, H, DH),
        A_Wk.reshape(D // 2, 2, H, DH),
        A_Wv.reshape(D // 2, 2, H, DH),
        A_Wo.reshape(H * DH, D),
        B_w_r,
        B_w_gate,
        B_w_up,
        B_w_down,
        c,
        w_mod,
    )
    return out.reshape(1, NSEG * SEG, D)
```

```python
import jax
import jax.numpy as jnp
import jax.experimental.pallas as pl
import jax.experimental.pallas.tpu as pltpu

F32 = jnp.float32
BF16 = jnp.bfloat16
U32 = jnp.uint32

D = 1024
H = 32
DH = 128
NP = H // 2
M = 8
SEG = 32
NSEG = 64
FF = 3584
NJ = SEG - M
NE = NSEG * M
EPS = 1.0013580322265625e-05
SCALE = DH ** (-0.5)
NEG = -1000000000.0
LOG2E = 1.4426950408889634
KQ = 128
NK = D // KQ
MB = 11
NG = 4
NS = 5
UNROLL = 2
NIT = NSEG // (2 * UNROLL)
OUT_SPLIT = NSEG - 2 * UNROLL - 2


def _rb(x):
    return x.astype(BF16).astype(F32)


def _layernorm(xf):
    m = jnp.mean(xf, axis=-1, keepdims=True)
    d = xf - m
    v = jnp.mean(d * d, axis=-1, keepdims=True)
    std = _rb(jnp.sqrt(_rb(_rb(v) + EPS)))
    return _rb(xf - _rb(m)) * (1.0 / std)


def _sigmoid(x):
    return _rb(1.0 / _rb(1.0 + _rb(jnp.exp(-x))))


def _dot(a, b):
    return jnp.dot(a, b, preferred_element_type=F32)


def _dot_nt(a, b):
    return jax.lax.dot_general(a, b, (((1,), (1,)), ((), ())), preferred_element_type=F32)


def _kernel(x_hbm, mem0_hbm, wq_hbm, wk_hbm, wv_hbm, wo_hbm, wr_hbm, wg_hbm, wu_hbm, wd_hbm,
            c_hbm, wm_hbm,
            out_hbm,
            wq, wk, wv, wo, wg, wu, wd, wm, cb, xv, x1v, h2v, outv, early, hn, he, hj, pend,
            mod, fill, keys, patch, zero, opnd, acc0, mem0_ref, wr_ref, c_ref,
            sem, sem_out):
    w_u32 = [w.bitcast(U32) for w in (wq_hbm, wk_hbm, wv_hbm)]
    wqkv = (wq, wk, wv)
    wo_hbm, wg_hbm, wu_hbm, wd_hbm, wm_hbm = [
        w.bitcast(U32) for w in (wo_hbm, wg_hbm, wu_hbm, wd_hbm, wm_hbm)]

    def wblk(w, j):
        return pltpu.bitcast(w[:, j * 128:(j + 1) * 128], BF16)

    def wo_blk(n, lo, hi):
        return pltpu.bitcast(wo[n, lo // 2:hi // 2, :], BF16)

    def w_copies(m, p, k):
        return [pltpu.make_async_copy(w_u32[m].at[:, par, p, :], wqkv[m].at[2 * p + par], sem.at[k])
                for par in range(2)]

    def col_copy(src, dst, j, k):
        lo = j * 128 if isinstance(j, int) else pl.multiple_of(j * 128, 128)
        return pltpu.make_async_copy(src.at[:, pl.ds(lo, 128)], dst.at[j], sem.at[k])

    def units(g):
        return [(m, 4 * g + t) for t in range(4) for m in range(2)]

    def xj_copy(g):
        segs = pl.ds(16 * g, 16)
        return pltpu.make_async_copy(x_hbm.at[segs, 0:3], xv.at[segs, 0:3], sem.at[16 + g])

    def qk_copies(g):
        return sum([w_copies(m, p, 16 + g) for m, p in units(g)], [])

    def wm1_copies(j):
        return [col_copy(wm_hbm, wm, j, 1 + j), col_copy(wm_hbm, wm, 8 + j, 1 + j)]

    def wv_copies(j):
        lo = j * (KQ // 2) if isinstance(j, int) else pl.multiple_of(j * (KQ // 2), KQ // 2)
        rows = pl.ds(lo, KQ // 2)
        return [pltpu.make_async_copy(w_u32[2].at[rows, par, p, :], wv.at[2 * p + par, rows],
                                      sem.at[24 + j]) for p in range(NP) for par in range(2)]

    def wm2_copies(lo, n, t):
        return [col_copy(wm_hbm, wm, lo + b, 20 + t) for b in range(n)]

    def wait_if(cond, cps):
        for cp in cps:
            pl.when(cond)(cp.wait)

    def start_if(cond, cps):
        for cp in cps:
            pl.when(cond)(cp.start)

    def start_if_below(i, n, cps):
        for k in range(0, len(cps), 4):
            start_if(i < n if k % 8 == 0 else i + 1 <= n, cps[k:k + 4])

    cp_c = pltpu.make_async_copy(c_hbm, c_ref, sem.at[9])
    cp_xe = pltpu.make_async_copy(x_hbm.at[:, 3], xv.at[:, 3], sem.at[0])
    cp_wo = [col_copy(wo_hbm, wo, n, 10) for n in range(8)]
    cp_small = [pltpu.make_async_copy(mem0_hbm, mem0_ref, sem.at[14]),
                pltpu.make_async_copy(wr_hbm, wr_ref, sem.at[15])]
    cp_ffn = [pltpu.make_async_copy(wg_hbm, wg.at[:, 0:FF], sem.at[11]),
              pltpu.make_async_copy(wu_hbm, wu.at[:, 0:FF], sem.at[12]),
              pltpu.make_async_copy(wd_hbm, wd.at[:, 0:D], sem.at[13])]

    for cp in ([cp_c, cp_xe] + wm1_copies(0) + wv_copies(0) + wm1_copies(1) + wm1_copies(2)
               + wv_copies(1) + cp_small):
        cp.start()

    ri = jax.lax.broadcasted_iota(jnp.int32, (80, 128), 0)
    ci = jax.lax.broadcasted_iota(jnp.int32, (80, 128), 1)

    def head_of(i):
        return jnp.where(i < 64, i >> 5, (i - 64) >> 3)

    def pos_of(i):
        return jnp.where(i < 64, i & 31, 32 + (i & 7))

    same = (head_of(ri) == head_of(ci)) & (ci < 80)
    allowed = (pos_of(ri) < M) | (pos_of(ri) >= pos_of(ci))
    fill[...] = jnp.where(same, jnp.where(allowed, 0.0, NEG / SCALE), -jnp.inf).astype(F32)
    keys[...] = jnp.zeros(keys.shape, F32)
    pend[M:, :] = jnp.zeros((SEG + M, D), F32)
    zero[...] = jnp.zeros(zero.shape, U32)

    def pin_zero(vals):
        acc = None
        for v in vals:
            v = pltpu.bitcast(v, U32)
            for r in range(0, v.shape[0], 8):
                acc = v[r:r + 8] if acc is None else acc | v[r:r + 8]
        return acc & zero[...]

    cp_c.wait()
    cf = c_ref[...].astype(F32)
    sc = _rb(cf * _sigmoid(cf))
    cb[0:D, :] = jnp.broadcast_to(sc, (128, D)).T
    cb[D:, :] = jnp.zeros((32, 128), F32)

    def mod_vec(k):
        return jnp.concatenate([mod[8 * k + b] for b in range(8)], axis=1)

    def mod_block_vpu(src, dst, is_scale, after=None):
        acc = None if after is None else pltpu.bitcast(pin_zero([after]), F32)
        for r in range(0, D // 2, 8):
            w = wm[src, r:r + 8, :]
            t0 = pltpu.bitcast(w << 16, F32) * cb[pl.ds(2 * r, 8, stride=2), :]
            t1 = pltpu.bitcast(w & U32(0xFFFF0000), F32) * cb[pl.ds(2 * r + 1, 8, stride=2), :]
            if after is not None:
                acc = (acc + t0) + t1
            else:
                acc = t0 + t1 if acc is None else acc + (t0 + t1)
        v = _rb(jnp.broadcast_to(jnp.sum(acc, axis=0, keepdims=True), (8, 128)))
        v = jnp.where(is_scale, _rb(1.0 + v), v)
        mod[dst] = v
        return v

    def ne_body(i, carry):
        n = _layernorm(xv[pl.ds(i * 16, 16), 3].astype(F32)).reshape(128, D).astype(BF16)
        for j in range(NK):
            hn[j, pl.ds(pl.multiple_of(i * 128, 128), 128), :] = n[:, j * KQ:(j + 1) * KQ]
        return carry

    cp_xe.wait()
    jax.lax.fori_loop(0, NSEG // 16, ne_body, 0)

    def w_head(m, h, lo=0, hi=D):
        return pltpu.bitcast(wqkv[m][h, lo // 2:hi // 2, :], BF16)

    def relayout(m, p, rows=slice(None)):
        w = wqkv[m]
        e = w[2 * p, rows, :]
        o = w[2 * p + 1, rows, :]
        w[2 * p, rows, :] = (e & U32(0xFFFF)) | (o << 16)
        w[2 * p + 1, rows, :] = (e >> 16) | (o & U32(0xFFFF0000))

    def store_early(m, p, row0, r1, r2):
        ns = r1.shape[0] // 8
        r12 = jnp.concatenate([r1.reshape(ns, 8, DH), r2.reshape(ns, 8, DH)], axis=1)
        v = pltpu.bitcast(r12.reshape(16 * ns, DH).astype(BF16), U32)
        early[row0 // 8:row0 // 8 + ns, m * NP + p] = v.reshape(ns, 8, DH)
        return v

    def modulate(src, dst, shift, scale):
        n = hn[src].astype(F32).reshape(NSEG, 8, KQ)
        h = (_rb(n * scale) + shift).reshape(NE, KQ)
        he[dst] = h.astype(BF16)
        return h

    def chunk_body(j, carry):
        @pl.when(j <= 1)
        def _():
            for cp in wm1_copies(j):
                cp.wait()
            modulate(j, j, mod_block_vpu(j, j, False), mod_block_vpu(8 + j, 8 + j, True))

        nxt = jnp.where(j >= 1, jnp.minimum(j + 1, NK - 1), 0)
        live = nxt == j + 1
        wait_if(live, wm1_copies(nxt))
        for cp in wv_copies(j):
            cp.wait()
        krows = pl.ds(pl.multiple_of(j * (KQ // 2), KQ // 2), KQ // 2)
        hb = [he[j, c * 256:(c + 1) * 256, :] for c in range(2)]
        pins = {}
        for c in range(2):
            rows = slice(c * 256, (c + 1) * 256)
            for q in range(NP // 2):
                i = 8 * c + q
                if c == 0:
                    relayout(2, 2 * q, krows)
                    relayout(2, 2 * q + 1, krows)
                w4 = [wv[4 * q + b, krows, :] for b in range(4)]
                if i in pins:
                    w4[0] = jnp.concatenate([w4[0][0:8] | pin_zero(pins[i]), w4[0][8:]], axis=0)
                r = _dot(hb[c], pltpu.bitcast(jnp.concatenate(w4, axis=1), BF16))
                for b in range(4):
                    acc0[4 * q + b, rows, :] = (r[:, b * DH:(b + 1) * DH]
                                                + jnp.where(j > 0, acc0[4 * q + b, rows, :], 0.0))
                if i == 7:
                    shift = mod_block_vpu(nxt, jnp.where(live, nxt, 48), False, r[0:8, 0:128])
                if i == 9:
                    scale = mod_block_vpu(8 + nxt, jnp.where(live, 8 + nxt, 49), True,
                                          r[0:8, 0:128])
                    h = modulate(nxt, jnp.where(live, nxt, NK), shift, scale)
                    pins = {13: [h[0:256]], 15: [h[256:512]]}
        pr = 1 + (j >> 1)
        t = jnp.maximum(j - 5, 0)
        start_if(j + 4 < NK, wm1_copies(jnp.minimum(j + 4, NK - 1)))
        start_if_below(j, NK - 3, wv_copies(jnp.minimum(j + 3, NK - 1)))
        start_if((j & 1) == 0, w_copies(0, pr, 16 + (pr >> 2)))
        start_if((j & 1) == 1, w_copies(1, pr, 16 + (pr >> 2)))
        start_if_below(4, j, [xj_copy(t)] + w_copies(0, 5 + t, 17) + w_copies(1, 5 + t, 17)
                       + wm2_copies(16 + 4 * t, 4, 0))
        return carry

    for cp in wm1_copies(3) + wv_copies(2) + w_copies(0, 0, 16) + w_copies(1, 0, 16):
        cp.start()
    jax.lax.fori_loop(0, NK, chunk_body, 0)

    def early_proj(m, p, pins):
        relayout(m, p)
        for c in range(2):
            rows = slice(c * 256, (c + 1) * 256)
            hc = jnp.concatenate([he[j, rows, :] for j in range(NK)], axis=1)
            r12 = []
            for b in range(2):
                halves = []
                for k in range(2):
                    wh = wqkv[m][2 * p + b, k * 256:(k + 1) * 256, :]
                    if pins.get(4 * c + 2 * b + k):
                        wh = jnp.concatenate(
                            [wh[0:8] | pin_zero(pins[4 * c + 2 * b + k]), wh[8:]], axis=0)
                    halves.append(wh)
                r12.append(_dot(hc, pltpu.bitcast(jnp.concatenate(halves, axis=0), BF16)))
            store_early(m, p, c * 256, *r12)

    def make_hj(s):
        n = _rb(_layernorm(xv[s, 0:3].astype(F32)))
        h = _rb(n * mod_vec(1)) + mod_vec(0)
        hj[s] = h
        return [h[g, :, 0:128] for g in range(3)]

    def pro_body(g, carry):
        wait_if(g == 1, wm2_copies(16, 12, 0))
        tb = jnp.maximum(g - 2, 0)
        wait_if(g >= 2, wm2_copies(28 + 10 * tb, 10, 1 + tb))
        for cp in qk_copies(g) + [xj_copy(g)]:
            cp.wait()
        lnp = sum([make_hj(g * 16 + t) for t in range(16)], [])
        mv = []
        for b in range(MB):
            blk = 16 + MB * (g - 1) + b
            live = (g > 0) & (blk < 48)
            mv.append(mod_block_vpu(jnp.where(live, blk, b), jnp.where(live, blk, 48 + b),
                                    (blk >= 32) & (blk < 40)))
        fin = [store_early(2, 4 * g + t, 0, acc0[8 * g + 2 * t], acc0[8 * g + 2 * t + 1])
               for t in range(4)]
        sites = {i: [] for i in range(64)}
        twice = [3, 4, 6, 7, 10, 11, 12, 14, 15, 18, 19, 20, 22, 23, 26, 27, 30, 31]
        for i, v in zip(sorted(list(range(2, 32)) + twice), lnp):
            sites[2 * i].append(v)
        for i, v in zip(range(1, 31, 2), mv + fin):
            sites[2 * i + 1].append(v)
        for u, (m, p) in enumerate(units(g)):
            early_proj(m, p, {i: sites[8 * u + i] for i in range(8)})
        gn = jnp.minimum(g, 1)
        start_if_below(g, 2, qk_copies(gn + 2))
        start_if(g == 1, [xj_copy(3)])
        start_if_below(g, 2, wm2_copies(28 + 10 * gn, 10, 1 + gn))
        start_if(g == 0, cp_wo[:1])
        start_if(g == 1, cp_wo[1:])
        return carry

    jax.lax.fori_loop(0, NG, pro_body, 0)

    for cp in cp_ffn:
        cp.start()
    for cp in cp_small + cp_wo:
        cp.wait()
    pend[0:M, :] = mem0_ref[...].astype(F32)

    wr = jnp.broadcast_to(wr_ref[...].astype(F32).reshape(1, D), (8, D))

    lane8 = jax.lax.broadcasted_iota(jnp.int32, (8, 128), 1)
    sub8 = jax.lax.broadcasted_iota(jnp.int32, (8, 128), 0)
    LAST = NSEG * SEG - 1

    def post(s, g0, g1, attn, record=True):
        attn = attn.reshape(g1 - g0, 8, D)
        x1 = _rb(xv[s, g0:g1].astype(F32) + _rb(mod_vec(2) * _rb(attn)))
        n = _rb(_layernorm(x1))
        h2 = _rb(_rb(n * mod_vec(4)) + mod_vec(3))
        r = _rb(jnp.sum(h2 * wr, axis=-1, keepdims=True)) + 0.0
        x1v[s, g0:g1] = x1.astype(BF16)
        h2v[s, g0:g1] = h2.astype(BF16)
        outv[s, g0:g1] = (x1 + _rb(mod_vec(5) * h2)).astype(BF16)
        pins = []
        for g in range(g0, g1):
            bits = pltpu.bitcast(jnp.broadcast_to(r[g - g0], (8, 128)), jnp.int32)
            hi = jax.lax.shift_right_logical(bits, 16)
            code = jnp.where(bits < 0, hi ^ 0xFFFF, hi | 0x8000)
            key = (code << 11) | (LAST - (s * SEG + g * 8) - sub8) | 0x40000000
            key = pltpu.bitcast(key, F32)
            if record:
                rows = slice(g * 8, (g + 1) * 8)
                keys[rows, :] = jnp.where(lane8 == s, key, keys[rows, :])
            pins.append(key)
        return pins

    def post_pair(a, rows, record=True):
        return post(a + 1, 0, 4, rows[0:SEG], record) + post(a, 3, 4, rows[SEG:], record)

    zpad = jnp.zeros((48, DH), BF16)
    G = 4
    KA = (NP - G) * 2 * DH
    KS = D - 128

    def segment(s, lhs, lhs_split, extra, pins):
        scales = {}

        def stash(p, m, v):
            opnd[p, m, 0:v.shape[0], :] = v.astype(BF16)

        def qkv_group(p):
            keys = [(m, 2 * p + b) for m in range(3) for b in range(2 * G)]
            nsplit = 6 if (p == 0 and lhs_split is not None) else 0
            part = [_dot(lhs_split[0], w_head(m, h, 0, KS)) for m, h in keys[:nsplit]]
            full = [_dot(lhs_split[1], w_head(m, h, KS, D)) + part[i]
                    for i, (m, h) in enumerate(keys[:nsplit])]
            full += [_dot(lhs, w_head(m, h)) for m, h in keys[nsplit:]]
            for m in range(3):
                for t in range(G):
                    i = 2 * G * m + 2 * t
                    stash(p + t, m, jnp.concatenate([full[i], full[i + 1]], axis=0))

        def operand(p, m):
            parts = [opnd[p, m, 0:64, :], pltpu.bitcast(early[s, m * NP + p], BF16)]
            if m > 0:
                parts.append(zpad)
            return jnp.concatenate(parts, axis=0)

        def scores(p):
            sc_ = _dot_nt(operand(p, 0), operand(p, 1))
            f = fill[...]
            if pins.get(p):
                f = jnp.concatenate([f[0:8] + pltpu.bitcast(pin_zero(pins[p]), F32), f[8:]], axis=0)
            sc_ = jnp.where(f == 0.0, sc_, f)
            mx = jnp.max(sc_, axis=-1, keepdims=True)
            e = jnp.exp2((sc_ - mx) * (SCALE * LOG2E))
            inv = pl.reciprocal(jnp.sum(e, axis=-1, keepdims=True), approx=True)
            if p // G == NP // G - 2:
                stash(p, 3, e * inv)
            else:
                stash(p, 3, e)
                scales[p] = inv

        oe = []

        def pv(p):
            o = _dot(opnd[p, 3], operand(p, 2))
            if p in scales:
                o = o * scales[p]
                pins.setdefault(p + G, []).append(o)
            res = []
            for b in range(2):
                rows, erows = o[32 * b:32 * b + 32], o[64 + 8 * b:72 + 8 * b]
                oe.append(erows)
                if extra is not None:
                    rows = jnp.concatenate([rows, erows, extra[2 * p + b]], axis=0)
                res.append(rows)
            return res

        os_ = []
        for p in range(0, NP, G):
            qkv_group(p)
            if p >= G:
                for t in range(G):
                    os_ += pv(p - G + t)
            for t in range(G):
                scores(p + t)
        oa = jnp.concatenate(os_, axis=1).astype(BF16)
        acc, ob = [], []
        for n in range(7):
            acc.append(_dot(oa, wo_blk(n, 0, KA)))
            if n == 1:
                for t in range(G):
                    ob += pv(NP - G + t)
        ob = jnp.concatenate(ob, axis=1).astype(BF16)
        res = [_dot(ob, wo_blk(n, KA, H * DH)) + acc[n] for n in range(7)]
        res.append(_dot(ob, wo_blk(7, KA, H * DH)) + _dot(oa, wo_blk(7, 0, KA)))
        return res, oe

    def make_lhs(mem, s):
        return jnp.concatenate([mem, hj[s].reshape(NJ, D)], axis=0)

    cp_o1 = pltpu.make_async_copy(outv.at[0:OUT_SPLIT], out_hbm.at[0:OUT_SPLIT], sem_out.at[0])
    cp_o2 = pltpu.make_async_copy(outv.at[OUT_SPLIT:NSEG], out_hbm.at[OUT_SPLIT:NSEG],
                                  sem_out.at[1])

    def split_lhs(lhs):
        return lhs.astype(BF16), (lhs[:, :KS].astype(BF16), lhs[:, KS:].astype(BF16))

    def step(i, carry):
        @pl.when(i == NIT - 1)
        def _():
            cp_o1.start()

        prev = pend[...]
        for u in range(UNROLL):
            a = 2 * (UNROLL * i + u)
            pins = post_pair(jnp.maximum(a - 2, 0) if u == 0 else a - 2, prev[M:])
            lhs_a = make_lhs(prev[0:M], a)
            lhs_a = (lhs_a.astype(BF16), None) if u == 0 else split_lhs(lhs_a)
            res_a, oe_a = segment(a, *lhs_a, None,
                                  {k: [v] for k, v in zip((2, 6, 10, 14), pins[:4])})
            res_a = jnp.concatenate(res_a, axis=1)
            pins = pins[4:] + post(a, 0, 3, res_a[M:])
            res_b, _ = segment(a + 1, *split_lhs(make_lhs(res_a[0:M], a + 1)), oe_a,
                               {k: [v] for k, v in zip((2, 6, 10, 14), pins)})
            prev = jnp.concatenate(res_b, axis=1)
        pend[...] = prev
        return carry

    jax.lax.fori_loop(0, NIT, step, 0)
    for cp in cp_ffn:
        cp.wait()

    def decode(k):
        kb = pltpu.bitcast(jnp.broadcast_to(k, (8, 128)), jnp.int32)
        code = (kb >> 11) & 0xFFFF
        hi = jnp.where(code >= 0x8000, code & 0x7FFF, code ^ 0xFFFF)
        tok = jnp.clip((LAST - (kb & LAST))[0, 0], 0, LAST)
        return tok, pltpu.bitcast(hi << 16, F32)[:, 0:1]

    def top2(kv):
        k1 = jnp.max(kv, axis=0, keepdims=True)
        k2 = jnp.max(jnp.where(kv == k1, 0.0, kv), axis=0, keepdims=True)
        return decode(k1), decode(k2)

    def rows_of(ref, a, b):
        return jnp.concatenate([ref[t >> 5, pl.ds((t >> 3) & 3, 1)] for t in (a, b)],
                               axis=0).astype(F32)

    def hidden(h, lo, hi):
        hl = h.reshape(16, D).astype(BF16)
        act = []
        for j in range(lo, hi):
            gt = _rb(_dot(hl, wblk(wg, j)))
            act.append(_rb(gt * _sigmoid(gt)) * _rb(_dot(hl, wblk(wu, j))))
        return jnp.concatenate(act, axis=1).astype(BF16)

    def down(act, lo, hi):
        return [_dot(act, pltpu.bitcast(wd[lo * 64:hi * 64, n * 128:(n + 1) * 128], BF16))
                for n in range(8)]

    kv = keys[...]
    o1 = jnp.max(jnp.max(kv, axis=0, keepdims=True), axis=1, keepdims=True)
    kv = jnp.where(kv == o1, 0.0, kv)
    o2 = jnp.max(jnp.max(kv, axis=0, keepdims=True), axis=1, keepdims=True)
    old = jnp.where(sub8 < 4, o1, o2)
    j1, j2 = [decode(jnp.broadcast_to(o, (1, 128)))[0] for o in (o1, o2)]
    act_s = hidden(rows_of(h2v, j1, j2), 0, NS)
    last_keys = post_pair(NSEG - 2, pend[M:, :], record=False)
    cp_o2.start()
    (i1, r1), (i2, r2) = top2(jnp.concatenate(last_keys + [old], axis=0))
    g1, g2 = i1 >> 3, i2 >> 3
    x1, h2 = rows_of(x1v, i1, i2), rows_of(h2v, i1, i2)
    act_r = hidden(h2, NS, FF // 128)
    y_s = down(act_s, 0, NS)
    y_r = jnp.concatenate(down(act_r, NS, FF // 128), axis=1)
    rowi = jax.lax.broadcasted_iota(jnp.int32, (2, 8, 1), 1)
    gsel = jax.lax.broadcasted_iota(jnp.int32, (2, 8, 1), 0)
    tokp = jnp.where(gsel == 0, g1, g2) * 8 + rowi
    gate = _sigmoid(jnp.where(tokp == i1, r1[None], r2[None]))

    def finish(y_first):
        y = (y_r + jnp.concatenate(y_first, axis=1)).reshape(2, 8, D)
        upd = jnp.where((tokp == i1) | (tokp == i2), _rb(_rb(y) * gate), 0.0)
        patch[...] = (x1 + _rb(mod_vec(5) * _rb(h2 + upd))).astype(BF16)

    finish(y_s)

    @pl.when((i1 != j1) | (i2 != j2))
    def _():
        finish(down(hidden(h2, 0, NS), 0, NS))

    cp_o1.wait()
    cp_o2.wait()
    cp1 = pltpu.make_async_copy(patch.at[0], out_hbm.at[g1 >> 2, g1 & 3], sem_out.at[0])
    cp1.start()

    @pl.when(g1 != g2)
    def _():
        cp2 = pltpu.make_async_copy(patch.at[1], out_hbm.at[g2 >> 2, g2 & 3], sem_out.at[1])
        cp2.start()
        cp2.wait()

    cp1.wait()


@jax.jit
def pallas_adaLN_cond__memory_aug_recurrent_mem_tr__moe_arch_mod__prompt_kernel(
    A_x: jax.Array,
    A_mem0: jax.Array,
    A_Wq: jax.Array,
    A_Wk: jax.Array,
    A_Wv: jax.Array,
    A_Wo: jax.Array,
    A_seg_len,
    B_x: jax.Array,
    B_w_r: jax.Array,
    B_w_gate: jax.Array,
    B_w_up: jax.Array,
    B_w_down: jax.Array,
    c: jax.Array,
    w_mod: jax.Array,
):
    assert A_x.shape == (1, NSEG * SEG, D)
    any_spec = pl.BlockSpec(memory_space=pl.ANY)
    out = pl.pallas_call(
        _kernel,
        out_shape=jax.ShapeDtypeStruct((NSEG, 4, 8, D), BF16),
        in_specs=[any_spec] * 12,
        out_specs=any_spec,
        scratch_shapes=[
            pltpu.VMEM((H, D // 2, DH), U32),
            pltpu.VMEM((H, D // 2, DH), U32),
            pltpu.VMEM((H, D // 2, DH), U32),
            pltpu.VMEM((8, H * DH // 2, 128), U32),
            pltpu.VMEM((D // 2, FF + 128), U32),
            pltpu.VMEM((D // 2, FF + 128), U32),
            pltpu.VMEM((FF // 2, D + 128), U32),
            pltpu.VMEM((48, D // 2, 128), U32),
            pltpu.VMEM((D + 32, 128), F32),
            pltpu.VMEM((NSEG, 4, 8, D), BF16),
            pltpu.VMEM((NSEG, 4, 8, D), BF16),
            pltpu.VMEM((NSEG, 4, 8, D), BF16),
            pltpu.VMEM((NSEG, 4, 8, D), BF16),
            pltpu.VMEM((NSEG, 3 * NP, 8, DH), U32),
            pltpu.VMEM((NK, NE, KQ), BF16),
            pltpu.VMEM((NK + 1, NE, KQ), BF16),
            pltpu.VMEM((NSEG, 3, 8, D), F32),
            pltpu.VMEM((M + SEG + M, D), F32),
            pltpu.VMEM((48 + 16, 8, 128), F32),
            pltpu.VMEM((80, 128), F32),
            pltpu.VMEM((SEG, 128), F32),
            pltpu.VMEM((2, 8, D), BF16),
            pltpu.VMEM((8, 128), U32),
            pltpu.VMEM((NP, 4, 80, DH), BF16),
            pltpu.VMEM((H, NE, DH), F32),
            pltpu.VMEM((M, D), BF16),
            pltpu.VMEM((D,), BF16),
            pltpu.VMEM((1, D), BF16),
            pltpu.SemaphoreType.DMA((24 + NK,)),
            pltpu.SemaphoreType.DMA((2,)),
        ],
        compiler_params=pltpu.CompilerParams(vmem_limit_bytes=124 * 1024 * 1024,
                                             disable_bounds_checks=True,
                                             disable_semaphore_checks=True),
    )(
        A_x.reshape(NSEG, 4, 8, D),
        A_mem0.reshape(M, D),
        A_Wq.reshape(D // 2, 2, H, DH),
        A_Wk.reshape(D // 2, 2, H, DH),
        A_Wv.reshape(D // 2, 2, H, DH),
        A_Wo.reshape(H * DH, D),
        B_w_r,
        B_w_gate,
        B_w_up,
        B_w_down,
        c,
        w_mod,
    )
    return out.reshape(1, NSEG * SEG, D)
```

```python
import jax
import jax.numpy as jnp
import jax.experimental.pallas as pl
import jax.experimental.pallas.tpu as pltpu

F32 = jnp.float32
BF16 = jnp.bfloat16
U32 = jnp.uint32

D = 1024
H = 32
DH = 128
NP = H // 2
M = 8
SEG = 32
NSEG = 64
FF = 3584
NJ = SEG - M
NE = NSEG * M
EPS = 1.0013580322265625e-05
SCALE = DH ** (-0.5)
NEG = -1000000000.0
LOG2E = 1.4426950408889634
KQ = 128
NK = D // KQ
MB = 11
NG = 4
NF = FF // 128
I0 = 2
ND = 4
UNROLL = 2
NIT = NSEG // (2 * UNROLL)
OUT_SPLIT = NSEG - 2 * UNROLL - 2


def _rb(x):
    return x.astype(BF16).astype(F32)


def _layernorm(xf):
    m = jnp.mean(xf, axis=-1, keepdims=True)
    d = xf - m
    v = jnp.mean(d * d, axis=-1, keepdims=True)
    std = _rb(jnp.sqrt(_rb(_rb(v) + EPS)))
    return _rb(xf - _rb(m)) * (1.0 / std)


def _sigmoid(x):
    return _rb(1.0 / _rb(1.0 + _rb(jnp.exp(-x))))


def _dot(a, b):
    return jnp.dot(a, b, preferred_element_type=F32)


def _dot_nt(a, b):
    return jax.lax.dot_general(a, b, (((1,), (1,)), ((), ())), preferred_element_type=F32)


def _kernel(x_hbm, mem0_hbm, wq_hbm, wk_hbm, wv_hbm, wo_hbm, wr_hbm, wg_hbm, wu_hbm, wd_hbm,
            c_hbm, wm_hbm,
            out_hbm,
            wq, wk, wv, wo, wg, wu, wd, wm, cb, xv, x1v, h2v, outv, early, hn, he, hj, pend,
            mod, fill, keys, patch, zero, opnd, xt, act, ys, acc0, mem0_ref, wr_ref, c_ref,
            sem, sem_out):
    w_u32 = [w.bitcast(U32) for w in (wq_hbm, wk_hbm, wv_hbm)]
    wqkv = (wq, wk, wv)
    wo_hbm, wg_hbm, wu_hbm, wd_hbm, wm_hbm = [
        w.bitcast(U32) for w in (wo_hbm, wg_hbm, wu_hbm, wd_hbm, wm_hbm)]

    def wo_blk(n, lo, hi):
        return pltpu.bitcast(wo[n, lo // 2:hi // 2, :], BF16)

    def w_copies(m, p, k):
        return [pltpu.make_async_copy(w_u32[m].at[:, par, p, :], wqkv[m].at[2 * p + par], sem.at[k])
                for par in range(2)]

    def col_copy(src, dst, j, k):
        lo = j * 128 if isinstance(j, int) else pl.multiple_of(j * 128, 128)
        return pltpu.make_async_copy(src.at[:, pl.ds(lo, 128)], dst.at[j], sem.at[k])

    def units(g):
        return [(m, 4 * g + t) for t in range(4) for m in range(2)]

    def xj_copy(g):
        segs = pl.ds(16 * g, 16)
        return pltpu.make_async_copy(x_hbm.at[segs, 0:3], xv.at[segs, 0:3], sem.at[16 + g])

    def qk_copies(g):
        return sum([w_copies(m, p, 16 + g) for m, p in units(g)], [])

    def wm1_copies(j):
        return [col_copy(wm_hbm, wm, j, 1 + j), col_copy(wm_hbm, wm, 8 + j, 1 + j)]

    def wv_copies(j):
        lo = j * (KQ // 2) if isinstance(j, int) else pl.multiple_of(j * (KQ // 2), KQ // 2)
        rows = pl.ds(lo, KQ // 2)
        return [pltpu.make_async_copy(w_u32[2].at[rows, par, p, :], wv.at[2 * p + par, rows],
                                      sem.at[24 + j]) for p in range(NP) for par in range(2)]

    def wm2_copies(lo, n, t):
        return [col_copy(wm_hbm, wm, lo + b, 20 + t) for b in range(n)]

    def wait_if(cond, cps):
        for cp in cps:
            pl.when(cond)(cp.wait)

    def start_if(cond, cps):
        for cp in cps:
            pl.when(cond)(cp.start)

    def start_if_below(i, n, cps):
        for k in range(0, len(cps), 4):
            start_if(i < n if k % 8 == 0 else i + 1 <= n, cps[k:k + 4])

    cp_c = pltpu.make_async_copy(c_hbm, c_ref, sem.at[9])
    cp_xe = pltpu.make_async_copy(x_hbm.at[:, 3], xv.at[:, 3], sem.at[0])
    cp_wo = [col_copy(wo_hbm, wo, n, 10) for n in range(8)]
    cp_small = [pltpu.make_async_copy(mem0_hbm, mem0_ref, sem.at[14]),
                pltpu.make_async_copy(wr_hbm, wr_ref, sem.at[15])]
    cp_glu = ([col_copy(wg_hbm, wg, j, 11) for j in range(NF)]
              + [col_copy(wu_hbm, wu, j, 11) for j in range(NF)])
    cp_wd = pltpu.make_async_copy(wd_hbm, wd.at[:, 0:D], sem.at[13])

    for cp in ([cp_c, cp_xe] + wm1_copies(0) + wv_copies(0) + wm1_copies(1) + wm1_copies(2)
               + wv_copies(1) + cp_small):
        cp.start()

    ri = jax.lax.broadcasted_iota(jnp.int32, (80, 128), 0)
    ci = jax.lax.broadcasted_iota(jnp.int32, (80, 128), 1)

    def head_of(i):
        return jnp.where(i < 64, i >> 5, (i - 64) >> 3)

    def pos_of(i):
        return jnp.where(i < 64, i & 31, 32 + (i & 7))

    same = (head_of(ri) == head_of(ci)) & (ci < 80)
    allowed = (pos_of(ri) < M) | (pos_of(ri) >= pos_of(ci))
    fill[...] = jnp.where(same, jnp.where(allowed, 0.0, NEG / SCALE), -jnp.inf).astype(F32)
    keys[...] = jnp.zeros(keys.shape, F32)
    pend[M:, :] = jnp.zeros((SEG + M, D), F32)
    zero[...] = jnp.zeros(zero.shape, U32)
    wg[NF] = jnp.zeros((D // 2, 128), U32)
    wu[NF] = jnp.zeros((D // 2, 128), U32)
    xt[...] = jnp.zeros(xt.shape, F32)
    act[...] = jnp.zeros(act.shape, F32)

    def pin_zero(vals):
        acc = None
        for v in vals:
            v = pltpu.bitcast(v, U32)
            for r in range(0, v.shape[0], 8):
                acc = v[r:r + 8] if acc is None else acc | v[r:r + 8]
        return acc & zero[...]

    cp_c.wait()
    cf = c_ref[...].astype(F32)
    sc = _rb(cf * _sigmoid(cf))
    cb[0:D, :] = jnp.broadcast_to(sc, (128, D)).T
    cb[D:, :] = jnp.zeros((32, 128), F32)

    def mod_vec(k):
        return jnp.concatenate([mod[8 * k + b] for b in range(8)], axis=1)

    def mod_block_vpu(src, dst, is_scale, after=None):
        acc = None if after is None else pltpu.bitcast(pin_zero([after]), F32)
        for r in range(0, D // 2, 8):
            w = wm[src, r:r + 8, :]
            t0 = pltpu.bitcast(w << 16, F32) * cb[pl.ds(2 * r, 8, stride=2), :]
            t1 = pltpu.bitcast(w & U32(0xFFFF0000), F32) * cb[pl.ds(2 * r + 1, 8, stride=2), :]
            if after is not None:
                acc = (acc + t0) + t1
            else:
                acc = t0 + t1 if acc is None else acc + (t0 + t1)
        v = _rb(jnp.broadcast_to(jnp.sum(acc, axis=0, keepdims=True), (8, 128)))
        v = jnp.where(is_scale, _rb(1.0 + v), v)
        mod[dst] = v
        return v

    def ne_body(i, carry):
        n = _layernorm(xv[pl.ds(i * 16, 16), 3].astype(F32)).reshape(128, D).astype(BF16)
        for j in range(NK):
            hn[j, pl.ds(pl.multiple_of(i * 128, 128), 128), :] = n[:, j * KQ:(j + 1) * KQ]
        return carry

    cp_xe.wait()
    jax.lax.fori_loop(0, NSEG // 16, ne_body, 0)

    def w_head(m, h, lo=0, hi=D):
        return pltpu.bitcast(wqkv[m][h, lo // 2:hi // 2, :], BF16)

    def relayout(m, p, rows=slice(None)):
        w = wqkv[m]
        e = w[2 * p, rows, :]
        o = w[2 * p + 1, rows, :]
        w[2 * p, rows, :] = (e & U32(0xFFFF)) | (o << 16)
        w[2 * p + 1, rows, :] = (e >> 16) | (o & U32(0xFFFF0000))

    def store_early(m, p, row0, r1, r2):
        ns = r1.shape[0] // 8
        r12 = jnp.concatenate([r1.reshape(ns, 8, DH), r2.reshape(ns, 8, DH)], axis=1)
        v = pltpu.bitcast(r12.reshape(16 * ns, DH).astype(BF16), U32)
        early[row0 // 8:row0 // 8 + ns, m * NP + p] = v.reshape(ns, 8, DH)
        return v

    def modulate(src, dst, shift, scale):
        n = hn[src].astype(F32).reshape(NSEG, 8, KQ)
        h = (_rb(n * scale) + shift).reshape(NE, KQ)
        he[dst] = h.astype(BF16)
        return h

    def chunk_body(j, carry):
        @pl.when(j <= 1)
        def _():
            for cp in wm1_copies(j):
                cp.wait()
            modulate(j, j, mod_block_vpu(j, j, False), mod_block_vpu(8 + j, 8 + j, True))

        nxt = jnp.where(j >= 1, jnp.minimum(j + 1, NK - 1), 0)
        live = nxt == j + 1
        wait_if(live, wm1_copies(nxt))
        for cp in wv_copies(j):
            cp.wait()
        krows = pl.ds(pl.multiple_of(j * (KQ // 2), KQ // 2), KQ // 2)
        hb = [he[j, c * 256:(c + 1) * 256, :] for c in range(2)]
        pins = {}
        for c in range(2):
            rows = slice(c * 256, (c + 1) * 256)
            for q in range(NP // 2):
                i = 8 * c + q
                if c == 0:
                    relayout(2, 2 * q, krows)
                    relayout(2, 2 * q + 1, krows)
                w4 = [wv[4 * q + b, krows, :] for b in range(4)]
                if i in pins:
                    w4[0] = jnp.concatenate([w4[0][0:8] | pin_zero(pins[i]), w4[0][8:]], axis=0)
                r = _dot(hb[c], pltpu.bitcast(jnp.concatenate(w4, axis=1), BF16))
                for b in range(4):
                    acc0[4 * q + b, rows, :] = (r[:, b * DH:(b + 1) * DH]
                                                + jnp.where(j > 0, acc0[4 * q + b, rows, :], 0.0))
                if i == 7:
                    shift = mod_block_vpu(nxt, jnp.where(live, nxt, 48), False, r[0:8, 0:128])
                if i == 9:
                    scale = mod_block_vpu(8 + nxt, jnp.where(live, 8 + nxt, 49), True,
                                          r[0:8, 0:128])
                    h = modulate(nxt, jnp.where(live, nxt, NK), shift, scale)
                    pins = {13: [h[0:256]], 15: [h[256:512]]}
        pr = 1 + (j >> 1)
        t = jnp.maximum(j - 5, 0)
        start_if(j + 4 < NK, wm1_copies(jnp.minimum(j + 4, NK - 1)))
        start_if_below(j, NK - 3, wv_copies(jnp.minimum(j + 3, NK - 1)))
        start_if((j & 1) == 0, w_copies(0, pr, 16 + (pr >> 2)))
        start_if((j & 1) == 1, w_copies(1, pr, 16 + (pr >> 2)))
        start_if_below(4, j, [xj_copy(t)] + w_copies(0, 5 + t, 17) + w_copies(1, 5 + t, 17)
                       + wm2_copies(16 + 4 * t, 4, 0))
        return carry

    for cp in wm1_copies(3) + wv_copies(2) + w_copies(0, 0, 16) + w_copies(1, 0, 16):
        cp.start()
    jax.lax.fori_loop(0, NK, chunk_body, 0)

    def early_proj(m, p, pins):
        relayout(m, p)
        for c in range(2):
            rows = slice(c * 256, (c + 1) * 256)
            hc = jnp.concatenate([he[j, rows, :] for j in range(NK)], axis=1)
            r12 = []
            for b in range(2):
                halves = []
                for k in range(2):
                    wh = wqkv[m][2 * p + b, k * 256:(k + 1) * 256, :]
                    if pins.get(4 * c + 2 * b + k):
                        wh = jnp.concatenate(
                            [wh[0:8] | pin_zero(pins[4 * c + 2 * b + k]), wh[8:]], axis=0)
                    halves.append(wh)
                r12.append(_dot(hc, pltpu.bitcast(jnp.concatenate(halves, axis=0), BF16)))
            store_early(m, p, c * 256, *r12)

    def make_hj(s):
        n = _rb(_layernorm(xv[s, 0:3].astype(F32)))
        h = _rb(n * mod_vec(1)) + mod_vec(0)
        hj[s] = h
        return [h[g, :, 0:128] for g in range(3)]

    def pro_body(g, carry):
        wait_if(g == 1, wm2_copies(16, 12, 0))
        tb = jnp.maximum(g - 2, 0)
        wait_if(g >= 2, wm2_copies(28 + 10 * tb, 10, 1 + tb))
        for cp in qk_copies(g) + [xj_copy(g)]:
            cp.wait()
        lnp = sum([make_hj(g * 16 + t) for t in range(16)], [])
        mv = []
        for b in range(MB):
            blk = 16 + MB * (g - 1) + b
            live = (g > 0) & (blk < 48)
            mv.append(mod_block_vpu(jnp.where(live, blk, b), jnp.where(live, blk, 48 + b),
                                    (blk >= 32) & (blk < 40)))
        fin = [store_early(2, 4 * g + t, 0, acc0[8 * g + 2 * t], acc0[8 * g + 2 * t + 1])
               for t in range(4)]
        sites = {i: [] for i in range(64)}
        twice = [3, 4, 6, 7, 10, 11, 12, 14, 15, 18, 19, 20, 22, 23, 26, 27, 30, 31]
        for i, v in zip(sorted(list(range(2, 32)) + twice), lnp):
            sites[2 * i].append(v)
        for i, v in zip(range(1, 31, 2), mv + fin):
            sites[2 * i + 1].append(v)
        for u, (m, p) in enumerate(units(g)):
            early_proj(m, p, {i: sites[8 * u + i] for i in range(8)})
        gn = jnp.minimum(g, 1)
        start_if_below(g, 2, qk_copies(gn + 2))
        start_if(g == 1, [xj_copy(3)])
        start_if_below(g, 2, wm2_copies(28 + 10 * gn, 10, 1 + gn))
        start_if(g == 0, cp_wo[:1])
        start_if(g == 1, cp_wo[1:])
        start_if_below(NG - 2, g, cp_glu)
        return carry

    jax.lax.fori_loop(0, NG, pro_body, 0)

    cp_wd.start()
    for cp in cp_small + cp_wo:
        cp.wait()
    pend[0:M, :] = mem0_ref[...].astype(F32)

    wr = jnp.broadcast_to(wr_ref[...].astype(F32).reshape(1, D), (8, D))

    lane8 = jax.lax.broadcasted_iota(jnp.int32, (8, 128), 1)
    sub8 = jax.lax.broadcasted_iota(jnp.int32, (8, 128), 0)
    LAST = NSEG * SEG - 1

    def post(s, g0, g1, attn, record=True):
        attn = attn.reshape(g1 - g0, 8, D)
        x1 = _rb(xv[s, g0:g1].astype(F32) + _rb(mod_vec(2) * _rb(attn)))
        n = _rb(_layernorm(x1))
        h2 = _rb(_rb(n * mod_vec(4)) + mod_vec(3))
        r = _rb(jnp.sum(h2 * wr, axis=-1, keepdims=True)) + 0.0
        x1v[s, g0:g1] = x1.astype(BF16)
        h2v[s, g0:g1] = h2.astype(BF16)
        outv[s, g0:g1] = (x1 + _rb(mod_vec(5) * h2)).astype(BF16)
        pins = []
        for g in range(g0, g1):
            bits = pltpu.bitcast(jnp.broadcast_to(r[g - g0], (8, 128)), jnp.int32)
            hi = jax.lax.shift_right_logical(bits, 16)
            code = jnp.where(bits < 0, hi ^ 0xFFFF, hi | 0x8000)
            key = (code << 11) | (LAST - (s * SEG + g * 8) - sub8) | 0x40000000
            key = pltpu.bitcast(key, F32)
            if record:
                rows = slice(g * 8, (g + 1) * 8)
                keys[rows, :] = jnp.where(lane8 == s, key, keys[rows, :])
            pins.append(key)
        return pins

    def post_pair(a, rows, record=True):
        return post(a + 1, 0, 4, rows[0:SEG], record) + post(a, 3, 4, rows[SEG:], record)

    zpad = jnp.zeros((48, DH), BF16)
    G = 4
    KA = (NP - G) * 2 * DH
    KS = D - 128

    def decode(k):
        kb = pltpu.bitcast(jnp.broadcast_to(k, (8, 128)), jnp.int32)
        code = (kb >> 11) & 0xFFFF
        hi = jnp.where(code >= 0x8000, code & 0x7FFF, code ^ 0xFFFF)
        tok = jnp.clip((LAST - (kb & LAST))[0, 0], 0, LAST)
        return tok, pltpu.bitcast(hi << 16, F32)[:, 0:1]

    def recorded_top2():
        kv = keys[...]
        o1 = jnp.max(jnp.max(kv, axis=0, keepdims=True), axis=1, keepdims=True)
        kv = jnp.where(kv == o1, 0.0, kv)
        return o1, jnp.max(jnp.max(kv, axis=0, keepdims=True), axis=1, keepdims=True)

    def group_of(ref, t):
        return ref[t >> 5, pl.ds((t >> 3) & 3, 1)].astype(F32)

    glu = {}

    def glu_act(gt, up):
        gt = _rb(gt)
        return _rb(gt * _sigmoid(gt)) * _rb(up)

    def glu_block(after):
        j = glu['first'] + glu['todo'].pop(0)
        src = jnp.where(glu['live'], j, NF)
        sums = []
        for w_ref in (wg, wu):
            acc = pltpu.bitcast(pin_zero([after]), F32)
            for r in range(0, D // 2, 8):
                w = w_ref[src, r:r + 8, :]
                acc = ((acc + pltpu.bitcast(w << 16, F32) * xt[pl.ds(2 * r, 8, stride=2), :])
                       + pltpu.bitcast(w & U32(0xFFFF0000), F32) * xt[pl.ds(2 * r + 1, 8, stride=2), :])
            after = acc
            sums.append(jnp.broadcast_to(jnp.sum(acc, axis=0, keepdims=True), (8, 128)))
        act[glu['slot'], j] = glu_act(*sums)

    def segment(s, lhs, lhs_split, extra, pins):
        scales = {}

        def stash(p, m, v):
            opnd[p, m, 0:v.shape[0], :] = v.astype(BF16)

        def qkv_group(p):
            keys = [(m, 2 * p + b) for m in range(3) for b in range(2 * G)]
            nsplit = 6 if (p == 0 and lhs_split is not None) else 0
            part = [_dot(lhs_split[0], w_head(m, h, 0, KS)) for m, h in keys[:nsplit]]
            full = [_dot(lhs_split[1], w_head(m, h, KS, D)) + part[i]
                    for i, (m, h) in enumerate(keys[:nsplit])]
            full += [_dot(lhs, w_head(m, h)) for m, h in keys[nsplit:]]
            if glu['todo']:
                glu_block(full[10][0:8])
            for m in range(3):
                for t in range(G):
                    i = 2 * G * m + 2 * t
                    stash(p + t, m, jnp.concatenate([full[i], full[i + 1]], axis=0))

        def operand(p, m):
            parts = [opnd[p, m, 0:64, :], pltpu.bitcast(early[s, m * NP + p], BF16)]
            if m > 0:
                parts.append(zpad)
            return jnp.concatenate(parts, axis=0)

        def scores(p):
            sc_ = _dot_nt(operand(p, 0), operand(p, 1))
            f = fill[...]
            if pins.get(p):
                f = jnp.concatenate([f[0:8] + pltpu.bitcast(pin_zero(pins[p]), F32), f[8:]], axis=0)
            sc_ = jnp.where(f == 0.0, sc_, f)
            mx = jnp.max(sc_, axis=-1, keepdims=True)
            e = jnp.exp2((sc_ - mx) * (SCALE * LOG2E))
            inv = pl.reciprocal(jnp.sum(e, axis=-1, keepdims=True), approx=True)
            if p // G == NP // G - 2:
                stash(p, 3, e * inv)
            else:
                stash(p, 3, e)
                scales[p] = inv

        oe = []

        def pv(p):
            o = _dot(opnd[p, 3], operand(p, 2))
            if p in scales:
                o = o * scales[p]
                pins.setdefault(p + G, []).append(o)
            res = []
            for b in range(2):
                rows, erows = o[32 * b:32 * b + 32], o[64 + 8 * b:72 + 8 * b]
                oe.append(erows)
                if extra is not None:
                    rows = jnp.concatenate([rows, erows, extra[2 * p + b]], axis=0)
                res.append(rows)
            return res

        os_ = []
        for p in range(0, NP, G):
            qkv_group(p)
            if p >= G:
                for t in range(G):
                    os_ += pv(p - G + t)
            for t in range(G):
                scores(p + t)
        oa = jnp.concatenate(os_, axis=1).astype(BF16)
        acc, ob = [], []
        for n in range(7):
            acc.append(_dot(oa, wo_blk(n, 0, KA)))
            if n == 1:
                for t in range(G):
                    ob += pv(NP - G + t)
        ob = jnp.concatenate(ob, axis=1).astype(BF16)
        res = [_dot(ob, wo_blk(n, KA, H * DH)) + acc[n] for n in range(7)]
        res.append(_dot(ob, wo_blk(7, KA, H * DH)) + _dot(oa, wo_blk(7, 0, KA)))
        return res, oe

    def make_lhs(mem, s):
        return jnp.concatenate([mem, hj[s].reshape(NJ, D)], axis=0)

    cp_o1 = pltpu.make_async_copy(outv.at[0:OUT_SPLIT], out_hbm.at[0:OUT_SPLIT], sem_out.at[0])
    cp_o2 = pltpu.make_async_copy(outv.at[OUT_SPLIT:NSEG], out_hbm.at[OUT_SPLIT:NSEG],
                                  sem_out.at[1])

    def split_lhs(lhs):
        return lhs.astype(BF16), (lhs[:, :KS].astype(BF16), lhs[:, KS:].astype(BF16))

    def step(i, carry):
        c0, c1, tok, slot, half = carry
        held = jnp.where(half == 1, tok, jnp.where(jnp.where(slot == 0, c0, c1) == tok, tok, -1))
        c0, c1 = jnp.where(slot == 0, held, c0), jnp.where(slot == 1, held, c1)
        glu.update(todo=list(range(NF // 2)), first=half * (NF // 2), slot=slot, live=i >= I0)

        @pl.when(i == I0)
        def _():
            for cp in cp_glu:
                cp.wait()

        @pl.when(i == NIT - 1)
        def _():
            cp_o1.start()

        prev = pend[...]
        for u in range(UNROLL):
            a = 2 * (UNROLL * i + u)
            pins = post_pair(jnp.maximum(a - 2, 0) if u == 0 else a - 2, prev[M:])
            lhs_a = make_lhs(prev[0:M], a)
            lhs_a = (lhs_a.astype(BF16), None) if u == 0 else split_lhs(lhs_a)
            res_a, oe_a = segment(a, *lhs_a, None,
                                  {k: [v] for k, v in zip((2, 6, 10, 14), pins[:4])})
            res_a = jnp.concatenate(res_a, axis=1)
            pins = pins[4:] + post(a, 0, 3, res_a[M:])
            res_b, _ = segment(a + 1, *split_lhs(make_lhs(res_a[0:M], a + 1)), oe_a,
                               {k: [v] for k, v in zip((2, 6, 10, 14), pins)})
            prev = jnp.concatenate(res_b, axis=1)
        pend[...] = prev
        assert not glu['todo']

        ta, tb = [decode(jnp.broadcast_to(o, (1, 128)))[0] for o in recorded_top2()]
        has_a = (c0 == ta) | (c1 == ta)
        more = (half == 0) & (held != tok) & ((tok == ta) | (tok == tb))
        nt = jnp.where(more, tok, jnp.where(has_a, tb, ta))
        ns = jnp.where(more, slot, jnp.where(c0 == jnp.where(has_a, ta, tb), 1, 0))
        rowi = jax.lax.broadcasted_iota(jnp.int32, (8, 1), 0)
        row = jnp.sum(jnp.where(rowi == (nt & 7), group_of(h2v, nt)[0], 0.0), axis=0, keepdims=True)
        xt[0:D, :] = jnp.broadcast_to(row, (128, D)).T
        return c0, c1, jnp.where(i + 1 >= I0, nt, -1), ns, more.astype(jnp.int32)

    c0, c1, tok, slot, half = jax.lax.fori_loop(
        0, NIT, step, (jnp.int32(-1), jnp.int32(-1), jnp.int32(-1), jnp.int32(0), jnp.int32(0)))
    cp_wd.wait()

    def down(lo, hi):
        ab = jnp.concatenate([act[:, j].reshape(16, 128) for j in range(NF)], axis=1).astype(BF16)
        return jnp.concatenate([_dot(ab, pltpu.bitcast(wd[:, n * 128:(n + 1) * 128], BF16))
                                for n in range(lo, hi)], axis=1)

    ys[:, 0:ND * 128] = down(0, ND)
    o1, o2 = recorded_top2()
    last_keys = post_pair(NSEG - 2, pend[M:, :], record=False)
    cp_o2.start()
    kv = jnp.concatenate(last_keys + [jnp.where(sub8 < 4, o1, o2)], axis=0)
    k1 = jnp.max(kv, axis=0, keepdims=True)
    k2 = jnp.max(jnp.where(kv == k1, 0.0, kv), axis=0, keepdims=True)
    (i1, r1), (i2, r2) = decode(k1), decode(k2)
    g1, g2 = i1 >> 3, i2 >> 3
    x1 = jnp.concatenate([group_of(x1v, i1), group_of(x1v, i2)], axis=0)
    h2 = jnp.concatenate([group_of(h2v, i1), group_of(h2v, i2)], axis=0)
    d0 = jnp.where((half == 1) & (slot == 0), tok, c0)
    d1 = jnp.where((half == 1) & (slot == 1), tok, c1)
    swapped = (d0 == i2) & (d1 == i1)
    found = swapped | ((d0 == i1) & (d1 == i2))

    @pl.when(jnp.logical_not(found) | (half == 1))
    def _():
        hl = jnp.where(swapped, jnp.concatenate([h2[1], h2[0]], axis=0), h2.reshape(16, D))
        hl = hl.astype(BF16)

        def redo(t, carry):
            for b in range(NF // 2):
                j = t * (NF // 2) + b
                act[:, j] = glu_act(_dot(hl, pltpu.bitcast(wg[j], BF16)),
                                    _dot(hl, pltpu.bitcast(wu[j], BF16))).reshape(2, 8, 128)
            return carry

        jax.lax.fori_loop(found.astype(jnp.int32), 2, redo, 0)
        ys[:, 0:ND * 128] = down(0, ND)

    y = _rb(jnp.concatenate([ys[:, 0:ND * 128], down(ND, 8)], axis=1))
    y1 = _rb(jnp.where(swapped, y[8:16], y[0:8]) * _sigmoid(r1))
    y2 = _rb(jnp.where(swapped, y[0:8], y[8:16]) * _sigmoid(r2))
    rowi = jax.lax.broadcasted_iota(jnp.int32, (2, 8, 1), 1)
    gsel = jax.lax.broadcasted_iota(jnp.int32, (2, 8, 1), 0)
    tokp = jnp.where(gsel == 0, g1, g2) * 8 + rowi
    upd = jnp.where(tokp == i1, y1[None], jnp.where(tokp == i2, y2[None], 0.0))
    patch[...] = (x1 + _rb(mod_vec(5) * _rb(h2 + upd))).astype(BF16)
    cp_o1.wait()
    cp_o2.wait()
    cp1 = pltpu.make_async_copy(patch.at[0], out_hbm.at[g1 >> 2, g1 & 3], sem_out.at[0])
    cp1.start()

    @pl.when(g1 != g2)
    def _():
        cp2 = pltpu.make_async_copy(patch.at[1], out_hbm.at[g2 >> 2, g2 & 3], sem_out.at[1])
        cp2.start()
        cp2.wait()

    cp1.wait()


@jax.jit
def pallas_adaLN_cond__memory_aug_recurrent_mem_tr__moe_arch_mod__prompt_kernel(
    A_x: jax.Array,
    A_mem0: jax.Array,
    A_Wq: jax.Array,
    A_Wk: jax.Array,
    A_Wv: jax.Array,
    A_Wo: jax.Array,
    A_seg_len,
    B_x: jax.Array,
    B_w_r: jax.Array,
    B_w_gate: jax.Array,
    B_w_up: jax.Array,
    B_w_down: jax.Array,
    c: jax.Array,
    w_mod: jax.Array,
):
    assert A_x.shape == (1, NSEG * SEG, D)
    any_spec = pl.BlockSpec(memory_space=pl.ANY)
    out = pl.pallas_call(
        _kernel,
        out_shape=jax.ShapeDtypeStruct((NSEG, 4, 8, D), BF16),
        in_specs=[any_spec] * 12,
        out_specs=any_spec,
        scratch_shapes=[
            pltpu.VMEM((H, D // 2, DH), U32),
            pltpu.VMEM((H, D // 2, DH), U32),
            pltpu.VMEM((H, D // 2, DH), U32),
            pltpu.VMEM((8, H * DH // 2, 128), U32),
            pltpu.VMEM((NF + 1, D // 2, 128), U32),
            pltpu.VMEM((NF + 1, D // 2, 128), U32),
            pltpu.VMEM((FF // 2, D + 128), U32),
            pltpu.VMEM((48, D // 2, 128), U32),
            pltpu.VMEM((D + 32, 128), F32),
            pltpu.VMEM((NSEG, 4, 8, D), BF16),
            pltpu.VMEM((NSEG, 4, 8, D), BF16),
            pltpu.VMEM((NSEG, 4, 8, D), BF16),
            pltpu.VMEM((NSEG, 4, 8, D), BF16),
            pltpu.VMEM((NSEG, 3 * NP, 8, DH), U32),
            pltpu.VMEM((NK, NE, KQ), BF16),
            pltpu.VMEM((NK + 1, NE, KQ), BF16),
            pltpu.VMEM((NSEG, 3, 8, D), F32),
            pltpu.VMEM((M + SEG + M, D), F32),
            pltpu.VMEM((48 + 16, 8, 128), F32),
            pltpu.VMEM((80, 128), F32),
            pltpu.VMEM((SEG, 128), F32),
            pltpu.VMEM((2, 8, D), BF16),
            pltpu.VMEM((8, 128), U32),
            pltpu.VMEM((NP, 4, 80, DH), BF16),
            pltpu.VMEM((D + 32, 128), F32),
            pltpu.VMEM((2, NF, 8, 128), F32),
            pltpu.VMEM((16, D), F32),
            pltpu.VMEM((H, NE, DH), F32),
            pltpu.VMEM((M, D), BF16),
            pltpu.VMEM((D,), BF16),
            pltpu.VMEM((1, D), BF16),
            pltpu.SemaphoreType.DMA((24 + NK,)),
            pltpu.SemaphoreType.DMA((2,)),
        ],
        compiler_params=pltpu.CompilerParams(vmem_limit_bytes=124 * 1024 * 1024,
                                             disable_bounds_checks=True,
                                             disable_semaphore_checks=True),
    )(
        A_x.reshape(NSEG, 4, 8, D),
        A_mem0.reshape(M, D),
        A_Wq.reshape(D // 2, 2, H, DH),
        A_Wk.reshape(D // 2, 2, H, DH),
        A_Wv.reshape(D // 2, 2, H, DH),
        A_Wo.reshape(H * DH, D),
        B_w_r,
        B_w_gate,
        B_w_up,
        B_w_down,
        c,
        w_mod,
    )
    return out.reshape(1, NSEG * SEG, D)
```

```python
import jax
import jax.numpy as jnp
import jax.experimental.pallas as pl
import jax.experimental.pallas.tpu as pltpu

F32 = jnp.float32
BF16 = jnp.bfloat16
U32 = jnp.uint32

D = 1024
H = 32
DH = 128
NP = H // 2
M = 8
SEG = 32
NSEG = 64
FF = 3584
NJ = SEG - M
NE = NSEG * M
EPS = 1.0013580322265625e-05
SCALE = 0.08837890625
NEG = -1000000000.0
LOG2E = 1.4426950408889634
KQ = 128
NK = D // KQ
MB = 11
NG = 4
NF = FF // 128
I0 = 2
ND = 4
UNROLL = 2
NIT = NSEG // (2 * UNROLL)
OUT_SPLIT = NSEG - 2 * UNROLL - 2


def _rb(x):
    return x.astype(BF16).astype(F32)


def _layernorm(xf):
    m = jnp.mean(xf, axis=-1, keepdims=True)
    d = xf - m
    v = jnp.mean(d * d, axis=-1, keepdims=True)
    std = _rb(jnp.sqrt(_rb(_rb(v) + EPS)))
    return _rb(xf - _rb(m)) * (1.0 / std)


def _sigmoid(x):
    return _rb(1.0 / _rb(1.0 + _rb(jnp.exp(-x))))


def _dot(a, b):
    return jnp.dot(a, b, preferred_element_type=F32)


def _dot_nt(a, b):
    return jax.lax.dot_general(a, b, (((1,), (1,)), ((), ())), preferred_element_type=F32)


def _kernel(x_hbm, mem0_hbm, wq_hbm, wk_hbm, wv_hbm, wo_hbm, wr_hbm, wg_hbm, wu_hbm, wd_hbm,
            c_hbm, wm_hbm,
            out_hbm,
            wq, wk, wv, wo, wg, wu, wd, wm, cb, xv, x1v, h2v, outv, early, hn, he, hj, pend,
            mod, fill, keys, patch, zero, opnd, xt, act, ys, acc0, mem0_ref, wr_ref, c_ref,
            sem, sem_out):
    w_u32 = [w.bitcast(U32) for w in (wq_hbm, wk_hbm, wv_hbm)]
    wqkv = (wq, wk, wv)
    wo_hbm, wg_hbm, wu_hbm, wd_hbm, wm_hbm = [
        w.bitcast(U32) for w in (wo_hbm, wg_hbm, wu_hbm, wd_hbm, wm_hbm)]

    def wo_blk(n, lo, hi):
        return pltpu.bitcast(wo[n, lo // 2:hi // 2, :], BF16)

    def w_copies(m, p, k):
        return [pltpu.make_async_copy(w_u32[m].at[:, par, p, :], wqkv[m].at[2 * p + par], sem.at[k])
                for par in range(2)]

    def col_copy(src, dst, j, k):
        lo = j * 128 if isinstance(j, int) else pl.multiple_of(j * 128, 128)
        return pltpu.make_async_copy(src.at[:, pl.ds(lo, 128)], dst.at[j], sem.at[k])

    def units(g):
        return [(m, 4 * g + t) for t in range(4) for m in range(2)]

    def xj_copy(g):
        segs = pl.ds(16 * g, 16)
        return pltpu.make_async_copy(x_hbm.at[segs, 0:3], xv.at[segs, 0:3], sem.at[16 + g])

    def qk_copies(g):
        return sum([w_copies(m, p, 16 + g) for m, p in units(g)], [])

    def wm1_copies(j):
        return [col_copy(wm_hbm, wm, j, 1 + j), col_copy(wm_hbm, wm, 8 + j, 1 + j)]

    def wv_copies(j):
        lo = j * (KQ // 2) if isinstance(j, int) else pl.multiple_of(j * (KQ // 2), KQ // 2)
        rows = pl.ds(lo, KQ // 2)
        return [pltpu.make_async_copy(w_u32[2].at[rows, par, p, :], wv.at[2 * p + par, rows],
                                      sem.at[24 + j]) for p in range(NP) for par in range(2)]

    def wm2_copies(lo, n, t):
        return [col_copy(wm_hbm, wm, lo + b, 20 + t) for b in range(n)]

    def wait_if(cond, cps):
        for cp in cps:
            pl.when(cond)(cp.wait)

    def start_if(cond, cps):
        for cp in cps:
            pl.when(cond)(cp.start)

    def start_if_below(i, n, cps):
        for k in range(0, len(cps), 4):
            start_if(i < n if k % 8 == 0 else i + 1 <= n, cps[k:k + 4])

    cp_c = pltpu.make_async_copy(c_hbm, c_ref, sem.at[9])
    cp_xe = pltpu.make_async_copy(x_hbm.at[:, 3], xv.at[:, 3], sem.at[0])
    cp_wo = [col_copy(wo_hbm, wo, n, 10) for n in range(8)]
    cp_small = [pltpu.make_async_copy(mem0_hbm, mem0_ref, sem.at[14]),
                pltpu.make_async_copy(wr_hbm, wr_ref, sem.at[15])]
    cp_glu = ([col_copy(wg_hbm, wg, j, 11) for j in range(NF)]
              + [col_copy(wu_hbm, wu, j, 11) for j in range(NF)])
    cp_wd = pltpu.make_async_copy(wd_hbm, wd.at[:, 0:D], sem.at[13])

    for cp in ([cp_c, cp_xe] + wm1_copies(0) + wv_copies(0) + wm1_copies(1) + wm1_copies(2)
               + wv_copies(1) + cp_small):
        cp.start()

    ri = jax.lax.broadcasted_iota(jnp.int32, (80, 128), 0)
    ci = jax.lax.broadcasted_iota(jnp.int32, (80, 128), 1)

    def head_of(i):
        return jnp.where(i < 64, i >> 5, (i - 64) >> 3)

    def pos_of(i):
        return jnp.where(i < 64, i & 31, 32 + (i & 7))

    same = (head_of(ri) == head_of(ci)) & (ci < 80)
    allowed = (pos_of(ri) < M) | (pos_of(ri) >= pos_of(ci))
    fill[...] = jnp.where(same, jnp.where(allowed, 0.0, NEG / SCALE), -jnp.inf).astype(F32)
    keys[...] = jnp.zeros(keys.shape, F32)
    pend[M:, :] = jnp.zeros((SEG + M, D), F32)
    zero[...] = jnp.zeros(zero.shape, U32)
    wg[NF] = jnp.zeros((D // 2, 128), U32)
    wu[NF] = jnp.zeros((D // 2, 128), U32)
    xt[...] = jnp.zeros(xt.shape, F32)
    act[...] = jnp.zeros(act.shape, F32)

    def pin_zero(vals):
        acc = None
        for v in vals:
            v = pltpu.bitcast(v, U32)
            for r in range(0, v.shape[0], 8):
                acc = v[r:r + 8] if acc is None else acc | v[r:r + 8]
        return acc & zero[...]

    cp_c.wait()
    cf = c_ref[...].astype(F32)
    sc = _rb(cf * _sigmoid(cf))
    cb[0:D, :] = jnp.broadcast_to(sc, (128, D)).T
    cb[D:, :] = jnp.zeros((32, 128), F32)

    def mod_vec(k):
        return jnp.concatenate([mod[8 * k + b] for b in range(8)], axis=1)

    def mod_block_vpu(src, dst, is_scale, after=None):
        acc = None if after is None else pltpu.bitcast(pin_zero([after]), F32)
        for r in range(0, D // 2, 8):
            w = wm[src, r:r + 8, :]
            t0 = pltpu.bitcast(w << 16, F32) * cb[pl.ds(2 * r, 8, stride=2), :]
            t1 = pltpu.bitcast(w & U32(0xFFFF0000), F32) * cb[pl.ds(2 * r + 1, 8, stride=2), :]
            if after is not None:
                acc = (acc + t0) + t1
            else:
                acc = t0 + t1 if acc is None else acc + (t0 + t1)
        v = _rb(jnp.broadcast_to(jnp.sum(acc, axis=0, keepdims=True), (8, 128)))
        v = jnp.where(is_scale, _rb(1.0 + v), v)
        mod[dst] = v
        return v

    def ne_body(i, carry):
        n = _layernorm(xv[pl.ds(i * 16, 16), 3].astype(F32)).reshape(128, D).astype(BF16)
        for j in range(NK):
            hn[j, pl.ds(pl.multiple_of(i * 128, 128), 128), :] = n[:, j * KQ:(j + 1) * KQ]
        return carry

    cp_xe.wait()
    jax.lax.fori_loop(0, NSEG // 16, ne_body, 0)

    def w_head(m, h, lo=0, hi=D):
        return pltpu.bitcast(wqkv[m][h, lo // 2:hi // 2, :], BF16)

    def relayout(m, p, rows=slice(None)):
        w = wqkv[m]
        e = w[2 * p, rows, :]
        o = w[2 * p + 1, rows, :]
        w[2 * p, rows, :] = (e & U32(0xFFFF)) | (o << 16)
        w[2 * p + 1, rows, :] = (e >> 16) | (o & U32(0xFFFF0000))

    def store_early(m, p, row0, r1, r2):
        ns = r1.shape[0] // 8
        r12 = jnp.concatenate([r1.reshape(ns, 8, DH), r2.reshape(ns, 8, DH)], axis=1)
        v = pltpu.bitcast(r12.reshape(16 * ns, DH).astype(BF16), U32)
        early[row0 // 8:row0 // 8 + ns, m * NP + p] = v.reshape(ns, 8, DH)
        return v

    def modulate(src, dst, shift, scale):
        n = hn[src].astype(F32).reshape(NSEG, 8, KQ)
        h = (_rb(n * scale) + shift).reshape(NE, KQ)
        he[dst] = h.astype(BF16)
        return h

    def chunk_body(j, carry):
        @pl.when(j <= 1)
        def _():
            for cp in wm1_copies(j):
                cp.wait()
            modulate(j, j, mod_block_vpu(j, j, False), mod_block_vpu(8 + j, 8 + j, True))

        nxt = jnp.where(j >= 1, jnp.minimum(j + 1, NK - 1), 0)
        live = nxt == j + 1
        wait_if(live, wm1_copies(nxt))
        for cp in wv_copies(j):
            cp.wait()
        krows = pl.ds(pl.multiple_of(j * (KQ // 2), KQ // 2), KQ // 2)
        hb = [he[j, c * 256:(c + 1) * 256, :] for c in range(2)]
        pins = {}
        for c in range(2):
            rows = slice(c * 256, (c + 1) * 256)
            for q in range(NP // 2):
                i = 8 * c + q
                if c == 0:
                    relayout(2, 2 * q, krows)
                    relayout(2, 2 * q + 1, krows)
                w4 = [wv[4 * q + b, krows, :] for b in range(4)]
                if i in pins:
                    w4[0] = jnp.concatenate([w4[0][0:8] | pin_zero(pins[i]), w4[0][8:]], axis=0)
                r = _dot(hb[c], pltpu.bitcast(jnp.concatenate(w4, axis=1), BF16))
                for b in range(4):
                    acc0[4 * q + b, rows, :] = (r[:, b * DH:(b + 1) * DH]
                                                + jnp.where(j > 0, acc0[4 * q + b, rows, :], 0.0))
                if i == 7:
                    shift = mod_block_vpu(nxt, jnp.where(live, nxt, 48), False, r[0:8, 0:128])
                if i == 9:
                    scale = mod_block_vpu(8 + nxt, jnp.where(live, 8 + nxt, 49), True,
                                          r[0:8, 0:128])
                    h = modulate(nxt, jnp.where(live, nxt, NK), shift, scale)
                    pins = {13: [h[0:256]], 15: [h[256:512]]}
        pr = 1 + (j >> 1)
        t = jnp.maximum(j - 5, 0)
        start_if(j + 4 < NK, wm1_copies(jnp.minimum(j + 4, NK - 1)))
        start_if_below(j, NK - 3, wv_copies(jnp.minimum(j + 3, NK - 1)))
        start_if((j & 1) == 0, w_copies(0, pr, 16 + (pr >> 2)))
        start_if((j & 1) == 1, w_copies(1, pr, 16 + (pr >> 2)))
        start_if_below(4, j, [xj_copy(t)] + w_copies(0, 5 + t, 17) + w_copies(1, 5 + t, 17)
                       + wm2_copies(16 + 4 * t, 4, 0))
        return carry

    for cp in wm1_copies(3) + wv_copies(2) + w_copies(0, 0, 16) + w_copies(1, 0, 16):
        cp.start()
    jax.lax.fori_loop(0, NK, chunk_body, 0)

    def early_proj(m, p, pins):
        relayout(m, p)
        for c in range(2):
            rows = slice(c * 256, (c + 1) * 256)
            hc = jnp.concatenate([he[j, rows, :] for j in range(NK)], axis=1)
            r12 = []
            for b in range(2):
                halves = []
                for k in range(2):
                    wh = wqkv[m][2 * p + b, k * 256:(k + 1) * 256, :]
                    if pins.get(4 * c + 2 * b + k):
                        wh = jnp.concatenate(
                            [wh[0:8] | pin_zero(pins[4 * c + 2 * b + k]), wh[8:]], axis=0)
                    halves.append(wh)
                r12.append(_dot(hc, pltpu.bitcast(jnp.concatenate(halves, axis=0), BF16)))
            store_early(m, p, c * 256, *r12)

    def make_hj(s):
        n = _rb(_layernorm(xv[s, 0:3].astype(F32)))
        h = _rb(n * mod_vec(1)) + mod_vec(0)
        hj[s] = h
        h2v[s] = jnp.concatenate([h, h[0:1]], axis=0).astype(BF16)
        return [h[g, :, 0:128] for g in range(3)]

    def pro_body(g, carry):
        wait_if(g == 1, wm2_copies(16, 12, 0))
        tb = jnp.maximum(g - 2, 0)
        wait_if(g >= 2, wm2_copies(28 + 10 * tb, 10, 1 + tb))
        for cp in qk_copies(g) + [xj_copy(g)]:
            cp.wait()
        lnp = sum([make_hj(g * 16 + t) for t in range(16)], [])
        mv = []
        for b in range(MB):
            blk = 16 + MB * (g - 1) + b
            live = (g > 0) & (blk < 48)
            mv.append(mod_block_vpu(jnp.where(live, blk, b), jnp.where(live, blk, 48 + b),
                                    (blk >= 32) & (blk < 40)))
        fin = [store_early(2, 4 * g + t, 0, acc0[8 * g + 2 * t], acc0[8 * g + 2 * t + 1])
               for t in range(4)]
        sites = {i: [] for i in range(64)}
        twice = [3, 4, 6, 7, 10, 11, 12, 14, 15, 18, 19, 20, 22, 23, 26, 27, 30, 31]
        for i, v in zip(sorted(list(range(2, 32)) + twice), lnp):
            sites[2 * i].append(v)
        for i, v in zip(range(1, 31, 2), mv + fin):
            sites[2 * i + 1].append(v)
        for u, (m, p) in enumerate(units(g)):
            early_proj(m, p, {i: sites[8 * u + i] for i in range(8)})
        gn = jnp.minimum(g, 1)
        start_if_below(g, 2, qk_copies(gn + 2))
        start_if(g == 1, [xj_copy(3)])
        start_if_below(g, 2, wm2_copies(28 + 10 * gn, 10, 1 + gn))
        start_if(g == 0, cp_wo[:1])
        start_if(g == 1, cp_wo[1:])
        start_if_below(NG - 2, g, cp_glu)
        return carry

    jax.lax.fori_loop(0, NG, pro_body, 0)

    cp_wd.start()
    for cp in cp_small + cp_wo:
        cp.wait()
    pend[0:M, :] = mem0_ref[...].astype(F32)

    wr = jnp.broadcast_to(wr_ref[...].astype(F32).reshape(1, D), (8, D))

    lane8 = jax.lax.broadcasted_iota(jnp.int32, (8, 128), 1)
    sub8 = jax.lax.broadcasted_iota(jnp.int32, (8, 128), 0)
    LAST = NSEG * SEG - 1

    def post(s, g0, g1, attn, record=True):
        attn = attn.reshape(g1 - g0, 8, D)
        x1 = _rb(xv[s, g0:g1].astype(F32) + _rb(mod_vec(2) * _rb(attn)))
        n = _rb(_layernorm(x1))
        h2 = _rb(_rb(n * mod_vec(4)) + mod_vec(3))
        r = _rb(jnp.sum(h2 * wr, axis=-1, keepdims=True)) + 0.0
        x1v[s, g0:g1] = x1.astype(BF16)
        h2v[s, g0:g1] = h2.astype(BF16)
        outv[s, g0:g1] = (x1 + _rb(mod_vec(5) * h2)).astype(BF16)
        pins = []
        for g in range(g0, g1):
            bits = pltpu.bitcast(jnp.broadcast_to(r[g - g0], (8, 128)), jnp.int32)
            hi = jax.lax.shift_right_logical(bits, 16)
            code = jnp.where(bits < 0, hi ^ 0xFFFF, hi | 0x8000)
            key = (code << 11) | (LAST - (s * SEG + g * 8) - sub8) | 0x40000000
            key = pltpu.bitcast(key, F32)
            if record:
                rows = slice(g * 8, (g + 1) * 8)
                keys[rows, :] = jnp.where(lane8 == s, key, keys[rows, :])
            pins.append(key)
        return pins

    def post_pair(a, rows, record=True):
        return post(a + 1, 0, 4, rows[0:SEG], record) + post(a, 3, 4, rows[SEG:], record)

    zpad = jnp.zeros((48, DH), BF16)
    G = 4
    KA = (NP - G) * 2 * DH
    KS = D - 128

    def decode(k):
        kb = pltpu.bitcast(jnp.broadcast_to(k, (8, 128)), jnp.int32)
        code = (kb >> 11) & 0xFFFF
        hi = jnp.where(code >= 0x8000, code & 0x7FFF, code ^ 0xFFFF)
        tok = jnp.clip((LAST - (kb & LAST))[0, 0], 0, LAST)
        return tok, pltpu.bitcast(hi << 16, F32)[:, 0:1]

    def recorded_top2():
        kv = keys[...]
        o1 = jnp.max(jnp.max(kv, axis=0, keepdims=True), axis=1, keepdims=True)
        kv = jnp.where(kv == o1, 0.0, kv)
        return o1, jnp.max(jnp.max(kv, axis=0, keepdims=True), axis=1, keepdims=True)

    def group_of(ref, t):
        return ref[t >> 5, pl.ds((t >> 3) & 3, 1)].astype(F32)

    glu = {}

    def glu_act(gt, up):
        gt = _rb(gt)
        return _rb(gt * _sigmoid(gt)) * _rb(up)

    def glu_block(after):
        j = glu['first'] + glu['todo'].pop(0)
        src = jnp.where(glu['live'], j, NF)
        sums = []
        for w_ref in (wg, wu):
            acc = pltpu.bitcast(pin_zero([after]), F32)
            for r in range(0, D // 2, 8):
                w = w_ref[src, r:r + 8, :]
                acc = ((acc + pltpu.bitcast(w << 16, F32) * xt[pl.ds(2 * r, 8, stride=2), :])
                       + pltpu.bitcast(w & U32(0xFFFF0000), F32) * xt[pl.ds(2 * r + 1, 8, stride=2), :])
            after = acc
            sums.append(jnp.broadcast_to(jnp.sum(acc, axis=0, keepdims=True), (8, 128)))
        act[glu['slot'], j] = glu_act(*sums)

    def segment(s, lhs, lhs_split, extra, pins):
        scales = {}

        def stash(p, m, v):
            opnd[p, m, 0:v.shape[0], :] = v.astype(BF16)

        def qkv_group(p):
            order = (1, 0, 2)
            keys = [(m, 2 * p + b) for m in order for b in range(2 * G)]
            nsplit = 6 if (p == 0 and lhs_split is not None) else 0
            part = [_dot(lhs_split[0], w_head(m, h, 0, KS)) for m, h in keys[:nsplit]]
            full = [_dot(lhs_split[1], w_head(m, h, KS, D)) + part[i]
                    for i, (m, h) in enumerate(keys[:nsplit])]
            full += [_dot(lhs, w_head(m, h)) for m, h in keys[nsplit:]]
            if glu['todo']:
                glu_block(full[(8, 11, 8, 8)[p // G]][0:8])
            for m in range(3):
                for t in range(G):
                    i = 2 * G * order.index(m) + 2 * t
                    stash(p + t, m, jnp.concatenate([full[i], full[i + 1]], axis=0))

        def operand(p, m):
            parts = [opnd[p, m, 0:64, :], pltpu.bitcast(early[s, m * NP + p], BF16)]
            if m > 0:
                parts.append(zpad)
            return jnp.concatenate(parts, axis=0)

        def scores(p):
            sc_ = _dot_nt(operand(p, 0), operand(p, 1))
            f = fill[...]
            if pins.get(p):
                f = jnp.concatenate([f[0:8] + pltpu.bitcast(pin_zero(pins[p]), F32), f[8:]], axis=0)
            sc_ = jnp.where(f == 0.0, sc_, f)
            mx = jnp.max(sc_, axis=-1, keepdims=True)
            e = jnp.exp2((sc_ - mx) * (SCALE * LOG2E))
            inv = pl.reciprocal(jnp.sum(e, axis=-1, keepdims=True), approx=True)
            if p // G == NP // G - 2:
                stash(p, 3, e * inv)
            else:
                stash(p, 3, e)
                scales[p] = inv

        oe = []

        def pv(p):
            o = _dot(opnd[p, 3], operand(p, 2))
            if p in scales:
                o = o * scales[p]
                pins.setdefault((p // G + 1) * G + (0, 2, 3, 1)[p % G], []).append(o)
            res = []
            for b in range(2):
                rows, erows = o[32 * b:32 * b + 32], o[64 + 8 * b:72 + 8 * b]
                oe.append(erows)
                if extra is not None:
                    rows = jnp.concatenate([rows, erows, extra[2 * p + b]], axis=0)
                res.append(rows)
            return res

        os_ = []
        for p in range(0, NP, G):
            qkv_group(p)
            if p >= G:
                for t in range(G):
                    os_ += pv(p - G + t)
            for t in (1, 2, 3, 0):
                scores(p + t)
        oa = jnp.concatenate(os_, axis=1).astype(BF16)
        acc, ob = [], []
        for n in range(7):
            acc.append(_dot(oa, wo_blk(n, 0, KA)))
            if n == (1 if extra is None else 0):
                for t in range(G):
                    ob += pv(NP - G + t)
        ob = jnp.concatenate(ob, axis=1).astype(BF16)
        res = [_dot(ob, wo_blk(n, KA, H * DH)) + acc[n] for n in range(7)]
        res.append(_dot(ob, wo_blk(7, KA, H * DH)) + _dot(oa, wo_blk(7, 0, KA)))
        return res, oe

    def make_lhs(mem, s):
        return jnp.concatenate([mem, hj[s].reshape(NJ, D)], axis=0)

    cp_o1 = pltpu.make_async_copy(outv.at[0:OUT_SPLIT], out_hbm.at[0:OUT_SPLIT], sem_out.at[0])
    cp_o2 = pltpu.make_async_copy(outv.at[OUT_SPLIT:NSEG], out_hbm.at[OUT_SPLIT:NSEG],
                                  sem_out.at[1])

    def split_lhs(lhs):
        return lhs.astype(BF16), (lhs[:, :KS].astype(BF16), lhs[:, KS:].astype(BF16))

    def step(i, carry):
        c0, c1, tok, slot, half = carry
        held = jnp.where(half == 1, tok, jnp.where(jnp.where(slot == 0, c0, c1) == tok, tok, -1))
        c0, c1 = jnp.where(slot == 0, held, c0), jnp.where(slot == 1, held, c1)
        glu.update(todo=list(range(NF // 2)), first=half * (NF // 2), slot=slot, live=i >= I0)

        @pl.when(i == I0)
        def _():
            for cp in cp_glu:
                cp.wait()

        @pl.when(i == NIT - 1)
        def _():
            cp_o1.start()

        prev = pend[...]
        for u in range(UNROLL):
            a = 2 * (UNROLL * i + u)
            pins = post_pair(jnp.maximum(a - 2, 0) if u == 0 else a - 2, prev[M:])
            lhs_a = make_lhs(prev[0:M], a)
            lhs_a = (lhs_a.astype(BF16), None) if u == 0 else split_lhs(lhs_a)
            res_a, oe_a = segment(a, *lhs_a, None,
                                  {k: [v] for k, v in zip((2, 6, 10, 14), pins[:4])})
            res_a = jnp.concatenate(res_a, axis=1)
            pins = pins[4:] + post(a, 0, 3, res_a[M:])
            res_b, _ = segment(a + 1, *split_lhs(make_lhs(res_a[0:M], a + 1)), oe_a,
                               {k: [v] for k, v in zip((2, 6, 10, 14), pins)})
            prev = jnp.concatenate(res_b, axis=1)
        pend[...] = prev
        assert not glu['todo']

        ta, tb = [decode(jnp.broadcast_to(o, (1, 128)))[0] for o in recorded_top2()]
        has_a = (c0 == ta) | (c1 == ta)
        more = (half == 0) & (held != tok) & ((tok == ta) | (tok == tb))
        nt = jnp.where(more, tok, jnp.where(has_a, tb, ta))
        ns = jnp.where(more, slot, jnp.where(c0 == jnp.where(has_a, ta, tb), 1, 0))
        rowi = jax.lax.broadcasted_iota(jnp.int32, (8, 1), 0)
        row = jnp.sum(jnp.where(rowi == (nt & 7), group_of(h2v, nt)[0], 0.0), axis=0, keepdims=True)
        xt[0:D, :] = jnp.broadcast_to(row, (128, D)).T
        return c0, c1, jnp.where(i + 1 >= I0, nt, -1), ns, more.astype(jnp.int32)

    c0, c1, tok, slot, half = jax.lax.fori_loop(
        0, NIT, step, (jnp.int32(-1), jnp.int32(-1), jnp.int32(-1), jnp.int32(0), jnp.int32(0)))
    cp_wd.wait()

    def down(lo, hi):
        ab = jnp.concatenate([act[:, j].reshape(16, 128) for j in range(NF)], axis=1).astype(BF16)
        return jnp.concatenate([_dot(ab, pltpu.bitcast(wd[:, n * 128:(n + 1) * 128], BF16))
                                for n in range(lo, hi)], axis=1)

    ys[:, 0:ND * 128] = down(0, ND)
    o1, o2 = recorded_top2()
    last_keys = post_pair(NSEG - 2, pend[M:, :], record=False)
    cp_o2.start()
    kv = jnp.concatenate(last_keys + [jnp.where(sub8 < 4, o1, o2)], axis=0)
    k1 = jnp.max(kv, axis=0, keepdims=True)
    k2 = jnp.max(jnp.where(kv == k1, 0.0, kv), axis=0, keepdims=True)
    (i1, r1), (i2, r2) = decode(k1), decode(k2)
    g1, g2 = i1 >> 3, i2 >> 3
    x1 = jnp.concatenate([group_of(x1v, i1), group_of(x1v, i2)], axis=0)
    h2 = jnp.concatenate([group_of(h2v, i1), group_of(h2v, i2)], axis=0)
    d0 = jnp.where((half == 1) & (slot == 0), tok, c0)
    d1 = jnp.where((half == 1) & (slot == 1), tok, c1)
    swapped = (d0 == i2) & (d1 == i1)
    found = swapped | ((d0 == i1) & (d1 == i2))

    @pl.when(jnp.logical_not(found) | (half == 1))
    def _():
        hl = jnp.where(swapped, jnp.concatenate([h2[1], h2[0]], axis=0), h2.reshape(16, D))
        hl = hl.astype(BF16)

        def redo(t, carry):
            for b in range(NF // 2):
                j = t * (NF // 2) + b
                act[:, j] = glu_act(_dot(hl, pltpu.bitcast(wg[j], BF16)),
                                    _dot(hl, pltpu.bitcast(wu[j], BF16))).reshape(2, 8, 128)
            return carry

        jax.lax.fori_loop(found.astype(jnp.int32), 2, redo, 0)
        ys[:, 0:ND * 128] = down(0, ND)

    y = _rb(jnp.concatenate([ys[:, 0:ND * 128], down(ND, 8)], axis=1))
    y1 = _rb(jnp.where(swapped, y[8:16], y[0:8]) * _sigmoid(r1))
    y2 = _rb(jnp.where(swapped, y[0:8], y[8:16]) * _sigmoid(r2))
    rowi = jax.lax.broadcasted_iota(jnp.int32, (2, 8, 1), 1)
    gsel = jax.lax.broadcasted_iota(jnp.int32, (2, 8, 1), 0)
    tokp = jnp.where(gsel == 0, g1, g2) * 8 + rowi
    upd = jnp.where(tokp == i1, y1[None], jnp.where(tokp == i2, y2[None], 0.0))
    patch[...] = (x1 + _rb(mod_vec(5) * _rb(h2 + upd))).astype(BF16)
    cp_o1.wait()
    cp_o2.wait()
    cp1 = pltpu.make_async_copy(patch.at[0], out_hbm.at[g1 >> 2, g1 & 3], sem_out.at[0])
    cp1.start()

    @pl.when(g1 != g2)
    def _():
        cp2 = pltpu.make_async_copy(patch.at[1], out_hbm.at[g2 >> 2, g2 & 3], sem_out.at[1])
        cp2.start()
        cp2.wait()

    cp1.wait()


@jax.jit
def pallas_adaLN_cond__memory_aug_recurrent_mem_tr__moe_arch_mod__prompt_kernel(
    A_x: jax.Array,
    A_mem0: jax.Array,
    A_Wq: jax.Array,
    A_Wk: jax.Array,
    A_Wv: jax.Array,
    A_Wo: jax.Array,
    A_seg_len,
    B_x: jax.Array,
    B_w_r: jax.Array,
    B_w_gate: jax.Array,
    B_w_up: jax.Array,
    B_w_down: jax.Array,
    c: jax.Array,
    w_mod: jax.Array,
):
    assert A_x.shape == (1, NSEG * SEG, D)
    any_spec = pl.BlockSpec(memory_space=pl.ANY)
    out = pl.pallas_call(
        _kernel,
        out_shape=jax.ShapeDtypeStruct((NSEG, 4, 8, D), BF16),
        in_specs=[any_spec] * 12,
        out_specs=any_spec,
        scratch_shapes=[
            pltpu.VMEM((H, D // 2, DH), U32),
            pltpu.VMEM((H, D // 2, DH), U32),
            pltpu.VMEM((H, D // 2, DH), U32),
            pltpu.VMEM((8, H * DH // 2, 128), U32),
            pltpu.VMEM((NF + 1, D // 2, 128), U32),
            pltpu.VMEM((NF + 1, D // 2, 128), U32),
            pltpu.VMEM((FF // 2, D + 128), U32),
            pltpu.VMEM((48, D // 2, 128), U32),
            pltpu.VMEM((D + 32, 128), F32),
            pltpu.VMEM((NSEG, 4, 8, D), BF16),
            pltpu.VMEM((NSEG, 4, 8, D), BF16),
            pltpu.VMEM((NSEG, 4, 8, D), BF16),
            pltpu.VMEM((NSEG, 4, 8, D), BF16),
            pltpu.VMEM((NSEG, 3 * NP, 8, DH), U32),
            pltpu.VMEM((NK, NE, KQ), BF16),
            pltpu.VMEM((NK + 1, NE, KQ), BF16),
            pltpu.VMEM((NSEG, 3, 8, D), F32),
            pltpu.VMEM((M + SEG + M, D), F32),
            pltpu.VMEM((48 + 16, 8, 128), F32),
            pltpu.VMEM((80, 128), F32),
            pltpu.VMEM((SEG, 128), F32),
            pltpu.VMEM((2, 8, D), BF16),
            pltpu.VMEM((8, 128), U32),
            pltpu.VMEM((NP, 4, 80, DH), BF16),
            pltpu.VMEM((D + 32, 128), F32),
            pltpu.VMEM((2, NF, 8, 128), F32),
            pltpu.VMEM((16, D), F32),
            pltpu.VMEM((H, NE, DH), F32),
            pltpu.VMEM((M, D), BF16),
            pltpu.VMEM((D,), BF16),
            pltpu.VMEM((1, D), BF16),
            pltpu.SemaphoreType.DMA((24 + NK,)),
            pltpu.SemaphoreType.DMA((2,)),
        ],
        compiler_params=pltpu.CompilerParams(vmem_limit_bytes=124 * 1024 * 1024,
                                             disable_bounds_checks=True,
                                             disable_semaphore_checks=True),
    )(
        A_x.reshape(NSEG, 4, 8, D),
        A_mem0.reshape(M, D),
        A_Wq.reshape(D // 2, 2, H, DH),
        A_Wk.reshape(D // 2, 2, H, DH),
        A_Wv.reshape(D // 2, 2, H, DH),
        A_Wo.reshape(H * DH, D),
        B_w_r,
        B_w_gate,
        B_w_up,
        B_w_down,
        c,
        w_mod,
    )
    return out.reshape(1, NSEG * SEG, D)
```
